```python
import jax
import jax.numpy as jnp

def _softmax(x, axis=-1):
    return jax.nn.softmax(x, axis=axis)
def _gelu(x):
    return jax.nn.gelu(x, approximate=True)
def _silu(x):
    return jax.nn.silu(x)
def _sigmoid(x):
    return jax.nn.sigmoid(x)
def _layernorm(x, axis=-1, eps=1e-5):
    m = jnp.mean(x, axis=axis, keepdims=True)
    v = jnp.var(x, axis=axis, keepdims=True)
    return (x - m) / jnp.sqrt(v + eps)
def _scatter_add(tgt, idx, src, axis=0):
    return tgt.at[idx].add(src)
def _segment_sum(src, seg, n):
    return jax.ops.segment_sum(src, seg, n)
class _Rng:
    def __init__(self, key):
        self._k = key
    def _next(self):
        self._k, sub = jax.random.split(self._k)
        return sub
    def normal(self, shape):
        return jax.random.normal(self._next(), shape, dtype=jnp.bfloat16)
    def randint(self, lo, hi, shape):
        return jax.random.randint(self._next(), shape, lo, hi, dtype=jnp.int32)
    def uniform(self, shape, lo=0.0, hi=1.0):
        return jax.random.uniform(self._next(), shape, jnp.bfloat16, lo, hi)
    def permutation(self, n):
        return jax.random.permutation(self._next(), n)


kernel_name = 'gated_mix__sliding_local_dilated__glu_gated_reglu__prompt'

def setup_inputs():
    _rng = _Rng(jax.random.key(int.from_bytes(__import__("os").urandom(4), "little")))
    _w = (lambda a: (lambda t: t.astype(jnp.bfloat16) if jnp.issubdtype(t.dtype, jnp.floating) else t)(jnp.asarray(a)))
    def _A_setup():
        B, S, D = 1, 2048, 1024
        return {
            "x": _w((lambda *s: _rng.normal(s) * 0.05)(B, S, D)),
            "wqkv": _w((lambda *s: _rng.normal(s) * 0.05)(D, 3 * D)),
            "wo": _w((lambda *s: _rng.normal(s) * 0.05)(D, D)),
        }
    _A_in = _A_setup()

    def _B_setup():
        B, S, D, F = 1, 2048, 1024, 3584
        return {
            "x": _w((lambda *s: _rng.normal(s) * 0.05)(B, S, D)),
            "W_gate": _w((lambda *s: _rng.normal(s) * 0.05)(D, F) * (2.0 / D) ** 0.5),
            "W_up": _w((lambda *s: _rng.normal(s) * 0.05)(D, F) * (2.0 / D) ** 0.5),
            "W_down": _w((lambda *s: _rng.normal(s) * 0.05)(F, D) * (1.0 / F) ** 0.5),
        }
    _B_in = _B_setup()

    return {
        "A_x": _A_in["x"],
        "A_wqkv": _A_in["wqkv"],
        "A_wo": _A_in["wo"],
        "B_x": _B_in["x"],
        "B_W_gate": _B_in["W_gate"],
        "B_W_up": _B_in["W_up"],
        "B_W_down": _B_in["W_down"],
        "gate_w": _w((lambda *s: _rng.normal(s) * 0.05)(1024)),
    }

def reference(A_x, A_wqkv, A_wo, B_x, B_W_gate, B_W_up, B_W_down, gate_w):
    def _A_ref(x, wqkv, wo):
        B, S, D = x.shape
        H = 32; Dh = D // H
        W, dil = 8, 2
        qkv = (lambda x, *d: x.transpose(*d))((x @ wqkv).reshape(B, S, 3, H, Dh), 2, 0, 3, 1, 4)
        q, k, v = qkv[0], qkv[1], qkv[2]
        scale = Dh ** -0.5
        pos = jnp.arange(S)
        off = jnp.arange(W) * dil
        idx = pos[:, None] - off[None, :]
        mask = idx >= 0
        idx_c = jnp.where(mask, idx, 0).reshape(-1)
        kg = k[:, :, idx_c, :].reshape(B, H, S, W, Dh)
        vg = v[:, :, idx_c, :].reshape(B, H, S, W, Dh)
        logits = jnp.einsum("bhsd,bhswd->bhsw", q, kg) * scale
        logits = jnp.where(mask[None, None, :, :], logits, -1e9)
        attn = _softmax(logits, axis=-1)
        o = jnp.einsum("bhsw,bhswd->bhsd", attn, vg)
        return (lambda x, *d: x.transpose(*d))(o, 0, 2, 1, 3).reshape(B, S, D) @ wo

    def _B_ref(x, W_gate, W_up, W_down):
        gate = jnp.einsum("bsd,df->bsf", x, W_gate)
        up = jnp.einsum("bsd,df->bsf", x, W_up)
        gate = gate * (lambda x, dt: x.astype(dt))(gate > 0, gate.dtype)
        h = gate * up
        return jnp.einsum("bsf,fd->bsd", h, W_down)

    x = A_x
    g = _sigmoid((x * gate_w).sum(-1, keepdims=True))
    a = _A_ref(x, A_wqkv, A_wo)
    b = _B_ref(x, B_W_gate, B_W_up, B_W_down)
    return g * a + (1 - g) * b
```

```python
import functools
import math

import jax
import jax.numpy as jnp
from jax import lax
import jax.experimental.pallas as pl
import jax.experimental.pallas.tpu as pltpu

f32 = jnp.float32
bf16 = jnp.bfloat16
i32 = jnp.int32

S = 2048
D = 1024
F = 3584
NH = 32
DH = D // NH
W = 8
DIL = 2
H = S // 2
KH = D // 2
FC = 512
CH = FC // 2
NC = F // FC
RB = 256
NRB = H // RB
PAD = 16
TP = DH + 1
AU = 16
UPC = 11

SCALE = DH ** -0.5
EXP2_SCALE = SCALE * math.log2(math.e)
NEG = -1e9 / SCALE


def _dot(a, b):
    return jnp.dot(a, b, preferred_element_type=f32)


def _a_combos(a11, a12, a21, a22):
    return [a11 + a22, a21 + a22, a11, a22, a11 + a12, a21 - a11, a12 - a22]


def _b_combos(b11, b12, b21, b22):
    return [b11 + b22, b11, b12 - b22, b21 - b11, b22, b11 + b12, b21 + b22]


def _c_combos(m):
    return (m[0] + m[3] - m[4] + m[6], m[2] + m[4], m[1] + m[3],
            m[0] - m[1] + m[2] + m[5])


_A_SLOT = {0: 0, 1: 1, 4: 2, 5: 3, 6: 4}
_B_SLOT = {0: 0, 2: 1, 3: 2, 5: 3, 6: 4}


def _interleave(main, side):
    n, m = len(main), len(side)
    done = 0
    for i, task in enumerate(main):
        task()
        upto = (i + 1) * m // n
        for t in side[done:upto]:
            t()
        done = upto


def _kernel(x_hbm, wqkv_hbm, wo_hbm, wg_hbm, wu_hbm, wd_hbm, gw_hbm, out_hbm,
            x_vm, xa, gw_vm, wgu, wd, bc, dc, acc, wqkv_vm, wp, tbuf, q_s, k_s, v_s,
            gs, oa, wo_vm, woc, vbc, sems):
    sem_ids = iter(range(1000))

    def cp(src, dst):
        return pltpu.make_async_copy(src, dst, sems.at[next(sem_ids)])

    x2 = x_hbm.at[0]
    o2 = out_hbm.at[0]
    cp_gw = cp(gw_hbm, gw_vm)
    cp_x = [[cp(x2.at[pl.ds(hf * H + rb * RB, RB), :], x_vm.at[pl.ds(hf * H + rb * RB, RB), :])
             for hf in range(2)] for rb in range(NRB)]
    cp_gu = [[cp((wg_hbm, wu_hbm)[p % 2].at[:, pl.ds(j * FC + (p // 2) * CH, CH)],
                 wgu.at[j, :, pl.ds(p * CH, CH)]) for p in range(4)] for j in range(NC)]
    cp_d = [cp(wd_hbm.at[pl.ds(j * FC, FC), :], wd.at[j]) for j in range(NC)]
    cp_qkv = [cp(wqkv_hbm.at[:, pl.ds(i * D, D)], wqkv_vm.at[:, pl.ds(i * D, D)]) for i in range(3)]
    cp_wo = cp(wo_hbm, wo_vm)
    cp_out = [[cp(x_vm.at[pl.ds(hf * H + rb * RB, RB), :], o2.at[pl.ds(hf * H + rb * RB, RB), :])
               for hf in range(2)] for rb in range(NRB)]

    def start(cs):
        for c in cs:
            c.start()

    def wait(cs):
        for c in cs:
            c.wait()

    start([cp_gw] + cp_x[0] + cp_gu[0])
    for rb in range(1, NRB):
        start(cp_x[rb])
    start([cp_d[0]] + cp_qkv + [cp_wo])
    for j in range(1, NC):
        start(cp_gu[j] + [cp_d[j]])

    def rows(rb, hf=0):
        return slice(hf * H + rb * RB, hf * H + (rb + 1) * RB)

    def x_lhs(t, rb):
        if t == 2:
            return x_vm[rows(rb, 0), :KH]
        if t == 3:
            return x_vm[rows(rb, 1), KH:]
        return xa[_A_SLOT[t], rows(rb), :]

    def prep_x(rb):
        gw = gw_vm[...].astype(f32)
        sub = 64
        for s0 in range(0, RB, sub):
            r = [slice(hf * H + rb * RB + s0, hf * H + rb * RB + s0 + sub) for hf in range(2)]
            a = [x_vm[r[0], :KH].astype(f32), x_vm[r[0], KH:].astype(f32),
                 x_vm[r[1], :KH].astype(f32), x_vm[r[1], KH:].astype(f32)]
            cs = _a_combos(*a)
            for t, slot in _A_SLOT.items():
                xa[slot, r[0], :] = cs[t].astype(bf16)
            for hf in range(2):
                z = None
                for c in range(8):
                    blk = a[2 * hf + c // 4][:, (c % 4) * 128:(c % 4 + 1) * 128]
                    term = blk * gw[c:c + 1, :]
                    z = term if z is None else z + term
                g = jax.nn.sigmoid(jnp.sum(z, axis=1, keepdims=True))
                gs[r[hf], :] = jnp.broadcast_to(g, (sub, 128))

    def b_combo_tasks(src, dst, kh, nh, sub=64):
        def task(r0):
            def run():
                b = [src(slice(a * kh + r0, a * kh + r0 + sub), slice(c * nh, (c + 1) * nh)).astype(f32)
                     for a in range(2) for c in range(2)]
                cs = _b_combos(*b)
                for t, slot in _B_SLOT.items():
                    dst[slot, r0:r0 + sub, :] = cs[t].astype(bf16)
            return run
        return [task(r0) for r0 in range(0, kh, sub)]

    def b_rhs(t, raw, comb, kh, nh):
        if t == 1:
            return raw(slice(0, kh), slice(0, nh))
        if t == 4:
            return raw(slice(kh, 2 * kh), slice(nh, 2 * nh))
        return comb[_B_SLOT[t]]

    ORDER = (1, 4, 2, 3, 0, 5, 6)

    def strassen_x(rb, raw, comb, nh):
        m = [None] * 7
        for t in ORDER:
            m[t] = _dot(x_lhs(t, rb), b_rhs(t, raw, comb, KH, nh))
        return _c_combos(m)

    def ffn_up(j, rb, ha):
        cs = strassen_x(rb, lambda r, c: wgu[j, r, c], bc, FC)
        hs = []
        for qd, cc in enumerate(cs):
            omg = 1.0 - gs[rows(rb, qd // 2), :]
            omg = jnp.concatenate([omg] * (CH // 128), axis=1)
            hs.append(jnp.maximum(cc[:, :CH], 0.0) * cc[:, CH:] * omg)
        ha[rb] = [c.astype(bf16) for c in _a_combos(*hs)]

    def ffn_down(j, rb, ha, first):
        for t in ORDER:
            p = _dot(ha[rb][t], b_rhs(t, lambda r, c: wd[j, r, c], dc, CH, KH))
            if first:
                acc[t, rows(rb), :] = p
            else:
                acc[t, rows(rb), :] += p

    def perm_tasks(i):
        def fwd(rb):
            def run():
                w32 = pltpu.bitcast(wqkv_vm[rb * 256:(rb + 1) * 256, i * D:(i + 1) * D], i32)
                for c in range(8):
                    tt = w32[:, c * 128:(c + 1) * 128].T
                    for hh in range(4):
                        tbuf[rb, pl.ds((4 * c + hh) * TP, DH), :] = tt[hh * DH:(hh + 1) * DH, :]
            return run

        def bwd(rb):
            def run():
                for j in range(8):
                    g = jnp.concatenate(
                        [tbuf[rb, pl.ds(4 * j + dd, NH, stride=TP), :] for dd in range(4)], axis=0)
                    wp[i, rb * 256:(rb + 1) * 256, j * 128:(j + 1) * 128] = pltpu.bitcast(g.T, bf16)
            return run
        return [fwd(rb) for rb in range(4)] + [bwd(rb) for rb in range(4)]

    def wo_tasks():
        def spread(h0):
            def run():
                for h in range(h0, h0 + 8):
                    blk = wo_vm[h * DH:(h + 1) * DH, :].astype(f32)
                    for c in range(8):
                        v_s[c, pl.ds(h * TP, DH), :] = blk[:, c * 128:(c + 1) * 128]
            return run

        def gather(d0):
            def run():
                for d in range(d0, d0 + 4):
                    b = [jnp.concatenate(
                        [v_s[4 * ch + c, pl.ds(16 * rh + d, NH, stride=TP), :] for c in range(4)], axis=1)
                        for rh in range(2) for ch in range(2)]
                    cs = _b_combos(*b)
                    for t in range(7):
                        woc[t, d * NH:(d + 1) * NH, :] = cs[t].astype(bf16)
            return run
        return [spread(h0) for h0 in range(0, NH, 8)] + [gather(d0) for d0 in range(0, 16, 4)]

    def proj(i, dst, pad, rb):
        r0 = rb * 2 * RB
        p = _dot(x_vm[r0:r0 + 2 * RB, :], wp[i])
        for j in range(8):
            dst[j, pad + r0:pad + r0 + 2 * RB, :] = p[:, j * 128:(j + 1) * 128]

    def v_proj(rb):
        cs = strassen_x(rb, lambda r, c: wp[2, r, c], vbc, KH)
        for qd, cc in enumerate(cs):
            r0 = PAD + (qd // 2) * H + rb * RB
            for j in range(4):
                v_s[(qd % 2) * 4 + j, r0:r0 + RB, :] = cc[:, j * 128:(j + 1) * 128]
        if rb == 0:
            for j in range(8):
                src = cs[j // 4][0:1, (j % 4) * 128:(j % 4 + 1) * 128]
                v_s[j, 0:PAD, :] = jnp.broadcast_to(src, (PAD, 128))

    def attn_group(row, masked):
        g = 8
        q = [q_s[j, pl.ds(row, g), :] for j in range(8)]
        ls = []
        for w in range(W):
            a = None
            for j in range(8):
                term = q[j] * k_s[j, pl.ds(row + (PAD - DIL * w), g), :]
                a = term if a is None else a + term
            ls.append(a)
        rs = [pltpu.roll(a, 64, 1) for a in ls]
        ls = [a + r for a, r in zip(ls, rs)]
        rs = [pltpu.roll(a, 32, 1) for a in ls]
        ls = [a + r for a, r in zip(ls, rs)]
        if masked:
            ri = row + lax.broadcasted_iota(i32, (g, 128), 0)
            ls = [ls[0]] + [jnp.where(ri >= DIL * w, ls[w], NEG) for w in range(1, W)]
        m = functools.reduce(jnp.maximum, ls)
        ps = [jnp.exp2((l - m) * EXP2_SCALE) for l in ls]
        r = gs[pl.ds(row, g), :] / functools.reduce(lambda a, b: a + b, ps)
        outs = []
        for j in range(8):
            a = None
            for w in range(W):
                term = ps[w] * v_s[j, pl.ds(row + (PAD - DIL * w), g), :]
                a = term if a is None else a + term
            outs.append(a * r)
        return jnp.concatenate(outs, axis=1)

    def attn_unit(row, masked):
        def run():
            o = [jnp.concatenate([attn_group(row + hf * H + r, masked and hf == 0)
                                  for r in range(0, AU, 8)], axis=0) for hf in range(2)]
            cs = _a_combos(o[0][:, :KH], o[0][:, KH:], o[1][:, :KH], o[1][:, KH:])
            for t in range(7):
                oa[t, pl.ds(row, AU), :] = cs[t].astype(bf16)
        return run

    def gu_tasks(j):
        return b_combo_tasks(lambda r, c: wgu[j, r, c], bc, KH, FC)

    def d_tasks(j):
        return b_combo_tasks(lambda r, c: wd[j, r, c], dc, CH, KH)

    wait([cp_gw] + cp_x[0] + cp_gu[0])
    prep_x(0)
    for t in gu_tasks(0):
        t()
    ha = {}
    ffn_up(0, 0, ha)
    for rb in range(1, NRB):
        wait(cp_x[rb])
    wait([cp_d[0]])
    for rb in range(1, NRB):
        prep_x(rb)
    _interleave([functools.partial(ffn_up, 0, rb, ha) for rb in range(1, NRB)], d_tasks(0))
    wait(cp_qkv + [cp_wo])
    _interleave([functools.partial(ffn_down, 0, rb, ha, True) for rb in range(NRB)], perm_tasks(0))

    for j in range(8):
        k_s[j, 0:PAD, :] = jnp.zeros((PAD, 128), f32)
    _interleave([functools.partial(proj, 0, q_s, 0, rb) for rb in range(NRB)],
                perm_tasks(1) + wo_tasks())
    _interleave([functools.partial(proj, 1, k_s, PAD, rb) for rb in range(NRB)],
                perm_tasks(2) + b_combo_tasks(lambda r, c: wp[2, r, c], vbc, KH, KH))
    for j in range(1, NC):
        wait(cp_gu[j] + [cp_d[j]])
    _interleave([functools.partial(v_proj, rb) for rb in range(NRB)], gu_tasks(1))

    def body(j, carry):
        base = pl.multiple_of(jnp.minimum((j - 1) * (UPC * AU), H - UPC * AU), AU)
        units = [attn_unit(base + u * AU, u == 0) for u in range(UPC)]
        ha = {}
        nup = (2 * UPC) // 3
        _interleave([functools.partial(ffn_up, j, rb, ha) for rb in range(NRB)],
                    d_tasks(j) + units[:nup])
        _interleave([functools.partial(ffn_down, j, rb, ha, False) for rb in range(NRB)],
                    gu_tasks(jnp.minimum(j + 1, NC - 1)) + units[nup:])
        return carry

    lax.fori_loop(1, NC, body, 0)

    for rb in range(NRB):
        m = [acc[t, rows(rb), :] + _dot(oa[t, rows(rb), :], woc[t]) for t in range(7)]
        cs = _c_combos(m)
        for qd, cc in enumerate(cs):
            x_vm[rows(rb, qd // 2), (qd % 2) * KH:(qd % 2 + 1) * KH] = cc.astype(bf16)
        start(cp_out[rb])
    for rb in range(NRB):
        wait(cp_out[rb])


_N_SEMS = 1 + 2 * NRB + 4 * NC + NC + 3 + 1 + 2 * NRB


@jax.jit
def pallas_gated_mix__sliding_local_dilated__glu_gated_reglu__prompt_kernel(
    A_x: jax.Array,
    A_wqkv: jax.Array,
    A_wo: jax.Array,
    B_x: jax.Array,
    B_W_gate: jax.Array,
    B_W_up: jax.Array,
    B_W_down: jax.Array,
    gate_w: jax.Array,
):
    del B_x
    hbm = pl.BlockSpec(memory_space=pl.ANY)
    scratch = [
        pltpu.VMEM((S, D), bf16),
        pltpu.VMEM((5, H, KH), bf16),
        pltpu.VMEM((8, 128), bf16),
        pltpu.VMEM((NC, D, 2 * FC), bf16),
        pltpu.VMEM((NC, FC, D), bf16),
        pltpu.VMEM((5, KH, FC), bf16),
        pltpu.VMEM((5, CH, KH), bf16),
        pltpu.VMEM((7, H, KH), f32),
        pltpu.VMEM((D, 3 * D), bf16),
        pltpu.VMEM((3, D, D), bf16),
        pltpu.VMEM((4, NH * TP, 128), i32),
        pltpu.VMEM((8, S, 128), f32),
        pltpu.VMEM((8, S + PAD, 128), f32),
        pltpu.VMEM((8, S + PAD, 128), f32),
        pltpu.VMEM((S, 128), f32),
        pltpu.VMEM((7, H, KH), bf16),
        pltpu.VMEM((D, D), bf16),
        pltpu.VMEM((7, KH, KH), bf16),
        pltpu.VMEM((5, KH, KH), bf16),
        pltpu.SemaphoreType.DMA((_N_SEMS,)),
    ]
    return pl.pallas_call(
        _kernel,
        in_specs=[hbm] * 7,
        out_specs=hbm,
        out_shape=jax.ShapeDtypeStruct((1, S, D), bf16),
        scratch_shapes=scratch,
        compiler_params=pltpu.CompilerParams(vmem_limit_bytes=124 * 1024 * 1024),
    )(A_x, A_wqkv, A_wo, B_W_gate, B_W_up, B_W_down, gate_w.reshape(8, 128))
```

```python
import functools
import math

import jax
import jax.numpy as jnp
from jax import lax
import jax.experimental.pallas as pl
import jax.experimental.pallas.tpu as pltpu

f32 = jnp.float32
bf16 = jnp.bfloat16
i32 = jnp.int32

S = 2048
D = 1024
F = 3584
NH = 32
DH = D // NH
W = 8
DIL = 2
H = S // 2
KH = D // 2
FC = 512
CH = FC // 2
NC = F // FC
RB = 256
NRB = H // RB
PAD = 16
TP = DH + 1
AR = 160
KPAD = 64

ATTN_SLOTS = (16, 168)
PACK_SLOTS = (118, 168)
DC_SLOTS = (16, 108)
BC_SLOTS = (2, 16)
ALIGN = 16
DEPTH = 3
PREP_LINK = True
PROFILE = ()
TIE = True

SCALE = DH ** -0.5
EXP2_SCALE = SCALE * math.log2(math.e)
NEG = -1e9 / SCALE


def _dot(a, b):
    return jnp.dot(a, b, preferred_element_type=f32)


def _a_combos(a11, a12, a21, a22):
    return [a11 + a22, a21 + a22, a11, a22, a11 + a12, a21 - a11, a12 - a22]


def _b_combos(b11, b12, b21, b22):
    return [b11 + b22, b11, b12 - b22, b21 - b11, b22, b11 + b12, b21 + b22]


_C_TERMS = (((1, 0), (1, 3), (-1, 4), (1, 6)), ((1, 2), (1, 4)), ((1, 1), (1, 3)),
            ((1, 0), (-1, 1), (1, 2), (1, 5)))


def _c_quadrant(m, qd):
    out = m[_C_TERMS[qd][0][1]]
    for sign, t in _C_TERMS[qd][1:]:
        out = out + m[t] if sign > 0 else out - m[t]
    return out


def _c_combos(m):
    return [_c_quadrant(m, qd) for qd in range(4)]


_A_SLOT = {0: 0, 1: 1, 4: 2, 5: 3, 6: 4}
_B_SLOT = {2: 0, 3: 1, 0: 2, 5: 3, 6: 4}
_ALL = {t: t for t in range(7)}


class _Scope:
    def __init__(self, name):
        self.cm = jax.named_scope(name) if (PROFILE is True or name in PROFILE) else None

    def __enter__(self):
        if self.cm is not None:
            self.cm.__enter__()

    def __exit__(self, *a):
        if self.cm is not None:
            self.cm.__exit__(*a)


def _tree(op, xs):
    xs = list(xs)
    while len(xs) > 1:
        xs = [op(xs[i], xs[i + 1]) if i + 1 < len(xs) else xs[i] for i in range(0, len(xs), 2)]
    return xs[0]


def _half(r):
    if isinstance(r, slice):
        return slice(r.start // 2, r.stop // 2)
    return pl.ds(r[0], r[1] // 2)


def _ld(ref, lead, r, c=slice(None)):
    return pltpu.bitcast(ref[lead + (_half(r), c)], bf16)


def _st(ref, lead, r, val, c=slice(None)):
    val = pltpu.bitcast(val, i32)
    ref[lead + (_half(r), c)] = val
    return val


SLOT = 256


class _Spreader:
    def __init__(self, zero_ref):
        self.zero_ref = zero_ref
        self.plan = {}
        self.now = 0

    def block(self):
        self.zero = self.zero_ref[...]
        self.never = self.zero != 0

    def link(self, after, x):
        if after is None or not TIE:
            return x
        if after.dtype != x.dtype:
            after = pltpu.bitcast(after, x.dtype)
        return jnp.where(self.never, after, x)

    def chain(self, vals, prev, depth):
        for v in vals:
            v = pltpu.bitcast(v, i32) if v.dtype != i32 else v
            for r in range(0, v.shape[0], 8):
                for c in range(0, v.shape[1], 128):
                    tile = v[r:r + 8, c:c + 128]
                    if prev is None:
                        prev = tile
                        continue
                    prev = (pltpu.bitcast(prev, i32) if prev.dtype != i32 else prev) | tile
                    for _ in range(depth - 1):
                        prev = (prev + self.zero) if _ % 2 == 0 else (prev ^ self.zero)
        return prev

    def schedule(self, tasks, first, last):
        n = len(tasks)
        for i, t in enumerate(tasks):
            pos = self.now + first + ((i + 1) * (last - first) - 1) // n
            self.plan.setdefault(pos, []).append(t)

    def dot(self, lhs, rhs):
        m, k = lhs.shape
        n = rhs.shape[1]
        tiles = [(r, c) for c in range(0, n, 128) for r in range(0, k, 128)]
        nslots = m * len(tiles) // (4 * SLOT)
        deps = {}
        for sl in range(nslots):
            ps = sl * SLOT // m
            for t in self.plan.pop(self.now + sl, []):
                tok = t(deps.get(ps))
                if tok is not None:
                    deps[ps] = tok
        self.now += nslots
        if deps and TIE:
            tied = {tile: d for ps, d in deps.items() for tile in tiles[4 * ps:4 * ps + 4]}
            parts = []
            for r in range(0, k, 128):
                top = [rhs[r:r + 16, c:c + 128] for c in range(0, n, 128)]
                for i, t0 in enumerate(top):
                    if (r, i * 128) in tied:
                        top[i] = pltpu.bitcast(
                            self.link(tied[r, i * 128], pltpu.bitcast(t0, i32)), bf16)
                parts += [jnp.concatenate(top, axis=1), rhs[r + 16:r + 128, :]]
            rhs = jnp.concatenate(parts, axis=0)
        return _dot(lhs, rhs)


def _kernel(x_hbm, wqkv_hbm, wo_hbm, wg_hbm, wu_hbm, wd_hbm, gw_hbm, out_hbm,
            x_vm, xn, xa, gw_vm, wgu, wd, bc, dc, acc, wqkv_vm, wp, q_s, k_s, v_s,
            gs, oa, wo_vm, woc, vbc, zs, zi, sems):
    sem_ids = iter(range(1000))

    def cp(src, dst):
        return pltpu.make_async_copy(src, dst, sems.at[next(sem_ids)])

    x2 = x_hbm.at[0]
    o2 = out_hbm.at[0]
    cp_gw = cp(gw_hbm, gw_vm)
    cp_x = [[cp(x2.at[pl.ds(hf * H + rb * RB, RB), :], x_vm.at[pl.ds(hf * H + rb * RB, RB), :])
             for hf in range(2)] for rb in range(NRB)]
    cp_gu = [[cp((wg_hbm, wu_hbm)[p % 2].at[:, pl.ds(j * FC + (p // 2) * CH, CH)],
                 wgu.at[j, :, pl.ds(p * CH, CH)]) for p in range(4)] for j in range(NC)]
    cp_d = [cp(wd_hbm.at[pl.ds(j * FC, FC), :], wd.at[j]) for j in range(NC)]
    cp_qkv = [cp(wqkv_hbm.at[:, pl.ds(i * D, D)], wqkv_vm.at[:, pl.ds(i * D, D)]) for i in range(3)]
    cp_wo = cp(wo_hbm, wo_vm)
    out_sem = _N_SEMS - 2 * NRB - 2
    cp_out = [[cp(x_vm.at[pl.ds(hf * H + rb * RB, RB), :], o2.at[pl.ds(hf * H + rb * RB, RB), :])
               for hf in range(2)] for rb in range(NRB - 1)]
    last = [(pl.ds((qd // 2) * H + H - RB, RB), pl.ds((qd % 2) * KH, KH)) for qd in range(4)]
    cp_out.append([cp(x_vm.at[idx], o2.at[idx]) for idx in last])

    def start(cs):
        for c in cs:
            c.start()

    def wait(cs):
        for c in cs:
            c.wait()

    start([cp_x[0][0]] + cp_gu[0] + [cp_x[0][1], cp_gw])

    zs[...] = jnp.zeros((8, 128), i32)
    zi[0] = 1
    sp = _Spreader(zs)

    def rows(rb, hf=0):
        return slice(hf * H + rb * RB, hf * H + (rb + 1) * RB)

    def x_lhs(t, rb):
        if t == 2:
            return _ld(xn, (), rows(rb, 0), slice(0, KH))
        if t == 3:
            return _ld(xn, (), rows(rb, 1), slice(KH, D))
        return _ld(xa, (_A_SLOT[t],), rows(rb))

    def prep_tasks(rb, sums=True, gate=True):
        def task(s0):
            def run(first):
                prev = None
                gw = gw_vm[...].astype(f32)
                r = [slice(hf * H + rb * RB + s0, hf * H + rb * RB + s0 + 16) for hf in range(2)]
                z = [None, None]
                for c in range(4):
                    cols = [slice(kh * KH + c * 128, kh * KH + (c + 1) * 128) for kh in range(2)]
                    xs = [sp.link(prev if PREP_LINK else None, pltpu.bitcast(x_vm[r[qd // 2], cols[qd % 2]], i32))
                          for qd in range(4)]
                    a = [pltpu.bitcast(t, bf16).astype(f32) for t in xs]
                    outs = []
                    if sums:
                        for qd in range(4):
                            xn[_half(r[qd // 2]), cols[qd % 2]] = xs[qd]
                        cs = _a_combos(*a)
                        outs = [_st(xa, (slot,), r[0], cs[t].astype(bf16), cols[0])
                                for t, slot in _A_SLOT.items()]
                    if gate:
                        for qd in range(4):
                            g0 = (qd % 2) * 4 + c
                            term = a[qd] * gw[g0:g0 + 1, :]
                            z[qd // 2] = term if z[qd // 2] is None else z[qd // 2] + term
                        outs += z
                    prev = sp.chain(outs, prev, 1)
                if gate:
                    for hf in range(2):
                        g = jax.nn.sigmoid(jnp.sum(z[hf], axis=1, keepdims=True))
                        g = jnp.broadcast_to(g, (16, 128))
                        gs[r[hf], :] = g
                        prev = sp.chain([g], prev, 1)
                return sp.chain([prev], first, 1)
            return run
        return [task(s0) for s0 in range(0, RB, 16)]

    def b_combo_tasks(src, dst, kh, nh, slots, sub=16):
        def task(r0):
            def run(prev):
                raw = [src(slice(a * kh + r0, a * kh + r0 + sub), slice(c * nh, (c + 1) * nh))
                       for a in range(2) for c in range(2)]
                cs = [c.astype(bf16) for c in _b_combos(*[b.astype(f32) for b in raw])]
                cs[1], cs[4] = raw[0], raw[3]
                return sp.chain([_st(dst, (slot,), slice(r0, r0 + sub), cs[t])
                                 for t, slot in slots.items()], prev, DEPTH)
            return run
        return [task(r0) for r0 in range(0, kh, sub)]

    ORDER = (1, 4, 2, 3, 0, 5, 6)

    def strassen_x(order, rhs, finish):
        m = {}
        for rb, t in order:
            m.setdefault(rb, {})[t] = sp.dot(x_lhs(t, rb), rhs(t))
            if len(m[rb]) == 7:
                finish(rb, _c_combos(m.pop(rb)))

    def gu_rhs(j):
        def rhs(t):
            if t == 1:
                return wgu[j, :KH, :FC]
            if t == 4:
                return wgu[j, KH:, FC:]
            return _ld(bc, (_B_SLOT[t],), slice(0, KH))
        return rhs

    def glu_tasks(ha, rb, cs, sub):
        ha[rb] = [[] for _ in range(7)]

        def task(r0):
            def run(prev=None):
                hs = []
                for qd, cc in enumerate(cs):
                    g0 = (qd // 2) * H + rb * RB + r0
                    omg = 1.0 - gs[g0:g0 + sub, :]
                    omg = jnp.concatenate([omg] * (CH // 128), axis=1)
                    hs.append(jnp.maximum(cc[r0:r0 + sub, :CH], 0.0) * cc[r0:r0 + sub, CH:] * omg)
                sums = _a_combos(*hs)
                for t in range(7):
                    ha[rb][t].append(sums[t].astype(bf16))
                if sub < RB:
                    return sp.chain([sums[t][:8, :] for t in (0, 1, 4, 5, 6)], prev, DEPTH)
            return run
        return [task(r0) for r0 in range(0, RB, sub)]

    def glu(ha):
        return lambda rb, cs: glu_tasks(ha, rb, cs, RB)[0]()

    def ffn_down(j, rb, ha, first):
        for t in ORDER:
            p = sp.dot(jnp.concatenate(ha[rb][t], axis=0), _ld(dc, (t,), slice(0, CH)))
            if first:
                acc[t, rows(rb), :] = p
            else:
                acc[t, rows(rb), :] += p

    def perm_tasks(i, tbuf):
        def fwd(rb, c):
            def run(prev):
                c0 = i * D + c * 128
                tt = pltpu.bitcast(wqkv_vm[rb * 256:(rb + 1) * 256, c0:c0 + 128], f32).T
                for hh in range(4):
                    tbuf[rb, pl.ds((4 * c + hh) * TP, DH), :] = tt[hh * DH:(hh + 1) * DH, :]
                return sp.chain([tt], prev, 1)
            return run

        def bwd(rb, j):
            def run(prev):
                g = jnp.concatenate(
                    [tbuf[rb, pl.ds(4 * j + dd, NH, stride=TP), :] for dd in range(4)], axis=0).T
                wp[i, rb * 128:(rb + 1) * 128, j * 128:(j + 1) * 128] = pltpu.bitcast(g, i32)
            return run
        tasks = []
        for rb in range(4):
            tasks += [fwd(rb, c) for c in range(8)] + [bwd(rb, j) for j in range(8)]
        return tasks

    def wo_tasks():
        def stage(c):
            return 4 + c % 4, (c // 4) * NH * TP

        def spread(h0):
            def run(prev):
                blk = wo_vm[h0 * DH:(h0 + 2) * DH, :].astype(f32)
                for h in range(2):
                    for c in range(8):
                        sl, r0 = stage(c)
                        v_s[sl, pl.ds(r0 + (h0 + h) * TP, DH), :] = (
                            blk[h * DH:(h + 1) * DH, c * 128:(c + 1) * 128])
                return sp.chain([blk], prev, 1)
            return run

        def gather(d):
            def run(prev):
                def tile(rh, c):
                    sl, r0 = stage(c)
                    return v_s[sl, pl.ds(r0 + 16 * rh + d, NH, stride=TP), :]
                b = [jnp.concatenate([tile(rh, 4 * ch + c) for c in range(4)], axis=1)
                     for rh in range(2) for ch in range(2)]
                cs = [c.astype(bf16) for c in _b_combos(*b)]
                return sp.chain([_st(woc, (t,), slice(d * NH, (d + 1) * NH), cs[t])
                                 for t in range(7)], prev, DEPTH)
            return run
        return [spread(h0) for h0 in range(0, NH, 2)], [gather(d) for d in range(16)]

    def proj(i, dst, pad, rb):
        r0 = rb * 2 * RB
        p = sp.dot(_ld(xn, (), slice(r0, r0 + 2 * RB)), _ld(wp, (i,), slice(0, D)))
        for j in range(8):
            dst[j, pad + r0:pad + r0 + 2 * RB, :] = p[:, j * 128:(j + 1) * 128]

    def v_finish(rb, cs):
        for qd, cc in enumerate(cs):
            r0 = PAD + (qd // 2) * H + rb * RB
            for j in range(4):
                v_s[(qd % 2) * 4 + j, r0:r0 + RB, :] = cc[:, j * 128:(j + 1) * 128]
        if rb == 0:
            for j in range(8):
                src = cs[j // 4][0:1, (j % 4) * 128:(j % 4 + 1) * 128]
                v_s[j, 0:PAD, :] = jnp.broadcast_to(src, (PAD, 128))

    def attn_group(row, masked):
        def run(prev):
            g = 8
            q = [q_s[j, pl.ds(row + AR, g), :] for j in range(8)]
            ls = []
            for w in range(W):
                a = None
                for j in range(8):
                    term = q[j] * k_s[j, pl.ds(row + (PAD - DIL * w), g), :]
                    a = sp.link(ls[-1] if ls else None, term) if a is None else a + term
                ls.append(a)
            rs = [pltpu.roll(a, 64, 1) for a in ls]
            ls = [a + r for a, r in zip(ls, rs)]
            rs = [pltpu.roll(a, 32, 1) for a in ls]
            ls = [a + r for a, r in zip(ls, rs)]
            if masked:
                ri = row + lax.broadcasted_iota(i32, (g, 128), 0)
                ls = [ls[0]] + [jnp.where(ri >= DIL * w, ls[w], NEG) for w in range(1, W)]
            m = _tree(jnp.maximum, ls)
            ps = [jnp.exp2((l - m) * EXP2_SCALE) for l in ls]
            r = gs[pl.ds(row, g), :] / _tree(jnp.add, ps)
            outs = []
            for j in range(8):
                a = None
                for w in range(W):
                    term = ps[w] * v_s[j, pl.ds(row + (PAD - DIL * w), g), :]
                    a = sp.link(outs[-1] if outs else None, term) if a is None else a + term
                outs.append(a * r)
            for j in range(8):
                q_s[j, pl.ds(row + AR, g), :] = outs[j]
            return sp.chain([outs[-1]], prev, 1)
        return run

    def attn_tasks(base, nrows, first=False):
        return [attn_group(base + (hf * H + r), first and hf == 0 and r < PAD)
                for r in range(0, nrows, 8) for hf in range(2)]

    def pack_tasks(base, hbase, nrows):
        def task(r):
            def run(prev):
                o = [jnp.concatenate([q_s[4 * ch + j, pl.ds(base + (hf * H + r), 16), :]
                                      for j in range(4)], axis=1)
                     for hf in range(2) for ch in range(2)]
                cs = [c.astype(bf16) for c in _a_combos(*o)]
                return sp.chain([_st(oa, (t,), (hbase + r // 2, 16), cs[t]) for t in range(7)],
                                prev, DEPTH)
            return run
        return [task(r) for r in range(0, nrows, 16)]

    def gu_tasks(j):
        return b_combo_tasks(lambda r, c: wgu[j, r, c], bc, KH, FC, _B_SLOT)

    def d_tasks(j):
        return b_combo_tasks(lambda r, c: wd[j, r, c], dc, CH, KH, _ALL)

    GS = RB * (KH // 128) * (FC // 128) * 7 // (4 * SLOT)
    DS = RB * (CH // 128) * (KH // 128) * 7 // (4 * SLOT)
    PS = 2 * RB * (D // 128) * (D // 128) // (4 * SLOT)

    def plain(rb, hf, p):
        return sp.dot(x_vm[rows(rb, hf), :], wgu[0, :, p * CH:(p + 1) * CH])

    def plain_finish(rb, c, sub):
        cs = [jnp.concatenate(c[2 * qd:2 * qd + 2], axis=1) for qd in range(4)]
        return glu_tasks(ha, rb, cs, sub)

    ha = {}
    c0 = []
    with _Scope("w0"):
        wait([cp_x[0][0], cp_gu[0][0]])
    with _Scope("p1a"):
        for p in range(4):
            if p:
                wait([cp_gu[0][p]])
            if p == 1:
                start(cp_x[1] + cp_x[2])
            c0.append(plain(0, 0, p))
        wait([cp_x[0][1], cp_gw])
        start(cp_x[3] + [cp_d[0]])
        sp.block()
        gu0 = gu_tasks(0)
        sp.schedule(gu0[:12], 3, 16)
        sp.schedule(prep_tasks(0, sums=False), 3, 16)
        c0 += [plain(0, 1, p) for p in range(4)]
    with _Scope("w1"):
        wait(cp_x[1] + cp_x[2])
        start(cp_qkv[:1])
    with _Scope("p1b"):
        sp.block()
        sp.schedule(gu0[12:], 3, 32)
        sp.schedule(prep_tasks(1, sums=False), 2, 10)
        sp.schedule(prep_tasks(2), 10, 32)
        c1 = [plain(1, hf, p) for hf in range(2) for p in range(4)]
    with _Scope("w2"):
        wait(cp_x[3] + [cp_d[0]] + cp_qkv[:1])
        start(cp_qkv[1:] + [cp_wo])
        for j in range(1, NC):
            start(cp_gu[j] + [cp_d[j]])
    with _Scope("p1c"):
        sp.block()
        for j in range(8):
            k_s[j, 0:PAD, :] = jnp.zeros((PAD, 128), f32)
            q_s[j, 0:AR, :] = jnp.zeros((AR, 128), f32)
        sp.schedule(prep_tasks(3), 2, GS)
        sp.schedule(plain_finish(0, c0, 16), 2, GS)
        sp.schedule(plain_finish(1, c1, 16), GS + 6, 2 * GS)
        sp.schedule(d_tasks(0), GS + 6, 2 * GS)
        sp.schedule(prep_tasks(0, gate=False) + prep_tasks(1, gate=False), 2 * GS + 6, 2 * GS + 4 * DS)
        sp.schedule(perm_tasks(0, q_s.at[:, AR:, :]), 2 * GS + 6, 2 * GS + 4 * DS - 8)
        strassen_x([(rb, t) for rb in (2, 3) for t in ORDER], gu_rhs(0), glu(ha))
        for rb in range(NRB):
            ffn_down(0, rb, ha, True)

    with _Scope("w2b"):
        wait(cp_qkv[1:] + [cp_wo])
    with _Scope("q"):
        sp.block()
        wo_spread, wo_gather = wo_tasks()
        sp.schedule(perm_tasks(1, k_s.at[:, PAD:, :]) + perm_tasks(2, v_s), 4, NRB * PS - 8)
        sp.schedule(wo_spread, 4, NRB * PS - 8)
        for rb in range(NRB):
            proj(0, q_s, AR, rb)
    with _Scope("w3"):
        for j in range(1, NC):
            wait(cp_gu[j] + [cp_d[j]])
    with _Scope("kv"):
        sp.block()
        sp.schedule(wo_gather + b_combo_tasks(lambda r, c: _ld(wp, (2,), r, c), vbc, KH, KH, _ALL),
                    4, NRB * PS)
        for rb in range(NRB):
            proj(1, k_s, PAD, rb)
        v_rhs = lambda t: _ld(vbc, (t,), slice(0, KH))
        strassen_x([(0, t) for t in ORDER], v_rhs, v_finish)

    def v_rest(_, carry):
        with _Scope("v"):
            strassen_x([(rb, t) for rb in range(1, NRB) for t in ORDER], v_rhs, v_finish)
        return carry

    lax.fori_loop(0, zi[0], v_rest, 0)

    def body(j, carry):
        with _Scope("chunk"):
            sp.block()
            base = pl.multiple_of((j - 1) * AR, ALIGN)
            ha = {}
            sp.schedule(gu_tasks(j), *BC_SLOTS)
            sp.schedule(attn_tasks(base, AR, True), *ATTN_SLOTS)
            sp.schedule(pack_tasks(base, pl.multiple_of((j - 1) * (AR // 2), ALIGN // 2), AR), *PACK_SLOTS)
            sp.schedule(d_tasks(j), *DC_SLOTS)
            strassen_x([(rb, t) for rb in (0, 1) for t in ORDER[:2]]
                       + [(rb, t) for rb in (0, 1) for t in ORDER[2:]]
                       + [(rb, t) for rb in (2, 3) for t in ORDER], gu_rhs(j), glu(ha))
            for rb in range(NRB):
                ffn_down(j, rb, ha, False)
        return carry

    lax.fori_loop(1, NC, body, 0)

    def out_block(r0, copies):
        m = {}
        r = [pl.ds(r0 + hf * H, RB) for hf in range(2)]
        for ts, qd in (((2, 4), 1), ((1, 3), 2), ((0, 6), 0), ((5,), 3)):
            for t in ts:
                lhs = _ld(oa, (t,), ((r0 + AR) // 2 if isinstance(r0, int)
                                     else pl.multiple_of((r0 + AR) // 2, 16), RB))
                m[t] = acc[t, r[0], :] + sp.dot(lhs, _ld(woc, (t,), slice(0, KH)))
            x_vm[r[qd // 2], (qd % 2) * KH:(qd % 2 + 1) * KH] = _c_quadrant(m, qd).astype(bf16)
            start(copies.get(qd, []))

    done = (NC - 1) * AR
    rest = H - done

    def out_copy(r0, hf, sem):
        idx = (pl.ds(r0 + hf * H, RB), slice(None))
        return pltpu.make_async_copy(x_vm.at[idx], o2.at[idx], sems.at[sem])

    def out_body(i, carry):
        with _Scope("p4a"):
            sp.block()
            arow = pl.multiple_of(done + i * (rest // 2), 32)
            prow = pl.multiple_of(i * (AR // 4), 8)
            sp.schedule(attn_tasks(arow, rest // 2), 2, GS)
            sp.schedule(pack_tasks(done + 2 * prow, done // 2 + prow, AR // 2), 2, GS)
            r0 = pl.multiple_of(i * RB, RB)
            out_block(r0, {3: [out_copy(r0, hf, out_sem + 2 * i + hf) for hf in range(2)]})
        return carry

    lax.fori_loop(0, 2, out_body, 0)
    with _Scope("p4b"):
        sp.block()
        sp.schedule(pack_tasks(done + AR, (done + AR) // 2, rest), 2, GS)
        out_block(2 * RB, {3: cp_out[2]})
        out_block(3 * RB, {qd: [cp_out[3][qd]] for qd in range(4)})
    with _Scope("w4"):
        for rb in range(NRB):
            wait(cp_out[rb])
    assert not sp.plan


_N_SEMS = 1 + 2 * NRB + 4 * NC + NC + 3 + 1 + 2 * NRB + 2


@jax.jit
def pallas_gated_mix__sliding_local_dilated__glu_gated_reglu__prompt_kernel(
    A_x: jax.Array,
    A_wqkv: jax.Array,
    A_wo: jax.Array,
    B_x: jax.Array,
    B_W_gate: jax.Array,
    B_W_up: jax.Array,
    B_W_down: jax.Array,
    gate_w: jax.Array,
):
    del B_x
    hbm = pl.BlockSpec(memory_space=pl.ANY)
    scratch = [
        pltpu.VMEM((S, D), bf16),
        pltpu.VMEM((S // 2, D), i32),
        pltpu.VMEM((5, H // 2, KH), i32),
        pltpu.VMEM((8, 128), bf16),
        pltpu.VMEM((NC, D, 2 * FC), bf16),
        pltpu.VMEM((NC, FC, D), bf16),
        pltpu.VMEM((5, KH // 2, FC), i32),
        pltpu.VMEM((7, CH // 2, KH), i32),
        pltpu.VMEM((7, H, KH), f32),
        pltpu.VMEM((D, 3 * D), bf16),
        pltpu.VMEM((3, D // 2, D), i32),
        pltpu.VMEM((8, AR + S, 128), f32),
        pltpu.VMEM((8, PAD + S + KPAD, 128), f32),
        pltpu.VMEM((8, PAD + S + KPAD, 128), f32),
        pltpu.VMEM((S, 128), f32),
        pltpu.VMEM((7, (AR + H) // 2, KH), i32),
        pltpu.VMEM((D, D), bf16),
        pltpu.VMEM((7, KH // 2, KH), i32),
        pltpu.VMEM((7, KH // 2, KH), i32),
        pltpu.VMEM((8, 128), i32),
        pltpu.SMEM((1,), i32),
        pltpu.SemaphoreType.DMA((_N_SEMS,)),
    ]
    return pl.pallas_call(
        _kernel,
        in_specs=[hbm] * 7,
        out_specs=hbm,
        out_shape=jax.ShapeDtypeStruct((1, S, D), bf16),
        scratch_shapes=scratch,
        compiler_params=pltpu.CompilerParams(vmem_limit_bytes=124 * 1024 * 1024),
    )(A_x, A_wqkv, A_wo, B_W_gate, B_W_up, B_W_down, gate_w.reshape(8, 128))
```

```python
import math

import jax
import jax.numpy as jnp
from jax import lax
import jax.experimental.pallas as pl
import jax.experimental.pallas.tpu as pltpu

f32 = jnp.float32
bf16 = jnp.bfloat16
i32 = jnp.int32

S = 2048
D = 1024
F = 3584
NH = 32
DH = D // NH
W = 8
DIL = 2
H = S // 2
Q = S // 4
KH = D // 2
KQ = D // 4
FC = 512
CH = FC // 2
CQ = FC // 4
NC = F // FC
RB = 256
NRB = H // RB
PB = 128
PAD = 16
TP = DH + 1
AR = 96
KPAD = 64

ATTN_SLOTS = (38, 112)
PACK_SLOTS = (16, 38)
DC_SLOTS = (38, 108)
BC_SLOTS = (2, 16)
DEPTH = 3
DEPTH2 = 3
H_DEPTH = 3
LEAD = 0
PROFILE = ()

SCALE = DH ** -0.5
EXP2_SCALE = SCALE * math.log2(math.e)
NEG = -1e9 / SCALE


def _a_combos(a11, a12, a21, a22):
    return [a11 + a22, a21 + a22, a11, a22, a11 + a12, a21 - a11, a12 - a22]


def _b_combos(b11, b12, b21, b22):
    return [b11 + b22, b11, b12 - b22, b21 - b11, b22, b11 + b12, b21 + b22]


_C_TERMS = (((1, 0), (1, 3), (-1, 4), (1, 6)), ((1, 2), (1, 4)), ((1, 1), (1, 3)),
            ((1, 0), (-1, 1), (1, 2), (1, 5)))
_C_ORDER = (((2, 4), 1), ((1, 3), 2), ((0, 6), 0), ((5,), 3))


def _c_quadrant(m, qd):
    out = m[_C_TERMS[qd][0][1]]
    for sign, t in _C_TERMS[qd][1:]:
        out = out + m[t] if sign > 0 else out - m[t]
    return out


def _c_combos(m):
    return [_c_quadrant(m, qd) for qd in range(4)]


_A_SLOT = {0: 0, 1: 1, 4: 2, 5: 3, 6: 4}
_B_SUMS = (2, 3, 0, 5, 6)
ORDER = (1, 4) + _B_SUMS


class _Scope:
    def __init__(self, name):
        self.cm = jax.named_scope(name) if (PROFILE is True or name in PROFILE) else None

    def __enter__(self):
        if self.cm is not None:
            self.cm.__enter__()

    def __exit__(self, *a):
        if self.cm is not None:
            self.cm.__exit__(*a)


def _tree(op, xs):
    xs = list(xs)
    while len(xs) > 1:
        xs = [op(xs[i], xs[i + 1]) if i + 1 < len(xs) else xs[i] for i in range(0, len(xs), 2)]
    return xs[0]


def _pack(x):
    return pltpu.bitcast(x.astype(bf16), i32)


def _unpack(x):
    return pltpu.bitcast(x, bf16)


def _half(r):
    return slice(r.start // 2, r.stop // 2)


SLOT = 256


class _Spreader:
    def __init__(self, zero_ref):
        self.zero_ref = zero_ref
        self.plan = {}
        self.tokens = {}
        self.now = 0

    def block(self):
        self.zero = self.zero_ref[...]
        self.never = self.zero != 0

    def link(self, after, x):
        if after is None:
            return x
        if after.dtype != x.dtype:
            after = pltpu.bitcast(after, x.dtype)
        return jnp.where(self.never, after, x)

    def chain(self, vals, prev, depth):
        for v in vals:
            v = pltpu.bitcast(v, i32) if v.dtype != i32 else v
            for r in range(0, v.shape[0], 8):
                for c in range(0, v.shape[1], 128):
                    tile = v[r:r + 8, c:c + 128]
                    if prev is None:
                        prev = tile
                        continue
                    prev = prev | tile
                    for i in range(depth - 1):
                        prev = (prev + self.zero) if i % 2 == 0 else (prev ^ self.zero)
        return prev

    def link_rows(self, after, x):
        return jnp.concatenate([self.link(after, x[r:r + 8, :]) for r in range(0, x.shape[0], 8)],
                               axis=0)

    def serial_combos(self, combos, x11, x12, x21, x22, after):
        return combos(self.link_rows(after, x11), x12, x21, self.link_rows(after, x22))

    def two_level(self, combos, blk, prev, depth):
        outer = [combos(*[blk(r1, r2, c1, c2) for r1 in range(2) for c1 in range(2)])
                 for r2 in range(2) for c2 in range(2)]
        outs, tok = [], None
        for t in range(7):
            outs += [_pack(x) for x in self.serial_combos(combos, *[o[t] for o in outer], tok)]
            tok = self.chain(outs[-7:], tok, depth)
        return outs, self.chain([tok], prev, 1)

    def schedule(self, tasks, first, last):
        n = len(tasks)
        for i, t in enumerate(tasks):
            pos = self.now + first + ((i + 1) * (last - first) - 1) // n
            self.plan.setdefault(pos, []).append(t)

    def dots(self, pairs):
        m = pairs[0][0].shape[0]
        tiles = [(i, r, c) for i, (_, rhs) in enumerate(pairs)
                 for c in range(0, rhs.shape[1], 128) for r in range(0, rhs.shape[0], 128)]
        nslots = m * len(tiles) // (4 * SLOT)
        for sl in range(self.now, self.now + nslots + LEAD):
            for t in self.plan.pop(sl, []):
                tok = t(self.tokens.get(sl))
                if tok is not None:
                    self.tokens[sl] = tok
        deps = {}
        for sl in range(nslots):
            ps = sl * SLOT // m
            tok = self.tokens.pop(self.now + sl, None)
            if tok is not None:
                deps[ps] = tok | deps[ps] if ps in deps else tok
        self.now += nslots
        tied = {tile: d for ps, d in deps.items() for tile in tiles[4 * ps:4 * ps + 4]}
        outs = []
        for i, (lhs, rhs) in enumerate(pairs):
            if any(key[0] == i for key in tied):
                parts = []
                for r in range(0, rhs.shape[0], 128):
                    top = [rhs[r:r + 16, c:c + 128] for c in range(0, rhs.shape[1], 128)]
                    top = [_unpack(self.link(tied[i, r, c * 128], _pack(t0)))
                           if (i, r, c * 128) in tied else t0 for c, t0 in enumerate(top)]
                    parts += [jnp.concatenate(top, axis=1), rhs[r + 16:r + 128, :]]
                rhs = jnp.concatenate(parts, axis=0)
            outs.append(jnp.dot(lhs, rhs, preferred_element_type=f32))
        return outs

    def dot(self, lhs, rhs):
        return self.dots([(lhs, rhs)])[0]


def _kernel(x_hbm, wqkv_hbm, wo_hbm, wg_hbm, wu_hbm, wd_hbm, gw_hbm, out_hbm,
            x_vm, xn, xa, gw_vm, wgu, wd, acc, q_s, k_s, v_s, gs, woc, zs, zi, sems):
    sem_ids = iter(range(10, 1000))

    def cp(src, dst, sem=None):
        return pltpu.make_async_copy(src, dst, sems.at[next(sem_ids) if sem is None else sem])

    def cp_gu(j, slot):
        col = j * FC if isinstance(j, int) else pl.multiple_of(j * FC, FC)
        return [cp((wg_hbm, wu_hbm)[p % 2].at[:, pl.ds(col + (p // 2) * CH, CH)],
                   wgu.at[slot, :, pl.ds(p * CH, CH)], slot * 5 + p) for p in range(4)]

    def cp_d(j, slot):
        row = j * FC if isinstance(j, int) else pl.multiple_of(j * FC, FC)
        return [cp(wd_hbm.at[pl.ds(row, FC), :], wd.at[slot], slot * 5 + 4)]

    x2 = x_hbm.at[0]
    o2 = out_hbm.at[0]
    cp_gw = cp(gw_hbm, gw_vm)
    cp_x = [[cp(x2.at[pl.ds(hf * H + rb * RB, RB), :], x_vm.at[pl.ds(hf * H + rb * RB, RB), :])
             for hf in range(2)] for rb in range(NRB)]
    out_sem = _N_SEMS - 20

    def start(cs):
        for c in cs:
            c.start()

    def wait(cs):
        for c in cs:
            c.wait()

    gu0 = cp_gu(0, 0)
    start([cp_x[0][0]] + gu0 + [cp_x[0][1], cp_gw])

    zs[...] = jnp.zeros((8, 128), i32)
    zi[0] = 1
    sp = _Spreader(zs)

    def rows(rb, hf=0):
        return slice(hf * H + rb * RB, hf * H + (rb + 1) * RB)

    def x_lhs(t, rb):
        if t == 2:
            return _unpack(xn[_half(rows(rb, 0)), :KH])
        if t == 3:
            return _unpack(xn[_half(rows(rb, 1)), KH:])
        return _unpack(xa[_A_SLOT[t], _half(rows(rb)), :])

    def prep_tasks(rb, sums=True, gate=True):
        def task(s0):
            def run(first):
                prev = None
                gw = gw_vm[...].astype(f32)
                r = [slice(hf * H + rb * RB + s0, hf * H + rb * RB + s0 + 16) for hf in range(2)]
                z = [None, None]
                for c in range(4):
                    cols = [slice(kh * KH + c * 128, kh * KH + (c + 1) * 128) for kh in range(2)]
                    xs = [sp.link(prev, _pack(x_vm[r[qd // 2], cols[qd % 2]])) for qd in range(4)]
                    a = [_unpack(t).astype(f32) for t in xs]
                    outs = []
                    if sums:
                        for qd in range(4):
                            xn[_half(r[qd // 2]), cols[qd % 2]] = xs[qd]
                        cs = _a_combos(*a)
                        for t, slot in _A_SLOT.items():
                            outs.append(_pack(cs[t]))
                            xa[slot, _half(r[0]), cols[0]] = outs[-1]
                    if gate:
                        for qd in range(4):
                            g0 = (qd % 2) * 4 + c
                            term = a[qd] * gw[g0:g0 + 1, :]
                            z[qd // 2] = term if z[qd // 2] is None else z[qd // 2] + term
                        outs += z
                    prev = sp.chain(outs, prev, 1)
                if gate:
                    for hf in range(2):
                        g = jax.nn.sigmoid(jnp.sum(z[hf], axis=1, keepdims=True))
                        g = jnp.broadcast_to(g, (16, 128))
                        gs[r[hf], :] = g
                        prev = sp.chain([g], prev, 1)
                return sp.chain([prev], first, 1)
            return run
        return [task(s0) for s0 in range(0, RB, 16)]

    def b_sum_tasks(src, dst):
        def task(r0):
            def run(prev):
                raw = [src(slice(a * KH + r0, a * KH + r0 + 16), slice(c * KH, (c + 1) * KH))
                       for a in range(2) for c in range(2)]
                cs = _b_combos(*[b.astype(f32) for b in raw])
                for t in _B_SUMS:
                    dst.setdefault(t, []).append(_pack(cs[t]))
                return sp.chain([dst[t][-1] for t in _B_SUMS], prev, DEPTH)
            return run
        return [task(r0) for r0 in range(0, KH, 16)]

    def b_rhs(src, sums):
        def rhs(t):
            if t == 1:
                return src(slice(0, KH), slice(0, KH))
            if t == 4:
                return src(slice(KH, D), slice(KH, D))
            return _unpack(jnp.concatenate(sums[t], axis=0))
        return rhs

    def strassen_x(order, rhs, finish):
        m = {}
        for rb, t in order:
            m.setdefault(rb, {})[t] = sp.dot(x_lhs(t, rb), rhs(t))
            if len(m[rb]) == 7:
                finish(rb, _c_combos(m.pop(rb)))

    def glu_tasks(hs, rb, cs, sub):
        hs[rb] = [[] for _ in range(7)]

        def task(r0):
            def run(prev=None):
                h = []
                for qd, cc in enumerate(cs):
                    g0 = (qd // 2) * H + rb * RB + r0
                    omg = 1.0 - gs[g0:g0 + sub, :]
                    omg = jnp.concatenate([omg] * (CH // 128), axis=1)
                    h.append(jnp.maximum(cc[r0:r0 + sub, :CH], 0.0) * cc[r0:r0 + sub, CH:] * omg)
                sums = _a_combos(*h)
                for t in range(7):
                    hs[rb][t].append(sums[t])
                if sub < RB:
                    return sp.chain([sums[t] for t in _A_SLOT], prev, DEPTH2)
            return run
        return [task(r0) for r0 in range(0, RB, sub)]

    def down_lhs(hs, b, ha):
        tok = None
        for t in range(7):
            s0, s1 = [jnp.concatenate(hs[rb][t], axis=0) for rb in (b, b + 2)]
            slabs = []
            for r in range(0, RB, 16):
                slabs.append(sp.serial_combos(
                    _a_combos, s0[r:r + 16, :CQ], s0[r:r + 16, CQ:],
                    s1[r:r + 16, :CQ], s1[r:r + 16, CQ:], tok))
                tok = sp.chain([slabs[-1][t2] for t2 in _A_SLOT], None, H_DEPTH)
            for t2 in range(7):
                ha[b, 7 * t + t2] = jnp.concatenate([sl[t2] for sl in slabs], axis=0).astype(bf16)

    def d_tasks(slot, dst):
        def task(r0, c):
            def run(prev):
                def blk(k1, k2, n1, n2):
                    r, c0 = k1 * CH + k2 * CQ + r0, n1 * KH + n2 * KQ + c * 128
                    return wd[slot, r:r + 16, c0:c0 + 128].astype(f32)
                cs, tok = sp.two_level(_b_combos, blk, prev, DEPTH2)
                for t in range(49):
                    dst.setdefault((t, c), []).append(cs[t])
                return tok
            return run
        return [task(r0, c) for r0 in range(0, CQ, 16) for c in range(2)]

    def ffn_down(ha, dc, first):
        rhs = [_unpack(jnp.concatenate([jnp.concatenate(dc[t, c], axis=0) for c in range(2)], axis=1))
               for t in range(49)]
        todo = [(b, t) for b in range(2) for t in range(49)]
        for i in range(0, len(todo), 2):
            pair = todo[i:i + 2]
            ps = sp.dots([(ha[b, t], rhs[t]) for b, t in pair])
            for (b, t), p in zip(pair, ps):
                if first:
                    acc[t, b * RB:(b + 1) * RB, :] = p
                else:
                    acc[t, b * RB:(b + 1) * RB, :] += p

    def perm_tasks(wqkv_vm, wp, i, tbuf):
        def fwd(rb, c):
            def run(prev):
                c0 = i * D + c * 128
                tt = pltpu.bitcast(wqkv_vm[rb * 256:(rb + 1) * 256, c0:c0 + 128], f32).T
                for hh in range(4):
                    tbuf[rb, pl.ds((4 * c + hh) * TP, DH), :] = tt[hh * DH:(hh + 1) * DH, :]
                return sp.chain([tt], prev, 1)
            return run

        def bwd(rb, j):
            def run(prev):
                g = jnp.concatenate(
                    [tbuf[rb, pl.ds(4 * j + dd, NH, stride=TP), :] for dd in range(4)], axis=0).T
                wp[i, rb * 128:(rb + 1) * 128, j * 128:(j + 1) * 128] = pltpu.bitcast(g, i32)
            return run
        tasks = []
        for rb in range(4):
            tasks += [fwd(rb, c) for c in range(8)] + [bwd(rb, j) for j in range(8)]
        return tasks

    def wo_tasks(wo_vm):
        def stage(c):
            return 4 + c % 4, (c // 4) * NH * TP

        def spread(h0):
            def run(prev):
                blk = wo_vm[h0 * DH:(h0 + 2) * DH, :].astype(f32)
                for h in range(2):
                    for c in range(8):
                        sl, r0 = stage(c)
                        v_s[sl, pl.ds(r0 + (h0 + h) * TP, DH), :] = (
                            blk[h * DH:(h + 1) * DH, c * 128:(c + 1) * 128])
                return sp.chain([blk], prev, 1)
            return run

        def gather(d, h0, c):
            def run(prev):
                def blk(k1, k2, n1, n2):
                    sl, r0 = stage(4 * n1 + 2 * n2 + c)
                    r0 += h0 * TP + 16 * k1 + 8 * k2 + d
                    return v_s[sl, pl.ds(r0, 16, stride=TP), :]
                cs, tok = sp.two_level(_b_combos, blk, prev, DEPTH2)
                r = (d * NH + h0) // 2
                for t in range(49):
                    woc[t, r:r + 8, c * 128:(c + 1) * 128] = cs[t]
                return tok
            return run
        return ([spread(h0) for h0 in range(0, NH, 2)],
                [gather(d, h0, c) for d in range(8) for h0 in (0, 16) for c in range(2)])

    def proj(wp, i, dst, pad, rb):
        r0 = rb * 2 * RB
        p = sp.dot(_unpack(xn[r0 // 2:r0 // 2 + RB, :]), _unpack(wp[i]))
        for j in range(8):
            dst[j, pad + r0:pad + r0 + 2 * RB, :] = p[:, j * 128:(j + 1) * 128]

    def v_finish(rb, cs):
        for qd, cc in enumerate(cs):
            r0 = PAD + (qd // 2) * H + rb * RB
            for j in range(4):
                v_s[(qd % 2) * 4 + j, r0:r0 + RB, :] = cc[:, j * 128:(j + 1) * 128]
        if rb == 0:
            for j in range(8):
                src = cs[j // 4][0:1, (j % 4) * 128:(j % 4 + 1) * 128]
                v_s[j, 0:PAD, :] = jnp.broadcast_to(src, (PAD, 128))

    def attn_group(row, masked):
        def run(prev):
            g = 8
            q = [q_s[j, pl.ds(row + AR, g), :] for j in range(8)]
            ls = []
            for w in range(W):
                a = None
                for j in range(8):
                    term = q[j] * k_s[j, pl.ds(row + (PAD - DIL * w), g), :]
                    a = sp.link(ls[-1] if ls else None, term) if a is None else a + term
                ls.append(a)
            rs = [pltpu.roll(a, 64, 1) for a in ls]
            ls = [a + r for a, r in zip(ls, rs)]
            rs = [pltpu.roll(a, 32, 1) for a in ls]
            ls = [a + r for a, r in zip(ls, rs)]
            if masked:
                ri = row + lax.broadcasted_iota(i32, (g, 128), 0)
                ls = [ls[0]] + [jnp.where(ri >= DIL * w, ls[w], NEG) for w in range(1, W)]
            m = _tree(jnp.maximum, ls)
            ps = [jnp.exp2((l - m) * EXP2_SCALE) for l in ls]
            r = gs[pl.ds(row, g), :] / _tree(jnp.add, ps)
            outs = []
            for j in range(8):
                a = None
                for w in range(W):
                    term = ps[w] * v_s[j, pl.ds(row + (PAD - DIL * w), g), :]
                    a = sp.link(outs[-1] if outs else None, term) if a is None else a + term
                outs.append(a * r)
            for j in range(8):
                q_s[j, pl.ds(row + AR, g), :] = outs[j]
            return sp.chain([outs[-1]], prev, 1)
        return run

    def attn_tasks(base, nrows, first=False):
        return [attn_group(base + (qq * Q + r), first and qq == 0 and r < PAD)
                for r in range(0, nrows, 8) for qq in range(4)]

    def pack_tasks(oa, base, hbase, nrows):
        def task(r, c):
            def run(prev):
                def blk(i1, i2, k1, k2):
                    return q_s[4 * k1 + 2 * k2 + c, pl.ds(base + (i1 * H + i2 * Q + r), 16), :]
                cs, tok = sp.two_level(_a_combos, blk, prev, DEPTH2)
                for t in range(49):
                    oa[t, pl.ds(hbase + r // 2, 8), c * 128:(c + 1) * 128] = cs[t]
                return tok
            return run
        return [task(r, c) for r in range(0, nrows, 16) for c in range(2)]

    GS = RB * (KH // 128) * (FC // 128) * 7 // (4 * SLOT)
    DS = 49
    PS = 2 * RB * (D // 128) * (D // 128) // (4 * SLOT)

    def glu(hs):
        return lambda rb, cs: glu_tasks(hs, rb, cs, RB)[0]()

    def gu_src(slot):
        return lambda r, c: wgu[slot, r, c]

    def front(wqkv_vm, wp, wo_vm):
        cp_qkv = [cp(wqkv_hbm.at[:, pl.ds(i * D, D)], wqkv_vm.at[:, pl.ds(i * D, D)])
                  for i in range(3)]
        cp_wo = cp(wo_hbm, wo_vm)

        def plain(rb, hf, p):
            return sp.dot(x_vm[rows(rb, hf), :], wgu[0, :, p * CH:(p + 1) * CH])

        def plain_finish(rb, c):
            cs = [jnp.concatenate(c[2 * qd:2 * qd + 2], axis=1) for qd in range(4)]
            return glu_tasks(hs, rb, cs, 16)

        hs, bc, dc, c0 = {}, {}, {}, []
        with _Scope("w0"):
            wait([cp_x[0][0], gu0[0]])
        with _Scope("p1a"):
            for p in range(4):
                if p:
                    wait([gu0[p]])
                if p == 1:
                    start(cp_x[1] + cp_x[2])
                c0.append(plain(0, 0, p))
            wait([cp_x[0][1], cp_gw])
            start(cp_x[3] + cp_d(0, 0))
            sp.block()
            bt = b_sum_tasks(gu_src(0), bc)
            sp.schedule(bt[:12], 3, 16)
            sp.schedule(prep_tasks(0, sums=False), 3, 16)
            c0 += [plain(0, 1, p) for p in range(4)]
        with _Scope("w1"):
            wait(cp_x[1] + cp_x[2])
            start(cp_qkv[:1])
        with _Scope("p1b"):
            sp.block()
            sp.schedule(bt[12:], 3, 32)
            sp.schedule(prep_tasks(1, sums=False), 2, 10)
            sp.schedule(prep_tasks(2), 10, 32)
            c1 = [plain(1, hf, p) for hf in range(2) for p in range(4)]
        with _Scope("w2"):
            wait(cp_x[3] + cp_d(0, 0) + cp_qkv[:1])
            start(cp_qkv[1:] + [cp_wo] + cp_gu(1, 1) + cp_d(1, 1))
        with _Scope("p1c"):
            sp.block()
            for j in range(8):
                k_s[j, 0:PAD, :] = jnp.zeros((PAD, 128), f32)
                q_s[j, 0:AR, :] = jnp.zeros((AR, 128), f32)
                for ref, r0 in ((q_s, AR + S), (k_s, PAD + S), (v_s, PAD + S)):
                    ref[j, r0:r0 + KPAD, :] = jnp.zeros((KPAD, 128), f32)
            gs[S:, :] = jnp.zeros((KPAD, 128), f32)
            ha = {}
            sp.schedule(prep_tasks(3), 2, GS)
            sp.schedule(plain_finish(0, c0), 2, GS)
            sp.schedule(plain_finish(1, c1), GS + 6, 2 * GS)
            sp.schedule(d_tasks(0, dc), 2, 2 * GS)
            sp.schedule(perm_tasks(wqkv_vm, wp, 0, q_s.at[:, AR:, :]), 2 * GS + 6, 2 * GS + DS - 8)
            strassen_x([(rb, t) for rb in (2, 3) for t in ORDER], b_rhs(gu_src(0), bc), glu(hs))
            down_lhs(hs, 0, ha)
            down_lhs(hs, 1, ha)
            ffn_down(ha, dc, True)

        with _Scope("w2b"):
            wait(cp_qkv[1:] + [cp_wo])
        with _Scope("q"):
            sp.block()
            wo_spread, wo_gather = wo_tasks(wo_vm)
            sp.schedule(perm_tasks(wqkv_vm, wp, 1, k_s.at[:, PAD:, :]) + perm_tasks(wqkv_vm, wp, 2, v_s), 4, NRB * PS - 8)
            sp.schedule(wo_spread, 2 * PS, NRB * PS - 8)
            sp.schedule(prep_tasks(0, gate=False) + prep_tasks(1, gate=False), 4, 2 * PS)
            for rb in (1, 3, 0, 2):
                proj(wp, 0, q_s, AR, rb)
        with _Scope("w3"):
            wait(cp_gu(1, 1) + cp_d(1, 1))
        with _Scope("kv"):
            sp.block()
            vb = {}
            v_src = lambda r, c: _unpack(wp[2, _half(r), c])
            sp.schedule(wo_gather + b_sum_tasks(v_src, vb), 4, NRB * PS)
            for rb in range(NRB):
                proj(wp, 1, k_s, PAD, rb)
            v_rhs = b_rhs(v_src, vb)
            strassen_x([(0, t) for t in ORDER], v_rhs, v_finish)

        def v_rest(_, carry):
            with _Scope("v"):
                strassen_x([(rb, t) for rb in range(1, NRB) for t in ORDER], v_rhs, v_finish)
            return carry

        lax.fori_loop(0, zi[0], v_rest, 0)

    def back(oa):
        def body(j, carry):
            with _Scope("chunk"):
                slot = j % 2
                nxt = jnp.minimum(j + 1, NC - 1)
                prefetch = cp_gu(nxt, 1 - slot) + cp_d(nxt, 1 - slot)
                start(prefetch)
                sp.block()
                base = pl.multiple_of((j - 1) * AR, 32)
                hs, ha, bc, dc = {}, {}, {}, {}
                sp.schedule(b_sum_tasks(gu_src(slot), bc), *BC_SLOTS)
                sp.schedule(attn_tasks(base, AR, True), *ATTN_SLOTS)
                sp.schedule(pack_tasks(oa, base, pl.multiple_of((j - 1) * (AR // 2), 16), AR), *PACK_SLOTS)
                sp.schedule(d_tasks(slot, dc), *DC_SLOTS)
                strassen_x([(rb, t) for rb in (0, 2) for t in ORDER[:2]]
                           + [(rb, t) for rb in (0, 2) for t in ORDER[2:]]
                           + [(rb, t) for rb in (1, 3) for t in ORDER], b_rhs(gu_src(slot), bc), glu(hs))
                down_lhs(hs, 0, ha)
                down_lhs(hs, 1, ha)
                ffn_down(ha, dc, False)
                wait(prefetch)
            return carry

        lax.fori_loop(1, NC, body, 0)

        def out_copies(r0, i1, cols, sem):
            cs = []
            for i2 in range(2):
                idx = (pl.ds(r0 + (i1 * H + i2 * Q), PB), cols)
                cs.append(cp(x_vm.at[idx], o2.at[idx], sem + i2))
            return cs

        def out_blocks(blocks):
            todo = [(blk, 7 * t1 + t2) for blk in range(len(blocks))
                    for ts1, _ in _C_ORDER for t1 in ts1 for ts2, _ in _C_ORDER for t2 in ts2]
            m = {}
            for i in range(0, len(todo), 2):
                pair = todo[i:i + 2]
                ps = sp.dots([(_unpack(oa[t, pl.ds(blocks[blk][1], PB // 2), :]), _unpack(woc[t]))
                              for blk, t in pair])
                for (blk, t), p in zip(pair, ps):
                    r0, _, copies = blocks[blk]
                    mm = m.setdefault(blk, ({}, {}))
                    mm[0][t] = acc[t, pl.ds(r0, PB), :] + p
                    t1 = t // 7
                    if t % 7 != _C_ORDER[-1][0][-1]:
                        continue
                    mm[1][t1] = _c_combos([mm[0].pop(7 * t1 + t2) for t2 in range(7)])
                    for ts, qd in _C_ORDER:
                        if t1 != ts[-1]:
                            continue
                        for q2 in range(4):
                            val = _c_quadrant({tt: v[q2] for tt, v in mm[1].items()}, qd)
                            r = pl.ds(r0 + ((qd // 2) * H + (q2 // 2) * Q), PB)
                            c = (qd % 2) * KH + (q2 % 2) * KQ
                            x_vm[r, c:c + KQ] = val.astype(bf16)
                        start(copies.get(qd, []))

        def whole(r0, sem):
            return [c for i1 in range(2) for c in out_copies(r0, i1, slice(None), sem + 2 * i1)]

        done = (NC - 1) * AR

        def out_body(i, carry):
            with _Scope("p4a"):
                sp.block()
                half = pl.multiple_of(done // 2 + i * 8, 8)
                sp.schedule(pack_tasks(oa, 2 * half, half, 16), 4, 24)
                r0 = pl.multiple_of(i * PB, PB)
                out_blocks([(r0, pl.multiple_of((AR + i * PB) // 2, 16),
                             {3: whole(r0, out_sem + 4 * i)})])
            return carry

        lax.fori_loop(0, 2, out_body, 0)
        with _Scope("p4b"):
            last = {qd: out_copies(3 * PB, qd // 2, pl.ds((qd % 2) * KH, KH), out_sem + 12 + 2 * qd)
                    for qd in range(4)}
            copies = [{3: whole(blk * PB, out_sem + 4 * blk)} for blk in range(3)] + [last]
            out_blocks([(blk * PB, (AR + blk * PB) // 2, copies[blk]) for blk in (2, 3)])
        with _Scope("w4"):
            for cs in copies:
                for qd in cs:
                    wait(cs[qd])

    pl.run_scoped(front, pltpu.VMEM((D, 3 * D), bf16), pltpu.VMEM((3, D // 2, D), i32),
                  pltpu.VMEM((D, D), bf16))
    pl.run_scoped(back, pltpu.VMEM((49, (AR + Q) // 2, KQ), i32))
    assert not sp.plan and not sp.tokens


_N_SEMS = 10 + 1 + 2 * NRB + 3 + 1 + 20


@jax.jit
def pallas_gated_mix__sliding_local_dilated__glu_gated_reglu__prompt_kernel(
    A_x: jax.Array,
    A_wqkv: jax.Array,
    A_wo: jax.Array,
    B_x: jax.Array,
    B_W_gate: jax.Array,
    B_W_up: jax.Array,
    B_W_down: jax.Array,
    gate_w: jax.Array,
):
    del B_x
    hbm = pl.BlockSpec(memory_space=pl.ANY)
    scratch = [
        pltpu.VMEM((S, D), bf16),
        pltpu.VMEM((S // 2, D), i32),
        pltpu.VMEM((5, H // 2, KH), i32),
        pltpu.VMEM((8, 128), bf16),
        pltpu.VMEM((2, D, 2 * FC), bf16),
        pltpu.VMEM((2, FC, D), bf16),
        pltpu.VMEM((49, Q, KQ), f32),
        pltpu.VMEM((8, AR + S + KPAD, 128), f32),
        pltpu.VMEM((8, PAD + S + KPAD, 128), f32),
        pltpu.VMEM((8, PAD + S + KPAD, 128), f32),
        pltpu.VMEM((S + KPAD, 128), f32),
        pltpu.VMEM((49, KQ // 2, KQ), i32),
        pltpu.VMEM((8, 128), i32),
        pltpu.SMEM((1,), i32),
        pltpu.SemaphoreType.DMA((_N_SEMS,)),
    ]
    return pl.pallas_call(
        _kernel,
        in_specs=[hbm] * 7,
        out_specs=hbm,
        out_shape=jax.ShapeDtypeStruct((1, S, D), bf16),
        scratch_shapes=scratch,
        compiler_params=pltpu.CompilerParams(vmem_limit_bytes=124 * 1024 * 1024),
    )(A_x, A_wqkv, A_wo, B_W_gate, B_W_up, B_W_down, gate_w.reshape(8, 128))
```

```python
import math

import jax
import jax.numpy as jnp
from jax import lax
import jax.experimental.pallas as pl
import jax.experimental.pallas.tpu as pltpu

f32 = jnp.float32
bf16 = jnp.bfloat16
i32 = jnp.int32

S = 2048
D = 1024
F = 3584
NH = 32
DH = D // NH
W = 8
DIL = 2
H = S // 2
Q = S // 4
KH = D // 2
KQ = D // 4
FC = 512
CH = FC // 2
CQ = FC // 4
NC = F // FC
RB = 256
NRB = H // RB
PB = 128
PAD = 16
TP = DH + 1
AR = 64
A0 = Q - 6 * AR
QA = 160
QPAD = 64

ATTN_SLOTS = (32, 112)
PACK_SLOTS = (16, 32)
DC_SLOTS = (32, 108)
BC_SLOTS = (2, 16)
DEPTH = 3
DEPTH2 = 3
H_DEPTH = 3
LEAD = 0
PROFILE = ()

SCALE = DH ** -0.5
EXP2_SCALE = SCALE * math.log2(math.e)
NEG = -1e9 / SCALE


def _a_combos(a11, a12, a21, a22):
    return [a11 + a22, a21 + a22, a11, a22, a11 + a12, a21 - a11, a12 - a22]


def _b_combos(b11, b12, b21, b22):
    return [b11 + b22, b11, b12 - b22, b21 - b11, b22, b11 + b12, b21 + b22]


_C_TERMS = (((1, 0), (1, 3), (-1, 4), (1, 6)), ((1, 2), (1, 4)), ((1, 1), (1, 3)),
            ((1, 0), (-1, 1), (1, 2), (1, 5)))
_C_ORDER = (((2, 4), 1), ((1, 3), 2), ((0, 6), 0), ((5,), 3))


def _c_quadrant(m, qd):
    out = m[_C_TERMS[qd][0][1]]
    for sign, t in _C_TERMS[qd][1:]:
        out = out + m[t] if sign > 0 else out - m[t]
    return out


def _c_combos(m):
    return [_c_quadrant(m, qd) for qd in range(4)]


_A_SLOT = {0: 0, 1: 1, 4: 2, 5: 3, 6: 4}
_B_SUMS = (2, 3, 0, 5, 6)
ORDER = (1, 4) + _B_SUMS


class _Scope:
    def __init__(self, name):
        self.cm = jax.named_scope(name) if (PROFILE is True or name in PROFILE) else None

    def __enter__(self):
        if self.cm is not None:
            self.cm.__enter__()

    def __exit__(self, *a):
        if self.cm is not None:
            self.cm.__exit__(*a)


def _tree(op, xs):
    xs = list(xs)
    while len(xs) > 1:
        xs = [op(xs[i], xs[i + 1]) if i + 1 < len(xs) else xs[i] for i in range(0, len(xs), 2)]
    return xs[0]


def _pack(x):
    return pltpu.bitcast(x.astype(bf16), i32)


def _unpack(x):
    return pltpu.bitcast(x, bf16)


def _half(r):
    return slice(r.start // 2, r.stop // 2)


SLOT = 256


class _Spreader:
    def __init__(self, zero_ref):
        self.zero_ref = zero_ref
        self.plan = {}
        self.tokens = {}
        self.now = 0

    def block(self):
        self.zero = self.zero_ref[...]
        self.never = self.zero != 0

    def link(self, after, x):
        if after is None:
            return x
        if after.dtype != x.dtype:
            after = pltpu.bitcast(after, x.dtype)
        return jnp.where(self.never, after, x)

    def chain(self, vals, prev, depth):
        for v in vals:
            v = pltpu.bitcast(v, i32) if v.dtype != i32 else v
            for r in range(0, v.shape[0], 8):
                for c in range(0, v.shape[1], 128):
                    tile = v[r:r + 8, c:c + 128]
                    if prev is None:
                        prev = tile
                        continue
                    prev = prev | tile
                    for i in range(depth - 1):
                        prev = (prev + self.zero) if i % 2 == 0 else (prev ^ self.zero)
        return prev

    def link_rows(self, after, x):
        return jnp.concatenate([self.link(after, x[r:r + 8, :]) for r in range(0, x.shape[0], 8)],
                               axis=0)

    def serial_combos(self, combos, x11, x12, x21, x22, after):
        return combos(self.link_rows(after, x11), x12, x21, self.link_rows(after, x22))

    def two_level(self, combos, blk, prev, depth):
        outer = [combos(*[blk(r1, r2, c1, c2) for r1 in range(2) for c1 in range(2)])
                 for r2 in range(2) for c2 in range(2)]
        outs, tok = [], None
        for t in range(7):
            wide = _pack(jnp.concatenate(
                self.serial_combos(combos, *[o[t] for o in outer], tok), axis=1))
            outs += [wide[:, c:c + 128] for c in range(0, 7 * 128, 128)]
            tok = self.chain(outs[-7:], tok, depth)
        return outs, self.chain([tok], prev, 1)

    def schedule(self, tasks, first, last):
        n = len(tasks)
        for i, t in enumerate(tasks):
            pos = self.now + first + ((i + 1) * (last - first) - 1) // n
            self.plan.setdefault(pos, []).append(t)

    def dots(self, pairs):
        m = pairs[0][0].shape[0]
        tiles = [(i, r, c) for i, (_, rhs) in enumerate(pairs)
                 for c in range(0, rhs.shape[1], 128) for r in range(0, rhs.shape[0], 128)]
        nslots = m * len(tiles) // (4 * SLOT)
        for sl in range(self.now, self.now + nslots + LEAD):
            for t in self.plan.pop(sl, []):
                tok = t(self.tokens.get(sl))
                if tok is not None:
                    self.tokens[sl] = tok
        deps = {}
        for sl in range(nslots):
            ps = sl * SLOT // m
            tok = self.tokens.pop(self.now + sl, None)
            if tok is not None:
                deps[ps] = tok | deps[ps] if ps in deps else tok
        self.now += nslots
        tied = {tile: d for ps, d in deps.items() for tile in tiles[4 * ps:4 * ps + 4]}
        outs = []
        for i, (lhs, rhs) in enumerate(pairs):
            if any(key[0] == i for key in tied):
                parts = []
                for r in range(0, rhs.shape[0], 128):
                    top = [rhs[r:r + 16, c:c + 128] for c in range(0, rhs.shape[1], 128)]
                    top = [_unpack(self.link(tied[i, r, c * 128], _pack(t0)))
                           if (i, r, c * 128) in tied else t0 for c, t0 in enumerate(top)]
                    parts += [jnp.concatenate(top, axis=1), rhs[r + 16:r + 128, :]]
                rhs = jnp.concatenate(parts, axis=0)
            outs.append(jnp.dot(lhs, rhs, preferred_element_type=f32))
        return outs

    def dot(self, lhs, rhs):
        return self.dots([(lhs, rhs)])[0]


def _kernel(x_hbm, wqkv_hbm, wo_hbm, wg_hbm, wu_hbm, wd_hbm, gw_hbm, out_hbm,
            x_vm, xn, xa, gw_vm, wgu, wd, acc, q_s, k_s, v_s, gs, woc, zs, zi, sems):
    sem_ids = iter(range(10, 1000))

    def cp(src, dst, sem=None):
        return pltpu.make_async_copy(src, dst, sems.at[next(sem_ids) if sem is None else sem])

    def cp_gu(j, slot):
        col = j * FC if isinstance(j, int) else pl.multiple_of(j * FC, FC)
        return [cp((wg_hbm, wu_hbm)[p % 2].at[:, pl.ds(col + (p // 2) * CH, CH)],
                   wgu.at[slot, :, pl.ds(p * CH, CH)], slot * 5 + p) for p in range(4)]

    def cp_d(j, slot):
        row = j * FC if isinstance(j, int) else pl.multiple_of(j * FC, FC)
        return [cp(wd_hbm.at[pl.ds(row, FC), :], wd.at[slot], slot * 5 + 4)]

    x2 = x_hbm.at[0]
    o2 = out_hbm.at[0]
    cp_gw = cp(gw_hbm, gw_vm)
    cp_x = [[cp(x2.at[pl.ds(hf * H + rb * RB, RB), :], x_vm.at[pl.ds(hf * H + rb * RB, RB), :])
             for hf in range(2)] for rb in range(NRB)]
    out_sem = _N_SEMS - 20

    def start(cs):
        for c in cs:
            c.start()

    def wait(cs):
        for c in cs:
            c.wait()

    gu0 = cp_gu(0, 0)
    start([cp_x[0][0]] + gu0 + [cp_x[0][1], cp_gw])

    zs[...] = jnp.zeros((8, 128), i32)
    zi[0] = 1
    sp = _Spreader(zs)

    def rows(rb, hf=0):
        return slice(hf * H + rb * RB, hf * H + (rb + 1) * RB)

    def x_lhs(t, rb):
        if t == 2:
            return _unpack(xn[_half(rows(rb, 0)), :KH])
        if t == 3:
            return _unpack(xn[_half(rows(rb, 1)), KH:])
        return _unpack(xa[_A_SLOT[t], _half(rows(rb)), :])

    def prep_tasks(rb, sums=True, gate=True):
        def task(s0):
            def run(first):
                prev = None
                gw = gw_vm[...].astype(f32)
                r = [slice(hf * H + rb * RB + s0, hf * H + rb * RB + s0 + 16) for hf in range(2)]
                z = [None, None]
                for c in range(4):
                    cols = [slice(kh * KH + c * 128, kh * KH + (c + 1) * 128) for kh in range(2)]
                    xs = [sp.link(prev, _pack(x_vm[r[qd // 2], cols[qd % 2]])) for qd in range(4)]
                    a = [_unpack(t).astype(f32) for t in xs]
                    outs = []
                    if sums:
                        for qd in range(4):
                            xn[_half(r[qd // 2]), cols[qd % 2]] = xs[qd]
                        cs = _a_combos(*a)
                        for t, slot in _A_SLOT.items():
                            outs.append(_pack(cs[t]))
                            xa[slot, _half(r[0]), cols[0]] = outs[-1]
                    if gate:
                        for qd in range(4):
                            g0 = (qd % 2) * 4 + c
                            term = a[qd] * gw[g0:g0 + 1, :]
                            z[qd // 2] = term if z[qd // 2] is None else z[qd // 2] + term
                        outs += z
                    prev = sp.chain(outs, prev, 1)
                if gate:
                    for hf in range(2):
                        g = jax.nn.sigmoid(jnp.sum(z[hf], axis=1, keepdims=True))
                        g = jnp.broadcast_to(g, (16, 128))
                        gs[r[hf], :] = g
                        prev = sp.chain([g], prev, 1)
                return sp.chain([prev], first, 1)
            return run
        return [task(s0) for s0 in range(0, RB, 16)]

    def b_sum_tasks(src, dst):
        def task(r0):
            def run(prev):
                raw = [src(slice(a * KH + r0, a * KH + r0 + 16), slice(c * KH, (c + 1) * KH))
                       for a in range(2) for c in range(2)]
                cs = _b_combos(*[b.astype(f32) for b in raw])
                for t in _B_SUMS:
                    dst.setdefault(t, []).append(_pack(cs[t]))
                return sp.chain([dst[t][-1] for t in _B_SUMS], prev, DEPTH)
            return run
        return [task(r0) for r0 in range(0, KH, 16)]

    def b_rhs(src, sums):
        def rhs(t):
            if t == 1:
                return src(slice(0, KH), slice(0, KH))
            if t == 4:
                return src(slice(KH, D), slice(KH, D))
            return _unpack(jnp.concatenate(sums[t], axis=0))
        return rhs

    def strassen_x(order, rhs, finish):
        m = {}
        for rb, t in order:
            m.setdefault(rb, {})[t] = sp.dot(x_lhs(t, rb), rhs(t))
            if len(m[rb]) == 7:
                finish(rb, _c_combos(m.pop(rb)))

    def glu_tasks(hs, rb, cs, sub):
        hs[rb] = [[] for _ in range(7)]

        def task(r0):
            def run(prev=None):
                h = []
                for qd, cc in enumerate(cs):
                    g0 = (qd // 2) * H + rb * RB + r0
                    omg = 1.0 - gs[g0:g0 + sub, :]
                    omg = jnp.concatenate([omg] * (CH // 128), axis=1)
                    h.append(jnp.maximum(cc[r0:r0 + sub, :CH], 0.0) * cc[r0:r0 + sub, CH:] * omg)
                sums = _a_combos(*h)
                for t in range(7):
                    hs[rb][t].append(sums[t])
                if sub < RB:
                    return sp.chain([sums[t] for t in _A_SLOT], prev, DEPTH2)
            return run
        return [task(r0) for r0 in range(0, RB, sub)]

    def down_lhs(hs, b, ha):
        tok = None
        for t in range(7):
            s0, s1 = [jnp.concatenate(hs[rb][t], axis=0) for rb in (b, b + 2)]
            slabs = []
            for r in range(0, RB, 16):
                slabs.append(sp.serial_combos(
                    _a_combos, s0[r:r + 16, :CQ], s0[r:r + 16, CQ:],
                    s1[r:r + 16, :CQ], s1[r:r + 16, CQ:], tok))
                tok = sp.chain([slabs[-1][t2] for t2 in _A_SLOT], None, H_DEPTH)
            for t2 in range(7):
                ha[b, 7 * t + t2] = jnp.concatenate([sl[t2] for sl in slabs], axis=0).astype(bf16)

    def d_tasks(slot, dst):
        def task(r0, c):
            def run(prev):
                def blk(k1, k2, n1, n2):
                    r, c0 = k1 * CH + k2 * CQ + r0, n1 * KH + n2 * KQ + c * 128
                    return wd[slot, r:r + 16, c0:c0 + 128].astype(f32)
                cs, tok = sp.two_level(_b_combos, blk, prev, DEPTH2)
                for t in range(49):
                    dst.setdefault((t, c), []).append(cs[t])
                return tok
            return run
        return [task(r0, c) for r0 in range(0, CQ, 16) for c in range(2)]

    def ffn_down(ha, dc, first):
        rhs = [_unpack(jnp.concatenate([jnp.concatenate(dc[t, c], axis=0) for c in range(2)], axis=1))
               for t in range(49)]
        todo = [(b, t) for b in range(2) for t in range(49)]
        for i in range(0, len(todo), 2):
            pair = todo[i:i + 2]
            ps = sp.dots([(ha[b, t], rhs[t]) for b, t in pair])
            for (b, t), p in zip(pair, ps):
                if first:
                    acc[t, b * RB:(b + 1) * RB, :] = p
                else:
                    acc[t, b * RB:(b + 1) * RB, :] += p

    def perm_tasks(wqkv_vm, wp, i, tbuf):
        def fwd(rb, c):
            def run(prev):
                c0 = i * D + c * 128
                tt = pltpu.bitcast(wqkv_vm[rb * 256:(rb + 1) * 256, c0:c0 + 128], f32).T
                for hh in range(4):
                    tbuf[rb, pl.ds((4 * c + hh) * TP, DH), :] = tt[hh * DH:(hh + 1) * DH, :]
                return sp.chain([tt], prev, 1)
            return run

        def bwd(rb, j):
            def run(prev):
                g = jnp.concatenate(
                    [tbuf[rb, pl.ds(4 * j + dd, NH, stride=TP), :] for dd in range(4)], axis=0).T
                wp[i, rb * 128:(rb + 1) * 128, j * 128:(j + 1) * 128] = pltpu.bitcast(g, i32)
            return run
        tasks = []
        for rb in range(4):
            tasks += [fwd(rb, c) for c in range(8)] + [bwd(rb, j) for j in range(8)]
        return tasks

    def wo_tasks(wo_vm):
        def stage(c):
            return 4 + c % 4, (c // 4) * NH * TP

        def spread(h0):
            def run(prev):
                blk = wo_vm[h0 * DH:(h0 + 2) * DH, :].astype(f32)
                for h in range(2):
                    for c in range(8):
                        sl, r0 = stage(c)
                        q_s[sl, pl.ds(r0 + (h0 + h) * TP, DH), :] = (
                            blk[h * DH:(h + 1) * DH, c * 128:(c + 1) * 128])
                return sp.chain([blk], prev, 1)
            return run

        def gather(d, h0, c):
            def run(prev):
                def blk(k1, k2, n1, n2):
                    sl, r0 = stage(4 * n1 + 2 * n2 + c)
                    r0 += h0 * TP + 16 * k1 + 8 * k2 + d
                    return q_s[sl, pl.ds(r0, 16, stride=TP), :]
                cs, tok = sp.two_level(_b_combos, blk, prev, DEPTH2)
                r = (d * NH + h0) // 2
                for t in range(49):
                    woc[t, r:r + 8, c * 128:(c + 1) * 128] = cs[t]
                return tok
            return run
        return ([spread(h0) for h0 in range(0, NH, 2)],
                [gather(d, h0, c) for d in range(8) for h0 in (0, 16) for c in range(2)])

    def proj(wp, i, dst, pad, slabs):
        lhs = jnp.concatenate([xn[r0 // 2:(r0 + n) // 2, :] for r0, n in slabs], axis=0)
        p = sp.dot(_unpack(lhs), _unpack(wp[i]))
        at = 0
        for r0, n in slabs:
            for j in range(8):
                dst[j, pad + r0:pad + r0 + n, :] = p[at:at + n, j * 128:(j + 1) * 128]
            at += n

    def v_finish(rb, cs):
        for qd, cc in enumerate(cs):
            r0 = PAD + (qd // 2) * H + rb * RB
            for j in range(4):
                v_s[(qd % 2) * 4 + j, r0:r0 + RB, :] = cc[:, j * 128:(j + 1) * 128]
        if rb == 0:
            for j in range(8):
                src = cs[j // 4][0:1, (j % 4) * 128:(j % 4 + 1) * 128]
                v_s[j, 0:PAD, :] = jnp.broadcast_to(src, (PAD, 128))

    def attn_group(row, masked):
        def run(prev):
            g = 8
            q = [q_s[j, pl.ds(row, g), :] for j in range(8)]
            ls = []
            for w in range(W):
                a = None
                for j in range(8):
                    term = q[j] * k_s[j, pl.ds(row + (PAD - DIL * w), g), :]
                    a = sp.link(ls[-1] if ls else None, term) if a is None else a + term
                ls.append(a)
            rs = [pltpu.roll(a, 64, 1) for a in ls]
            ls = [a + r for a, r in zip(ls, rs)]
            rs = [pltpu.roll(a, 32, 1) for a in ls]
            ls = [a + r for a, r in zip(ls, rs)]
            if masked:
                ri = row + lax.broadcasted_iota(i32, (g, 128), 0)
                ls = [ls[0]] + [jnp.where(ri >= DIL * w, ls[w], NEG) for w in range(1, W)]
            m = _tree(jnp.maximum, ls)
            ps = [jnp.exp2((l - m) * EXP2_SCALE) for l in ls]
            r = gs[pl.ds(row, g), :] / _tree(jnp.add, ps)
            outs = []
            for j in range(8):
                a = None
                for w in range(W):
                    term = ps[w] * v_s[j, pl.ds(row + (PAD - DIL * w), g), :]
                    a = sp.link(outs[-1] if outs else None, term) if a is None else a + term
                outs.append(a * r)
            for j in range(8):
                q_s[j, pl.ds(row, g), :] = outs[j]
            return sp.chain([outs[-1]], prev, 1)
        return run

    def attn_tasks(base, nrows, first=False):
        return [attn_group(base + (qq * Q + r), first and qq == 0 and r < PAD)
                for r in range(0, nrows, 8) for qq in range(4)]

    def pack_tasks(oa, base, hbase, nrows):
        def task(r, c):
            def run(prev):
                def blk(i1, i2, k1, k2):
                    return q_s[4 * k1 + 2 * k2 + c, pl.ds(base + (i1 * H + i2 * Q + r), 16), :]
                cs, tok = sp.two_level(_a_combos, blk, prev, DEPTH2)
                for t in range(49):
                    oa[t, pl.ds(hbase + r // 2, 8), c * 128:(c + 1) * 128] = cs[t]
                return tok
            return run
        return [task(r, c) for r in range(0, nrows, 16) for c in range(2)]

    GS = RB * (KH // 128) * (FC // 128) * 7 // (4 * SLOT)
    DS = 49
    PS = 2 * RB * (D // 128) * (D // 128) // (4 * SLOT)

    def glu(hs):
        return lambda rb, cs: glu_tasks(hs, rb, cs, RB)[0]()

    def raw_first(first, rest):
        return ([(rb, t) for rb in first for t in ORDER[:2]]
                + [(rb, t) for rb in first for t in ORDER[2:]]
                + [(rb, t) for rb in rest for t in ORDER])

    def gu_src(slot):
        return lambda r, c: wgu[slot, r, c]

    def front(wqkv_vm, wp, wo_vm):
        cp_qkv = [cp(wqkv_hbm.at[:, pl.ds(i * D, D)], wqkv_vm.at[:, pl.ds(i * D, D)])
                  for i in range(3)]
        cp_wo = cp(wo_hbm, wo_vm)

        def plain(rb, hf, p):
            return sp.dot(x_vm[rows(rb, hf), :], wgu[0, :, p * CH:(p + 1) * CH])

        def plain_finish(rb, c):
            cs = [jnp.concatenate(c[2 * qd:2 * qd + 2], axis=1) for qd in range(4)]
            return glu_tasks(hs, rb, cs, 16)

        hs, bc, dc, c0 = {}, {}, {}, []
        with _Scope("w0"):
            wait([cp_x[0][0], gu0[0]])
        with _Scope("p1a"):
            for p in range(4):
                if p:
                    wait([gu0[p]])
                if p == 1:
                    start(cp_x[1] + cp_x[2])
                c0.append(plain(0, 0, p))
            wait([cp_x[0][1], cp_gw])
            start(cp_x[3] + cp_d(0, 0))
            sp.block()
            bt = b_sum_tasks(gu_src(0), bc)
            sp.schedule(bt[:12], 3, 16)
            sp.schedule(prep_tasks(0, sums=False), 3, 16)
            c0 += [plain(0, 1, p) for p in range(4)]
        with _Scope("w1"):
            wait(cp_x[1] + cp_x[2])
            start(cp_qkv[2:])
        with _Scope("p1b"):
            sp.block()
            sp.schedule(bt[12:], 3, 32)
            sp.schedule(prep_tasks(1, sums=False), 2, 10)
            sp.schedule(prep_tasks(2), 10, 32)
            c1 = [plain(1, hf, p) for hf in range(2) for p in range(4)]
        with _Scope("w2"):
            wait(cp_x[3] + cp_d(0, 0) + cp_qkv[2:])
            start([cp_qkv[1], cp_wo, cp_qkv[0]] + cp_gu(1, 1) + cp_d(1, 1))
        with _Scope("p1c"):
            sp.block()
            for j in range(8):
                k_s[j, 0:PAD, :] = jnp.zeros((PAD, 128), f32)
            ha = {}
            sp.schedule(prep_tasks(3), 2, GS)
            sp.schedule(plain_finish(0, c0), 2, GS)
            sp.schedule(plain_finish(1, c1), GS + 6, 2 * GS)
            sp.schedule(d_tasks(0, dc), 2, 2 * GS)
            sp.schedule(perm_tasks(wqkv_vm, wp, 2, q_s), 2 * GS + 6, 2 * GS + DS - 8)
            strassen_x([(rb, t) for rb in (2, 3) for t in ORDER], b_rhs(gu_src(0), bc), glu(hs))
            down_lhs(hs, 0, ha)
            down_lhs(hs, 1, ha)
            ffn_down(ha, dc, True)

        with _Scope("w2b"):
            wait([cp_qkv[1], cp_wo])
        with _Scope("v"):
            sp.block()
            vb = {}
            v_src = lambda r, c: _unpack(wp[2, _half(r), c])
            wo_spread, wo_gather = wo_tasks(wo_vm)
            sp.schedule(b_sum_tasks(v_src, vb), *BC_SLOTS)
            sp.schedule(prep_tasks(0, gate=False) + prep_tasks(1, gate=False), 16, 2 * GS)
            sp.schedule(perm_tasks(wqkv_vm, wp, 1, k_s.at[:, PAD:, :]), 2 * GS, 4 * GS - 8)
            sp.schedule(wo_spread, 2 * GS, 4 * GS)
            strassen_x(raw_first((2, 3), (0, 1)), b_rhs(v_src, vb), v_finish)
        with _Scope("w3"):
            wait(cp_qkv[:1] + cp_gu(1, 1) + cp_d(1, 1))
        with _Scope("kq"):
            sp.block()
            sp.schedule(perm_tasks(wqkv_vm, wp, 0, q_s), 4, 3 * PS)
            sp.schedule(wo_gather, 4, NRB * PS)
            for rb in range(NRB):
                proj(wp, 1, k_s, PAD, [(rb * Q, Q)])
            proj(wp, 0, q_s, 0, [(qq * Q, QA) for qq in range(4)])

        def q_rest(_, carry):
            with _Scope("q"):
                sp.block()
                n = (Q - QA) // 2
                total = 4 * (Q - QA) * 64 // (4 * SLOT)
                sp.schedule(attn_tasks(0, A0, True), 4, total)
                for r0 in (QA, QA + n):
                    proj(wp, 0, q_s, 0, [(qq * Q + r0, n) for qq in range(4)])
            return carry

        lax.fori_loop(0, zi[0], q_rest, 0)

    def back(oa):
        def body(j, carry):
            with _Scope("chunk"):
                slot = j % 2
                nxt = jnp.minimum(j + 1, NC - 1)
                prefetch = cp_gu(nxt, 1 - slot) + cp_d(nxt, 1 - slot)
                sp.block()
                base = pl.multiple_of((j - 1) * AR, AR)
                hs, ha, bc, dc = {}, {}, {}, {}
                sp.schedule(b_sum_tasks(gu_src(slot), bc), *BC_SLOTS)
                sp.schedule(attn_tasks(base + A0, AR), *ATTN_SLOTS)
                sp.schedule(pack_tasks(oa, base, pl.multiple_of((j - 1) * (AR // 2), AR // 2), AR),
                            *PACK_SLOTS)
                sp.schedule(d_tasks(slot, dc), *DC_SLOTS)
                start(prefetch)
                strassen_x(raw_first((0, 2), (1, 3)), b_rhs(gu_src(slot), bc), glu(hs))
                down_lhs(hs, 0, ha)
                down_lhs(hs, 1, ha)
                ffn_down(ha, dc, False)
                wait(prefetch)
            return carry

        lax.fori_loop(1, NC, body, 0)

        def out_copies(r0, i1, cols, sem):
            cs = []
            for i2 in range(2):
                idx = (pl.ds(r0 + (i1 * H + i2 * Q), PB), cols)
                cs.append(cp(x_vm.at[idx], o2.at[idx], sem + i2))
            return cs

        def out_blocks(blocks):
            todo = [(blk, 7 * t1 + t2) for blk in range(len(blocks))
                    for ts1, _ in _C_ORDER for t1 in ts1 for ts2, _ in _C_ORDER for t2 in ts2]
            m = {}
            for i in range(0, len(todo), 2):
                pair = todo[i:i + 2]
                ps = sp.dots([(_unpack(oa[t, pl.ds(blocks[blk][1], PB // 2), :]), _unpack(woc[t]))
                              for blk, t in pair])
                for (blk, t), p in zip(pair, ps):
                    r0, _, copies = blocks[blk]
                    mm = m.setdefault(blk, ({}, {}))
                    mm[0][t] = acc[t, pl.ds(r0, PB), :] + p
                    t1 = t // 7
                    if t % 7 != _C_ORDER[-1][0][-1]:
                        continue
                    mm[1][t1] = _c_combos([mm[0].pop(7 * t1 + t2) for t2 in range(7)])
                    for ts, qd in _C_ORDER:
                        if t1 != ts[-1]:
                            continue
                        for q2 in range(4):
                            val = _c_quadrant({tt: v[q2] for tt, v in mm[1].items()}, qd)
                            r = pl.ds(r0 + ((qd // 2) * H + (q2 // 2) * Q), PB)
                            c = (qd % 2) * KH + (q2 % 2) * KQ
                            x_vm[r, c:c + KQ] = val.astype(bf16)
                        start(copies.get(qd, []))

        def whole(r0, sem):
            return [c for i1 in range(2) for c in out_copies(r0, i1, slice(None), sem + 2 * i1)]

        done = (NC - 1) * AR

        def out_body(i, carry):
            with _Scope("p4a"):
                sp.block()
                half = pl.multiple_of(done // 2 + i * 24, 8)
                sp.schedule(pack_tasks(oa, 2 * half, half, 48), 4, 24)
                r0 = pl.multiple_of(i * PB, PB)
                out_blocks([(r0, pl.multiple_of(i * (PB // 2), PB // 2),
                             {3: whole(r0, out_sem + 4 * i)})])
            return carry

        lax.fori_loop(0, 2, out_body, 0)
        with _Scope("p4b"):
            sp.block()
            sp.schedule(pack_tasks(oa, done + 96, (done + 96) // 2, Q - done - 96), 4, 22)
            last = {qd: out_copies(3 * PB, qd // 2, pl.ds((qd % 2) * KH, KH), out_sem + 12 + 2 * qd)
                    for qd in range(4)}
            copies = [{3: whole(blk * PB, out_sem + 4 * blk)} for blk in range(3)] + [last]
            out_blocks([(blk * PB, blk * PB // 2, copies[blk]) for blk in (2, 3)])
        with _Scope("w4"):
            for cs in copies:
                for qd in cs:
                    wait(cs[qd])

    pl.run_scoped(front, pltpu.VMEM((D, 3 * D), bf16), pltpu.VMEM((3, D // 2, D), i32),
                  pltpu.VMEM((D, D), bf16))
    pl.run_scoped(back, pltpu.VMEM((49, Q // 2, KQ), i32))
    assert not sp.plan and not sp.tokens


_N_SEMS = 10 + 1 + 2 * NRB + 3 + 1 + 20


@jax.jit
def pallas_gated_mix__sliding_local_dilated__glu_gated_reglu__prompt_kernel(
    A_x: jax.Array,
    A_wqkv: jax.Array,
    A_wo: jax.Array,
    B_x: jax.Array,
    B_W_gate: jax.Array,
    B_W_up: jax.Array,
    B_W_down: jax.Array,
    gate_w: jax.Array,
):
    del B_x
    hbm = pl.BlockSpec(memory_space=pl.ANY)
    scratch = [
        pltpu.VMEM((S, D), bf16),
        pltpu.VMEM((S // 2, D), i32),
        pltpu.VMEM((5, H // 2, KH), i32),
        pltpu.VMEM((8, 128), bf16),
        pltpu.VMEM((2, D, 2 * FC), bf16),
        pltpu.VMEM((2, FC, D), bf16),
        pltpu.VMEM((49, Q, KQ), f32),
        pltpu.VMEM((8, S + QPAD + 16, 128), f32),
        pltpu.VMEM((8, PAD + S, 128), f32),
        pltpu.VMEM((8, PAD + S, 128), f32),
        pltpu.VMEM((S, 128), f32),
        pltpu.VMEM((49, KQ // 2, KQ), i32),
        pltpu.VMEM((8, 128), i32),
        pltpu.SMEM((1,), i32),
        pltpu.SemaphoreType.DMA((_N_SEMS,)),
    ]
    return pl.pallas_call(
        _kernel,
        in_specs=[hbm] * 7,
        out_specs=hbm,
        out_shape=jax.ShapeDtypeStruct((1, S, D), bf16),
        scratch_shapes=scratch,
        compiler_params=pltpu.CompilerParams(vmem_limit_bytes=124 * 1024 * 1024),
    )(A_x, A_wqkv, A_wo, B_W_gate, B_W_up, B_W_down, gate_w.reshape(8, 128))
```

```python
import math

import jax
import jax.numpy as jnp
from jax import lax
import jax.experimental.pallas as pl
import jax.experimental.pallas.tpu as pltpu

f32 = jnp.float32
bf16 = jnp.bfloat16
i32 = jnp.int32

S = 2048
D = 1024
F = 3584
NH = 32
DH = D // NH
W = 8
DIL = 2
H = S // 2
Q = S // 4
KH = D // 2
KQ = D // 4
FC = 512
CH = FC // 2
CQ = FC // 4
NC = F // FC
RB = 256
NRB = H // RB
PB = 128
PAD = 16
TP = DH + 1
AR = 64
A0 = Q - 6 * AR
QA = 160
QPAD = 64

ATTN_SLOTS = (32, 112)
PACK_SLOTS = (16, 32)
DC_SLOTS = (32, 108)
BC_SLOTS = (2, 16)
DEPTH = 3
H_ORDER = (0, 1, 2, 3, 4, 5, 6)
DEPTH2 = 3
H_DEPTH = 3
PROFILE = ()

SCALE = DH ** -0.5
EXP2_SCALE = SCALE * math.log2(math.e)
NEG = -1e9 / SCALE


def _a_combos(a11, a12, a21, a22):
    return [a11 + a22, a21 + a22, a11, a22, a11 + a12, a21 - a11, a12 - a22]


def _b_combos(b11, b12, b21, b22):
    return [b11 + b22, b11, b12 - b22, b21 - b11, b22, b11 + b12, b21 + b22]


_C_TERMS = (((1, 0), (1, 3), (-1, 4), (1, 6)), ((1, 2), (1, 4)), ((1, 1), (1, 3)),
            ((1, 0), (-1, 1), (1, 2), (1, 5)))
_C_ORDER = (((2, 4), 1), ((1, 3), 2), ((0, 6), 0), ((5,), 3))


def _c_quadrant(m, qd):
    out = m[_C_TERMS[qd][0][1]]
    for sign, t in _C_TERMS[qd][1:]:
        out = out + m[t] if sign > 0 else out - m[t]
    return out


def _c_combos(m):
    return [_c_quadrant(m, qd) for qd in range(4)]


_A_SLOT = {0: 0, 1: 1, 4: 2, 5: 3, 6: 4}
_B_SUMS = (2, 3, 0, 5, 6)
ORDER = (1, 4) + _B_SUMS


class _Scope:
    def __init__(self, name):
        self.cm = jax.named_scope(name) if (PROFILE is True or name in PROFILE) else None

    def __enter__(self):
        if self.cm is not None:
            self.cm.__enter__()

    def __exit__(self, *a):
        if self.cm is not None:
            self.cm.__exit__(*a)


def _tree(op, xs):
    xs = list(xs)
    while len(xs) > 1:
        xs = [op(xs[i], xs[i + 1]) if i + 1 < len(xs) else xs[i] for i in range(0, len(xs), 2)]
    return xs[0]


def _pack(x):
    return pltpu.bitcast(x.astype(bf16), i32)


def _unpack(x):
    return pltpu.bitcast(x, bf16)


def _half(r):
    return slice(r.start // 2, r.stop // 2)


SLOT = 256


class _Spreader:
    def __init__(self, zero_ref):
        self.zero_ref = zero_ref
        self.plan = {}
        self.now = 0

    def block(self):
        self.zero = self.zero_ref[...]
        self.never = self.zero != 0

    def link(self, after, x):
        if after is None:
            return x
        if after.dtype != x.dtype:
            after = pltpu.bitcast(after, x.dtype)
        return jnp.where(self.never, after, x)

    def chain(self, vals, prev, depth):
        for v in vals:
            v = pltpu.bitcast(v, i32) if v.dtype != i32 else v
            for r in range(0, v.shape[0], 8):
                for c in range(0, v.shape[1], 128):
                    tile = v[r:r + 8, c:c + 128]
                    if prev is None:
                        prev = tile
                        continue
                    prev = prev | tile
                    for i in range(depth - 1):
                        prev = (prev + self.zero) if i % 2 == 0 else (prev ^ self.zero)
        return prev

    def link_rows(self, after, x):
        return jnp.concatenate([self.link(after, x[r:r + 8, :]) for r in range(0, x.shape[0], 8)],
                               axis=0)

    def serial_combos(self, combos, x11, x12, x21, x22, after):
        return combos(self.link_rows(after, x11), x12, x21, self.link_rows(after, x22))

    def two_level(self, combos, blk, prev, depth):
        outer = [combos(*[blk(r1, r2, c1, c2) for r1 in range(2) for c1 in range(2)])
                 for r2 in range(2) for c2 in range(2)]
        outs, tok = [], None
        for t in range(7):
            wide = _pack(jnp.concatenate(
                self.serial_combos(combos, *[o[t] for o in outer], tok), axis=1))
            outs += [wide[:, c:c + 128] for c in range(0, 7 * 128, 128)]
            tok = self.chain(outs[-7:], tok, depth)
        return outs, self.chain([tok], prev, 1)

    def schedule(self, tasks, first, last):
        n = len(tasks)
        for i, t in enumerate(tasks):
            pos = self.now + first + ((i + 1) * (last - first) - 1) // n
            self.plan.setdefault(pos, []).append((t, id(tasks)))

    def dots(self, pairs):
        m = pairs[0][0].shape[0]
        tiles = [(i, r, c) for i, (_, rhs) in enumerate(pairs)
                 for c in range(0, rhs.shape[1], 128) for r in range(0, rhs.shape[0], 128)]
        nslots = m * len(tiles) // (4 * SLOT)
        deps = {}
        for sl in range(nslots):
            ps = sl * SLOT // m
            toks = {}
            for t, lane in self.plan.pop(self.now + sl, []):
                tok = t(toks.get(lane))
                if tok is not None:
                    toks[lane] = tok
            for tok in toks.values():
                deps[ps] = tok | deps[ps] if ps in deps else tok
        self.now += nslots
        tied = {tile: d for ps, d in deps.items() for tile in tiles[4 * ps:4 * ps + 4]}
        outs = []
        for i, (lhs, rhs) in enumerate(pairs):
            if any(key[0] == i for key in tied):
                parts = []
                for r in range(0, rhs.shape[0], 128):
                    top = [rhs[r:r + 16, c:c + 128] for c in range(0, rhs.shape[1], 128)]
                    top = [_unpack(self.link(tied[i, r, c * 128], _pack(t0)))
                           if (i, r, c * 128) in tied else t0 for c, t0 in enumerate(top)]
                    parts += [jnp.concatenate(top, axis=1), rhs[r + 16:r + 128, :]]
                rhs = jnp.concatenate(parts, axis=0)
            outs.append(jnp.dot(lhs, rhs, preferred_element_type=f32))
        return outs

    def dot(self, lhs, rhs):
        return self.dots([(lhs, rhs)])[0]


def _kernel(x_hbm, wqkv_hbm, wo_hbm, wg_hbm, wu_hbm, wd_hbm, gw_hbm, out_hbm,
            x_vm, xn, xa, gw_vm, wgu, wd, acc, q_s, k_s, v_s, gs, woc, zs, zi, sems):
    sem_ids = iter(range(10, 1000))

    def cp(src, dst, sem=None):
        return pltpu.make_async_copy(src, dst, sems.at[next(sem_ids) if sem is None else sem])

    def cp_gu(j, slot):
        col = j * FC if isinstance(j, int) else pl.multiple_of(j * FC, FC)
        return [cp((wg_hbm, wu_hbm)[p % 2].at[:, pl.ds(col + (p // 2) * CH, CH)],
                   wgu.at[slot, :, pl.ds(p * CH, CH)], slot * 5 + p) for p in range(4)]

    def cp_d(j, slot):
        row = j * FC if isinstance(j, int) else pl.multiple_of(j * FC, FC)
        return [cp(wd_hbm.at[pl.ds(row, FC), :], wd.at[slot], slot * 5 + 4)]

    x2 = x_hbm.at[0]
    o2 = out_hbm.at[0]
    cp_gw = cp(gw_hbm, gw_vm)
    cp_x = [[cp(x2.at[pl.ds(hf * H + rb * RB, RB), :], x_vm.at[pl.ds(hf * H + rb * RB, RB), :])
             for hf in range(2)] for rb in range(NRB)]
    out_sem = _N_SEMS - 20

    def start(cs):
        for c in cs:
            c.start()

    def wait(cs):
        for c in cs:
            c.wait()

    gu0 = cp_gu(0, 0)
    start([cp_x[0][0]] + gu0 + [cp_x[0][1], cp_gw])

    zs[...] = jnp.zeros((8, 128), i32)
    zi[0] = 1
    sp = _Spreader(zs)

    def rows(rb, hf=0):
        return slice(hf * H + rb * RB, hf * H + (rb + 1) * RB)

    def x_lhs(t, rb):
        if t == 2:
            return _unpack(xn[_half(rows(rb, 0)), :KH])
        if t == 3:
            return _unpack(xn[_half(rows(rb, 1)), KH:])
        return _unpack(xa[_A_SLOT[t], _half(rows(rb)), :])

    def prep_tasks(rb, sums=True, gate=True):
        def task(s0):
            def run(first):
                prev = None
                gw = gw_vm[...].astype(f32)
                r = [slice(hf * H + rb * RB + s0, hf * H + rb * RB + s0 + 16) for hf in range(2)]
                z = [None, None]
                for c in range(4):
                    cols = [slice(kh * KH + c * 128, kh * KH + (c + 1) * 128) for kh in range(2)]
                    xs = [sp.link(prev, _pack(x_vm[r[qd // 2], cols[qd % 2]])) for qd in range(4)]
                    a = [_unpack(t).astype(f32) for t in xs]
                    outs = []
                    if sums:
                        for qd in range(4):
                            xn[_half(r[qd // 2]), cols[qd % 2]] = xs[qd]
                        cs = _a_combos(*a)
                        for t, slot in _A_SLOT.items():
                            outs.append(_pack(cs[t]))
                            xa[slot, _half(r[0]), cols[0]] = outs[-1]
                    if gate:
                        for qd in range(4):
                            g0 = (qd % 2) * 4 + c
                            term = a[qd] * gw[g0:g0 + 1, :]
                            z[qd // 2] = term if z[qd // 2] is None else z[qd // 2] + term
                        outs += z
                    prev = sp.chain(outs, prev, 1)
                if gate:
                    for hf in range(2):
                        g = jax.nn.sigmoid(jnp.sum(z[hf], axis=1, keepdims=True))
                        g = jnp.broadcast_to(g, (16, 128))
                        gs[r[hf], :] = g
                        prev = sp.chain([g], prev, 1)
                return sp.chain([prev], first, 1)
            return run
        return [task(s0) for s0 in range(0, RB, 16)]

    def b_sum_tasks(src, dst):
        def task(r0):
            def run(prev):
                raw = [src(slice(a * KH + r0, a * KH + r0 + 16), slice(c * KH, (c + 1) * KH))
                       for a in range(2) for c in range(2)]
                cs = _b_combos(*[b.astype(f32) for b in raw])
                for t in _B_SUMS:
                    dst.setdefault(t, []).append(_pack(cs[t]))
                return sp.chain([dst[t][-1] for t in _B_SUMS], prev, DEPTH)
            return run
        return [task(r0) for r0 in range(0, KH, 16)]

    def b_rhs(src, sums):
        def rhs(t):
            if t == 1:
                return src(slice(0, KH), slice(0, KH))
            if t == 4:
                return src(slice(KH, D), slice(KH, D))
            return _unpack(jnp.concatenate(sums[t], axis=0))
        return rhs

    def strassen_x(order, rhs, finish):
        m = {}
        for rb, t in order:
            m.setdefault(rb, {})[t] = sp.dot(x_lhs(t, rb), rhs(t))
            if len(m[rb]) == 7:
                finish(rb, _c_combos(m.pop(rb)))

    def glu_tasks(hs, rb, cs, sub):
        hs[rb] = [[] for _ in range(7)]

        def task(r0):
            def run(prev=None):
                h = []
                for qd, cc in enumerate(cs):
                    g0 = (qd // 2) * H + rb * RB + r0
                    omg = 1.0 - gs[g0:g0 + sub, :]
                    omg = jnp.concatenate([omg] * (CH // 128), axis=1)
                    h.append(jnp.maximum(cc[r0:r0 + sub, :CH], 0.0) * cc[r0:r0 + sub, CH:] * omg)
                sums = _a_combos(*h)
                for t in range(7):
                    hs[rb][t].append(sums[t])
                if sub < RB:
                    return sp.chain([sums[t] for t in _A_SLOT], prev, DEPTH2)
            return run
        return [task(r0) for r0 in range(0, RB, sub)]

    def down_lhs(hs, b, ha):
        tok = None
        for t in H_ORDER:
            s0, s1 = [jnp.concatenate(hs[rb][t], axis=0) for rb in (b, b + 2)]
            slabs = []
            for r in range(0, RB, 16):
                slabs.append(sp.serial_combos(
                    _a_combos, s0[r:r + 16, :CQ], s0[r:r + 16, CQ:],
                    s1[r:r + 16, :CQ], s1[r:r + 16, CQ:], tok))
                tok = sp.chain([slabs[-1][t2] for t2 in _A_SLOT], None, H_DEPTH)
            for t2 in range(7):
                ha[b, 7 * t + t2] = jnp.concatenate([sl[t2] for sl in slabs], axis=0).astype(bf16)

    def d_tasks(slot, dst):
        def task(r0, c):
            def run(prev):
                def blk(k1, k2, n1, n2):
                    r, c0 = k1 * CH + k2 * CQ + r0, n1 * KH + n2 * KQ + c * 128
                    return wd[slot, r:r + 16, c0:c0 + 128].astype(f32)
                cs, tok = sp.two_level(_b_combos, blk, prev, DEPTH2)
                for t in range(49):
                    dst.setdefault((t, c), []).append(cs[t])
                return tok
            return run
        return [task(r0, c) for r0 in range(0, CQ, 16) for c in range(2)]

    def ffn_down(ha, dc, first):
        rhs = [_unpack(jnp.concatenate([jnp.concatenate(dc[t, c], axis=0) for c in range(2)], axis=1))
               for t in range(49)]
        todo = [(b, 7 * t + t2) for b in range(2) for t in H_ORDER for t2 in range(7)]
        for i in range(0, len(todo), 2):
            pair = todo[i:i + 2]
            ps = sp.dots([(ha[b, t], rhs[t]) for b, t in pair])
            for (b, t), p in zip(pair, ps):
                if first:
                    acc[t, b * RB:(b + 1) * RB, :] = p
                else:
                    acc[t, b * RB:(b + 1) * RB, :] += p

    def perm_tasks(wqkv_vm, wp, i, tbuf):
        def fwd(rb, c):
            def run(prev):
                c0 = i * D + c * 128
                tt = pltpu.bitcast(wqkv_vm[rb * 256:(rb + 1) * 256, c0:c0 + 128], f32).T
                for hh in range(4):
                    tbuf[rb, pl.ds((4 * c + hh) * TP, DH), :] = tt[hh * DH:(hh + 1) * DH, :]
                return sp.chain([tt], prev, 1)
            return run

        def bwd(rb, j):
            def run(prev):
                g = jnp.concatenate(
                    [tbuf[rb, pl.ds(4 * j + dd, NH, stride=TP), :] for dd in range(4)], axis=0).T
                wp[i, rb * 128:(rb + 1) * 128, j * 128:(j + 1) * 128] = pltpu.bitcast(g, i32)
            return run
        tasks = []
        for rb in range(4):
            tasks += [fwd(rb, c) for c in range(8)] + [bwd(rb, j) for j in range(8)]
        return tasks

    def wo_tasks(wo_vm):
        def stage(c):
            return 4 + c % 4, (c // 4) * NH * TP

        def spread(h0):
            def run(prev):
                blk = wo_vm[h0 * DH:(h0 + 2) * DH, :].astype(f32)
                for h in range(2):
                    for c in range(8):
                        sl, r0 = stage(c)
                        q_s[sl, pl.ds(r0 + (h0 + h) * TP, DH), :] = (
                            blk[h * DH:(h + 1) * DH, c * 128:(c + 1) * 128])
                return sp.chain([blk], prev, 1)
            return run

        def gather(d, h0, c):
            def run(prev):
                def blk(k1, k2, n1, n2):
                    sl, r0 = stage(4 * n1 + 2 * n2 + c)
                    r0 += h0 * TP + 16 * k1 + 8 * k2 + d
                    return q_s[sl, pl.ds(r0, 16, stride=TP), :]
                cs, tok = sp.two_level(_b_combos, blk, prev, DEPTH2)
                r = (d * NH + h0) // 2
                for t in range(49):
                    woc[t, r:r + 8, c * 128:(c + 1) * 128] = cs[t]
                return tok
            return run
        return ([spread(h0) for h0 in range(0, NH, 2)],
                [gather(d, h0, c) for d in range(8) for h0 in (0, 16) for c in range(2)])

    def proj(wp, i, dst, pad, slabs):
        lhs = jnp.concatenate([xn[r0 // 2:(r0 + n) // 2, :] for r0, n in slabs], axis=0)
        p = sp.dot(_unpack(lhs), _unpack(wp[i]))
        at = 0
        for r0, n in slabs:
            for j in range(8):
                dst[j, pad + r0:pad + r0 + n, :] = p[at:at + n, j * 128:(j + 1) * 128]
            at += n

    def v_finish(rb, cs):
        for qd, cc in enumerate(cs):
            r0 = PAD + (qd // 2) * H + rb * RB
            for j in range(4):
                v_s[(qd % 2) * 4 + j, r0:r0 + RB, :] = cc[:, j * 128:(j + 1) * 128]
        if rb == 0:
            for j in range(8):
                src = cs[j // 4][0:1, (j % 4) * 128:(j % 4 + 1) * 128]
                v_s[j, 0:PAD, :] = jnp.broadcast_to(src, (PAD, 128))

    def attn_group(row, masked):
        def run(prev):
            g = 8
            q = [q_s[j, pl.ds(row, g), :] for j in range(8)]
            ls = []
            for w in range(W):
                a = None
                for j in range(8):
                    term = q[j] * k_s[j, pl.ds(row + (PAD - DIL * w), g), :]
                    a = sp.link(ls[-1] if ls else None, term) if a is None else a + term
                ls.append(a)
            rs = [pltpu.roll(a, 64, 1) for a in ls]
            ls = [a + r for a, r in zip(ls, rs)]
            rs = [pltpu.roll(a, 32, 1) for a in ls]
            ls = [a + r for a, r in zip(ls, rs)]
            if masked:
                ri = row + lax.broadcasted_iota(i32, (g, 128), 0)
                ls = [ls[0]] + [jnp.where(ri >= DIL * w, ls[w], NEG) for w in range(1, W)]
            m = _tree(jnp.maximum, ls)
            ps = [jnp.exp2((l - m) * EXP2_SCALE) for l in ls]
            r = gs[pl.ds(row, g), :] / _tree(jnp.add, ps)
            outs = []
            for j in range(8):
                a = None
                for w in range(W):
                    term = ps[w] * v_s[j, pl.ds(row + (PAD - DIL * w), g), :]
                    a = sp.link(outs[-1] if outs else None, term) if a is None else a + term
                outs.append(a * r)
            for j in range(8):
                q_s[j, pl.ds(row, g), :] = outs[j]
            return sp.chain([outs[-1]], prev, 1)
        return run

    def attn_tasks(base, nrows, first=False):
        return [attn_group(base + (qq * Q + r), first and qq == 0 and r < PAD)
                for r in range(0, nrows, 8) for qq in range(4)]

    def pack_tasks(oa, base, hbase, nrows):
        def task(r, c):
            def run(prev):
                def blk(i1, i2, k1, k2):
                    return q_s[4 * k1 + 2 * k2 + c, pl.ds(base + (i1 * H + i2 * Q + r), 16), :]
                cs, tok = sp.two_level(_a_combos, blk, prev, DEPTH2)
                for t in range(49):
                    oa[t, pl.ds(hbase + r // 2, 8), c * 128:(c + 1) * 128] = cs[t]
                return tok
            return run
        return [task(r, c) for r in range(0, nrows, 16) for c in range(2)]

    GS = RB * (KH // 128) * (FC // 128) * 7 // (4 * SLOT)
    DS = 49
    PS = 2 * RB * (D // 128) * (D // 128) // (4 * SLOT)

    def glu(hs):
        return lambda rb, cs: glu_tasks(hs, rb, cs, RB)[0]()

    def raw_first(first, rest):
        return ([(rb, t) for rb in first for t in ORDER[:2]]
                + [(rb, t) for rb in first for t in ORDER[2:]]
                + [(rb, t) for rb in rest for t in ORDER])

    def gu_src(slot):
        return lambda r, c: wgu[slot, r, c]

    def front(wqkv_vm, wp, wo_vm):
        cp_qkv = [cp(wqkv_hbm.at[:, pl.ds(i * D, D)], wqkv_vm.at[:, pl.ds(i * D, D)])
                  for i in range(3)]
        cp_wo = cp(wo_hbm, wo_vm)

        def plain(rb, hf, p):
            return sp.dot(x_vm[rows(rb, hf), :], wgu[0, :, p * CH:(p + 1) * CH])

        def plain_finish(rb, c):
            cs = [jnp.concatenate(c[2 * qd:2 * qd + 2], axis=1) for qd in range(4)]
            return glu_tasks(hs, rb, cs, 16)

        hs, bc, dc, c0 = {}, {}, {}, []
        with _Scope("w0"):
            wait([cp_x[0][0], gu0[0]])
        with _Scope("p1a"):
            for p in range(4):
                if p:
                    wait([gu0[p]])
                if p == 1:
                    start(cp_x[1] + cp_x[2])
                c0.append(plain(0, 0, p))
            wait([cp_x[0][1], cp_gw])
            start(cp_x[3] + cp_d(0, 0))
            sp.block()
            bt = b_sum_tasks(gu_src(0), bc)
            sp.schedule(bt[:12], 3, 16)
            sp.schedule(prep_tasks(0, sums=False), 3, 16)
            c0 += [plain(0, 1, p) for p in range(4)]
        with _Scope("w1"):
            wait(cp_x[1] + cp_x[2])
            start(cp_qkv[2:])
        with _Scope("p1b"):
            sp.block()
            sp.schedule(bt[12:], 3, 32)
            sp.schedule(prep_tasks(1, sums=False), 2, 10)
            sp.schedule(prep_tasks(2), 10, 32)
            c1 = [plain(1, hf, p) for hf in range(2) for p in range(4)]
        with _Scope("w2"):
            wait(cp_x[3] + cp_d(0, 0) + cp_qkv[2:])
            start([cp_qkv[1], cp_wo, cp_qkv[0]] + cp_gu(1, 1) + cp_d(1, 1))
        with _Scope("p1c"):
            sp.block()
            for j in range(8):
                k_s[j, 0:PAD, :] = jnp.zeros((PAD, 128), f32)
            ha = {}
            sp.schedule(prep_tasks(3), 2, GS)
            sp.schedule(plain_finish(0, c0), 2, GS)
            sp.schedule(plain_finish(1, c1), GS + 6, 2 * GS)
            sp.schedule(d_tasks(0, dc), GS - 2, 2 * GS)
            sp.schedule(perm_tasks(wqkv_vm, wp, 2, q_s), 2 * GS + 6, 2 * GS + DS - 8)
            strassen_x([(rb, t) for rb in (2, 3) for t in ORDER], b_rhs(gu_src(0), bc), glu(hs))
            down_lhs(hs, 0, ha)
            down_lhs(hs, 1, ha)
            ffn_down(ha, dc, True)

        with _Scope("w2b"):
            wait([cp_qkv[1], cp_wo])
        with _Scope("v"):
            sp.block()
            vb = {}
            v_src = lambda r, c: _unpack(wp[2, _half(r), c])
            wo_spread, wo_gather = wo_tasks(wo_vm)
            sp.schedule(b_sum_tasks(v_src, vb), *BC_SLOTS)
            sp.schedule(prep_tasks(0, gate=False) + prep_tasks(1, gate=False), 16, 2 * GS)
            sp.schedule(perm_tasks(wqkv_vm, wp, 1, k_s.at[:, PAD:, :]), 2 * GS, 4 * GS - 8)
            sp.schedule(wo_spread, 2 * GS, 4 * GS)
            strassen_x(raw_first((2, 3), (0, 1)), b_rhs(v_src, vb), v_finish)
        with _Scope("w3"):
            wait(cp_qkv[:1] + cp_gu(1, 1) + cp_d(1, 1))
        with _Scope("kq"):
            sp.block()
            sp.schedule(perm_tasks(wqkv_vm, wp, 0, q_s), 4, 3 * PS)
            sp.schedule(wo_gather, 4, NRB * PS)
            for rb in range(NRB):
                proj(wp, 1, k_s, PAD, [(rb * Q, Q)])
            proj(wp, 0, q_s, 0, [(qq * Q, QA) for qq in range(4)])

        def q_rest(_, carry):
            with _Scope("q"):
                sp.block()
                n = (Q - QA) // 2
                total = 4 * (Q - QA) * 64 // (4 * SLOT)
                sp.schedule(attn_tasks(0, A0, True), 4, total)
                for r0 in (QA, QA + n):
                    proj(wp, 0, q_s, 0, [(qq * Q + r0, n) for qq in range(4)])
            return carry

        lax.fori_loop(0, zi[0], q_rest, 0)

    def back(oa):
        def body(j, carry):
            with _Scope("chunk"):
                slot = j % 2
                nxt = jnp.minimum(j + 1, NC - 1)
                prefetch = cp_gu(nxt, 1 - slot) + cp_d(nxt, 1 - slot)
                sp.block()
                base = pl.multiple_of((j - 1) * AR, AR)
                hs, ha, bc, dc = {}, {}, {}, {}
                sp.schedule(b_sum_tasks(gu_src(slot), bc), *BC_SLOTS)
                sp.schedule(attn_tasks(base + A0, AR), *ATTN_SLOTS)
                sp.schedule(pack_tasks(oa, base, pl.multiple_of((j - 1) * (AR // 2), AR // 2), AR),
                            *PACK_SLOTS)
                sp.schedule(d_tasks(slot, dc), *DC_SLOTS)
                start(prefetch)
                strassen_x(raw_first((0, 2), (1, 3)), b_rhs(gu_src(slot), bc), glu(hs))
                down_lhs(hs, 0, ha)
                down_lhs(hs, 1, ha)
                ffn_down(ha, dc, False)
                wait(prefetch)
            return carry

        lax.fori_loop(1, NC, body, 0)

        def out_copies(r0, i1, cols, sem):
            cs = []
            for i2 in range(2):
                idx = (pl.ds(r0 + (i1 * H + i2 * Q), PB), cols)
                cs.append(cp(x_vm.at[idx], o2.at[idx], sem + i2))
            return cs

        def out_blocks(blocks):
            todo = [(blk, 7 * t1 + t2) for blk in range(len(blocks))
                    for ts1, _ in _C_ORDER for t1 in ts1 for ts2, _ in _C_ORDER for t2 in ts2]
            m = {}
            for i in range(0, len(todo), 2):
                pair = todo[i:i + 2]
                ps = sp.dots([(_unpack(oa[t, pl.ds(blocks[blk][1], PB // 2), :]), _unpack(woc[t]))
                              for blk, t in pair])
                for (blk, t), p in zip(pair, ps):
                    r0, _, copies = blocks[blk]
                    mm = m.setdefault(blk, ({}, {}))
                    mm[0][t] = acc[t, pl.ds(r0, PB), :] + p
                    t1 = t // 7
                    if t % 7 != _C_ORDER[-1][0][-1]:
                        continue
                    mm[1][t1] = _c_combos([mm[0].pop(7 * t1 + t2) for t2 in range(7)])
                    for ts, qd in _C_ORDER:
                        if t1 != ts[-1]:
                            continue
                        for q2 in range(4):
                            val = _c_quadrant({tt: v[q2] for tt, v in mm[1].items()}, qd)
                            r = pl.ds(r0 + ((qd // 2) * H + (q2 // 2) * Q), PB)
                            c = (qd % 2) * KH + (q2 % 2) * KQ
                            x_vm[r, c:c + KQ] = val.astype(bf16)
                        start(copies.get(qd, []))

        def whole(r0, sem):
            return [c for i1 in range(2) for c in out_copies(r0, i1, slice(None), sem + 2 * i1)]

        done = (NC - 1) * AR

        def out_body(i, carry):
            with _Scope("p4a"):
                sp.block()
                half = pl.multiple_of(done // 2 + i * 24, 8)
                sp.schedule(pack_tasks(oa, 2 * half, half, 48), 4, 24)
                r0 = pl.multiple_of(i * PB, PB)
                out_blocks([(r0, pl.multiple_of(i * (PB // 2), PB // 2),
                             {3: whole(r0, out_sem + 4 * i)})])
            return carry

        lax.fori_loop(0, 2, out_body, 0)
        with _Scope("p4b"):
            sp.block()
            sp.schedule(pack_tasks(oa, done + 96, (done + 96) // 2, Q - done - 96), 4, 22)
            last = {qd: out_copies(3 * PB, qd // 2, pl.ds((qd % 2) * KH, KH), out_sem + 12 + 2 * qd)
                    for qd in range(4)}
            copies = [{3: whole(blk * PB, out_sem + 4 * blk)} for blk in range(3)] + [last]
            out_blocks([(blk * PB, blk * PB // 2, copies[blk]) for blk in (2, 3)])
        with _Scope("w4"):
            for cs in copies:
                for qd in cs:
                    wait(cs[qd])

    pl.run_scoped(front, pltpu.VMEM((D, 3 * D), bf16), pltpu.VMEM((3, D // 2, D), i32),
                  pltpu.VMEM((D, D), bf16))
    pl.run_scoped(back, pltpu.VMEM((49, Q // 2, KQ), i32))
    assert not sp.plan


_N_SEMS = 10 + 1 + 2 * NRB + 3 + 1 + 20


@jax.jit
def pallas_gated_mix__sliding_local_dilated__glu_gated_reglu__prompt_kernel(
    A_x: jax.Array,
    A_wqkv: jax.Array,
    A_wo: jax.Array,
    B_x: jax.Array,
    B_W_gate: jax.Array,
    B_W_up: jax.Array,
    B_W_down: jax.Array,
    gate_w: jax.Array,
):
    del B_x
    hbm = pl.BlockSpec(memory_space=pl.ANY)
    scratch = [
        pltpu.VMEM((S, D), bf16),
        pltpu.VMEM((S // 2, D), i32),
        pltpu.VMEM((5, H // 2, KH), i32),
        pltpu.VMEM((8, 128), bf16),
        pltpu.VMEM((2, D, 2 * FC), bf16),
        pltpu.VMEM((2, FC, D), bf16),
        pltpu.VMEM((49, Q, KQ), f32),
        pltpu.VMEM((8, S + QPAD + 16, 128), f32),
        pltpu.VMEM((8, PAD + S, 128), f32),
        pltpu.VMEM((8, PAD + S, 128), f32),
        pltpu.VMEM((S, 128), f32),
        pltpu.VMEM((49, KQ // 2, KQ), i32),
        pltpu.VMEM((8, 128), i32),
        pltpu.SMEM((1,), i32),
        pltpu.SemaphoreType.DMA((_N_SEMS,)),
    ]
    return pl.pallas_call(
        _kernel,
        in_specs=[hbm] * 7,
        out_specs=hbm,
        out_shape=jax.ShapeDtypeStruct((1, S, D), bf16),
        scratch_shapes=scratch,
        compiler_params=pltpu.CompilerParams(vmem_limit_bytes=124 * 1024 * 1024),
    )(A_x, A_wqkv, A_wo, B_W_gate, B_W_up, B_W_down, gate_w.reshape(8, 128))
```

```python
import math

import jax
import jax.numpy as jnp
from jax import lax
import jax.experimental.pallas as pl
import jax.experimental.pallas.tpu as pltpu

f32 = jnp.float32
bf16 = jnp.bfloat16
i32 = jnp.int32

S = 2048
D = 1024
F = 3584
NH = 32
DH = D // NH
W = 8
DIL = 2
H = S // 2
Q = S // 4
KH = D // 2
KQ = D // 4
FC = 512
CH = FC // 2
CQ = FC // 4
NC = F // FC
RB = 256
NRB = H // RB
PB = 128
PAD = 16
TP = DH + 1
AR = 64
A0 = Q - 6 * AR
QA = 160
QPAD = 64

ATTN_SLOTS = (32, 112)
PACK_SLOTS = (16, 32)
DC_SLOTS = (32, 108)
BC_SLOTS = (2, 16)
DEPTH = 3
H_ORDER = (0, 1, 2, 3, 4, 5, 6)
DEPTH2 = 3
H_DEPTH = 3
PROFILE = ()

SCALE = DH ** -0.5
EXP2_SCALE = SCALE * math.log2(math.e)
NEG = -1e9 / SCALE


def _a_combos(a11, a12, a21, a22):
    return [a11 + a22, a21 + a22, a11, a22, a11 + a12, a21 - a11, a12 - a22]


def _b_combos(b11, b12, b21, b22):
    return [b11 + b22, b11, b12 - b22, b21 - b11, b22, b11 + b12, b21 + b22]


_C_TERMS = (((1, 0), (1, 3), (-1, 4), (1, 6)), ((1, 2), (1, 4)), ((1, 1), (1, 3)),
            ((1, 0), (-1, 1), (1, 2), (1, 5)))
_C_ORDER = (((2, 4), 1), ((1, 3), 2), ((0, 6), 0), ((5,), 3))


def _c_quadrant(m, qd):
    out = m[_C_TERMS[qd][0][1]]
    for sign, t in _C_TERMS[qd][1:]:
        out = out + m[t] if sign > 0 else out - m[t]
    return out


def _c_combos(m):
    return [_c_quadrant(m, qd) for qd in range(4)]


_A_SLOT = {0: 0, 1: 1, 4: 2, 5: 3, 6: 4}
_B_SUMS = (2, 3, 0, 5, 6)
ORDER = (1, 4) + _B_SUMS


class _Scope:
    def __init__(self, name):
        self.cm = jax.named_scope(name) if (PROFILE is True or name in PROFILE) else None

    def __enter__(self):
        if self.cm is not None:
            self.cm.__enter__()

    def __exit__(self, *a):
        if self.cm is not None:
            self.cm.__exit__(*a)


def _tree(op, xs):
    xs = list(xs)
    while len(xs) > 1:
        xs = [op(xs[i], xs[i + 1]) if i + 1 < len(xs) else xs[i] for i in range(0, len(xs), 2)]
    return xs[0]


def _pack(x):
    return pltpu.bitcast(x.astype(bf16), i32)


def _unpack(x):
    return pltpu.bitcast(x, bf16)


def _half(r):
    return slice(r.start // 2, r.stop // 2)


SLOT = 256


class _Spreader:
    def __init__(self, zero_ref):
        self.zero_ref = zero_ref
        self.plan = {}
        self.now = 0

    def block(self):
        self.zero = self.zero_ref[...]
        self.never = self.zero != 0

    def link(self, after, x):
        if after is None:
            return x
        if after.dtype != x.dtype:
            after = pltpu.bitcast(after, x.dtype)
        return jnp.where(self.never, after, x)

    def chain(self, vals, prev, depth):
        for v in vals:
            v = pltpu.bitcast(v, i32) if v.dtype != i32 else v
            for r in range(0, v.shape[0], 8):
                for c in range(0, v.shape[1], 128):
                    tile = v[r:r + 8, c:c + 128]
                    if prev is None:
                        prev = tile
                        continue
                    prev = prev | tile
                    for i in range(depth - 1):
                        prev = (prev + self.zero) if i % 2 == 0 else (prev ^ self.zero)
        return prev

    def link_rows(self, after, x):
        return jnp.concatenate([self.link(after, x[r:r + 8, :]) for r in range(0, x.shape[0], 8)],
                               axis=0)

    def serial_combos(self, combos, x11, x12, x21, x22, after):
        return combos(self.link_rows(after, x11), x12, x21, self.link_rows(after, x22))

    def two_level(self, combos, blk, prev, depth):
        outer = [combos(*[blk(r1, r2, c1, c2) for r1 in range(2) for c1 in range(2)])
                 for r2 in range(2) for c2 in range(2)]
        outs, tok = [], None
        for t in range(7):
            wide = _pack(jnp.concatenate(
                self.serial_combos(combos, *[o[t] for o in outer], tok), axis=1))
            outs += [wide[:, c:c + 128] for c in range(0, 7 * 128, 128)]
            tok = self.chain(outs[-7:], tok, depth)
        return outs, self.chain([tok], prev, 1)

    def schedule(self, tasks, first, last):
        n = len(tasks)
        for i, t in enumerate(tasks):
            pos = self.now + first + ((i + 1) * (last - first) - 1) // n
            self.plan.setdefault(pos, []).append((t, id(tasks)))

    def dots(self, pairs):
        m = pairs[0][0].shape[0]
        tiles = [(i, r, c) for i, (_, rhs) in enumerate(pairs)
                 for c in range(0, rhs.shape[1], 128) for r in range(0, rhs.shape[0], 128)]
        nslots = m * len(tiles) // (4 * SLOT)
        deps = {}
        for sl in range(nslots):
            ps = sl * SLOT // m
            toks = {}
            for t, lane in self.plan.pop(self.now + sl, []):
                tok = t(toks.get(lane))
                if tok is not None:
                    toks[lane] = tok
            for tok in toks.values():
                deps[ps] = tok | deps[ps] if ps in deps else tok
        self.now += nslots
        tied = {tile: d for ps, d in deps.items() for tile in tiles[4 * ps:4 * ps + 4]}
        outs = []
        for i, (lhs, rhs) in enumerate(pairs):
            if any(key[0] == i for key in tied):
                parts = []
                for r in range(0, rhs.shape[0], 128):
                    top = [rhs[r:r + 16, c:c + 128] for c in range(0, rhs.shape[1], 128)]
                    top = [_unpack(self.link(tied[i, r, c * 128], _pack(t0)))
                           if (i, r, c * 128) in tied else t0 for c, t0 in enumerate(top)]
                    parts += [jnp.concatenate(top, axis=1), rhs[r + 16:r + 128, :]]
                rhs = jnp.concatenate(parts, axis=0)
            outs.append(jnp.dot(lhs, rhs, preferred_element_type=f32))
        return outs

    def dot(self, lhs, rhs):
        return self.dots([(lhs, rhs)])[0]


def _kernel(x_hbm, wqkv_hbm, wo_hbm, wg_hbm, wu_hbm, wd_hbm, gw_hbm, out_hbm,
            x_vm, xn, xa, gw_vm, wgu, wd, acc, q_s, k_s, v_s, gs, woc, zs, zi, sems):
    def cp(src, dst, sem):
        return pltpu.make_async_copy(src, dst, sems.at[sem])

    def cp_gu(j, p, sem):
        return cp((wg_hbm, wu_hbm)[p % 2].at[:, pl.ds(j * FC + (p // 2) * CH, CH)],
                  wgu.at[j, :, pl.ds(p * CH, CH)], sem)

    def cp_d(j, sem):
        return cp(wd_hbm.at[pl.ds(j * FC, FC), :], wd.at[j], sem)

    def cp_x(rb, hf, sem):
        idx = (pl.ds(hf * H + rb * RB, RB), slice(None))
        return cp(x_hbm.at[0].at[idx], x_vm.at[idx], sem)

    o2 = out_hbm.at[0]
    in0 = [cp_x(0, 0, 0), cp_gu(0, 0, 0)]
    in1 = [cp_x(0, 1, 1)]
    in2 = [cp_gu(0, 1, 2)]
    in3 = [cp_gu(0, 2, 3), cp_gu(0, 3, 3), cp(gw_hbm, gw_vm, 3)]
    in4 = [cp_x(rb, hf, 4) for rb in (1, 2) for hf in range(2)]
    in5 = [cp_x(3, 0, 5), cp_x(3, 1, 5), cp_d(0, 5)]
    in_ffn = [c for j in range(1, NC) for c in [cp_gu(j, p, 8) for p in range(4)] + [cp_d(j, 8)]]
    out_sem = 9

    def start(cs):
        for c in cs:
            c.start()

    def wait(cs):
        for c in cs:
            c.wait()

    start(in0 + in1 + in2)

    zs[...] = jnp.zeros((8, 128), i32)
    zi[0] = 1
    sp = _Spreader(zs)

    def rows(rb, hf=0):
        return slice(hf * H + rb * RB, hf * H + (rb + 1) * RB)

    def x_lhs(t, rb):
        if t == 2:
            return _unpack(xn[_half(rows(rb, 0)), :KH])
        if t == 3:
            return _unpack(xn[_half(rows(rb, 1)), KH:])
        return _unpack(xa[_A_SLOT[t], _half(rows(rb)), :])

    def prep_tasks(rb, sums=True, gate=True):
        def task(s0):
            def run(first):
                prev = None
                gw = gw_vm[...].astype(f32)
                r = [slice(hf * H + rb * RB + s0, hf * H + rb * RB + s0 + 16) for hf in range(2)]
                z = [None, None]
                for c in range(4):
                    cols = [slice(kh * KH + c * 128, kh * KH + (c + 1) * 128) for kh in range(2)]
                    xs = [sp.link(prev, _pack(x_vm[r[qd // 2], cols[qd % 2]])) for qd in range(4)]
                    a = [_unpack(t).astype(f32) for t in xs]
                    outs = []
                    if sums:
                        for qd in range(4):
                            xn[_half(r[qd // 2]), cols[qd % 2]] = xs[qd]
                        cs = _a_combos(*a)
                        for t, slot in _A_SLOT.items():
                            outs.append(_pack(cs[t]))
                            xa[slot, _half(r[0]), cols[0]] = outs[-1]
                    if gate:
                        for qd in range(4):
                            g0 = (qd % 2) * 4 + c
                            term = a[qd] * gw[g0:g0 + 1, :]
                            z[qd // 2] = term if z[qd // 2] is None else z[qd // 2] + term
                        outs += z
                    prev = sp.chain(outs, prev, 1)
                if gate:
                    for hf in range(2):
                        g = jax.nn.sigmoid(jnp.sum(z[hf], axis=1, keepdims=True))
                        g = jnp.broadcast_to(g, (16, 128))
                        gs[r[hf], :] = g
                        prev = sp.chain([g], prev, 1)
                return sp.chain([prev], first, 1)
            return run
        return [task(s0) for s0 in range(0, RB, 16)]

    def b_sum_tasks(src, dst):
        def task(r0):
            def run(prev):
                raw = [src(slice(a * KH + r0, a * KH + r0 + 16), slice(c * KH, (c + 1) * KH))
                       for a in range(2) for c in range(2)]
                cs = _b_combos(*[b.astype(f32) for b in raw])
                for t in _B_SUMS:
                    dst.setdefault(t, []).append(_pack(cs[t]))
                return sp.chain([dst[t][-1] for t in _B_SUMS], prev, DEPTH)
            return run
        return [task(r0) for r0 in range(0, KH, 16)]

    def b_rhs(src, sums):
        def rhs(t):
            if t == 1:
                return src(slice(0, KH), slice(0, KH))
            if t == 4:
                return src(slice(KH, D), slice(KH, D))
            return _unpack(jnp.concatenate(sums[t], axis=0))
        return rhs

    def strassen_x(order, rhs, finish):
        m = {}
        for rb, t in order:
            m.setdefault(rb, {})[t] = sp.dot(x_lhs(t, rb), rhs(t))
            if len(m[rb]) == 7:
                finish(rb, _c_combos(m.pop(rb)))

    def glu_tasks(hs, rb, cs, sub):
        hs[rb] = [[] for _ in range(7)]

        def task(r0):
            def run(prev=None):
                h = []
                for qd, cc in enumerate(cs):
                    g0 = (qd // 2) * H + rb * RB + r0
                    omg = 1.0 - gs[g0:g0 + sub, :]
                    omg = jnp.concatenate([omg] * (CH // 128), axis=1)
                    h.append(jnp.maximum(cc[r0:r0 + sub, :CH], 0.0) * cc[r0:r0 + sub, CH:] * omg)
                sums = _a_combos(*h)
                for t in range(7):
                    hs[rb][t].append(sums[t])
                if sub < RB:
                    return sp.chain([sums[t] for t in _A_SLOT], prev, DEPTH2)
            return run
        return [task(r0) for r0 in range(0, RB, sub)]

    def down_lhs(hs, b, ha):
        tok = None
        for t in H_ORDER:
            s0, s1 = [jnp.concatenate(hs[rb][t], axis=0) for rb in (b, b + 2)]
            slabs = []
            for r in range(0, RB, 16):
                slabs.append(sp.serial_combos(
                    _a_combos, s0[r:r + 16, :CQ], s0[r:r + 16, CQ:],
                    s1[r:r + 16, :CQ], s1[r:r + 16, CQ:], tok))
                tok = sp.chain([slabs[-1][t2] for t2 in _A_SLOT], None, H_DEPTH)
            for t2 in range(7):
                ha[b, 7 * t + t2] = jnp.concatenate([sl[t2] for sl in slabs], axis=0).astype(bf16)

    def d_tasks(j, dst):
        def task(r0, c):
            def run(prev):
                def blk(k1, k2, n1, n2):
                    r, c0 = k1 * CH + k2 * CQ + r0, n1 * KH + n2 * KQ + c * 128
                    return wd[j, r:r + 16, c0:c0 + 128].astype(f32)
                cs, tok = sp.two_level(_b_combos, blk, prev, DEPTH2)
                for t in range(49):
                    dst.setdefault((t, c), []).append(cs[t])
                return tok
            return run
        return [task(r0, c) for r0 in range(0, CQ, 16) for c in range(2)]

    def ffn_down(ha, dc, first):
        rhs = [_unpack(jnp.concatenate([jnp.concatenate(dc[t, c], axis=0) for c in range(2)], axis=1))
               for t in range(49)]
        todo = [(b, 7 * t + t2) for b in range(2) for t in H_ORDER for t2 in range(7)]
        for i in range(0, len(todo), 2):
            pair = todo[i:i + 2]
            ps = sp.dots([(ha[b, t], rhs[t]) for b, t in pair])
            for (b, t), p in zip(pair, ps):
                if first:
                    acc[t, b * RB:(b + 1) * RB, :] = p
                else:
                    acc[t, b * RB:(b + 1) * RB, :] += p

    def perm_tasks(wqkv_vm, wp, i, tbuf):
        def fwd(rb, c):
            def run(prev):
                c0 = i * D + c * 128
                tt = pltpu.bitcast(wqkv_vm[rb * 256:(rb + 1) * 256, c0:c0 + 128], f32).T
                for hh in range(4):
                    tbuf[rb, pl.ds((4 * c + hh) * TP, DH), :] = tt[hh * DH:(hh + 1) * DH, :]
                return sp.chain([tt], prev, 1)
            return run

        def bwd(rb, j):
            def run(prev):
                g = jnp.concatenate(
                    [tbuf[rb, pl.ds(4 * j + dd, NH, stride=TP), :] for dd in range(4)], axis=0).T
                wp[i, rb * 128:(rb + 1) * 128, j * 128:(j + 1) * 128] = pltpu.bitcast(g, i32)
            return run
        tasks = []
        for rb in range(4):
            tasks += [fwd(rb, c) for c in range(8)] + [bwd(rb, j) for j in range(8)]
        return tasks

    def wo_tasks(wo_vm):
        def stage(c):
            return 4 + c % 4, (c // 4) * NH * TP

        def spread(h0):
            def run(prev):
                blk = wo_vm[h0 * DH:(h0 + 2) * DH, :].astype(f32)
                for h in range(2):
                    for c in range(8):
                        sl, r0 = stage(c)
                        q_s[sl, pl.ds(r0 + (h0 + h) * TP, DH), :] = (
                            blk[h * DH:(h + 1) * DH, c * 128:(c + 1) * 128])
                return sp.chain([blk], prev, 1)
            return run

        def gather(d, h0, c):
            def run(prev):
                def blk(k1, k2, n1, n2):
                    sl, r0 = stage(4 * n1 + 2 * n2 + c)
                    r0 += h0 * TP + 16 * k1 + 8 * k2 + d
                    return q_s[sl, pl.ds(r0, 16, stride=TP), :]
                cs, tok = sp.two_level(_b_combos, blk, prev, DEPTH2)
                r = (d * NH + h0) // 2
                for t in range(49):
                    woc[t, r:r + 8, c * 128:(c + 1) * 128] = cs[t]
                return tok
            return run
        return ([spread(h0) for h0 in range(0, NH, 2)],
                [gather(d, h0, c) for d in range(8) for h0 in (0, 16) for c in range(2)])

    def proj(wp, i, dst, pad, slabs):
        lhs = jnp.concatenate([xn[r0 // 2:(r0 + n) // 2, :] for r0, n in slabs], axis=0)
        p = sp.dot(_unpack(lhs), _unpack(wp[i]))
        at = 0
        for r0, n in slabs:
            for j in range(8):
                dst[j, pad + r0:pad + r0 + n, :] = p[at:at + n, j * 128:(j + 1) * 128]
            at += n

    def v_finish(rb, cs):
        for qd, cc in enumerate(cs):
            r0 = PAD + (qd // 2) * H + rb * RB
            for j in range(4):
                v_s[(qd % 2) * 4 + j, r0:r0 + RB, :] = cc[:, j * 128:(j + 1) * 128]
        if rb == 0:
            for j in range(8):
                src = cs[j // 4][0:1, (j % 4) * 128:(j % 4 + 1) * 128]
                v_s[j, 0:PAD, :] = jnp.broadcast_to(src, (PAD, 128))

    def attn_group(row, masked):
        def run(prev):
            g = 8
            q = [q_s[j, pl.ds(row, g), :] for j in range(8)]
            ls = []
            for w in range(W):
                a = None
                for j in range(8):
                    term = q[j] * k_s[j, pl.ds(row + (PAD - DIL * w), g), :]
                    a = sp.link(ls[-1] if ls else None, term) if a is None else a + term
                ls.append(a)
            rs = [pltpu.roll(a, 64, 1) for a in ls]
            ls = [a + r for a, r in zip(ls, rs)]
            rs = [pltpu.roll(a, 32, 1) for a in ls]
            ls = [a + r for a, r in zip(ls, rs)]
            if masked:
                ri = row + lax.broadcasted_iota(i32, (g, 128), 0)
                ls = [ls[0]] + [jnp.where(ri >= DIL * w, ls[w], NEG) for w in range(1, W)]
            m = _tree(jnp.maximum, ls)
            ps = [jnp.exp2((l - m) * EXP2_SCALE) for l in ls]
            r = gs[pl.ds(row, g), :] / _tree(jnp.add, ps)
            outs = []
            for j in range(8):
                a = None
                for w in range(W):
                    term = ps[w] * v_s[j, pl.ds(row + (PAD - DIL * w), g), :]
                    a = sp.link(outs[-1] if outs else None, term) if a is None else a + term
                outs.append(a * r)
            for j in range(8):
                q_s[j, pl.ds(row, g), :] = outs[j]
            return sp.chain([outs[-1]], prev, 1)
        return run

    def attn_tasks(base, nrows, first=False):
        return [attn_group(base + (qq * Q + r), first and qq == 0 and r < PAD)
                for r in range(0, nrows, 8) for qq in range(4)]

    def pack_tasks(oa, base, hbase, nrows):
        def task(r, c):
            def run(prev):
                def blk(i1, i2, k1, k2):
                    return q_s[4 * k1 + 2 * k2 + c, pl.ds(base + (i1 * H + i2 * Q + r), 16), :]
                cs, tok = sp.two_level(_a_combos, blk, prev, DEPTH2)
                for t in range(49):
                    oa[t, pl.ds(hbase + r // 2, 8), c * 128:(c + 1) * 128] = cs[t]
                return tok
            return run
        return [task(r, c) for r in range(0, nrows, 16) for c in range(2)]

    GS = RB * (KH // 128) * (FC // 128) * 7 // (4 * SLOT)
    DS = 49
    PS = 2 * RB * (D // 128) * (D // 128) // (4 * SLOT)

    def glu(hs):
        return lambda rb, cs: glu_tasks(hs, rb, cs, RB)[0]()

    def raw_first(first, rest):
        return ([(rb, t) for rb in first for t in ORDER[:2]]
                + [(rb, t) for rb in first for t in ORDER[2:]]
                + [(rb, t) for rb in rest for t in ORDER])

    def gu_src(j):
        return lambda r, c: wgu[j, r, c]

    def front(wqkv_vm, wp, wo_vm):
        in_q, in_k, in_v = [
            cp(wqkv_hbm.at[:, pl.ds(i * D, D)], wqkv_vm.at[:, pl.ds(i * D, D)], 7 - i)
            for i in range(3)]
        in_wo = cp(wo_hbm, wo_vm, 6)

        def plain(rb, hf, p):
            return sp.dot(x_vm[rows(rb, hf), :], wgu[0, :, p * CH:(p + 1) * CH])

        def plain_finish(rb, c):
            cs = [jnp.concatenate(c[2 * qd:2 * qd + 2], axis=1) for qd in range(4)]
            return glu_tasks(hs, rb, cs, 16)

        hs, bc, dc = {}, {}, {}
        with _Scope("w0"):
            wait(in0)
        start(in3)
        c0 = {(0, 0): plain(0, 0, 0)}
        with _Scope("wa"):
            wait(in1)
        c0[1, 0] = plain(0, 1, 0)
        with _Scope("wb"):
            wait(in2)
        start(in4)
        for hf in range(2):
            c0[hf, 1] = plain(0, hf, 1)
        with _Scope("wc"):
            wait(in3)
        with _Scope("p1a"):
            start(in5)
            sp.block()
            bt = b_sum_tasks(gu_src(0), bc)
            sp.schedule(bt[:12], 3, 16)
            sp.schedule(prep_tasks(0, sums=False), 3, 16)
            for p in (2, 3):
                for hf in range(2):
                    c0[hf, p] = plain(0, hf, p)
            c0 = [c0[hf, p] for hf in range(2) for p in range(4)]
        with _Scope("w1"):
            wait(in4)
            start([in_v])
        with _Scope("p1b"):
            sp.block()
            sp.schedule(bt[12:], 3, 32)
            sp.schedule(prep_tasks(1, sums=False), 2, 10)
            sp.schedule(prep_tasks(2), 10, 32)
            c1 = [plain(1, hf, p) for hf in range(2) for p in range(4)]
        with _Scope("w2"):
            wait(in5 + [in_v])
            start([in_k, in_wo, in_q])
        with _Scope("p1c"):
            sp.block()
            for j in range(8):
                k_s[j, 0:PAD, :] = jnp.zeros((PAD, 128), f32)
            ha = {}
            sp.schedule(prep_tasks(3), 2, GS)
            sp.schedule(plain_finish(0, c0), 2, GS)
            sp.schedule(plain_finish(1, c1), GS + 6, 2 * GS)
            sp.schedule(d_tasks(0, dc), GS - 2, 2 * GS)
            sp.schedule(perm_tasks(wqkv_vm, wp, 2, q_s), 2 * GS + 6, 2 * GS + DS - 8)
            strassen_x([(rb, t) for rb in (2, 3) for t in ORDER], b_rhs(gu_src(0), bc), glu(hs))
            down_lhs(hs, 0, ha)
            down_lhs(hs, 1, ha)
            ffn_down(ha, dc, True)

        with _Scope("w2b"):
            wait([in_k, in_wo])
            start(in_ffn)
        with _Scope("v"):
            sp.block()
            vb = {}
            v_src = lambda r, c: _unpack(wp[2, _half(r), c])
            wo_spread, wo_gather = wo_tasks(wo_vm)
            sp.schedule(b_sum_tasks(v_src, vb), *BC_SLOTS)
            sp.schedule(prep_tasks(0, gate=False) + prep_tasks(1, gate=False), 16, 2 * GS)
            sp.schedule(perm_tasks(wqkv_vm, wp, 1, k_s.at[:, PAD:, :]), 2 * GS, 4 * GS - 8)
            sp.schedule(wo_spread, 2 * GS, 4 * GS)
            strassen_x(raw_first((2, 3), (0, 1)), b_rhs(v_src, vb), v_finish)
        with _Scope("w3"):
            wait([in_q])
        with _Scope("kq"):
            sp.block()
            sp.schedule(perm_tasks(wqkv_vm, wp, 0, q_s), 4, 3 * PS)
            sp.schedule(wo_gather, 4, NRB * PS)
            for rb in range(NRB):
                proj(wp, 1, k_s, PAD, [(rb * Q, Q)])
            proj(wp, 0, q_s, 0, [(qq * Q, QA) for qq in range(4)])

        def q_rest(_, carry):
            with _Scope("q"):
                sp.block()
                n = (Q - QA) // 2
                total = 4 * (Q - QA) * 64 // (4 * SLOT)
                sp.schedule(attn_tasks(0, A0, True), 4, total)
                for r0 in (QA, QA + n):
                    proj(wp, 0, q_s, 0, [(qq * Q + r0, n) for qq in range(4)])
            return carry

        lax.fori_loop(0, zi[0], q_rest, 0)
        wait(in_ffn)

    def back(oa):
        def body(j, carry):
            with _Scope("chunk"):
                sp.block()
                base = pl.multiple_of((j - 1) * AR, AR)
                hs, ha, bc, dc = {}, {}, {}, {}
                sp.schedule(b_sum_tasks(gu_src(j), bc), *BC_SLOTS)
                sp.schedule(attn_tasks(base + A0, AR), *ATTN_SLOTS)
                sp.schedule(pack_tasks(oa, base, pl.multiple_of((j - 1) * (AR // 2), AR // 2), AR),
                            *PACK_SLOTS)
                sp.schedule(d_tasks(j, dc), *DC_SLOTS)
                strassen_x(raw_first((0, 2), (1, 3)), b_rhs(gu_src(j), bc), glu(hs))
                down_lhs(hs, 0, ha)
                down_lhs(hs, 1, ha)
                ffn_down(ha, dc, False)
            return carry

        lax.fori_loop(1, NC, body, 0)

        def out_copies(r0, i1, cols):
            cs = []
            for i2 in range(2):
                idx = (pl.ds(r0 + (i1 * H + i2 * Q), PB), cols)
                cs.append(cp(x_vm.at[idx], o2.at[idx], out_sem))
            return cs

        def out_blocks(blocks):
            todo = [(blk, 7 * t1 + t2) for blk in range(len(blocks))
                    for ts1, _ in _C_ORDER for t1 in ts1 for ts2, _ in _C_ORDER for t2 in ts2]
            m = {}
            for i in range(0, len(todo), 2):
                pair = todo[i:i + 2]
                ps = sp.dots([(_unpack(oa[t, pl.ds(blocks[blk][1], PB // 2), :]), _unpack(woc[t]))
                              for blk, t in pair])
                for (blk, t), p in zip(pair, ps):
                    r0, _, copies = blocks[blk]
                    mm = m.setdefault(blk, ({}, {}))
                    mm[0][t] = acc[t, pl.ds(r0, PB), :] + p
                    t1 = t // 7
                    if t % 7 != _C_ORDER[-1][0][-1]:
                        continue
                    mm[1][t1] = _c_combos([mm[0].pop(7 * t1 + t2) for t2 in range(7)])
                    for ts, qd in _C_ORDER:
                        if t1 != ts[-1]:
                            continue
                        for q2 in range(4):
                            val = _c_quadrant({tt: v[q2] for tt, v in mm[1].items()}, qd)
                            r = pl.ds(r0 + ((qd // 2) * H + (q2 // 2) * Q), PB)
                            c = (qd % 2) * KH + (q2 % 2) * KQ
                            x_vm[r, c:c + KQ] = val.astype(bf16)
                        start(copies.get(qd, []))

        def whole(r0):
            return [c for i1 in range(2) for c in out_copies(r0, i1, slice(None))]

        done = (NC - 1) * AR

        def out_body(i, carry):
            with _Scope("p4a"):
                sp.block()
                half = pl.multiple_of(done // 2 + i * 24, 8)
                sp.schedule(pack_tasks(oa, 2 * half, half, 48), 4, 24)
                r0 = pl.multiple_of(i * PB, PB)
                out_blocks([(r0, pl.multiple_of(i * (PB // 2), PB // 2),
                             {3: whole(r0)})])
            return carry

        lax.fori_loop(0, 2, out_body, 0)
        with _Scope("p4b"):
            sp.block()
            sp.schedule(pack_tasks(oa, done + 96, (done + 96) // 2, Q - done - 96), 4, 22)
            last = {qd: out_copies(3 * PB, qd // 2, pl.ds((qd % 2) * KH, KH))
                    for qd in range(4)}
            copies = [{3: whole(blk * PB)} for blk in range(3)] + [last]
            out_blocks([(blk * PB, blk * PB // 2, copies[blk]) for blk in (2, 3)])
        with _Scope("w4"):
            for cs in copies:
                for qd in cs:
                    wait(cs[qd])

    pl.run_scoped(front, pltpu.VMEM((D, 3 * D), bf16), pltpu.VMEM((3, D // 2, D), i32),
                  pltpu.VMEM((D, D), bf16))
    pl.run_scoped(back, pltpu.VMEM((49, Q // 2, KQ), i32))
    assert not sp.plan


_N_SEMS = 10


@jax.jit
def pallas_gated_mix__sliding_local_dilated__glu_gated_reglu__prompt_kernel(
    A_x: jax.Array,
    A_wqkv: jax.Array,
    A_wo: jax.Array,
    B_x: jax.Array,
    B_W_gate: jax.Array,
    B_W_up: jax.Array,
    B_W_down: jax.Array,
    gate_w: jax.Array,
):
    del B_x
    hbm = pl.BlockSpec(memory_space=pl.ANY)
    scratch = [
        pltpu.VMEM((S, D), bf16),
        pltpu.VMEM((S // 2, D), i32),
        pltpu.VMEM((5, H // 2, KH), i32),
        pltpu.VMEM((8, 128), bf16),
        pltpu.VMEM((NC, D, 2 * FC), bf16),
        pltpu.VMEM((NC, FC, D), bf16),
        pltpu.VMEM((49, Q, KQ), f32),
        pltpu.VMEM((8, S + QPAD + 16, 128), f32),
        pltpu.VMEM((8, PAD + S, 128), f32),
        pltpu.VMEM((8, PAD + S, 128), f32),
        pltpu.VMEM((S, 128), f32),
        pltpu.VMEM((49, KQ // 2, KQ), i32),
        pltpu.VMEM((8, 128), i32),
        pltpu.SMEM((1,), i32),
        pltpu.SemaphoreType.DMA((_N_SEMS,)),
    ]
    return pl.pallas_call(
        _kernel,
        in_specs=[hbm] * 7,
        out_specs=hbm,
        out_shape=jax.ShapeDtypeStruct((1, S, D), bf16),
        scratch_shapes=scratch,
        compiler_params=pltpu.CompilerParams(vmem_limit_bytes=124 * 1024 * 1024),
    )(A_x, A_wqkv, A_wo, B_W_gate, B_W_up, B_W_down, gate_w.reshape(8, 128))
```

```python
import math

import jax
import jax.numpy as jnp
from jax import lax
import jax.experimental.pallas as pl
import jax.experimental.pallas.tpu as pltpu

f32 = jnp.float32
bf16 = jnp.bfloat16
i32 = jnp.int32

S = 2048
D = 1024
F = 3584
NH = 32
DH = D // NH
W = 8
DIL = 2
H = S // 2
Q = S // 4
KH = D // 2
KQ = D // 4
FC = 512
CH = FC // 2
CQ = FC // 4
NC = F // FC
RB = 256
NRB = H // RB
PB = 128
PAD = 16
TP = DH + 1
AR = 64
A0 = Q - 6 * AR
QA = 160
QPAD = 112

ATTN_SLOTS = (20, 96)
PACK_SLOTS = (96, 112)
DC_SLOTS = (24, 96)
BC_SLOTS = (2, 24)
DEPTH = 3
H_ORDER = (0, 1, 2, 3, 4, 5, 6)
NRAW = 3
VBC_SLOTS = (2, 16)
G_DEPTH = 0
G_LINK = 1
PREP01 = (16, 56)
PERMK = (64, 106)
WOS = (70, 112)
PACK4 = (4, 24)
DEPTH2 = 3
H_DEPTH = 3
PROFILE = ()

SCALE = DH ** -0.5
EXP2_SCALE = SCALE * math.log2(math.e)
NEG = -1e9 / SCALE


def _a_combos(a11, a12, a21, a22):
    return [a11 + a22, a21 + a22, a11, a22, a11 + a12, a21 - a11, a12 - a22]


def _b_combos(b11, b12, b21, b22):
    return [b11 + b22, b11, b12 - b22, b21 - b11, b22, b11 + b12, b21 + b22]


_C_TERMS = (((1, 0), (1, 3), (-1, 4), (1, 6)), ((1, 2), (1, 4)), ((1, 1), (1, 3)),
            ((1, 0), (-1, 1), (1, 2), (1, 5)))
_C_ORDER = (((2, 4), 1), ((1, 3), 2), ((0, 6), 0), ((5,), 3))


def _c_quadrant(m, qd):
    out = m[_C_TERMS[qd][0][1]]
    for sign, t in _C_TERMS[qd][1:]:
        out = out + m[t] if sign > 0 else out - m[t]
    return out


def _c_combos(m):
    return [_c_quadrant(m, qd) for qd in range(4)]


_A_SLOT = {0: 0, 1: 1, 4: 2, 5: 3, 6: 4}
_B_SUMS = (2, 3, 0, 5, 6)
ORDER = (1, 4) + _B_SUMS


class _Scope:
    def __init__(self, name):
        self.cm = jax.named_scope(name) if (PROFILE is True or name in PROFILE) else None

    def __enter__(self):
        if self.cm is not None:
            self.cm.__enter__()

    def __exit__(self, *a):
        if self.cm is not None:
            self.cm.__exit__(*a)


def _tree(op, xs):
    xs = list(xs)
    while len(xs) > 1:
        xs = [op(xs[i], xs[i + 1]) if i + 1 < len(xs) else xs[i] for i in range(0, len(xs), 2)]
    return xs[0]


def _pack(x):
    return pltpu.bitcast(x.astype(bf16), i32)


def _unpack(x):
    return pltpu.bitcast(x, bf16)


def _half(r):
    return slice(r.start // 2, r.stop // 2)


SLOT = 256


class _Spreader:
    def __init__(self, zero_ref):
        self.zero_ref = zero_ref
        self.plan = {}
        self.now = 0

    def block(self):
        self.zero = self.zero_ref[...]
        self.never = self.zero != 0

    def link(self, after, x):
        if after is None:
            return x
        if after.dtype != x.dtype:
            after = pltpu.bitcast(after, x.dtype)
        return jnp.where(self.never, after, x)

    def chain(self, vals, prev, depth):
        for v in vals:
            v = pltpu.bitcast(v, i32) if v.dtype != i32 else v
            for r in range(0, v.shape[0], 8):
                for c in range(0, v.shape[1], 128):
                    tile = v[r:r + 8, c:c + 128]
                    if prev is None:
                        prev = tile
                        continue
                    prev = prev | tile
                    for i in range(depth - 1):
                        prev = (prev + self.zero) if i % 2 == 0 else (prev ^ self.zero)
        return prev

    def link_rows(self, after, x):
        return jnp.concatenate([self.link(after, x[r:r + 8, :]) for r in range(0, x.shape[0], 8)],
                               axis=0)

    def serial_combos(self, combos, x11, x12, x21, x22, after):
        return combos(self.link_rows(after, x11), x12, x21, self.link_rows(after, x22))

    def two_level(self, combos, blk, prev, depth):
        outer = [combos(*[blk(r1, r2, c1, c2) for r1 in range(2) for c1 in range(2)])
                 for r2 in range(2) for c2 in range(2)]
        outs, tok = [], None
        for t in range(7):
            wide = _pack(jnp.concatenate(
                self.serial_combos(combos, *[o[t] for o in outer], tok), axis=1))
            outs += [wide[:, c:c + 128] for c in range(0, 7 * 128, 128)]
            tok = self.chain(outs[-7:], tok, depth)
        return outs, self.chain([tok], prev, 1)

    def schedule(self, tasks, first, last):
        n = len(tasks)
        for i, t in enumerate(tasks):
            pos = self.now + first + ((i + 1) * (last - first) - 1) // n
            self.plan.setdefault(pos, []).append((t, id(tasks)))

    def dots(self, pairs):
        m = pairs[0][0].shape[0]
        tiles = [(i, r, c) for i, (_, rhs) in enumerate(pairs)
                 for c in range(0, rhs.shape[1], 128) for r in range(0, rhs.shape[0], 128)]
        nslots = m * len(tiles) // (4 * SLOT)
        deps = {}
        for sl in range(nslots):
            ps = sl * SLOT // m
            toks = {}
            for t, lane in self.plan.pop(self.now + sl, []):
                tok = t(toks.get(lane))
                if tok is not None:
                    toks[lane] = tok
            for tok in toks.values():
                deps[ps] = tok | deps[ps] if ps in deps else tok
        self.now += nslots
        tied = {tile: d for ps, d in deps.items() for tile in tiles[4 * ps:4 * ps + 4]}
        outs = []
        for i, (lhs, rhs) in enumerate(pairs):
            if any(key[0] == i for key in tied):
                parts = []
                for r in range(0, rhs.shape[0], 128):
                    top = [rhs[r:r + 16, c:c + 128] for c in range(0, rhs.shape[1], 128)]
                    top = [_unpack(self.link(tied[i, r, c * 128], _pack(t0)))
                           if (i, r, c * 128) in tied else t0 for c, t0 in enumerate(top)]
                    parts += [jnp.concatenate(top, axis=1), rhs[r + 16:r + 128, :]]
                rhs = jnp.concatenate(parts, axis=0)
            outs.append(jnp.dot(lhs, rhs, preferred_element_type=f32))
        return outs

    def dot(self, lhs, rhs):
        return self.dots([(lhs, rhs)])[0]


def _kernel(x_hbm, wqkv_hbm, wo_hbm, wg_hbm, wu_hbm, wd_hbm, gw_hbm, out_hbm,
            x_vm, xn, xa, gw_vm, wgu, wd, acc, q_s, k_s, v_s, gs, woc, zs, zi, sems):
    def cp(src, dst, sem):
        return pltpu.make_async_copy(src, dst, sems.at[sem])

    def cp_gu(j, p, sem):
        return cp((wg_hbm, wu_hbm)[p % 2].at[:, pl.ds(j * FC + (p // 2) * CH, CH)],
                  wgu.at[j, :, pl.ds(p * CH, CH)], sem)

    def cp_d(j, sem):
        return cp(wd_hbm.at[pl.ds(j * FC, FC), :], wd.at[j], sem)

    def cp_x(rb, hf, sem):
        idx = (pl.ds(hf * H + rb * RB, RB), slice(None))
        return cp(x_hbm.at[0].at[idx], x_vm.at[idx], sem)

    o2 = out_hbm.at[0]
    in0 = [cp_x(0, 0, 0), cp_gu(0, 0, 0)]
    in1 = [cp_x(0, 1, 1)]
    in2 = [cp_gu(0, 1, 2)]
    in3 = [cp_gu(0, 2, 3), cp_gu(0, 3, 3), cp(gw_hbm, gw_vm, 3)]
    in4 = [cp_x(rb, hf, 4) for rb in (1, 2) for hf in range(2)]
    in5 = [cp_x(3, 0, 5), cp_x(3, 1, 5), cp_d(0, 5)]
    in_ffn = [c for j in range(1, NC) for c in [cp_gu(j, p, 8) for p in range(4)] + [cp_d(j, 8)]]
    out_sem = 9

    def start(cs):
        for c in cs:
            c.start()

    def wait(cs):
        for c in cs:
            c.wait()

    start(in0 + in1 + in2)

    zs[...] = jnp.zeros((8, 128), i32)
    zi[0] = 1
    sp = _Spreader(zs)

    def rows(rb, hf=0):
        return slice(hf * H + rb * RB, hf * H + (rb + 1) * RB)

    def x_lhs(t, rb):
        if t == 2:
            return _unpack(xn[_half(rows(rb, 0)), :KH])
        if t == 3:
            return _unpack(xn[_half(rows(rb, 1)), KH:])
        return _unpack(xa[_A_SLOT[t], _half(rows(rb)), :])

    def prep_tasks(rb, sums=True, gate=True):
        def task(s0):
            def run(first):
                prev = None
                gw = gw_vm[...].astype(f32)
                r = [slice(hf * H + rb * RB + s0, hf * H + rb * RB + s0 + 16) for hf in range(2)]
                z = [None, None]
                for c in range(4):
                    cols = [slice(kh * KH + c * 128, kh * KH + (c + 1) * 128) for kh in range(2)]
                    xs = [sp.link(prev, _pack(x_vm[r[qd // 2], cols[qd % 2]])) for qd in range(4)]
                    a = [_unpack(t).astype(f32) for t in xs]
                    outs = []
                    if sums:
                        for qd in range(4):
                            xn[_half(r[qd // 2]), cols[qd % 2]] = xs[qd]
                        cs = _a_combos(*a)
                        for t, slot in _A_SLOT.items():
                            outs.append(_pack(cs[t]))
                            xa[slot, _half(r[0]), cols[0]] = outs[-1]
                    if gate:
                        for qd in range(4):
                            g0 = (qd % 2) * 4 + c
                            term = a[qd] * gw[g0:g0 + 1, :]
                            z[qd // 2] = term if z[qd // 2] is None else z[qd // 2] + term
                        outs += z
                    prev = sp.chain(outs, prev, 1)
                if gate:
                    for hf in range(2):
                        g = jax.nn.sigmoid(jnp.sum(z[hf], axis=1, keepdims=True))
                        g = jnp.broadcast_to(g, (16, 128))
                        gs[r[hf], :] = g
                        prev = sp.chain([g], prev, 1)
                return sp.chain([prev], first, 1)
            return run
        return [task(s0) for s0 in range(0, RB, 16)]

    def b_sum_tasks(src, dst):
        def task(r0):
            def run(prev):
                raw = [src(slice(a * KH + r0, a * KH + r0 + 16), slice(c * KH, (c + 1) * KH))
                       for a in range(2) for c in range(2)]
                cs = _b_combos(*[b.astype(f32) for b in raw])
                for t in _B_SUMS:
                    dst.setdefault(t, []).append(_pack(cs[t]))
                return sp.chain([dst[t][-1] for t in _B_SUMS], prev, DEPTH)
            return run
        return [task(r0) for r0 in range(0, KH, 16)]

    def b_rhs(src, sums):
        def rhs(t):
            if t == 1:
                return src(slice(0, KH), slice(0, KH))
            if t == 4:
                return src(slice(KH, D), slice(KH, D))
            return _unpack(jnp.concatenate(sums[t], axis=0))
        return rhs

    def strassen_x(order, rhs, finish):
        m = {}
        for rb, t in order:
            m.setdefault(rb, {})[t] = sp.dot(x_lhs(t, rb), rhs(t))
            if len(m[rb]) == 7:
                finish(rb, m.pop(rb))

    def h_sums(rb, cs, r0, sub):
        h = []
        for qd, cc in enumerate(cs):
            g0 = (qd // 2) * H + rb * RB + r0
            omg = 1.0 - gs[g0:g0 + sub, :]
            omg = jnp.concatenate([omg] * (CH // 128), axis=1)
            h.append(jnp.maximum(cc[:, :CH], 0.0) * cc[:, CH:] * omg)
        return _a_combos(*h)

    def glu_tasks(hs, rb, cs, sub):
        hs[rb] = [[] for _ in range(7)]

        def task(r0):
            def run(prev=None):
                sums = h_sums(rb, [cc[r0:r0 + sub] for cc in cs], r0, sub)
                for t in range(7):
                    hs[rb][t].append(sums[t])
                if sub < RB:
                    return sp.chain([sums[t] for t in _A_SLOT], prev, DEPTH2)
            return run
        return [task(r0) for r0 in range(0, RB, sub)]

    def down_lhs(hs, b, ha, tok):
        for t in H_ORDER:
            s0, s1 = [jnp.concatenate(hs[rb][t], axis=0) for rb in (b, b + 2)]
            slabs = []
            for r in range(0, RB, 16):
                slabs.append(sp.serial_combos(
                    _a_combos, s0[r:r + 16, :CQ], s0[r:r + 16, CQ:],
                    s1[r:r + 16, :CQ], s1[r:r + 16, CQ:], tok))
                tok = sp.chain([slabs[-1][t2] for t2 in _A_SLOT], None, H_DEPTH)
            for t2 in range(7):
                ha[b, 7 * t + t2] = jnp.concatenate([sl[t2] for sl in slabs], axis=0).astype(bf16)

    def d_tasks(j, dst):
        def task(r0, c):
            def run(prev):
                def blk(k1, k2, n1, n2):
                    r, c0 = k1 * CH + k2 * CQ + r0, n1 * KH + n2 * KQ + c * 128
                    return wd[j, r:r + 16, c0:c0 + 128].astype(f32)
                cs, tok = sp.two_level(_b_combos, blk, prev, DEPTH2)
                for t in range(49):
                    dst.setdefault((t, c), []).append(cs[t])
                return tok
            return run
        return [task(r0, c) for r0 in range(0, CQ, 16) for c in range(2)]

    def ffn_down(ha, dc, first):
        rhs = [_unpack(jnp.concatenate([jnp.concatenate(dc[t, c], axis=0) for c in range(2)], axis=1))
               for t in range(49)]
        todo = [(b, 7 * t + t2) for b in range(2) for t in H_ORDER for t2 in range(7)]
        for i in range(0, len(todo), 2):
            pair = todo[i:i + 2]
            ps = sp.dots([(ha[b, t], rhs[t]) for b, t in pair])
            for (b, t), p in zip(pair, ps):
                if first:
                    acc[t, b * RB:(b + 1) * RB, :] = p
                else:
                    acc[t, b * RB:(b + 1) * RB, :] += p

    def perm_tasks(wqkv_vm, wp, i, tbuf):
        def fwd(rb, c):
            def run(prev):
                c0 = i * D + c * 128
                tt = pltpu.bitcast(wqkv_vm[rb * 256:(rb + 1) * 256, c0:c0 + 128], f32).T
                for hh in range(4):
                    tbuf[rb, pl.ds((4 * c + hh) * TP, DH), :] = tt[hh * DH:(hh + 1) * DH, :]
                return sp.chain([tt], prev, 1)
            return run

        def bwd(rb, j):
            def run(prev):
                g = jnp.concatenate(
                    [tbuf[rb, pl.ds(4 * j + dd, NH, stride=TP), :] for dd in range(4)], axis=0).T
                wp[i, rb * 128:(rb + 1) * 128, j * 128:(j + 1) * 128] = pltpu.bitcast(g, i32)
            return run
        tasks = []
        for rb in range(4):
            tasks += [fwd(rb, c) for c in range(8)] + [bwd(rb, j) for j in range(8)]
        return tasks

    def wo_tasks(wo_vm):
        def stage(c):
            return 4 + c % 4, (c // 4) * NH * TP

        def spread(h0):
            def run(prev):
                blk = wo_vm[h0 * DH:(h0 + 2) * DH, :].astype(f32)
                for h in range(2):
                    for c in range(8):
                        sl, r0 = stage(c)
                        q_s[sl, pl.ds(r0 + (h0 + h) * TP, DH), :] = (
                            blk[h * DH:(h + 1) * DH, c * 128:(c + 1) * 128])
                return sp.chain([blk], prev, 1)
            return run

        def gather(d, h0, c):
            def run(prev):
                def blk(k1, k2, n1, n2):
                    sl, r0 = stage(4 * n1 + 2 * n2 + c)
                    r0 += h0 * TP + 16 * k1 + 8 * k2 + d
                    return q_s[sl, pl.ds(r0, 16, stride=TP), :]
                cs, tok = sp.two_level(_b_combos, blk, prev, DEPTH2)
                r = (d * NH + h0) // 2
                for t in range(49):
                    woc[t, r:r + 8, c * 128:(c + 1) * 128] = cs[t]
                return tok
            return run
        return ([spread(h0) for h0 in range(0, NH, 2)],
                [gather(d, h0, c) for d in range(8) for h0 in (0, 16) for c in range(2)])

    def proj(wp, i, dst, pad, slabs):
        lhs = jnp.concatenate([xn[r0 // 2:(r0 + n) // 2, :] for r0, n in slabs], axis=0)
        p = sp.dot(_unpack(lhs), _unpack(wp[i]))
        at = 0
        for r0, n in slabs:
            for j in range(8):
                dst[j, pad + r0:pad + r0 + n, :] = p[at:at + n, j * 128:(j + 1) * 128]
            at += n

    def v_finish(rb, m):
        cs = _c_combos(m)
        for qd, cc in enumerate(cs):
            r0 = PAD + (qd // 2) * H + rb * RB
            for j in range(4):
                v_s[(qd % 2) * 4 + j, r0:r0 + RB, :] = cc[:, j * 128:(j + 1) * 128]
        if rb == 0:
            for j in range(8):
                src = cs[j // 4][0:1, (j % 4) * 128:(j % 4 + 1) * 128]
                v_s[j, 0:PAD, :] = jnp.broadcast_to(src, (PAD, 128))

    def attn_group(row, masked):
        def run(prev):
            g = 8
            q = [q_s[j, pl.ds(row, g), :] for j in range(8)]
            ls = []
            for w in range(W):
                a = None
                for j in range(8):
                    term = q[j] * k_s[j, pl.ds(row + (PAD - DIL * w), g), :]
                    a = sp.link(ls[-1] if ls else None, term) if a is None else a + term
                ls.append(a)
            rs = [pltpu.roll(a, 64, 1) for a in ls]
            ls = [a + r for a, r in zip(ls, rs)]
            rs = [pltpu.roll(a, 32, 1) for a in ls]
            ls = [a + r for a, r in zip(ls, rs)]
            if masked:
                ri = row + lax.broadcasted_iota(i32, (g, 128), 0)
                ls = [ls[0]] + [jnp.where(ri >= DIL * w, ls[w], NEG) for w in range(1, W)]
            m = _tree(jnp.maximum, ls)
            ps = [jnp.exp2((l - m) * EXP2_SCALE) for l in ls]
            r = gs[pl.ds(row, g), :] / _tree(jnp.add, ps)
            outs = []
            for j in range(8):
                a = None
                for w in range(W):
                    term = ps[w] * v_s[j, pl.ds(row + (PAD - DIL * w), g), :]
                    a = sp.link(outs[-1] if outs else None, term) if a is None else a + term
                outs.append(a * r)
            for j in range(8):
                q_s[j, pl.ds(row, g), :] = outs[j]
            return sp.chain([outs[-1]], prev, 1)
        return run

    def attn_tasks(base, nrows, first=False):
        return [attn_group(base + (qq * Q + r), first and qq == 0 and r < PAD)
                for r in range(0, nrows, 8) for qq in range(4)]

    def pack_tasks(oa, base, hbase, nrows):
        def task(r, c):
            def run(prev):
                def blk(i1, i2, k1, k2):
                    return q_s[4 * k1 + 2 * k2 + c, pl.ds(base + (i1 * H + i2 * Q + r), 16), :]
                cs, tok = sp.two_level(_a_combos, blk, prev, DEPTH2)
                for t in range(49):
                    oa[t, pl.ds(hbase + r // 2, 8), c * 128:(c + 1) * 128] = cs[t]
                return tok
            return run
        return [task(r, c) for r in range(0, nrows, 16) for c in range(2)]

    GS = RB * (KH // 128) * (FC // 128) * 7 // (4 * SLOT)
    DS = 49
    PS = 2 * RB * (D // 128) * (D // 128) // (4 * SLOT)

    def glu(hs, ha):
        def finish(rb, m):
            if rb < 2 or not G_DEPTH:
                glu_tasks(hs, rb, _c_combos(m), RB)[0]()
                tok = None
            else:
                tok, pieces = None, []
                for r in range(0, RB, 16):
                    mm = {t: v[r:r + 16] for t, v in m.items()}
                    for t in ORDER[-G_LINK:]:
                        mm[t] = jnp.concatenate([sp.link_rows(tok, mm[t][:, c:c + 128])
                                                 for c in range(0, FC, 128)], axis=1)
                    pieces.append(h_sums(rb, _c_combos(mm), r, 16))
                    tok = sp.chain([pieces[-1][t] for t in _A_SLOT], None, G_DEPTH)
                hs[rb] = [[pc[t] for pc in pieces] for t in range(7)]
            if rb >= 2:
                down_lhs(hs, rb - 2, ha, tok)
        return finish

    def raw_first(rbs, NRAW):
        lead = [(rb, t) for rb in rbs[:NRAW] for t in ORDER[:2]]
        return lead + [(rb, t) for rb in rbs for t in ORDER if (rb, t) not in lead]

    def gu_src(j):
        return lambda r, c: wgu[j, r, c]

    def front(wqkv_vm, wp, wo_vm):
        in_q, in_k, in_v = [
            cp(wqkv_hbm.at[:, pl.ds(i * D, D)], wqkv_vm.at[:, pl.ds(i * D, D)], 7 - i)
            for i in range(3)]
        in_wo = cp(wo_hbm, wo_vm, 6)

        def plain(rb, hf, p):
            return sp.dot(x_vm[rows(rb, hf), :], wgu[0, :, p * CH:(p + 1) * CH])

        def plain_finish(rb, c):
            cs = [jnp.concatenate(c[2 * qd:2 * qd + 2], axis=1) for qd in range(4)]
            return glu_tasks(hs, rb, cs, 16)

        hs, bc, dc = {}, {}, {}
        with _Scope("w0"):
            wait(in0)
        start(in3)
        c0 = {(0, 0): plain(0, 0, 0)}
        with _Scope("wa"):
            wait(in1)
        c0[1, 0] = plain(0, 1, 0)
        with _Scope("wb"):
            wait(in2)
        start(in4)
        for hf in range(2):
            c0[hf, 1] = plain(0, hf, 1)
        with _Scope("wc"):
            wait(in3)
        with _Scope("p1a"):
            start(in5)
            sp.block()
            bt = b_sum_tasks(gu_src(0), bc)
            sp.schedule(bt[:12], 3, 16)
            sp.schedule(prep_tasks(0, sums=False), 3, 16)
            for p in (2, 3):
                for hf in range(2):
                    c0[hf, p] = plain(0, hf, p)
            c0 = [c0[hf, p] for hf in range(2) for p in range(4)]
        with _Scope("w1"):
            wait(in4)
            start([in_v])
        with _Scope("p1b"):
            sp.block()
            sp.schedule(bt[12:], 3, 32)
            sp.schedule(prep_tasks(1, sums=False), 2, 10)
            sp.schedule(prep_tasks(2), 10, 32)
            c1 = [plain(1, hf, p) for hf in range(2) for p in range(4)]
        with _Scope("w2"):
            wait(in5 + [in_v])
            start([in_k, in_wo, in_q])
        with _Scope("p1c"):
            sp.block()
            for j in range(8):
                k_s[j, 0:PAD, :] = jnp.zeros((PAD, 128), f32)
            ha = {}
            sp.schedule(prep_tasks(3), 2, GS)
            sp.schedule(plain_finish(0, c0), 2, GS)
            sp.schedule(plain_finish(1, c1), GS + 6, 2 * GS)
            sp.schedule(d_tasks(0, dc), GS - 2, 2 * GS)
            sp.schedule(perm_tasks(wqkv_vm, wp, 2, q_s), 2 * GS + 6, 2 * GS + DS - 8)
            strassen_x([(rb, t) for rb in (2, 3) for t in ORDER], b_rhs(gu_src(0), bc),
                       glu(hs, ha))
            ffn_down(ha, dc, True)

        with _Scope("w2b"):
            wait([in_k, in_wo])
            start(in_ffn)
        with _Scope("v"):
            sp.block()
            vb = {}
            v_src = lambda r, c: _unpack(wp[2, _half(r), c])
            wo_spread, wo_gather = wo_tasks(wo_vm)
            sp.schedule(b_sum_tasks(v_src, vb), *VBC_SLOTS)
            sp.schedule(prep_tasks(0, gate=False) + prep_tasks(1, gate=False), *PREP01)
            sp.schedule(perm_tasks(wqkv_vm, wp, 1, k_s.at[:, PAD:, :]), *PERMK)
            sp.schedule(wo_spread, *WOS)
            strassen_x(raw_first((2, 3, 0, 1), 2), b_rhs(v_src, vb), v_finish)
        with _Scope("w3"):
            wait([in_q])
        with _Scope("kq"):
            sp.block()
            sp.schedule(perm_tasks(wqkv_vm, wp, 0, q_s), 4, 3 * PS)
            sp.schedule(wo_gather, 4, NRB * PS)
            for rb in range(NRB):
                proj(wp, 1, k_s, PAD, [(rb * Q, Q)])
            proj(wp, 0, q_s, 0, [(qq * Q, QA) for qq in range(4)])

        def q_rest(_, carry):
            with _Scope("q"):
                sp.block()
                n = (Q - QA) // 2
                total = 4 * (Q - QA) * 64 // (4 * SLOT)
                sp.schedule(attn_tasks(0, A0, True), 4, total)
                for r0 in (QA, QA + n):
                    proj(wp, 0, q_s, 0, [(qq * Q + r0, n) for qq in range(4)])
            return carry

        lax.fori_loop(0, zi[0], q_rest, 0)
        wait(in_ffn)

    def back(oa):
        def body(j, carry):
            with _Scope("chunk"):
                sp.block()
                base = pl.multiple_of((j - 1) * AR, AR)
                hs, ha, bc, dc = {}, {}, {}, {}
                sp.schedule(b_sum_tasks(gu_src(j), bc), *BC_SLOTS)
                sp.schedule(attn_tasks(base + A0, AR), *ATTN_SLOTS)
                sp.schedule(pack_tasks(oa, base, pl.multiple_of((j - 1) * (AR // 2), AR // 2), AR),
                            *PACK_SLOTS)
                sp.schedule(d_tasks(j, dc), *DC_SLOTS)
                strassen_x(raw_first((0, 2, 1, 3), NRAW), b_rhs(gu_src(j), bc), glu(hs, ha))
                ffn_down(ha, dc, False)
            return carry

        lax.fori_loop(1, NC, body, 0)

        def out_copies(r0, i1, cols):
            cs = []
            for i2 in range(2):
                idx = (pl.ds(r0 + (i1 * H + i2 * Q), PB), cols)
                cs.append(cp(x_vm.at[idx], o2.at[idx], out_sem))
            return cs

        def out_blocks(blocks):
            todo = [(blk, 7 * t1 + t2) for blk in range(len(blocks))
                    for ts1, _ in _C_ORDER for t1 in ts1 for ts2, _ in _C_ORDER for t2 in ts2]
            m = {}
            for i in range(0, len(todo), 2):
                pair = todo[i:i + 2]
                ps = sp.dots([(_unpack(oa[t, pl.ds(blocks[blk][1], PB // 2), :]), _unpack(woc[t]))
                              for blk, t in pair])
                for (blk, t), p in zip(pair, ps):
                    r0, _, copies = blocks[blk]
                    mm = m.setdefault(blk, ({}, {}))
                    mm[0][t] = acc[t, pl.ds(r0, PB), :] + p
                    t1 = t // 7
                    if t % 7 != _C_ORDER[-1][0][-1]:
                        continue
                    mm[1][t1] = _c_combos([mm[0].pop(7 * t1 + t2) for t2 in range(7)])
                    for ts, qd in _C_ORDER:
                        if t1 != ts[-1]:
                            continue
                        for q2 in range(4):
                            val = _c_quadrant({tt: v[q2] for tt, v in mm[1].items()}, qd)
                            r = pl.ds(r0 + ((qd // 2) * H + (q2 // 2) * Q), PB)
                            c = (qd % 2) * KH + (q2 % 2) * KQ
                            x_vm[r, c:c + KQ] = val.astype(bf16)
                        start(copies.get(qd, []))

        def whole(r0):
            return [c for i1 in range(2) for c in out_copies(r0, i1, slice(None))]

        done = (NC - 1) * AR

        def out_body(i, carry):
            with _Scope("p4a"):
                sp.block()
                half = pl.multiple_of(done // 2 + i * 24, 8)
                sp.schedule(pack_tasks(oa, 2 * half, half, 48), *PACK4)
                r0 = pl.multiple_of(i * PB, PB)
                out_blocks([(r0, pl.multiple_of(i * (PB // 2), PB // 2),
                             {3: whole(r0)})])
            return carry

        lax.fori_loop(0, 2, out_body, 0)
        with _Scope("p4b"):
            sp.block()
            sp.schedule(pack_tasks(oa, done + 96, (done + 96) // 2, Q - done - 96), 4, 22)
            last = {qd: out_copies(3 * PB, qd // 2, pl.ds((qd % 2) * KH, KH))
                    for qd in range(4)}
            copies = [{3: whole(blk * PB)} for blk in range(3)] + [last]
            out_blocks([(blk * PB, blk * PB // 2, copies[blk]) for blk in (2, 3)])
        with _Scope("w4"):
            for cs in copies:
                for qd in cs:
                    wait(cs[qd])

    pl.run_scoped(front, pltpu.VMEM((D, 3 * D), bf16), pltpu.VMEM((3, D // 2, D), i32),
                  pltpu.VMEM((D, D), bf16))
    pl.run_scoped(back, pltpu.VMEM((49, Q // 2, KQ), i32))
    assert not sp.plan


_N_SEMS = 10


@jax.jit
def pallas_gated_mix__sliding_local_dilated__glu_gated_reglu__prompt_kernel(
    A_x: jax.Array,
    A_wqkv: jax.Array,
    A_wo: jax.Array,
    B_x: jax.Array,
    B_W_gate: jax.Array,
    B_W_up: jax.Array,
    B_W_down: jax.Array,
    gate_w: jax.Array,
):
    del B_x
    hbm = pl.BlockSpec(memory_space=pl.ANY)
    scratch = [
        pltpu.VMEM((S, D), bf16),
        pltpu.VMEM((S // 2, D), i32),
        pltpu.VMEM((5, H // 2, KH), i32),
        pltpu.VMEM((8, 128), bf16),
        pltpu.VMEM((NC, D, 2 * FC), bf16),
        pltpu.VMEM((NC, FC, D), bf16),
        pltpu.VMEM((49, Q, KQ), f32),
        pltpu.VMEM((8, S + QPAD, 128), f32),
        pltpu.VMEM((8, PAD + S, 128), f32),
        pltpu.VMEM((8, PAD + S, 128), f32),
        pltpu.VMEM((S, 128), f32),
        pltpu.VMEM((49, KQ // 2, KQ), i32),
        pltpu.VMEM((8, 128), i32),
        pltpu.SMEM((1,), i32),
        pltpu.SemaphoreType.DMA((_N_SEMS,)),
    ]
    return pl.pallas_call(
        _kernel,
        in_specs=[hbm] * 7,
        out_specs=hbm,
        out_shape=jax.ShapeDtypeStruct((1, S, D), bf16),
        scratch_shapes=scratch,
        compiler_params=pltpu.CompilerParams(vmem_limit_bytes=124 * 1024 * 1024),
    )(A_x, A_wqkv, A_wo, B_W_gate, B_W_up, B_W_down, gate_w.reshape(8, 128))
```

```python
import math

import jax
import jax.numpy as jnp
from jax import lax
import jax.experimental.pallas as pl
import jax.experimental.pallas.tpu as pltpu

f32 = jnp.float32
bf16 = jnp.bfloat16
i32 = jnp.int32

S = 2048
D = 1024
F = 3584
NH = 32
DH = D // NH
W = 8
DIL = 2
H = S // 2
Q = S // 4
KH = D // 2
KQ = D // 4
FC = 512
CH = FC // 2
CQ = FC // 4
NC = F // FC
RB = 256
NRB = H // RB
PB = 128
PAD = 16
TP = DH + 1
AR = 64
A0 = Q - 6 * AR
QA = 160
QPAD = 112

ATTN_SLOTS = (20, 96)
PACK_SLOTS = (96, 112)
DC_SLOTS = (24, 96)
BC_SLOTS = (2, 24)
DEPTH = 3
H_ORDER = (0, 1, 2, 3, 4, 5, 6)
NRAW = 3
VBC_SLOTS = (2, 16)
G_DEPTH = 0
G_LINK = 1
PREP01 = (16, 56)
PERMK = (64, 106)
WOS = (70, 112)
PACK4 = (4, 24)
DEPTH2 = 3
H_DEPTH = 3
PROFILE = ()

SCALE = DH ** -0.5
EXP2_SCALE = SCALE * math.log2(math.e)
NEG = -1e9 / SCALE


def _a_combos(a11, a12, a21, a22):
    return [a11 + a22, a21 + a22, a11, a22, a11 + a12, a21 - a11, a12 - a22]


def _b_combos(b11, b12, b21, b22):
    return [b11 + b22, b11, b12 - b22, b21 - b11, b22, b11 + b12, b21 + b22]


_C_TERMS = (((1, 0), (1, 3), (-1, 4), (1, 6)), ((1, 2), (1, 4)), ((1, 1), (1, 3)),
            ((1, 0), (-1, 1), (1, 2), (1, 5)))
_C_ORDER = (((2, 4), 1), ((1, 3), 2), ((0, 6), 0), ((5,), 3))


def _c_quadrant(m, qd):
    out = m[_C_TERMS[qd][0][1]]
    for sign, t in _C_TERMS[qd][1:]:
        out = out + m[t] if sign > 0 else out - m[t]
    return out


def _c_combos(m):
    return [_c_quadrant(m, qd) for qd in range(4)]


_A_SLOT = {0: 0, 1: 1, 4: 2, 5: 3, 6: 4}
_B_SUMS = (2, 3, 0, 5, 6)
ORDER = (1, 4) + _B_SUMS


class _Scope:
    def __init__(self, name):
        self.cm = jax.named_scope(name) if (PROFILE is True or name in PROFILE) else None

    def __enter__(self):
        if self.cm is not None:
            self.cm.__enter__()

    def __exit__(self, *a):
        if self.cm is not None:
            self.cm.__exit__(*a)


def _tree(op, xs):
    xs = list(xs)
    while len(xs) > 1:
        xs = [op(xs[i], xs[i + 1]) if i + 1 < len(xs) else xs[i] for i in range(0, len(xs), 2)]
    return xs[0]


def _pack(x):
    return pltpu.bitcast(x.astype(bf16), i32)


def _unpack(x):
    return pltpu.bitcast(x, bf16)


def _half(r):
    return slice(r.start // 2, r.stop // 2)


SLOT = 256


class _Spreader:
    def __init__(self, zero_ref):
        self.zero_ref = zero_ref
        self.plan = {}
        self.now = 0

    def block(self):
        self.zero = self.zero_ref[...]
        self.never = self.zero != 0

    def link(self, after, x):
        if after is None:
            return x
        if after.dtype != x.dtype:
            after = pltpu.bitcast(after, x.dtype)
        return jnp.where(self.never, after, x)

    def chain(self, vals, prev, depth):
        for v in vals:
            v = pltpu.bitcast(v, i32) if v.dtype != i32 else v
            for r in range(0, v.shape[0], 8):
                for c in range(0, v.shape[1], 128):
                    tile = v[r:r + 8, c:c + 128]
                    if prev is None:
                        prev = tile
                        continue
                    prev = prev | tile
                    for i in range(depth - 1):
                        prev = (prev + self.zero) if i % 2 == 0 else (prev ^ self.zero)
        return prev

    def link_rows(self, after, x):
        return jnp.concatenate([self.link(after, x[r:r + 8, :]) for r in range(0, x.shape[0], 8)],
                               axis=0)

    def serial_combos(self, combos, x11, x12, x21, x22, after):
        return combos(self.link_rows(after, x11), x12, x21, self.link_rows(after, x22))

    def two_level(self, combos, blk, prev, depth, after=None):
        outer = [self.serial_combos(
            combos, *[blk(r1, r2, c1, c2) for r1 in range(2) for c1 in range(2)], after)
            for r2 in range(2) for c2 in range(2)]
        outs, tok = [], None
        for t in range(7):
            wide = _pack(jnp.concatenate(
                self.serial_combos(combos, *[o[t] for o in outer], tok), axis=1))
            outs += [wide[:, c:c + 128] for c in range(0, 7 * 128, 128)]
            tok = self.chain(outs[-7:], tok, depth)
        return outs, self.chain([tok], prev, 1)

    def schedule(self, tasks, first, last):
        n = len(tasks)
        for i, t in enumerate(tasks):
            pos = self.now + first + ((i + 1) * (last - first) - 1) // n
            self.plan.setdefault(pos, []).append((t, id(tasks)))

    def dots(self, pairs):
        m = pairs[0][0].shape[0]
        tiles = [(i, r, c) for i, (_, rhs) in enumerate(pairs)
                 for c in range(0, rhs.shape[1], 128) for r in range(0, rhs.shape[0], 128)]
        nslots = m * len(tiles) // (4 * SLOT)
        deps = {}
        for sl in range(nslots):
            ps = sl * SLOT // m
            toks = {}
            for t, lane in self.plan.pop(self.now + sl, []):
                tok = t(toks.get(lane))
                if tok is not None:
                    toks[lane] = tok
            for tok in toks.values():
                deps[ps] = tok | deps[ps] if ps in deps else tok
        self.now += nslots
        tied = {tile: d for ps, d in deps.items() for tile in tiles[4 * ps:4 * ps + 4]}
        outs = []
        for i, (lhs, rhs) in enumerate(pairs):
            if any(key[0] == i for key in tied):
                parts = []
                for r in range(0, rhs.shape[0], 128):
                    top = [rhs[r:r + 16, c:c + 128] for c in range(0, rhs.shape[1], 128)]
                    top = [_unpack(self.link(tied[i, r, c * 128], _pack(t0)))
                           if (i, r, c * 128) in tied else t0 for c, t0 in enumerate(top)]
                    parts += [jnp.concatenate(top, axis=1), rhs[r + 16:r + 128, :]]
                rhs = jnp.concatenate(parts, axis=0)
            outs.append(jnp.dot(lhs, rhs, preferred_element_type=f32))
        return outs

    def dot(self, lhs, rhs):
        return self.dots([(lhs, rhs)])[0]


def _kernel(x_hbm, wqkv_hbm, wo_hbm, wg_hbm, wu_hbm, wd_hbm, gw_hbm, out_hbm,
            x_vm, xn, xa, gw_vm, wgu, wd, acc, q_s, k_s, v_s, gs, woc, zs, zi, sems):
    def cp(src, dst, sem):
        return pltpu.make_async_copy(src, dst, sems.at[sem])

    def cp_gu(j, p, sem):
        return cp((wg_hbm, wu_hbm)[p % 2].at[:, pl.ds(j * FC + (p // 2) * CH, CH)],
                  wgu.at[j, :, pl.ds(p * CH, CH)], sem)

    def cp_d(j, sem):
        return cp(wd_hbm.at[pl.ds(j * FC, FC), :], wd.at[j], sem)

    def cp_x(rb, hf, sem):
        idx = (pl.ds(hf * H + rb * RB, RB), slice(None))
        return cp(x_hbm.at[0].at[idx], x_vm.at[idx], sem)

    o2 = out_hbm.at[0]
    in0 = [cp_x(0, 0, 0), cp_gu(0, 0, 0)]
    in1 = [cp_x(0, 1, 1)]
    in2 = [cp_gu(0, 1, 2)]
    in3 = [cp_gu(0, 2, 3), cp_gu(0, 3, 3), cp(gw_hbm, gw_vm, 3)]
    in4 = [cp_x(rb, hf, 4) for rb in (1, 2) for hf in range(2)]
    in5 = [cp_x(3, 0, 5), cp_x(3, 1, 5), cp_d(0, 5)]
    in_ffn = [c for j in range(1, NC) for c in [cp_gu(j, p, 7) for p in range(4)] + [cp_d(j, 7)]]
    out_sem = 8

    def start(cs):
        for c in cs:
            c.start()

    def wait(cs):
        for c in cs:
            c.wait()

    start(in0 + in1 + in2)

    zs[...] = jnp.zeros((8, 128), i32)
    zi[0] = 1
    sp = _Spreader(zs)

    def rows(rb, hf=0):
        return slice(hf * H + rb * RB, hf * H + (rb + 1) * RB)

    def x_lhs(t, rb):
        if t == 2:
            return _unpack(xn[_half(rows(rb, 0)), :KH])
        if t == 3:
            return _unpack(xn[_half(rows(rb, 1)), KH:])
        return _unpack(xa[_A_SLOT[t], _half(rows(rb)), :])

    def prep_tasks(rb, sums=True, gate=True):
        def task(s0):
            def run(first):
                prev = None
                gw = gw_vm[...].astype(f32)
                r = [slice(hf * H + rb * RB + s0, hf * H + rb * RB + s0 + 16) for hf in range(2)]
                z = [None, None]
                for c in range(4):
                    cols = [slice(kh * KH + c * 128, kh * KH + (c + 1) * 128) for kh in range(2)]
                    xs = [sp.link(prev, _pack(x_vm[r[qd // 2], cols[qd % 2]])) for qd in range(4)]
                    a = [_unpack(t).astype(f32) for t in xs]
                    outs = []
                    if sums:
                        for qd in range(4):
                            xn[_half(r[qd // 2]), cols[qd % 2]] = xs[qd]
                        cs = _a_combos(*a)
                        for t, slot in _A_SLOT.items():
                            outs.append(_pack(cs[t]))
                            xa[slot, _half(r[0]), cols[0]] = outs[-1]
                    if gate:
                        for qd in range(4):
                            g0 = (qd % 2) * 4 + c
                            term = a[qd] * gw[g0:g0 + 1, :]
                            z[qd // 2] = term if z[qd // 2] is None else z[qd // 2] + term
                        outs += z
                    prev = sp.chain(outs, prev, 1)
                if gate:
                    for hf in range(2):
                        g = jax.nn.sigmoid(jnp.sum(z[hf], axis=1, keepdims=True))
                        g = jnp.broadcast_to(g, (16, 128))
                        gs[r[hf], :] = g
                        prev = sp.chain([g], prev, 1)
                return sp.chain([prev], first, 1)
            return run
        return [task(s0) for s0 in range(0, RB, 16)]

    def b_sum_tasks(src, dst):
        def task(r0):
            def run(prev):
                raw = [src(slice(a * KH + r0, a * KH + r0 + 16), slice(c * KH, (c + 1) * KH))
                       for a in range(2) for c in range(2)]
                cs = _b_combos(*[b.astype(f32) for b in raw])
                for t in _B_SUMS:
                    dst.setdefault(t, []).append(_pack(cs[t]))
                return sp.chain([dst[t][-1] for t in _B_SUMS], prev, DEPTH)
            return run
        return [task(r0) for r0 in range(0, KH, 16)]

    def b_rhs(src, sums):
        def rhs(t):
            if t == 1:
                return src(slice(0, KH), slice(0, KH))
            if t == 4:
                return src(slice(KH, D), slice(KH, D))
            return _unpack(jnp.concatenate(sums[t], axis=0))
        return rhs

    def strassen_x(order, rhs, finish):
        m = {}
        for rb, t in order:
            m.setdefault(rb, {})[t] = sp.dot(x_lhs(t, rb), rhs(t))
            if len(m[rb]) == 7:
                finish(rb, m.pop(rb))

    def h_sums(rb, cs, r0, sub):
        h = []
        for qd, cc in enumerate(cs):
            g0 = (qd // 2) * H + rb * RB + r0
            omg = 1.0 - gs[g0:g0 + sub, :]
            omg = jnp.concatenate([omg] * (CH // 128), axis=1)
            h.append(jnp.maximum(cc[:, :CH], 0.0) * cc[:, CH:] * omg)
        return _a_combos(*h)

    def glu_tasks(hs, rb, cs, sub):
        hs[rb] = [[] for _ in range(7)]

        def task(r0):
            def run(prev=None):
                sums = h_sums(rb, [cc[r0:r0 + sub] for cc in cs], r0, sub)
                for t in range(7):
                    hs[rb][t].append(sums[t])
                if sub < RB:
                    return sp.chain([sums[t] for t in _A_SLOT], prev, DEPTH2)
            return run
        return [task(r0) for r0 in range(0, RB, sub)]

    def down_lhs(hs, b, ha, tok):
        for t in H_ORDER:
            s0, s1 = [jnp.concatenate(hs[rb][t], axis=0) for rb in (b, b + 2)]
            slabs = []
            for r in range(0, RB, 16):
                slabs.append(sp.serial_combos(
                    _a_combos, s0[r:r + 16, :CQ], s0[r:r + 16, CQ:],
                    s1[r:r + 16, :CQ], s1[r:r + 16, CQ:], tok))
                tok = sp.chain([slabs[-1][t2] for t2 in _A_SLOT], None, H_DEPTH)
            for t2 in range(7):
                ha[b, 7 * t + t2] = jnp.concatenate([sl[t2] for sl in slabs], axis=0).astype(bf16)

    def d_tasks(j, dst):
        def task(r0, c):
            def run(prev):
                def blk(k1, k2, n1, n2):
                    r, c0 = k1 * CH + k2 * CQ + r0, n1 * KH + n2 * KQ + c * 128
                    return wd[j, r:r + 16, c0:c0 + 128].astype(f32)
                cs, tok = sp.two_level(_b_combos, blk, prev, DEPTH2)
                for t in range(49):
                    dst.setdefault((t, c), []).append(cs[t])
                return tok
            return run
        return [task(r0, c) for r0 in range(0, CQ, 16) for c in range(2)]

    def ffn_down(ha, dc, first):
        rhs = [_unpack(jnp.concatenate([jnp.concatenate(dc[t, c], axis=0) for c in range(2)], axis=1))
               for t in range(49)]
        todo = [(b, 7 * t + t2) for b in range(2) for t in H_ORDER for t2 in range(7)]
        for i in range(0, len(todo), 2):
            pair = todo[i:i + 2]
            ps = sp.dots([(ha[b, t], rhs[t]) for b, t in pair])
            for (b, t), p in zip(pair, ps):
                if first:
                    acc[t, b * RB:(b + 1) * RB, :] = p
                else:
                    acc[t, b * RB:(b + 1) * RB, :] += p

    def perm_tasks(wqkv_vm, wp, i, tbuf):
        def fwd(rb, c):
            def run(prev):
                c0 = i * D + c * 128
                tt = pltpu.bitcast(wqkv_vm[rb * 256:(rb + 1) * 256, c0:c0 + 128], f32).T
                for hh in range(4):
                    tbuf[rb, pl.ds((4 * c + hh) * TP, DH), :] = tt[hh * DH:(hh + 1) * DH, :]
                return sp.chain([tt], prev, 1)
            return run

        def bwd(rb, j):
            def run(prev):
                g = jnp.concatenate(
                    [tbuf[rb, pl.ds(4 * j + dd, NH, stride=TP), :] for dd in range(4)], axis=0).T
                wp[i, rb * 128:(rb + 1) * 128, j * 128:(j + 1) * 128] = pltpu.bitcast(g, i32)
            return run
        tasks = []
        for rb in range(4):
            tasks += [fwd(rb, c) for c in range(8)] + [bwd(rb, j) for j in range(8)]
        return tasks

    def wo_tasks(wo_vm):
        def stage(c):
            return 4 + c % 4, (c // 4) * NH * TP

        def spread(h0):
            def run(prev):
                blk = wo_vm[h0 * DH:(h0 + 2) * DH, :].astype(f32)
                for h in range(2):
                    for c in range(8):
                        sl, r0 = stage(c)
                        q_s[sl, pl.ds(r0 + (h0 + h) * TP, DH), :] = (
                            blk[h * DH:(h + 1) * DH, c * 128:(c + 1) * 128])
                return sp.chain([blk], prev, 1)
            return run

        def gather(d, h0, c):
            def run(after):
                def blk(k1, k2, n1, n2):
                    sl, r0 = stage(4 * n1 + 2 * n2 + c)
                    r0 += h0 * TP + 16 * k1 + 8 * k2 + d
                    return q_s[sl, pl.ds(r0, 16, stride=TP), :]
                cs, tok = sp.two_level(_b_combos, blk, None, DEPTH2, after)
                r = (d * NH + h0) // 2
                for t in range(49):
                    woc[t, r:r + 8, c * 128:(c + 1) * 128] = cs[t]
                return tok
            return run
        return ([spread(h0) for h0 in range(0, NH, 2)],
                [gather(d, h0, c) for d in range(8) for h0 in (0, 16) for c in range(2)])

    def proj(wp, i, dst, pad, slabs):
        lhs = jnp.concatenate([xn[r0 // 2:(r0 + n) // 2, :] for r0, n in slabs], axis=0)
        p = sp.dot(_unpack(lhs), _unpack(wp[i]))
        at = 0
        for r0, n in slabs:
            for j in range(8):
                dst[j, pad + r0:pad + r0 + n, :] = p[at:at + n, j * 128:(j + 1) * 128]
            at += n

    def v_finish(rb, m):
        cs = _c_combos(m)
        for qd, cc in enumerate(cs):
            r0 = PAD + (qd // 2) * H + rb * RB
            for j in range(4):
                v_s[(qd % 2) * 4 + j, r0:r0 + RB, :] = cc[:, j * 128:(j + 1) * 128]
        if rb == 0:
            for j in range(8):
                src = cs[j // 4][0:1, (j % 4) * 128:(j % 4 + 1) * 128]
                v_s[j, 0:PAD, :] = jnp.broadcast_to(src, (PAD, 128))

    def attn_group(row, masked):
        def run(prev):
            g = 8
            q = [q_s[j, pl.ds(row, g), :] for j in range(8)]
            ls = []
            for w in range(W):
                a = None
                for j in range(8):
                    term = q[j] * k_s[j, pl.ds(row + (PAD - DIL * w), g), :]
                    a = sp.link(ls[-1] if ls else None, term) if a is None else a + term
                ls.append(a)
            rs = [pltpu.roll(a, 64, 1) for a in ls]
            ls = [a + r for a, r in zip(ls, rs)]
            rs = [pltpu.roll(a, 32, 1) for a in ls]
            ls = [a + r for a, r in zip(ls, rs)]
            if masked:
                ri = row + lax.broadcasted_iota(i32, (g, 128), 0)
                ls = [ls[0]] + [jnp.where(ri >= DIL * w, ls[w], NEG) for w in range(1, W)]
            m = _tree(jnp.maximum, ls)
            ps = [jnp.exp2((l - m) * EXP2_SCALE) for l in ls]
            r = gs[pl.ds(row, g), :] / _tree(jnp.add, ps)
            outs = []
            for j in range(8):
                a = None
                for w in range(W):
                    term = ps[w] * v_s[j, pl.ds(row + (PAD - DIL * w), g), :]
                    a = sp.link(outs[-1] if outs else None, term) if a is None else a + term
                outs.append(a * r)
            for j in range(8):
                q_s[j, pl.ds(row, g), :] = outs[j]
            return sp.chain([outs[-1]], prev, 1)
        return run

    def attn_tasks(base, nrows, first=False):
        return [attn_group(base + (qq * Q + r), first and qq == 0 and r < PAD)
                for r in range(0, nrows, 8) for qq in range(4)]

    def pack_tasks(oa, base, hbase, nrows):
        def task(r, c):
            def run(prev):
                def blk(i1, i2, k1, k2):
                    return q_s[4 * k1 + 2 * k2 + c, pl.ds(base + (i1 * H + i2 * Q + r), 16), :]
                cs, tok = sp.two_level(_a_combos, blk, prev, DEPTH2)
                for t in range(49):
                    oa[t, pl.ds(hbase + r // 2, 8), c * 128:(c + 1) * 128] = cs[t]
                return tok
            return run
        return [task(r, c) for r in range(0, nrows, 16) for c in range(2)]

    GS = RB * (KH // 128) * (FC // 128) * 7 // (4 * SLOT)
    DS = 49
    PS = 2 * RB * (D // 128) * (D // 128) // (4 * SLOT)

    def glu(hs, ha):
        def finish(rb, m):
            if rb < 2 or not G_DEPTH:
                glu_tasks(hs, rb, _c_combos(m), RB)[0]()
                tok = None
            else:
                tok, pieces = None, []
                for r in range(0, RB, 16):
                    mm = {t: v[r:r + 16] for t, v in m.items()}
                    for t in ORDER[-G_LINK:]:
                        mm[t] = jnp.concatenate([sp.link_rows(tok, mm[t][:, c:c + 128])
                                                 for c in range(0, FC, 128)], axis=1)
                    pieces.append(h_sums(rb, _c_combos(mm), r, 16))
                    tok = sp.chain([pieces[-1][t] for t in _A_SLOT], None, G_DEPTH)
                hs[rb] = [[pc[t] for pc in pieces] for t in range(7)]
            if rb >= 2:
                down_lhs(hs, rb - 2, ha, tok)
        return finish

    def raw_first(rbs, NRAW):
        lead = [(rb, t) for rb in rbs[:NRAW] for t in ORDER[:2]]
        return lead + [(rb, t) for rb in rbs for t in ORDER if (rb, t) not in lead]

    def gu_src(j):
        return lambda r, c: wgu[j, r, c]

    def front(wqkv_vm, wp, wo_vm):
        in_q, in_k, in_v = [
            cp(wqkv_hbm.at[:, pl.ds(i * D, D)], wqkv_vm.at[:, pl.ds(i * D, D)], (6, 6, 5)[i])
            for i in range(3)]
        in_wo = cp(wo_hbm, wo_vm, 6)

        def plain(rb, hf, p):
            return sp.dot(x_vm[rows(rb, hf), :], wgu[0, :, p * CH:(p + 1) * CH])

        def plain_finish(rb, c):
            cs = [jnp.concatenate(c[2 * qd:2 * qd + 2], axis=1) for qd in range(4)]
            return glu_tasks(hs, rb, cs, 16)

        hs, bc, dc = {}, {}, {}
        with _Scope("w0"):
            wait(in0)
        start(in3)
        c0 = {(0, 0): plain(0, 0, 0)}
        with _Scope("wa"):
            wait(in1)
        c0[1, 0] = plain(0, 1, 0)
        with _Scope("wb"):
            wait(in2)
        start(in4)
        for hf in range(2):
            c0[hf, 1] = plain(0, hf, 1)
        with _Scope("wc"):
            wait(in3)
        with _Scope("p1a"):
            start(in5)
            sp.block()
            bt = b_sum_tasks(gu_src(0), bc)
            sp.schedule(bt[:12], 3, 16)
            sp.schedule(prep_tasks(0, sums=False), 3, 16)
            for p in (2, 3):
                for hf in range(2):
                    c0[hf, p] = plain(0, hf, p)
            c0 = [c0[hf, p] for hf in range(2) for p in range(4)]
        with _Scope("w1"):
            wait(in4)
            start([in_v])
        with _Scope("p1b"):
            sp.block()
            sp.schedule(bt[12:], 3, 32)
            sp.schedule(prep_tasks(1, sums=False), 2, 10)
            sp.schedule(prep_tasks(2), 10, 32)
            c1 = [plain(1, hf, p) for hf in range(2) for p in range(4)]
        with _Scope("w2"):
            wait(in5 + [in_v])
            start([in_k, in_wo, in_q])
        with _Scope("p1c"):
            sp.block()
            for j in range(8):
                k_s[j, 0:PAD, :] = jnp.zeros((PAD, 128), f32)
            ha = {}
            sp.schedule(prep_tasks(3), 2, GS)
            sp.schedule(plain_finish(0, c0), 2, GS)
            sp.schedule(plain_finish(1, c1), GS + 6, 2 * GS)
            sp.schedule(d_tasks(0, dc), GS - 2, 2 * GS)
            sp.schedule(perm_tasks(wqkv_vm, wp, 2, q_s), 2 * GS + 6, 2 * GS + DS - 8)
            strassen_x([(rb, t) for rb in (2, 3) for t in ORDER], b_rhs(gu_src(0), bc),
                       glu(hs, ha))
            ffn_down(ha, dc, True)

        with _Scope("w2b"):
            wait([in_k, in_wo, in_q])
            start(in_ffn)
        with _Scope("v"):
            sp.block()
            vb = {}
            v_src = lambda r, c: _unpack(wp[2, _half(r), c])
            wo_spread, wo_gather = wo_tasks(wo_vm)
            sp.schedule(b_sum_tasks(v_src, vb), *VBC_SLOTS)
            sp.schedule(prep_tasks(0, gate=False) + prep_tasks(1, gate=False), *PREP01)
            sp.schedule(perm_tasks(wqkv_vm, wp, 1, k_s.at[:, PAD:, :]), *PERMK)
            sp.schedule(wo_spread, *WOS)
            strassen_x(raw_first((2, 3, 0, 1), 2), b_rhs(v_src, vb), v_finish)
            sp.schedule(perm_tasks(wqkv_vm, wp, 0, q_s), 4, 3 * PS)
            tok = None
            for t in wo_gather:
                tok = t(tok)
            for rb in range(NRB):
                proj(wp, 1, k_s, PAD, [(rb * Q, Q)])
            proj(wp, 0, q_s, 0, [(qq * Q, QA) for qq in range(4)])

        def q_rest(_, carry):
            with _Scope("q"):
                sp.block()
                n = (Q - QA) // 2
                total = 4 * (Q - QA) * 64 // (4 * SLOT)
                sp.schedule(attn_tasks(0, A0, True), 4, total)
                for r0 in (QA, QA + n):
                    proj(wp, 0, q_s, 0, [(qq * Q + r0, n) for qq in range(4)])
            return carry

        lax.fori_loop(0, zi[0], q_rest, 0)
        wait(in_ffn)

    def back(oa):
        def body(j, carry):
            with _Scope("chunk"):
                sp.block()
                base = pl.multiple_of((j - 1) * AR, AR)
                hs, ha, bc, dc = {}, {}, {}, {}
                sp.schedule(b_sum_tasks(gu_src(j), bc), *BC_SLOTS)
                sp.schedule(attn_tasks(base + A0, AR), *ATTN_SLOTS)
                sp.schedule(pack_tasks(oa, base, pl.multiple_of((j - 1) * (AR // 2), AR // 2), AR),
                            *PACK_SLOTS)
                sp.schedule(d_tasks(j, dc), *DC_SLOTS)
                strassen_x(raw_first((0, 2, 1, 3), NRAW), b_rhs(gu_src(j), bc), glu(hs, ha))
                ffn_down(ha, dc, False)
            return carry

        lax.fori_loop(1, NC, body, 0)

        def out_copies(r0, i1, cols):
            cs = []
            for i2 in range(2):
                idx = (pl.ds(r0 + (i1 * H + i2 * Q), PB), cols)
                cs.append(cp(x_vm.at[idx], o2.at[idx], out_sem))
            return cs

        def out_blocks(blocks):
            todo = [(blk, 7 * t1 + t2) for blk in range(len(blocks))
                    for ts1, _ in _C_ORDER for t1 in ts1 for ts2, _ in _C_ORDER for t2 in ts2]
            m = {}
            for i in range(0, len(todo), 2):
                pair = todo[i:i + 2]
                ps = sp.dots([(_unpack(oa[t, pl.ds(blocks[blk][1], PB // 2), :]), _unpack(woc[t]))
                              for blk, t in pair])
                for (blk, t), p in zip(pair, ps):
                    r0, _, copies = blocks[blk]
                    mm = m.setdefault(blk, ({}, {}))
                    mm[0][t] = acc[t, pl.ds(r0, PB), :] + p
                    t1 = t // 7
                    if t % 7 != _C_ORDER[-1][0][-1]:
                        continue
                    mm[1][t1] = _c_combos([mm[0].pop(7 * t1 + t2) for t2 in range(7)])
                    for ts, qd in _C_ORDER:
                        if t1 != ts[-1]:
                            continue
                        for q2 in range(4):
                            val = _c_quadrant({tt: v[q2] for tt, v in mm[1].items()}, qd)
                            r = pl.ds(r0 + ((qd // 2) * H + (q2 // 2) * Q), PB)
                            c = (qd % 2) * KH + (q2 % 2) * KQ
                            x_vm[r, c:c + KQ] = val.astype(bf16)
                        start(copies.get(qd, []))

        def whole(r0):
            return [c for i1 in range(2) for c in out_copies(r0, i1, slice(None))]

        done = (NC - 1) * AR

        def out_body(i, carry):
            with _Scope("p4a"):
                sp.block()
                half = pl.multiple_of(done // 2 + i * 24, 8)
                sp.schedule(pack_tasks(oa, 2 * half, half, 48), *PACK4)
                r0 = pl.multiple_of(i * PB, PB)
                out_blocks([(r0, pl.multiple_of(i * (PB // 2), PB // 2),
                             {3: whole(r0)})])
            return carry

        lax.fori_loop(0, 2, out_body, 0)
        with _Scope("p4b"):
            sp.block()
            sp.schedule(pack_tasks(oa, done + 96, (done + 96) // 2, Q - done - 96), 4, 22)
            last = {qd: out_copies(3 * PB, qd // 2, pl.ds((qd % 2) * KH, KH))
                    for qd in range(4)}
            copies = [{3: whole(blk * PB)} for blk in range(3)] + [last]
            out_blocks([(blk * PB, blk * PB // 2, copies[blk]) for blk in (2, 3)])
        with _Scope("w4"):
            for cs in copies:
                for qd in cs:
                    wait(cs[qd])

    pl.run_scoped(front, pltpu.VMEM((D, 3 * D), bf16), pltpu.VMEM((3, D // 2, D), i32),
                  pltpu.VMEM((D, D), bf16))
    pl.run_scoped(back, pltpu.VMEM((49, Q // 2, KQ), i32))
    assert not sp.plan


_N_SEMS = 9


@jax.jit
def pallas_gated_mix__sliding_local_dilated__glu_gated_reglu__prompt_kernel(
    A_x: jax.Array,
    A_wqkv: jax.Array,
    A_wo: jax.Array,
    B_x: jax.Array,
    B_W_gate: jax.Array,
    B_W_up: jax.Array,
    B_W_down: jax.Array,
    gate_w: jax.Array,
):
    del B_x
    hbm = pl.BlockSpec(memory_space=pl.ANY)
    scratch = [
        pltpu.VMEM((S, D), bf16),
        pltpu.VMEM((S // 2, D), i32),
        pltpu.VMEM((5, H // 2, KH), i32),
        pltpu.VMEM((8, 128), bf16),
        pltpu.VMEM((NC, D, 2 * FC), bf16),
        pltpu.VMEM((NC, FC, D), bf16),
        pltpu.VMEM((49, Q, KQ), f32),
        pltpu.VMEM((8, S + QPAD, 128), f32),
        pltpu.VMEM((8, PAD + S, 128), f32),
        pltpu.VMEM((8, PAD + S, 128), f32),
        pltpu.VMEM((S, 128), f32),
        pltpu.VMEM((49, KQ // 2, KQ), i32),
        pltpu.VMEM((8, 128), i32),
        pltpu.SMEM((1,), i32),
        pltpu.SemaphoreType.DMA((_N_SEMS,)),
    ]
    return pl.pallas_call(
        _kernel,
        in_specs=[hbm] * 7,
        out_specs=hbm,
        out_shape=jax.ShapeDtypeStruct((1, S, D), bf16),
        scratch_shapes=scratch,
        compiler_params=pltpu.CompilerParams(vmem_limit_bytes=124 * 1024 * 1024),
    )(A_x, A_wqkv, A_wo, B_W_gate, B_W_up, B_W_down, gate_w.reshape(8, 128))
```

```python
import math

import jax
import jax.numpy as jnp
from jax import lax
import jax.experimental.pallas as pl
import jax.experimental.pallas.tpu as pltpu

f32 = jnp.float32
bf16 = jnp.bfloat16
i32 = jnp.int32

S = 2048
D = 1024
F = 3584
NH = 32
DH = D // NH
W = 8
DIL = 2
H = S // 2
Q = S // 4
KH = D // 2
KQ = D // 4
FC = 512
CH = FC // 2
CQ = FC // 4
NC = F // FC
RB = 256
NRB = H // RB
PB = 128
PAD = 16
TP = DH + 1
AR = 64
A0 = Q - 6 * AR
QA = 160
QPAD = 112

BC_SLOTS = (2, 24)
ATTN_SLOTS = (20, 96)
DC_SLOTS = (24, 96)
PACK_SLOTS = (96, 112)
VBC_SLOTS = (2, 16)
PREP01 = (16, 56)
PERMK = (64, 106)
WOS = (70, 112)
PACK4 = (4, 24)
NRAW = 3
DEPTH = 3
DEPTH2 = 3
H_DEPTH = 3

SCALE = DH ** -0.5
EXP2_SCALE = SCALE * math.log2(math.e)
NEG = -1e9 / SCALE


def _a_combos(a11, a12, a21, a22):
    return [a11 + a22, a21 + a22, a11, a22, a11 + a12, a21 - a11, a12 - a22]


def _b_combos(b11, b12, b21, b22):
    return [b11 + b22, b11, b12 - b22, b21 - b11, b22, b11 + b12, b21 + b22]


_C_TERMS = (((1, 0), (1, 3), (-1, 4), (1, 6)), ((1, 2), (1, 4)), ((1, 1), (1, 3)),
            ((1, 0), (-1, 1), (1, 2), (1, 5)))
_C_ORDER = (((2, 4), 1), ((1, 3), 2), ((0, 6), 0), ((5,), 3))


def _c_quadrant(m, qd):
    out = m[_C_TERMS[qd][0][1]]
    for sign, t in _C_TERMS[qd][1:]:
        out = out + m[t] if sign > 0 else out - m[t]
    return out


def _c_combos(m):
    return [_c_quadrant(m, qd) for qd in range(4)]


_A_SLOT = {0: 0, 1: 1, 4: 2, 5: 3, 6: 4}
_B_SUMS = (2, 3, 0, 5, 6)
ORDER = (1, 4) + _B_SUMS


def _tree(op, xs):
    xs = list(xs)
    while len(xs) > 1:
        xs = [op(xs[i], xs[i + 1]) if i + 1 < len(xs) else xs[i] for i in range(0, len(xs), 2)]
    return xs[0]


def _pack(x):
    return pltpu.bitcast(x.astype(bf16), i32)


def _unpack(x):
    return pltpu.bitcast(x, bf16)


def _half(r):
    return slice(r.start // 2, r.stop // 2)


SLOT = 256


class _Spreader:
    def __init__(self, zero_ref):
        self.zero_ref = zero_ref
        self.plan = {}
        self.lists = 0
        self.now = 0

    def block(self):
        self.zero = self.zero_ref[...]
        self.never = self.zero != 0

    def link(self, after, x):
        if after is None:
            return x
        if after.dtype != x.dtype:
            after = pltpu.bitcast(after, x.dtype)
        return jnp.where(self.never, after, x)

    def chain(self, vals, prev, depth):
        for v in vals:
            v = pltpu.bitcast(v, i32) if v.dtype != i32 else v
            for r in range(0, v.shape[0], 8):
                for c in range(0, v.shape[1], 128):
                    tile = v[r:r + 8, c:c + 128]
                    if prev is None:
                        prev = tile
                        continue
                    prev = prev | tile
                    for i in range(depth - 1):
                        prev = (prev + self.zero) if i % 2 == 0 else (prev ^ self.zero)
        return prev

    def link_rows(self, after, x):
        return jnp.concatenate([self.link(after, x[r:r + 8, :]) for r in range(0, x.shape[0], 8)],
                               axis=0)

    def serial_combos(self, combos, x11, x12, x21, x22, after):
        return combos(self.link_rows(after, x11), x12, x21, self.link_rows(after, x22))

    def two_level(self, combos, blk, prev, depth, after=None):
        outer = [self.serial_combos(
            combos, *[blk(r1, r2, c1, c2) for r1 in range(2) for c1 in range(2)], after)
            for r2 in range(2) for c2 in range(2)]
        outs, tok = [], None
        for t in range(7):
            wide = _pack(jnp.concatenate(
                self.serial_combos(combos, *[o[t] for o in outer], tok), axis=1))
            outs += [wide[:, c:c + 128] for c in range(0, 7 * 128, 128)]
            tok = self.chain(outs[-7:], tok, depth)
        return outs, self.chain([tok], prev, 1)

    def schedule(self, tasks, first, last):
        n = len(tasks)
        self.lists += 1
        for i, t in enumerate(tasks):
            pos = self.now + first + ((i + 1) * (last - first) - 1) // n
            self.plan.setdefault(pos, []).append((t, self.lists))

    def dots(self, pairs):
        m = pairs[0][0].shape[0]
        tiles = [(i, r, c) for i, (_, rhs) in enumerate(pairs)
                 for c in range(0, rhs.shape[1], 128) for r in range(0, rhs.shape[0], 128)]
        nslots = m * len(tiles) // (4 * SLOT)
        deps = {}
        for sl in range(nslots):
            ps = sl * SLOT // m
            toks = {}
            for t, lane in self.plan.pop(self.now + sl, []):
                tok = t(toks.get(lane))
                if tok is not None:
                    toks[lane] = tok
            for tok in toks.values():
                deps[ps] = tok | deps[ps] if ps in deps else tok
        self.now += nslots
        tied = {tile: d for ps, d in deps.items() for tile in tiles[4 * ps:4 * ps + 4]}
        outs = []
        for i, (lhs, rhs) in enumerate(pairs):
            if any(key[0] == i for key in tied):
                parts = []
                for r in range(0, rhs.shape[0], 128):
                    top = [rhs[r:r + 16, c:c + 128] for c in range(0, rhs.shape[1], 128)]
                    top = [_unpack(self.link(tied[i, r, c * 128], _pack(t0)))
                           if (i, r, c * 128) in tied else t0 for c, t0 in enumerate(top)]
                    parts += [jnp.concatenate(top, axis=1), rhs[r + 16:r + 128, :]]
                rhs = jnp.concatenate(parts, axis=0)
            outs.append(jnp.dot(lhs, rhs, preferred_element_type=f32))
        return outs

    def dot(self, lhs, rhs):
        return self.dots([(lhs, rhs)])[0]


def _kernel(x_hbm, wqkv_hbm, wo_hbm, wg_hbm, wu_hbm, wd_hbm, gw_hbm, out_hbm,
            x_vm, xn, xa, gw_vm, wgu, wd, acc, q_s, k_s, v_s, gs, woc, zs, zi, sems):
    def cp(src, dst, sem):
        return pltpu.make_async_copy(src, dst, sems.at[sem])

    def cp_gu(j, p, sem):
        return cp((wg_hbm, wu_hbm)[p % 2].at[:, pl.ds(j * FC + (p // 2) * CH, CH)],
                  wgu.at[j, :, pl.ds(p * CH, CH)], sem)

    def cp_d(j, sem):
        return cp(wd_hbm.at[pl.ds(j * FC, FC), :], wd.at[j], sem)

    def cp_x(rb, hf, sem):
        idx = (pl.ds(hf * H + rb * RB, RB), slice(None))
        return cp(x_hbm.at[0].at[idx], x_vm.at[idx], sem)

    o2 = out_hbm.at[0]
    in0 = [cp_x(0, 0, 0), cp_gu(0, 0, 0)]
    in1 = [cp_x(0, 1, 1)]
    in2 = [cp_gu(0, 1, 2)]
    in3 = [cp_gu(0, 2, 3), cp_gu(0, 3, 3), cp(gw_hbm, gw_vm, 3)]
    in4 = [cp_x(rb, hf, 4) for rb in (1, 2) for hf in range(2)]
    in5 = [cp_x(3, 0, 5), cp_x(3, 1, 5), cp_d(0, 5)]
    in_ffn = [c for j in range(1, NC) for c in [cp_gu(j, p, 7) for p in range(4)] + [cp_d(j, 7)]]
    out_sem = 8

    def start(cs):
        for c in cs:
            c.start()

    def wait(cs):
        for c in cs:
            c.wait()

    start(in0 + in1 + in2)

    zs[...] = jnp.zeros((8, 128), i32)
    zi[0] = 1
    sp = _Spreader(zs)

    def rows(rb, hf=0):
        return slice(hf * H + rb * RB, hf * H + (rb + 1) * RB)

    def x_lhs(t, rb):
        if t == 2:
            return _unpack(xn[_half(rows(rb, 0)), :KH])
        if t == 3:
            return _unpack(xn[_half(rows(rb, 1)), KH:])
        return _unpack(xa[_A_SLOT[t], _half(rows(rb)), :])

    def prep_tasks(rb, sums=True, gate=True):
        def task(s0):
            def run(first):
                prev = None
                gw = gw_vm[...].astype(f32)
                r = [slice(hf * H + rb * RB + s0, hf * H + rb * RB + s0 + 16) for hf in range(2)]
                z = [None, None]
                for c in range(4):
                    cols = [slice(kh * KH + c * 128, kh * KH + (c + 1) * 128) for kh in range(2)]
                    xs = [sp.link(prev, _pack(x_vm[r[qd // 2], cols[qd % 2]])) for qd in range(4)]
                    a = [_unpack(t).astype(f32) for t in xs]
                    outs = []
                    if sums:
                        for qd in range(4):
                            xn[_half(r[qd // 2]), cols[qd % 2]] = xs[qd]
                        cs = _a_combos(*a)
                        for t, slot in _A_SLOT.items():
                            outs.append(_pack(cs[t]))
                            xa[slot, _half(r[0]), cols[0]] = outs[-1]
                    if gate:
                        for qd in range(4):
                            g0 = (qd % 2) * 4 + c
                            term = a[qd] * gw[g0:g0 + 1, :]
                            z[qd // 2] = term if z[qd // 2] is None else z[qd // 2] + term
                        outs += z
                    prev = sp.chain(outs, prev, 1)
                if gate:
                    for hf in range(2):
                        g = jax.nn.sigmoid(jnp.sum(z[hf], axis=1, keepdims=True))
                        g = jnp.broadcast_to(g, (16, 128))
                        gs[r[hf], :] = g
                        prev = sp.chain([g], prev, 1)
                return sp.chain([prev], first, 1)
            return run
        return [task(s0) for s0 in range(0, RB, 16)]

    def b_sum_tasks(src, dst):
        def task(r0):
            def run(prev):
                raw = [src(slice(a * KH + r0, a * KH + r0 + 16), slice(c * KH, (c + 1) * KH))
                       for a in range(2) for c in range(2)]
                cs = _b_combos(*[b.astype(f32) for b in raw])
                for t in _B_SUMS:
                    dst.setdefault(t, []).append(_pack(cs[t]))
                return sp.chain([dst[t][-1] for t in _B_SUMS], prev, DEPTH)
            return run
        return [task(r0) for r0 in range(0, KH, 16)]

    def b_rhs(src, sums):
        def rhs(t):
            if t == 1:
                return src(slice(0, KH), slice(0, KH))
            if t == 4:
                return src(slice(KH, D), slice(KH, D))
            return _unpack(jnp.concatenate(sums[t], axis=0))
        return rhs

    def strassen_x(order, rhs, finish):
        m = {}
        for rb, t in order:
            m.setdefault(rb, {})[t] = sp.dot(x_lhs(t, rb), rhs(t))
            if len(m[rb]) == 7:
                finish(rb, m.pop(rb))

    def h_sums(rb, cs, r0, sub):
        h = []
        for qd, cc in enumerate(cs):
            g0 = (qd // 2) * H + rb * RB + r0
            omg = 1.0 - gs[g0:g0 + sub, :]
            omg = jnp.concatenate([omg] * (CH // 128), axis=1)
            h.append(jnp.maximum(cc[:, :CH], 0.0) * cc[:, CH:] * omg)
        return _a_combos(*h)

    def glu_tasks(hs, rb, cs, sub):
        hs[rb] = [[] for _ in range(7)]

        def task(r0):
            def run(prev):
                sums = h_sums(rb, [cc[r0:r0 + sub] for cc in cs], r0, sub)
                for t in range(7):
                    hs[rb][t].append(sums[t])
                if sub < RB:
                    return sp.chain([sums[t] for t in _A_SLOT], prev, DEPTH2)
            return run
        return [task(r0) for r0 in range(0, RB, sub)]

    def down_lhs(hs, b, ha):
        tok = None
        for t in range(7):
            s0, s1 = [jnp.concatenate(hs[rb][t], axis=0) for rb in (b, b + 2)]
            slabs = []
            for r in range(0, RB, 16):
                slabs.append(sp.serial_combos(
                    _a_combos, s0[r:r + 16, :CQ], s0[r:r + 16, CQ:],
                    s1[r:r + 16, :CQ], s1[r:r + 16, CQ:], tok))
                tok = sp.chain([slabs[-1][t2] for t2 in _A_SLOT], None, H_DEPTH)
            for t2 in range(7):
                ha[b, 7 * t + t2] = jnp.concatenate([sl[t2] for sl in slabs], axis=0).astype(bf16)

    def d_tasks(j, dst):
        def task(r0, c):
            def run(prev):
                def blk(k1, k2, n1, n2):
                    r, c0 = k1 * CH + k2 * CQ + r0, n1 * KH + n2 * KQ + c * 128
                    return wd[j, r:r + 16, c0:c0 + 128].astype(f32)
                cs, tok = sp.two_level(_b_combos, blk, prev, DEPTH2)
                for t in range(49):
                    dst.setdefault((t, c), []).append(cs[t])
                return tok
            return run
        return [task(r0, c) for r0 in range(0, CQ, 16) for c in range(2)]

    def ffn_down(ha, dc, first):
        rhs = [_unpack(jnp.concatenate([jnp.concatenate(dc[t, c], axis=0) for c in range(2)], axis=1))
               for t in range(49)]
        todo = [(b, t) for b in range(2) for t in range(49)]
        for i in range(0, len(todo), 2):
            pair = todo[i:i + 2]
            ps = sp.dots([(ha[b, t], rhs[t]) for b, t in pair])
            for (b, t), p in zip(pair, ps):
                if first:
                    acc[t, b * RB:(b + 1) * RB, :] = p
                else:
                    acc[t, b * RB:(b + 1) * RB, :] += p

    def perm_tasks(wqkv_vm, wp, i, tbuf):
        def fwd(rb, c):
            def run(prev):
                c0 = i * D + c * 128
                tt = pltpu.bitcast(wqkv_vm[rb * 256:(rb + 1) * 256, c0:c0 + 128], f32).T
                for hh in range(4):
                    tbuf[rb, pl.ds((4 * c + hh) * TP, DH), :] = tt[hh * DH:(hh + 1) * DH, :]
                return sp.chain([tt], prev, 1)
            return run

        def bwd(rb, j):
            def run(prev):
                g = jnp.concatenate(
                    [tbuf[rb, pl.ds(4 * j + dd, NH, stride=TP), :] for dd in range(4)], axis=0).T
                wp[i, rb * 128:(rb + 1) * 128, j * 128:(j + 1) * 128] = pltpu.bitcast(g, i32)
            return run
        tasks = []
        for rb in range(4):
            tasks += [fwd(rb, c) for c in range(8)] + [bwd(rb, j) for j in range(8)]
        return tasks

    def wo_tasks(wo_vm):
        def stage(c):
            return 4 + c % 4, (c // 4) * NH * TP

        def spread(h0):
            def run(prev):
                blk = wo_vm[h0 * DH:(h0 + 2) * DH, :].astype(f32)
                for h in range(2):
                    for c in range(8):
                        sl, r0 = stage(c)
                        q_s[sl, pl.ds(r0 + (h0 + h) * TP, DH), :] = (
                            blk[h * DH:(h + 1) * DH, c * 128:(c + 1) * 128])
                return sp.chain([blk], prev, 1)
            return run

        def gather(d, h0, c):
            def run(after):
                def blk(k1, k2, n1, n2):
                    sl, r0 = stage(4 * n1 + 2 * n2 + c)
                    r0 += h0 * TP + 16 * k1 + 8 * k2 + d
                    return q_s[sl, pl.ds(r0, 16, stride=TP), :]
                cs, tok = sp.two_level(_b_combos, blk, None, DEPTH2, after)
                r = (d * NH + h0) // 2
                for t in range(49):
                    woc[t, r:r + 8, c * 128:(c + 1) * 128] = cs[t]
                return tok
            return run
        return ([spread(h0) for h0 in range(0, NH, 2)],
                [gather(d, h0, c) for d in range(8) for h0 in (0, 16) for c in range(2)])

    def proj(wp, i, dst, pad, slabs):
        lhs = jnp.concatenate([xn[r0 // 2:(r0 + n) // 2, :] for r0, n in slabs], axis=0)
        p = sp.dot(_unpack(lhs), _unpack(wp[i]))
        at = 0
        for r0, n in slabs:
            for j in range(8):
                dst[j, pad + r0:pad + r0 + n, :] = p[at:at + n, j * 128:(j + 1) * 128]
            at += n

    def v_finish(rb, m):
        cs = _c_combos(m)
        for qd, cc in enumerate(cs):
            r0 = PAD + (qd // 2) * H + rb * RB
            for j in range(4):
                v_s[(qd % 2) * 4 + j, r0:r0 + RB, :] = cc[:, j * 128:(j + 1) * 128]
        if rb == 0:
            for j in range(8):
                src = cs[j // 4][0:1, (j % 4) * 128:(j % 4 + 1) * 128]
                v_s[j, 0:PAD, :] = jnp.broadcast_to(src, (PAD, 128))

    def attn_group(row, masked):
        def run(prev):
            g = 8
            q = [q_s[j, pl.ds(row, g), :] for j in range(8)]
            ls = []
            for w in range(W):
                a = None
                for j in range(8):
                    term = q[j] * k_s[j, pl.ds(row + (PAD - DIL * w), g), :]
                    a = sp.link(ls[-1] if ls else None, term) if a is None else a + term
                ls.append(a)
            rs = [pltpu.roll(a, 64, 1) for a in ls]
            ls = [a + r for a, r in zip(ls, rs)]
            rs = [pltpu.roll(a, 32, 1) for a in ls]
            ls = [a + r for a, r in zip(ls, rs)]
            if masked:
                ri = row + lax.broadcasted_iota(i32, (g, 128), 0)
                ls = [ls[0]] + [jnp.where(ri >= DIL * w, ls[w], NEG) for w in range(1, W)]
            m = _tree(jnp.maximum, ls)
            ps = [jnp.exp2((l - m) * EXP2_SCALE) for l in ls]
            r = gs[pl.ds(row, g), :] / _tree(jnp.add, ps)
            outs = []
            for j in range(8):
                a = None
                for w in range(W):
                    term = ps[w] * v_s[j, pl.ds(row + (PAD - DIL * w), g), :]
                    a = sp.link(outs[-1] if outs else None, term) if a is None else a + term
                outs.append(a * r)
            for j in range(8):
                q_s[j, pl.ds(row, g), :] = outs[j]
            return sp.chain([outs[-1]], prev, 1)
        return run

    def attn_tasks(base, nrows, first=False):
        return [attn_group(base + (qq * Q + r), first and qq == 0 and r < PAD)
                for r in range(0, nrows, 8) for qq in range(4)]

    def pack_tasks(oa, base, hbase, nrows):
        def task(r, c):
            def run(prev):
                def blk(i1, i2, k1, k2):
                    return q_s[4 * k1 + 2 * k2 + c, pl.ds(base + (i1 * H + i2 * Q + r), 16), :]
                cs, tok = sp.two_level(_a_combos, blk, prev, DEPTH2)
                for t in range(49):
                    oa[t, pl.ds(hbase + r // 2, 8), c * 128:(c + 1) * 128] = cs[t]
                return tok
            return run
        return [task(r, c) for r in range(0, nrows, 16) for c in range(2)]

    GS = RB * (KH // 128) * (FC // 128) * 7 // (4 * SLOT)
    DS = 49
    PS = 2 * RB * (D // 128) * (D // 128) // (4 * SLOT)

    def glu(hs, ha):
        def finish(rb, m):
            glu_tasks(hs, rb, _c_combos(m), RB)[0](None)
            if rb >= 2:
                down_lhs(hs, rb - 2, ha)
        return finish

    def raw_first(rbs, n):
        lead = [(rb, t) for rb in rbs[:n] for t in ORDER[:2]]
        return lead + [(rb, t) for rb in rbs for t in ORDER if (rb, t) not in lead]

    def gu_src(j):
        return lambda r, c: wgu[j, r, c]

    def front(wqkv_vm, wp, wo_vm):
        in_q, in_k, in_v = [
            cp(wqkv_hbm.at[:, pl.ds(i * D, D)], wqkv_vm.at[:, pl.ds(i * D, D)], (6, 6, 5)[i])
            for i in range(3)]
        in_wo = cp(wo_hbm, wo_vm, 6)

        def plain(rb, hf, p):
            return sp.dot(x_vm[rows(rb, hf), :], wgu[0, :, p * CH:(p + 1) * CH])

        def plain_finish(rb, c):
            cs = [jnp.concatenate(c[2 * qd:2 * qd + 2], axis=1) for qd in range(4)]
            return glu_tasks(hs, rb, cs, 16)

        hs, bc, dc = {}, {}, {}
        wait(in0)
        start(in3)
        c0 = {(0, 0): plain(0, 0, 0)}
        wait(in1)
        c0[1, 0] = plain(0, 1, 0)
        wait(in2)
        start(in4)
        for hf in range(2):
            c0[hf, 1] = plain(0, hf, 1)
        wait(in3)
        start(in5)
        sp.block()
        bt = b_sum_tasks(gu_src(0), bc)
        sp.schedule(bt[:12], 3, 16)
        sp.schedule(prep_tasks(0, sums=False), 3, 16)
        for p in (2, 3):
            for hf in range(2):
                c0[hf, p] = plain(0, hf, p)
        c0 = [c0[hf, p] for hf in range(2) for p in range(4)]
        wait(in4)
        start([in_v])
        sp.block()
        sp.schedule(bt[12:], 3, 32)
        sp.schedule(prep_tasks(1, sums=False), 2, 10)
        sp.schedule(prep_tasks(2), 10, 32)
        c1 = [plain(1, hf, p) for hf in range(2) for p in range(4)]
        wait(in5 + [in_v])
        start([in_k, in_wo, in_q])
        sp.block()
        for j in range(8):
            k_s[j, 0:PAD, :] = jnp.zeros((PAD, 128), f32)
        ha = {}
        sp.schedule(prep_tasks(3), 2, GS)
        sp.schedule(plain_finish(0, c0), 2, GS)
        sp.schedule(plain_finish(1, c1), GS + 6, 2 * GS)
        sp.schedule(d_tasks(0, dc), GS - 2, 2 * GS)
        sp.schedule(perm_tasks(wqkv_vm, wp, 2, q_s), 2 * GS + 6, 2 * GS + DS - 8)
        strassen_x([(rb, t) for rb in (2, 3) for t in ORDER], b_rhs(gu_src(0), bc),
                   glu(hs, ha))
        ffn_down(ha, dc, True)

        wait([in_k, in_wo, in_q])
        start(in_ffn)
        sp.block()
        vb = {}
        v_src = lambda r, c: _unpack(wp[2, _half(r), c])
        wo_spread, wo_gather = wo_tasks(wo_vm)
        sp.schedule(b_sum_tasks(v_src, vb), *VBC_SLOTS)
        sp.schedule(prep_tasks(0, gate=False) + prep_tasks(1, gate=False), *PREP01)
        sp.schedule(perm_tasks(wqkv_vm, wp, 1, k_s.at[:, PAD:, :]), *PERMK)
        sp.schedule(wo_spread, *WOS)
        strassen_x(raw_first((2, 3, 0, 1), 2), b_rhs(v_src, vb), v_finish)
        sp.schedule(perm_tasks(wqkv_vm, wp, 0, q_s), 4, 3 * PS)
        tok = None
        for t in wo_gather:
            tok = t(tok)
        for rb in range(NRB):
            proj(wp, 1, k_s, PAD, [(rb * Q, Q)])
        proj(wp, 0, q_s, 0, [(qq * Q, QA) for qq in range(4)])

        def q_rest(_, carry):
            sp.block()
            n = (Q - QA) // 2
            total = 4 * (Q - QA) * 64 // (4 * SLOT)
            sp.schedule(attn_tasks(0, A0, True), 4, total)
            for r0 in (QA, QA + n):
                proj(wp, 0, q_s, 0, [(qq * Q + r0, n) for qq in range(4)])
            return carry

        lax.fori_loop(0, zi[0], q_rest, 0)
        wait(in_ffn)

    def back(oa):
        def body(j, carry):
            sp.block()
            base = pl.multiple_of((j - 1) * AR, AR)
            hs, ha, bc, dc = {}, {}, {}, {}
            sp.schedule(b_sum_tasks(gu_src(j), bc), *BC_SLOTS)
            sp.schedule(attn_tasks(base + A0, AR), *ATTN_SLOTS)
            sp.schedule(pack_tasks(oa, base, pl.multiple_of((j - 1) * (AR // 2), AR // 2), AR),
                        *PACK_SLOTS)
            sp.schedule(d_tasks(j, dc), *DC_SLOTS)
            strassen_x(raw_first((0, 2, 1, 3), NRAW), b_rhs(gu_src(j), bc), glu(hs, ha))
            ffn_down(ha, dc, False)
            return carry

        lax.fori_loop(1, NC, body, 0)

        def out_copies(r0, i1, cols):
            cs = []
            for i2 in range(2):
                idx = (pl.ds(r0 + (i1 * H + i2 * Q), PB), cols)
                cs.append(cp(x_vm.at[idx], o2.at[idx], out_sem))
            return cs

        def out_blocks(blocks):
            todo = [(blk, 7 * t1 + t2) for blk in range(len(blocks))
                    for ts1, _ in _C_ORDER for t1 in ts1 for ts2, _ in _C_ORDER for t2 in ts2]
            m = {}
            for i in range(0, len(todo), 2):
                pair = todo[i:i + 2]
                ps = sp.dots([(_unpack(oa[t, pl.ds(blocks[blk][1], PB // 2), :]), _unpack(woc[t]))
                              for blk, t in pair])
                for (blk, t), p in zip(pair, ps):
                    r0, _, copies = blocks[blk]
                    mm = m.setdefault(blk, ({}, {}))
                    mm[0][t] = acc[t, pl.ds(r0, PB), :] + p
                    t1 = t // 7
                    if t % 7 != _C_ORDER[-1][0][-1]:
                        continue
                    mm[1][t1] = _c_combos([mm[0].pop(7 * t1 + t2) for t2 in range(7)])
                    for ts, qd in _C_ORDER:
                        if t1 != ts[-1]:
                            continue
                        for q2 in range(4):
                            val = _c_quadrant({tt: v[q2] for tt, v in mm[1].items()}, qd)
                            r = pl.ds(r0 + ((qd // 2) * H + (q2 // 2) * Q), PB)
                            c = (qd % 2) * KH + (q2 % 2) * KQ
                            x_vm[r, c:c + KQ] = val.astype(bf16)
                        start(copies.get(qd, []))

        def whole(r0):
            return [c for i1 in range(2) for c in out_copies(r0, i1, slice(None))]

        done = (NC - 1) * AR

        def out_body(i, carry):
            sp.block()
            half = pl.multiple_of(done // 2 + i * 24, 8)
            sp.schedule(pack_tasks(oa, 2 * half, half, 48), *PACK4)
            r0 = pl.multiple_of(i * PB, PB)
            out_blocks([(r0, pl.multiple_of(i * (PB // 2), PB // 2),
                         {3: whole(r0)})])
            return carry

        lax.fori_loop(0, 2, out_body, 0)
        sp.block()
        sp.schedule(pack_tasks(oa, done + 96, (done + 96) // 2, Q - done - 96), 4, 22)
        last = {qd: out_copies(3 * PB, qd // 2, pl.ds((qd % 2) * KH, KH))
                for qd in range(4)}
        copies = [{3: whole(blk * PB)} for blk in range(3)] + [last]
        out_blocks([(blk * PB, blk * PB // 2, copies[blk]) for blk in (2, 3)])
        for cs in copies:
            for qd in cs:
                wait(cs[qd])

    pl.run_scoped(front, pltpu.VMEM((D, 3 * D), bf16), pltpu.VMEM((3, D // 2, D), i32),
                  pltpu.VMEM((D, D), bf16))
    pl.run_scoped(back, pltpu.VMEM((49, Q // 2, KQ), i32))
    assert not sp.plan


_N_SEMS = 9


@jax.jit
def pallas_gated_mix__sliding_local_dilated__glu_gated_reglu__prompt_kernel(
    A_x: jax.Array,
    A_wqkv: jax.Array,
    A_wo: jax.Array,
    B_x: jax.Array,
    B_W_gate: jax.Array,
    B_W_up: jax.Array,
    B_W_down: jax.Array,
    gate_w: jax.Array,
):
    del B_x
    hbm = pl.BlockSpec(memory_space=pl.ANY)
    scratch = [
        pltpu.VMEM((S, D), bf16),
        pltpu.VMEM((S // 2, D), i32),
        pltpu.VMEM((5, H // 2, KH), i32),
        pltpu.VMEM((8, 128), bf16),
        pltpu.VMEM((NC, D, 2 * FC), bf16),
        pltpu.VMEM((NC, FC, D), bf16),
        pltpu.VMEM((49, Q, KQ), f32),
        pltpu.VMEM((8, S + QPAD, 128), f32),
        pltpu.VMEM((8, PAD + S, 128), f32),
        pltpu.VMEM((8, PAD + S, 128), f32),
        pltpu.VMEM((S, 128), f32),
        pltpu.VMEM((49, KQ // 2, KQ), i32),
        pltpu.VMEM((8, 128), i32),
        pltpu.SMEM((1,), i32),
        pltpu.SemaphoreType.DMA((_N_SEMS,)),
    ]
    return pl.pallas_call(
        _kernel,
        in_specs=[hbm] * 7,
        out_specs=hbm,
        out_shape=jax.ShapeDtypeStruct((1, S, D), bf16),
        scratch_shapes=scratch,
        compiler_params=pltpu.CompilerParams(vmem_limit_bytes=124 * 1024 * 1024),
    )(A_x, A_wqkv, A_wo, B_W_gate, B_W_up, B_W_down, gate_w.reshape(8, 128))
```

```python
import math

import jax
import jax.numpy as jnp
from jax import lax
import jax.experimental.pallas as pl
import jax.experimental.pallas.tpu as pltpu

f32 = jnp.float32
bf16 = jnp.bfloat16
i32 = jnp.int32

S = 2048
D = 1024
F = 3584
NH = 32
DH = D // NH
W = 8
DIL = 2
H = S // 2
Q = S // 4
KH = D // 2
KQ = D // 4
FC = 512
CH = FC // 2
CQ = FC // 4
NC = F // FC
RB = 256
NRB = H // RB
PB = 128
PAD = 16
TP = DH + 1
AR = 64
A0 = Q - 6 * AR
QA = 160
QPAD = 112

BC_SLOTS = (2, 24)
ATTN_SLOTS = (20, 96)
DC_SLOTS = (24, 96)
PACK_SLOTS = (96, 112)
VBC_SLOTS = (2, 16)
PREP01 = (16, 56)
PERMK = (64, 106)
WOS = (70, 112)
PACK4 = (4, 24)
NRAW = 3
DEPTH = 3
DEPTH2 = 3
H_DEPTH = 3

SCALE = DH ** -0.5
EXP2_SCALE = SCALE * math.log2(math.e)
NEG = -1e9 / SCALE


def _a_combos(a11, a12, a21, a22):
    return [a11 + a22, a21 + a22, a11, a22, a11 + a12, a21 - a11, a12 - a22]


def _b_combos(b11, b12, b21, b22):
    return [b11 + b22, b11, b12 - b22, b21 - b11, b22, b11 + b12, b21 + b22]


_C_TERMS = (((1, 0), (1, 3), (-1, 4), (1, 6)), ((1, 2), (1, 4)), ((1, 1), (1, 3)),
            ((1, 0), (-1, 1), (1, 2), (1, 5)))
_C_ORDER = (((2, 4), 1), ((1, 3), 2), ((0, 6), 0), ((5,), 3))


def _c_quadrant(m, qd):
    out = m[_C_TERMS[qd][0][1]]
    for sign, t in _C_TERMS[qd][1:]:
        out = out + m[t] if sign > 0 else out - m[t]
    return out


def _c_combos(m):
    return [_c_quadrant(m, qd) for qd in range(4)]


_A_SLOT = {0: 0, 1: 1, 4: 2, 5: 3, 6: 4}
_B_SUMS = (2, 3, 0, 5, 6)
ORDER = (1, 4) + _B_SUMS


def _tree(op, xs):
    xs = list(xs)
    while len(xs) > 1:
        xs = [op(xs[i], xs[i + 1]) if i + 1 < len(xs) else xs[i] for i in range(0, len(xs), 2)]
    return xs[0]


def _pack(x):
    return pltpu.bitcast(x.astype(bf16), i32)


def _unpack(x):
    return pltpu.bitcast(x, bf16)


def _half(r):
    return slice(r.start // 2, r.stop // 2)


SLOT = 256


class _Spreader:
    def __init__(self, zero_ref):
        self.zero_ref = zero_ref
        self.plan = {}
        self.lists = 0
        self.now = 0

    def block(self):
        self.zero = self.zero_ref[...]
        self.never = self.zero != 0

    def link(self, after, x):
        if after is None:
            return x
        if after.dtype != x.dtype:
            after = pltpu.bitcast(after, x.dtype)
        return jnp.where(self.never, after, x)

    def chain(self, vals, prev, depth):
        for v in vals:
            v = pltpu.bitcast(v, i32) if v.dtype != i32 else v
            for r in range(0, v.shape[0], 8):
                for c in range(0, v.shape[1], 128):
                    tile = v[r:r + 8, c:c + 128]
                    if prev is None:
                        prev = tile
                        continue
                    prev = prev | tile
                    for i in range(depth - 1):
                        prev = (prev + self.zero) if i % 2 == 0 else (prev ^ self.zero)
        return prev

    def link_rows(self, after, x):
        return jnp.concatenate([self.link(after, x[r:r + 8, :]) for r in range(0, x.shape[0], 8)],
                               axis=0)

    def serial_combos(self, combos, x11, x12, x21, x22, after):
        return combos(self.link_rows(after, x11), x12, x21, self.link_rows(after, x22))

    def two_level(self, combos, blk, prev, depth, after=None):
        outer = [self.serial_combos(
            combos, *[blk(r1, r2, c1, c2) for r1 in range(2) for c1 in range(2)], after)
            for r2 in range(2) for c2 in range(2)]
        outs, tok = [], None
        for t in range(7):
            wide = _pack(jnp.concatenate(
                self.serial_combos(combos, *[o[t] for o in outer], tok), axis=1))
            outs += [wide[:, c:c + 128] for c in range(0, 7 * 128, 128)]
            tok = self.chain(outs[-7:], tok, depth)
        return outs, self.chain([tok], prev, 1)

    def schedule(self, tasks, first, last):
        n = len(tasks)
        self.lists += 1
        for i, t in enumerate(tasks):
            pos = self.now + first + ((i + 1) * (last - first) - 1) // n
            self.plan.setdefault(pos, []).append((t, self.lists))

    def dots(self, pairs):
        m = pairs[0][0].shape[0]
        tiles = [(i, r, c) for i, (_, rhs) in enumerate(pairs)
                 for c in range(0, rhs.shape[1], 128) for r in range(0, rhs.shape[0], 128)]
        nslots = m * len(tiles) // (4 * SLOT)
        deps = {}
        for sl in range(nslots):
            ps = sl * SLOT // m
            toks = {}
            for t, lane in self.plan.pop(self.now + sl, []):
                tok = t(toks.get(lane))
                if tok is not None:
                    toks[lane] = tok
            for tok in toks.values():
                deps[ps] = tok | deps[ps] if ps in deps else tok
        self.now += nslots
        tied = {tile: d for ps, d in deps.items() for tile in tiles[4 * ps:4 * ps + 4]}
        outs = []
        for i, (lhs, rhs) in enumerate(pairs):
            if any(key[0] == i for key in tied):
                parts = []
                for r in range(0, rhs.shape[0], 128):
                    top = [rhs[r:r + 16, c:c + 128] for c in range(0, rhs.shape[1], 128)]
                    top = [_unpack(self.link(tied[i, r, c * 128], _pack(t0)))
                           if (i, r, c * 128) in tied else t0 for c, t0 in enumerate(top)]
                    parts += [jnp.concatenate(top, axis=1), rhs[r + 16:r + 128, :]]
                rhs = jnp.concatenate(parts, axis=0)
            outs.append(jnp.dot(lhs, rhs, preferred_element_type=f32))
        return outs

    def dot(self, lhs, rhs):
        return self.dots([(lhs, rhs)])[0]


def _kernel(x_hbm, wqkv_hbm, wo_hbm, wg_hbm, wu_hbm, wd_hbm, gw_hbm, out_hbm,
            x_vm, xn, xa, gw_vm, wgu, wd, acc, q_s, k_s, v_s, gs, woc, zs, zi, sems):
    def cp(src, dst, sem):
        return pltpu.make_async_copy(src, dst, sems.at[sem])

    def cp_gu(j, p, sem):
        return cp((wg_hbm, wu_hbm)[p % 2].at[:, pl.ds(j * FC + (p // 2) * CH, CH)],
                  wgu.at[j, :, pl.ds(p * CH, CH)], sem)

    def cp_d(j, sem):
        return cp(wd_hbm.at[pl.ds(j * FC, FC), :], wd.at[j], sem)

    def cp_x(rb, hf, sem):
        idx = (pl.ds(hf * H + rb * RB, RB), slice(None))
        return cp(x_hbm.at[0].at[idx], x_vm.at[idx], sem)

    o2 = out_hbm.at[0]
    in0 = [cp_x(0, 0, 0), cp_gu(0, 0, 0)]
    in1 = [cp_x(0, 1, 1)]
    in2 = [cp_gu(0, 1, 2)]
    in3 = [cp_gu(0, 2, 3), cp_gu(0, 3, 3), cp(gw_hbm, gw_vm, 3)]
    in4 = [cp_x(rb, hf, 4) for rb in (1, 2) for hf in range(2)]
    in5 = [cp_x(3, 0, 5), cp_x(3, 1, 5), cp_d(0, 5)]
    in_ffn = [c for j in range(1, NC) for c in [cp_gu(j, p, 7) for p in range(4)] + [cp_d(j, 7)]]
    out_sem = 8

    def start(cs):
        for c in cs:
            c.start()

    def wait(cs):
        for c in cs:
            c.wait()

    start(in0 + in1 + in2)

    zs[...] = jnp.zeros((8, 128), i32)
    zi[0] = 1
    sp = _Spreader(zs)

    def rows(rb, hf=0):
        return slice(hf * H + rb * RB, hf * H + (rb + 1) * RB)

    def x_lhs(t, rb):
        if t == 2:
            return _unpack(xn[_half(rows(rb, 0)), :KH])
        if t == 3:
            return _unpack(xn[_half(rows(rb, 1)), KH:])
        return _unpack(xa[_A_SLOT[t], _half(rows(rb)), :])

    def prep_tasks(rb, sums=True, gate=True):
        def task(s0):
            def run(first):
                prev = None
                gw = gw_vm[...].astype(f32)
                r = [slice(hf * H + rb * RB + s0, hf * H + rb * RB + s0 + 16) for hf in range(2)]
                z = [None, None]
                for c in range(4):
                    cols = [slice(kh * KH + c * 128, kh * KH + (c + 1) * 128) for kh in range(2)]
                    xs = [sp.link(prev, _pack(x_vm[r[qd // 2], cols[qd % 2]])) for qd in range(4)]
                    a = [_unpack(t).astype(f32) for t in xs]
                    outs = []
                    if sums:
                        for qd in range(4):
                            xn[_half(r[qd // 2]), cols[qd % 2]] = xs[qd]
                        cs = _a_combos(*a)
                        for t, slot in _A_SLOT.items():
                            outs.append(_pack(cs[t]))
                            xa[slot, _half(r[0]), cols[0]] = outs[-1]
                    if gate:
                        for qd in range(4):
                            g0 = (qd % 2) * 4 + c
                            term = a[qd] * gw[g0:g0 + 1, :]
                            z[qd // 2] = term if z[qd // 2] is None else z[qd // 2] + term
                        outs += z
                    prev = sp.chain(outs, prev, 1)
                if gate:
                    for hf in range(2):
                        g = jax.nn.sigmoid(jnp.sum(z[hf], axis=1, keepdims=True))
                        g = jnp.broadcast_to(g, (16, 128))
                        gs[r[hf], :] = g
                        prev = sp.chain([g], prev, 1)
                return sp.chain([prev], first, 1)
            return run
        return [task(s0) for s0 in range(0, RB, 16)]

    def b_sum_tasks(src, dst):
        def task(r0):
            def run(prev):
                raw = [src(slice(a * KH + r0, a * KH + r0 + 16), slice(c * KH, (c + 1) * KH))
                       for a in range(2) for c in range(2)]
                cs = _b_combos(*[b.astype(f32) for b in raw])
                for t in _B_SUMS:
                    dst.setdefault(t, []).append(_pack(cs[t]))
                return sp.chain([dst[t][-1] for t in _B_SUMS], prev, DEPTH)
            return run
        return [task(r0) for r0 in range(0, KH, 16)]

    def b_rhs(src, sums):
        def rhs(t):
            if t == 1:
                return src(slice(0, KH), slice(0, KH))
            if t == 4:
                return src(slice(KH, D), slice(KH, D))
            return _unpack(jnp.concatenate(sums[t], axis=0))
        return rhs

    def strassen_x(order, rhs, finish):
        m = {}
        for rb, t in order:
            m.setdefault(rb, {})[t] = sp.dot(x_lhs(t, rb), rhs(t))
            if len(m[rb]) == 7:
                finish(rb, m.pop(rb))

    def h_sums(rb, cs, r0, sub):
        h = []
        for qd, cc in enumerate(cs):
            g0 = (qd // 2) * H + rb * RB + r0
            omg = 1.0 - gs[g0:g0 + sub, :]
            omg = jnp.concatenate([omg] * (CH // 128), axis=1)
            h.append(jnp.maximum(cc[:, :CH], 0.0) * cc[:, CH:] * omg)
        return _a_combos(*h)

    def glu_tasks(hs, rb, cs, sub):
        hs[rb] = [[] for _ in range(7)]

        def task(r0):
            def run(prev):
                sums = h_sums(rb, [cc[r0:r0 + sub] for cc in cs], r0, sub)
                for t in range(7):
                    hs[rb][t].append(sums[t])
                if sub < RB:
                    return sp.chain([sums[t] for t in _A_SLOT], prev, DEPTH2)
            return run
        return [task(r0) for r0 in range(0, RB, sub)]

    def down_lhs(hs, b, ha):
        tok = None
        for t in range(7):
            s0, s1 = [jnp.concatenate(hs[rb][t], axis=0) for rb in (b, b + 2)]
            slabs = []
            for r in range(0, RB, 16):
                slabs.append(sp.serial_combos(
                    _a_combos, s0[r:r + 16, :CQ], s0[r:r + 16, CQ:],
                    s1[r:r + 16, :CQ], s1[r:r + 16, CQ:], tok))
                tok = sp.chain([slabs[-1][t2] for t2 in _A_SLOT], None, H_DEPTH)
            for t2 in range(7):
                ha[b, 7 * t + t2] = jnp.concatenate([sl[t2] for sl in slabs], axis=0).astype(bf16)

    def d_tasks(j, dst):
        def task(r0, c):
            def run(prev):
                def blk(k1, k2, n1, n2):
                    r, c0 = k1 * CH + k2 * CQ + r0, n1 * KH + n2 * KQ + c * 128
                    return wd[j, r:r + 16, c0:c0 + 128].astype(f32)
                cs, tok = sp.two_level(_b_combos, blk, prev, DEPTH2)
                for t in range(49):
                    dst.setdefault((t, c), []).append(cs[t])
                return tok
            return run
        return [task(r0, c) for r0 in range(0, CQ, 16) for c in range(2)]

    def ffn_down(ha, dc, first):
        rhs = [_unpack(jnp.concatenate([jnp.concatenate(dc[t, c], axis=0) for c in range(2)], axis=1))
               for t in range(49)]
        todo = [(b, t) for b in range(2) for t in range(49)]
        for i in range(0, len(todo), 2):
            pair = todo[i:i + 2]
            ps = sp.dots([(ha[b, t], rhs[t]) for b, t in pair])
            for (b, t), p in zip(pair, ps):
                if first:
                    acc[t, b * RB:(b + 1) * RB, :] = p
                else:
                    acc[t, b * RB:(b + 1) * RB, :] += p

    def perm_tasks(wqkv_vm, wp, i, tbuf):
        def fwd(rb, c):
            def run(prev):
                c0 = i * D + c * 128
                tt = pltpu.bitcast(wqkv_vm[rb * 256:(rb + 1) * 256, c0:c0 + 128], f32).T
                for hh in range(4):
                    tbuf[rb, pl.ds((4 * c + hh) * TP, DH), :] = tt[hh * DH:(hh + 1) * DH, :]
                return sp.chain([tt], prev, 1)
            return run

        def bwd(rb, j):
            def run(prev):
                g = jnp.concatenate(
                    [tbuf[rb, pl.ds(4 * j + dd, NH, stride=TP), :] for dd in range(4)], axis=0).T
                wp[i, rb * 128:(rb + 1) * 128, j * 128:(j + 1) * 128] = pltpu.bitcast(g, i32)
            return run
        tasks = []
        for rb in range(4):
            tasks += [fwd(rb, c) for c in range(8)] + [bwd(rb, j) for j in range(8)]
        return tasks

    def wo_tasks(wo_vm):
        def stage(c):
            return 4 + c % 4, (c // 4) * NH * TP

        def spread(h0):
            def run(prev):
                blk = wo_vm[h0 * DH:(h0 + 2) * DH, :].astype(f32)
                for h in range(2):
                    for c in range(8):
                        sl, r0 = stage(c)
                        q_s[sl, pl.ds(r0 + (h0 + h) * TP, DH), :] = (
                            blk[h * DH:(h + 1) * DH, c * 128:(c + 1) * 128])
                return sp.chain([blk], prev, 1)
            return run

        def gather(d, h0, c):
            def run(after):
                def blk(k1, k2, n1, n2):
                    sl, r0 = stage(4 * n1 + 2 * n2 + c)
                    r0 += h0 * TP + 16 * k1 + 8 * k2 + d
                    return q_s[sl, pl.ds(r0, 16, stride=TP), :]
                cs, tok = sp.two_level(_b_combos, blk, None, DEPTH2, after)
                r = (d * NH + h0) // 2
                for t in range(49):
                    woc[t, r:r + 8, c * 128:(c + 1) * 128] = cs[t]
                return tok
            return run
        return ([spread(h0) for h0 in range(0, NH, 2)],
                [gather(d, h0, c) for d in range(8) for h0 in (0, 16) for c in range(2)])

    def proj(wp, i, dst, pad, slabs):
        lhs = jnp.concatenate([xn[r0 // 2:(r0 + n) // 2, :] for r0, n in slabs], axis=0)
        p = sp.dot(_unpack(lhs), _unpack(wp[i]))
        at = 0
        for r0, n in slabs:
            for j in range(8):
                dst[j, pad + r0:pad + r0 + n, :] = p[at:at + n, j * 128:(j + 1) * 128]
            at += n

    def v_finish(rb, m):
        cs = _c_combos(m)
        for qd, cc in enumerate(cs):
            r0 = PAD + (qd // 2) * H + rb * RB
            for j in range(4):
                v_s[(qd % 2) * 4 + j, r0:r0 + RB, :] = cc[:, j * 128:(j + 1) * 128]
        if rb == 0:
            for j in range(8):
                src = cs[j // 4][0:1, (j % 4) * 128:(j % 4 + 1) * 128]
                v_s[j, 0:PAD, :] = jnp.broadcast_to(src, (PAD, 128))

    def attn_group(row, masked):
        def run(prev):
            g = 8
            q = [q_s[j, pl.ds(row, g), :] for j in range(8)]
            ls = []
            for w in range(W):
                a = None
                for j in range(8):
                    term = q[j] * k_s[j, pl.ds(row + (PAD - DIL * w), g), :]
                    a = sp.link(ls[-1] if ls else None, term) if a is None else a + term
                ls.append(a)
            rs = [pltpu.roll(a, 64, 1) for a in ls]
            ls = [a + r for a, r in zip(ls, rs)]
            rs = [pltpu.roll(a, 32, 1) for a in ls]
            ls = [a + r for a, r in zip(ls, rs)]
            if masked:
                ri = row + lax.broadcasted_iota(i32, (g, 128), 0)
                ls = [ls[0]] + [jnp.where(ri >= DIL * w, ls[w], NEG) for w in range(1, W)]
            m = _tree(jnp.maximum, ls)
            ps = [jnp.exp2((l - m) * EXP2_SCALE) for l in ls]
            r = gs[pl.ds(row, g), :] / _tree(jnp.add, ps)
            outs = []
            for j in range(8):
                a = None
                for w in range(W):
                    term = ps[w] * v_s[j, pl.ds(row + (PAD - DIL * w), g), :]
                    a = sp.link(outs[-1] if outs else None, term) if a is None else a + term
                outs.append(a * r)
            for j in range(8):
                q_s[j, pl.ds(row, g), :] = outs[j]
            return sp.chain([outs[-1]], prev, 1)
        return run

    def attn_tasks(base, nrows, first=False):
        return [attn_group(base + (qq * Q + r), first and qq == 0 and r < PAD)
                for r in range(0, nrows, 8) for qq in range(4)]

    def pack_tasks(oa, base, hbase, nrows):
        def task(r, c):
            def run(prev):
                def blk(i1, i2, k1, k2):
                    return q_s[4 * k1 + 2 * k2 + c, pl.ds(base + (i1 * H + i2 * Q + r), 16), :]
                cs, tok = sp.two_level(_a_combos, blk, prev, DEPTH2)
                for t in range(49):
                    oa[t, pl.ds(hbase + r // 2, 8), c * 128:(c + 1) * 128] = cs[t]
                return tok
            return run
        return [task(r, c) for r in range(0, nrows, 16) for c in range(2)]

    GS = RB * (KH // 128) * (FC // 128) * 7 // (4 * SLOT)
    DS = 49
    PS = 2 * RB * (D // 128) * (D // 128) // (4 * SLOT)

    def glu(hs, ha):
        def finish(rb, m):
            glu_tasks(hs, rb, _c_combos(m), RB)[0](None)
            if rb >= 2:
                down_lhs(hs, rb - 2, ha)
        return finish

    def raw_first(rbs, n):
        lead = [(rb, t) for rb in rbs[:n] for t in ORDER[:2]]
        return lead + [(rb, t) for rb in rbs for t in ORDER if (rb, t) not in lead]

    def gu_src(j):
        return lambda r, c: wgu[j, r, c]

    def front(wqkv_vm, wp, wo_vm):
        in_q, in_k, in_v = [
            cp(wqkv_hbm.at[:, pl.ds(i * D, D)], wqkv_vm.at[:, pl.ds(i * D, D)], (6, 6, 5)[i])
            for i in range(3)]
        in_wo = cp(wo_hbm, wo_vm, 6)

        def plain(rb, hf, p):
            return sp.dot(x_vm[rows(rb, hf), :], wgu[0, :, p * CH:(p + 1) * CH])

        def plain_finish(rb, c):
            cs = [jnp.concatenate(c[2 * qd:2 * qd + 2], axis=1) for qd in range(4)]
            return glu_tasks(hs, rb, cs, 16)

        hs, bc, dc = {}, {}, {}
        wait(in0)
        start(in3)
        c0 = {(0, 0): plain(0, 0, 0)}
        wait(in1)
        c0[1, 0] = plain(0, 1, 0)
        wait(in2)
        start(in4)
        for hf in range(2):
            c0[hf, 1] = plain(0, hf, 1)
        wait(in3)
        start(in5)
        sp.block()
        bt = b_sum_tasks(gu_src(0), bc)
        sp.schedule(bt[:12], 3, 16)
        sp.schedule(prep_tasks(0, sums=False), 3, 16)
        for p in (2, 3):
            for hf in range(2):
                c0[hf, p] = plain(0, hf, p)
        c0 = [c0[hf, p] for hf in range(2) for p in range(4)]
        wait(in4)
        start([in_v])
        sp.block()
        sp.schedule(bt[12:], 3, 32)
        sp.schedule(prep_tasks(1, sums=False), 2, 10)
        sp.schedule(prep_tasks(2), 10, 32)
        c1 = [plain(1, hf, p) for hf in range(2) for p in range(4)]
        wait(in5 + [in_v])
        start([in_k, in_wo, in_q])
        sp.block()
        for j in range(8):
            k_s[j, 0:PAD, :] = jnp.zeros((PAD, 128), f32)
        ha = {}
        sp.schedule(prep_tasks(3), 2, GS)
        sp.schedule(plain_finish(0, c0), 2, GS)
        sp.schedule(plain_finish(1, c1), GS + 6, 2 * GS)
        sp.schedule(d_tasks(0, dc), GS - 2, 2 * GS)
        sp.schedule(perm_tasks(wqkv_vm, wp, 2, q_s), 2 * GS + 6, 2 * GS + DS - 8)
        strassen_x([(rb, t) for rb in (2, 3) for t in ORDER], b_rhs(gu_src(0), bc),
                   glu(hs, ha))
        ffn_down(ha, dc, True)

        wait([in_k, in_wo, in_q])
        start(in_ffn)
        sp.block()
        vb = {}
        v_src = lambda r, c: _unpack(wp[2, _half(r), c])
        wo_spread, wo_gather = wo_tasks(wo_vm)
        sp.schedule(b_sum_tasks(v_src, vb), *VBC_SLOTS)
        sp.schedule(prep_tasks(0, gate=False) + prep_tasks(1, gate=False), *PREP01)
        sp.schedule(perm_tasks(wqkv_vm, wp, 1, k_s.at[:, PAD:, :]), *PERMK)
        sp.schedule(wo_spread, *WOS)
        strassen_x(raw_first((2, 3, 0, 1), 2), b_rhs(v_src, vb), v_finish)
        sp.schedule(perm_tasks(wqkv_vm, wp, 0, q_s), 4, 3 * PS)
        tok = None
        for t in wo_gather:
            tok = t(tok)
        for rb in range(NRB):
            proj(wp, 1, k_s, PAD, [(rb * Q, Q)])
        proj(wp, 0, q_s, 0, [(qq * Q, QA) for qq in range(4)])

        def q_rest(_, carry):
            sp.block()
            n = (Q - QA) // 2
            total = 4 * (Q - QA) * 64 // (4 * SLOT)
            sp.schedule(attn_tasks(0, A0, True), 4, total)
            for r0 in (QA, QA + n):
                proj(wp, 0, q_s, 0, [(qq * Q + r0, n) for qq in range(4)])
            return carry

        lax.fori_loop(0, zi[0], q_rest, 0)
        wait(in_ffn)

    def back(oa):
        def body(j, carry):
            sp.block()
            base = pl.multiple_of((j - 1) * AR, AR)
            hs, ha, bc, dc = {}, {}, {}, {}
            sp.schedule(b_sum_tasks(gu_src(j), bc), *BC_SLOTS)
            sp.schedule(attn_tasks(base + A0, AR), *ATTN_SLOTS)
            sp.schedule(pack_tasks(oa, base, pl.multiple_of((j - 1) * (AR // 2), AR // 2), AR),
                        *PACK_SLOTS)
            sp.schedule(d_tasks(j, dc), *DC_SLOTS)
            strassen_x(raw_first((0, 2, 1, 3), NRAW), b_rhs(gu_src(j), bc), glu(hs, ha))
            ffn_down(ha, dc, False)
            return carry

        lax.fori_loop(1, NC, body, 0)

        def out_copy(r0, i1, i2, cols):
            idx = (pl.ds(r0 + (i1 * H + i2 * Q), PB), cols)
            return cp(x_vm.at[idx], o2.at[idx], out_sem)

        def out_blocks(blocks):
            done_by = {ts[-1]: qd for ts, qd in _C_ORDER}
            todo = [(blk, t1, t2) for blk in range(len(blocks))
                    for ts1, _ in _C_ORDER for t1 in ts1 for ts2, _ in _C_ORDER for t2 in ts2]
            m, inner = {}, {}
            for i in range(0, len(todo), 2):
                pair = todo[i:i + 2]
                ps = sp.dots([(_unpack(oa[7 * t1 + t2, pl.ds(blocks[blk][1], PB // 2), :]),
                               _unpack(woc[7 * t1 + t2])) for blk, t1, t2 in pair])
                for (blk, t1, t2), p in zip(pair, ps):
                    r0, _, copies = blocks[blk]
                    m.setdefault((blk, t1), {})[t2] = acc[7 * t1 + t2, pl.ds(r0, PB), :] + p
                    if t2 not in done_by:
                        continue
                    q2 = done_by[t2]
                    inner.setdefault((blk, q2), {})[t1] = _c_quadrant(m[blk, t1], q2)
                    if t1 not in done_by:
                        continue
                    q1 = done_by[t1]
                    r = pl.ds(r0 + ((q1 // 2) * H + (q2 // 2) * Q), PB)
                    c = (q1 % 2) * KH + (q2 % 2) * KQ
                    x_vm[r, c:c + KQ] = _c_quadrant(inner[blk, q2], q1).astype(bf16)
                    start(copies.get((q1, q2), []))

        def whole(r0):
            return {(3, 3): [out_copy(r0, i1, i2, slice(None)) for i1 in range(2) for i2 in range(2)]}

        done = (NC - 1) * AR

        def out_body(i, carry):
            sp.block()
            half = pl.multiple_of(done // 2 + i * 24, 8)
            sp.schedule(pack_tasks(oa, 2 * half, half, 48), *PACK4)
            r0 = pl.multiple_of(i * PB, PB)
            out_blocks([(r0, pl.multiple_of(i * (PB // 2), PB // 2),
                         whole(r0))])
            return carry

        lax.fori_loop(0, 2, out_body, 0)
        sp.block()
        sp.schedule(pack_tasks(oa, done + 96, (done + 96) // 2, Q - done - 96), 4, 22)
        last = {(q1, 3): [out_copy(3 * PB, q1 // 2, i2, pl.ds((q1 % 2) * KH, KH))
                          for i2 in range(2)] for q1 in range(3)}
        for q2 in range(4):
            last[3, q2] = [out_copy(3 * PB, 1, q2 // 2, pl.ds(KH + (q2 % 2) * KQ, KQ))]
        copies = [whole(blk * PB) for blk in range(3)] + [last]
        out_blocks([(blk * PB, blk * PB // 2, copies[blk]) for blk in (2, 3)])
        for cs in copies:
            for key in cs:
                wait(cs[key])

    pl.run_scoped(front, pltpu.VMEM((D, 3 * D), bf16), pltpu.VMEM((3, D // 2, D), i32),
                  pltpu.VMEM((D, D), bf16))
    pl.run_scoped(back, pltpu.VMEM((49, Q // 2, KQ), i32))
    assert not sp.plan


_N_SEMS = 9


@jax.jit
def pallas_gated_mix__sliding_local_dilated__glu_gated_reglu__prompt_kernel(
    A_x: jax.Array,
    A_wqkv: jax.Array,
    A_wo: jax.Array,
    B_x: jax.Array,
    B_W_gate: jax.Array,
    B_W_up: jax.Array,
    B_W_down: jax.Array,
    gate_w: jax.Array,
):
    del B_x
    hbm = pl.BlockSpec(memory_space=pl.ANY)
    scratch = [
        pltpu.VMEM((S, D), bf16),
        pltpu.VMEM((S // 2, D), i32),
        pltpu.VMEM((5, H // 2, KH), i32),
        pltpu.VMEM((8, 128), bf16),
        pltpu.VMEM((NC, D, 2 * FC), bf16),
        pltpu.VMEM((NC, FC, D), bf16),
        pltpu.VMEM((49, Q, KQ), f32),
        pltpu.VMEM((8, S + QPAD, 128), f32),
        pltpu.VMEM((8, PAD + S, 128), f32),
        pltpu.VMEM((8, PAD + S, 128), f32),
        pltpu.VMEM((S, 128), f32),
        pltpu.VMEM((49, KQ // 2, KQ), i32),
        pltpu.VMEM((8, 128), i32),
        pltpu.SMEM((1,), i32),
        pltpu.SemaphoreType.DMA((_N_SEMS,)),
    ]
    return pl.pallas_call(
        _kernel,
        in_specs=[hbm] * 7,
        out_specs=hbm,
        out_shape=jax.ShapeDtypeStruct((1, S, D), bf16),
        scratch_shapes=scratch,
        compiler_params=pltpu.CompilerParams(vmem_limit_bytes=124 * 1024 * 1024),
    )(A_x, A_wqkv, A_wo, B_W_gate, B_W_up, B_W_down, gate_w.reshape(8, 128))
```

```python
import math

import jax
import jax.numpy as jnp
from jax import lax
import jax.experimental.pallas as pl
import jax.experimental.pallas.tpu as pltpu

f32 = jnp.float32
bf16 = jnp.bfloat16
i32 = jnp.int32

S = 2048
D = 1024
F = 3584
NH = 32
DH = D // NH
W = 8
DIL = 2
H = S // 2
Q = S // 4
KH = D // 2
KQ = D // 4
FC = 512
CH = FC // 2
CQ = FC // 4
NC = F // FC
RB = 256
NRB = H // RB
PB = 128
PAD = 16
TP = DH + 1
AR = 64
A0 = Q - 6 * AR
QA = 160
QPAD = 112

BC_SLOTS = (2, 24)
ATTN_SLOTS = (22, 92)
DC_SLOTS = (26, 90)
PACK_SLOTS = (92, 112)
VDEPTH = 2
VBC_SLOTS = (2, 16)
PREP01 = (16, 56)
PERMK = (64, 106)
WOS = (70, 112)
PACK4 = (4, 24)
NRAW = 3
DEPTH = 3
DEPTH2 = 3
H_DEPTH = 3

SCALE = DH ** -0.5
EXP2_SCALE = SCALE * math.log2(math.e)
NEG = -1e9 / SCALE


def _a_combos(a11, a12, a21, a22):
    return [a11 + a22, a21 + a22, a11, a22, a11 + a12, a21 - a11, a12 - a22]


def _b_combos(b11, b12, b21, b22):
    return [b11 + b22, b11, b12 - b22, b21 - b11, b22, b11 + b12, b21 + b22]


_C_TERMS = (((1, 0), (1, 3), (-1, 4), (1, 6)), ((1, 2), (1, 4)), ((1, 1), (1, 3)),
            ((1, 0), (-1, 1), (1, 2), (1, 5)))
_C_ORDER = (((2, 4), 1), ((1, 3), 2), ((0, 6), 0), ((5,), 3))


def _c_quadrant(m, qd):
    out = m[_C_TERMS[qd][0][1]]
    for sign, t in _C_TERMS[qd][1:]:
        out = out + m[t] if sign > 0 else out - m[t]
    return out


def _c_combos(m):
    return [_c_quadrant(m, qd) for qd in range(4)]


_A_SLOT = {0: 0, 1: 1, 4: 2, 5: 3, 6: 4}
_B_SUMS = (2, 3, 0, 5, 6)
ORDER = (1, 4) + _B_SUMS


def _tree(op, xs):
    xs = list(xs)
    while len(xs) > 1:
        xs = [op(xs[i], xs[i + 1]) if i + 1 < len(xs) else xs[i] for i in range(0, len(xs), 2)]
    return xs[0]


def _pack(x):
    return pltpu.bitcast(x.astype(bf16), i32)


def _unpack(x):
    return pltpu.bitcast(x, bf16)


def _half(r):
    return slice(r.start // 2, r.stop // 2)


SLOT = 256


class _Spreader:
    def __init__(self, zero_ref):
        self.zero_ref = zero_ref
        self.plan = {}
        self.lists = 0
        self.now = 0

    def block(self):
        self.zero = self.zero_ref[...]
        self.never = self.zero != 0

    def link(self, after, x):
        if after is None:
            return x
        if after.dtype != x.dtype:
            after = pltpu.bitcast(after, x.dtype)
        return jnp.where(self.never, after, x)

    def chain(self, vals, prev, depth):
        for v in vals:
            v = pltpu.bitcast(v, i32) if v.dtype != i32 else v
            for r in range(0, v.shape[0], 8):
                for c in range(0, v.shape[1], 128):
                    tile = v[r:r + 8, c:c + 128]
                    if prev is None:
                        prev = tile
                        continue
                    prev = prev | tile
                    for i in range(depth - 1):
                        prev = (prev + self.zero) if i % 2 == 0 else (prev ^ self.zero)
        return prev

    def link_rows(self, after, x):
        return jnp.concatenate([self.link(after, x[r:r + 8, :]) for r in range(0, x.shape[0], 8)],
                               axis=0)

    def serial_combos(self, combos, x11, x12, x21, x22, after):
        return combos(self.link_rows(after, x11), x12, x21, self.link_rows(after, x22))

    def two_level(self, combos, blk, prev, depth, after=None):
        outer = [self.serial_combos(
            combos, *[blk(r1, r2, c1, c2) for r1 in range(2) for c1 in range(2)], after)
            for r2 in range(2) for c2 in range(2)]
        outs, tok = [], None
        for t in range(7):
            wide = _pack(jnp.concatenate(
                self.serial_combos(combos, *[o[t] for o in outer], tok), axis=1))
            outs += [wide[:, c:c + 128] for c in range(0, 7 * 128, 128)]
            tok = self.chain(outs[-7:], tok, depth)
        return outs, self.chain([tok], prev, 1)

    def schedule(self, tasks, first, last):
        self.lists += 1
        for i, t in enumerate(tasks):
            pos = self.now + first + ((i + 1) * (last - first) - 1) // len(tasks)
            self.plan.setdefault(pos, []).append((t, self.lists))

    def dots(self, pairs):
        m = pairs[0][0].shape[0]
        tiles = [(i, r, c) for i, (_, rhs) in enumerate(pairs)
                 for c in range(0, rhs.shape[1], 128) for r in range(0, rhs.shape[0], 128)]
        nslots = m * len(tiles) // (4 * SLOT)
        deps = {}
        for sl in range(nslots):
            ps = sl * SLOT // m
            toks = {}
            for t, lane in self.plan.pop(self.now + sl, []):
                tok = t(toks.get(lane))
                if tok is not None:
                    toks[lane] = tok
            for tok in toks.values():
                deps[ps] = tok | deps[ps] if ps in deps else tok
        self.now += nslots
        tied = {tile: d for ps, d in deps.items() for tile in tiles[4 * ps:4 * ps + 4]}
        outs = []
        for i, (lhs, rhs) in enumerate(pairs):
            if any(key[0] == i for key in tied):
                parts = []
                for r in range(0, rhs.shape[0], 128):
                    top = [rhs[r:r + 16, c:c + 128] for c in range(0, rhs.shape[1], 128)]
                    top = [_unpack(self.link(tied[i, r, c * 128], _pack(t0)))
                           if (i, r, c * 128) in tied else t0 for c, t0 in enumerate(top)]
                    parts += [jnp.concatenate(top, axis=1), rhs[r + 16:r + 128, :]]
                rhs = jnp.concatenate(parts, axis=0)
            outs.append(jnp.dot(lhs, rhs, preferred_element_type=f32))
        return outs

    def dot(self, lhs, rhs):
        return self.dots([(lhs, rhs)])[0]


def _kernel(x_hbm, wqkv_hbm, wo_hbm, wg_hbm, wu_hbm, wd_hbm, gw_hbm, out_hbm,
            x_vm, xn, xa, gw_vm, wgu, wd, acc, q_s, k_s, v_s, gs, woc, zs, zi, sems):
    def cp(src, dst, sem):
        return pltpu.make_async_copy(src, dst, sems.at[sem])

    def cp_gu(j, p, sem):
        return cp((wg_hbm, wu_hbm)[p % 2].at[:, pl.ds(j * FC + (p // 2) * CH, CH)],
                  wgu.at[j, :, pl.ds(p * CH, CH)], sem)

    def cp_d(j, sem):
        return cp(wd_hbm.at[pl.ds(j * FC, FC), :], wd.at[j], sem)

    def cp_x(rb, hf, sem):
        idx = (pl.ds(hf * H + rb * RB, RB), slice(None))
        return cp(x_hbm.at[0].at[idx], x_vm.at[idx], sem)

    o2 = out_hbm.at[0]
    in0 = [cp_x(0, 0, 0), cp_gu(0, 0, 0)]
    in1 = [cp_x(0, 1, 1)]
    in2 = [cp_gu(0, 1, 2)]
    in3 = [cp_gu(0, 2, 3), cp_gu(0, 3, 3), cp(gw_hbm, gw_vm, 3)]
    in4 = [cp_x(rb, hf, 4) for rb in (1, 2) for hf in range(2)]
    in5 = [cp_x(3, 0, 5), cp_x(3, 1, 5), cp_d(0, 5)]
    in_ffn = [c for j in range(1, NC) for c in [cp_gu(j, p, 7) for p in range(4)] + [cp_d(j, 7)]]
    out_sem = 8

    def start(cs):
        for c in cs:
            c.start()

    def wait(cs):
        for c in cs:
            c.wait()

    start(in0 + in1 + in2)

    zs[...] = jnp.zeros((8, 128), i32)
    zi[0] = 1
    sp = _Spreader(zs)

    def rows(rb, hf=0):
        return slice(hf * H + rb * RB, hf * H + (rb + 1) * RB)

    def x_lhs(t, rb):
        if t == 2:
            return _unpack(xn[_half(rows(rb, 0)), :KH])
        if t == 3:
            return _unpack(xn[_half(rows(rb, 1)), KH:])
        return _unpack(xa[_A_SLOT[t], _half(rows(rb)), :])

    def prep_tasks(rb, sums=True, gate=True):
        def task(s0):
            def run(first):
                prev = None
                gw = gw_vm[...].astype(f32)
                r = [slice(hf * H + rb * RB + s0, hf * H + rb * RB + s0 + 16) for hf in range(2)]
                z = [None, None]
                for c in range(4):
                    cols = [slice(kh * KH + c * 128, kh * KH + (c + 1) * 128) for kh in range(2)]
                    xs = [sp.link(prev, _pack(x_vm[r[qd // 2], cols[qd % 2]])) for qd in range(4)]
                    a = [_unpack(t).astype(f32) for t in xs]
                    outs = []
                    if sums:
                        for qd in range(4):
                            xn[_half(r[qd // 2]), cols[qd % 2]] = xs[qd]
                        cs = _a_combos(*a)
                        for t, slot in _A_SLOT.items():
                            outs.append(_pack(cs[t]))
                            xa[slot, _half(r[0]), cols[0]] = outs[-1]
                    if gate:
                        for qd in range(4):
                            g0 = (qd % 2) * 4 + c
                            term = a[qd] * gw[g0:g0 + 1, :]
                            z[qd // 2] = term if z[qd // 2] is None else z[qd // 2] + term
                        outs += z
                    prev = sp.chain(outs, prev, 1)
                if gate:
                    for hf in range(2):
                        g = jax.nn.sigmoid(jnp.sum(z[hf], axis=1, keepdims=True))
                        g = jnp.broadcast_to(g, (16, 128))
                        gs[r[hf], :] = g
                        prev = sp.chain([g], prev, 1)
                return sp.chain([prev], first, 1)
            return run
        return [task(s0) for s0 in range(0, RB, 16)]

    def b_sum_tasks(src, dst, depth=DEPTH):
        def task(r0):
            def run(prev):
                raw = [src(slice(a * KH + r0, a * KH + r0 + 16), slice(c * KH, (c + 1) * KH))
                       for a in range(2) for c in range(2)]
                cs = _b_combos(*[b.astype(f32) for b in raw])
                for t in _B_SUMS:
                    dst.setdefault(t, []).append(_pack(cs[t]))
                return sp.chain([dst[t][-1] for t in _B_SUMS], prev, depth)
            return run
        return [task(r0) for r0 in range(0, KH, 16)]

    def b_rhs(src, sums):
        def rhs(t):
            if t == 1:
                return src(slice(0, KH), slice(0, KH))
            if t == 4:
                return src(slice(KH, D), slice(KH, D))
            return _unpack(jnp.concatenate(sums[t], axis=0))
        return rhs

    def strassen_x(order, rhs, finish):
        m = {}
        for rb, t in order:
            m.setdefault(rb, {})[t] = sp.dot(x_lhs(t, rb), rhs(t))
            if len(m[rb]) == 7:
                finish(rb, m.pop(rb))

    def h_sums(rb, cs, r0, sub):
        h = []
        for qd, cc in enumerate(cs):
            g0 = (qd // 2) * H + rb * RB + r0
            omg = 1.0 - gs[g0:g0 + sub, :]
            omg = jnp.concatenate([omg] * (CH // 128), axis=1)
            h.append(jnp.maximum(cc[:, :CH], 0.0) * cc[:, CH:] * omg)
        return _a_combos(*h)

    def glu_tasks(hs, rb, cs, sub):
        hs[rb] = [[] for _ in range(7)]

        def task(r0):
            def run(prev):
                sums = h_sums(rb, [cc[r0:r0 + sub] for cc in cs], r0, sub)
                for t in range(7):
                    hs[rb][t].append(sums[t])
                if sub < RB:
                    return sp.chain([sums[t] for t in _A_SLOT], prev, DEPTH2)
            return run
        return [task(r0) for r0 in range(0, RB, sub)]

    def down_lhs(hs, b, ha):
        tok = None
        for t in range(7):
            s0, s1 = [jnp.concatenate(hs[rb][t], axis=0) for rb in (b, b + 2)]
            slabs = []
            for r in range(0, RB, 16):
                slabs.append(sp.serial_combos(
                    _a_combos, s0[r:r + 16, :CQ], s0[r:r + 16, CQ:],
                    s1[r:r + 16, :CQ], s1[r:r + 16, CQ:], tok))
                tok = sp.chain([slabs[-1][t2] for t2 in _A_SLOT], None, H_DEPTH)
            for t2 in range(7):
                ha[b, 7 * t + t2] = jnp.concatenate([sl[t2] for sl in slabs], axis=0).astype(bf16)

    def d_tasks(j, dst):
        def task(r0, c):
            def run(prev):
                def blk(k1, k2, n1, n2):
                    r, c0 = k1 * CH + k2 * CQ + r0, n1 * KH + n2 * KQ + c * 128
                    return wd[j, r:r + 16, c0:c0 + 128].astype(f32)
                cs, tok = sp.two_level(_b_combos, blk, prev, DEPTH2)
                for t in range(49):
                    dst.setdefault((t, c), []).append(cs[t])
                return tok
            return run
        return [task(r0, c) for r0 in range(0, CQ, 16) for c in range(2)]

    def ffn_down(ha, dc, first):
        rhs = [_unpack(jnp.concatenate([jnp.concatenate(dc[t, c], axis=0) for c in range(2)], axis=1))
               for t in range(49)]
        todo = [(b, t) for b in range(2) for t in range(49)]
        for i in range(0, len(todo), 2):
            pair = todo[i:i + 2]
            ps = sp.dots([(ha[b, t], rhs[t]) for b, t in pair])
            for (b, t), p in zip(pair, ps):
                if first:
                    acc[t, b * RB:(b + 1) * RB, :] = p
                else:
                    acc[t, b * RB:(b + 1) * RB, :] += p

    def perm_tasks(wqkv_vm, wp, i, tbuf):
        def fwd(rb, c):
            def run(prev):
                c0 = i * D + c * 128
                tt = pltpu.bitcast(wqkv_vm[rb * 256:(rb + 1) * 256, c0:c0 + 128], f32).T
                for hh in range(4):
                    tbuf[rb, pl.ds((4 * c + hh) * TP, DH), :] = tt[hh * DH:(hh + 1) * DH, :]
                return sp.chain([tt], prev, 1)
            return run

        def bwd(rb, j):
            def run(prev):
                g = jnp.concatenate(
                    [tbuf[rb, pl.ds(4 * j + dd, NH, stride=TP), :] for dd in range(4)], axis=0).T
                wp[i, rb * 128:(rb + 1) * 128, j * 128:(j + 1) * 128] = pltpu.bitcast(g, i32)
            return run
        tasks = []
        for rb in range(4):
            tasks += [fwd(rb, c) for c in range(8)] + [bwd(rb, j) for j in range(8)]
        return tasks

    def wo_tasks(wo_vm):
        def stage(c):
            return 4 + c % 4, (c // 4) * NH * TP

        def spread(h0):
            def run(prev):
                blk = wo_vm[h0 * DH:(h0 + 2) * DH, :].astype(f32)
                for h in range(2):
                    for c in range(8):
                        sl, r0 = stage(c)
                        q_s[sl, pl.ds(r0 + (h0 + h) * TP, DH), :] = (
                            blk[h * DH:(h + 1) * DH, c * 128:(c + 1) * 128])
                return sp.chain([blk], prev, 1)
            return run

        def gather(d, h0, c):
            def run(after):
                def blk(k1, k2, n1, n2):
                    sl, r0 = stage(4 * n1 + 2 * n2 + c)
                    r0 += h0 * TP + 16 * k1 + 8 * k2 + d
                    return q_s[sl, pl.ds(r0, 16, stride=TP), :]
                cs, tok = sp.two_level(_b_combos, blk, None, DEPTH2, after)
                r = (d * NH + h0) // 2
                for t in range(49):
                    woc[t, r:r + 8, c * 128:(c + 1) * 128] = cs[t]
                return tok
            return run
        return ([spread(h0) for h0 in range(0, NH, 2)],
                [gather(d, h0, c) for d in range(8) for h0 in (0, 16) for c in range(2)])

    def proj(wp, i, dst, pad, slabs):
        lhs = jnp.concatenate([xn[r0 // 2:(r0 + n) // 2, :] for r0, n in slabs], axis=0)
        p = sp.dot(_unpack(lhs), _unpack(wp[i]))
        at = 0
        for r0, n in slabs:
            for j in range(8):
                dst[j, pad + r0:pad + r0 + n, :] = p[at:at + n, j * 128:(j + 1) * 128]
            at += n

    def v_finish(rb, m):
        cs = _c_combos(m)
        for qd, cc in enumerate(cs):
            r0 = PAD + (qd // 2) * H + rb * RB
            for j in range(4):
                v_s[(qd % 2) * 4 + j, r0:r0 + RB, :] = cc[:, j * 128:(j + 1) * 128]
        if rb == 0:
            for j in range(8):
                src = cs[j // 4][0:1, (j % 4) * 128:(j % 4 + 1) * 128]
                v_s[j, 0:PAD, :] = jnp.broadcast_to(src, (PAD, 128))

    def attn_group(row, masked):
        def run(prev):
            g = 8
            q = [q_s[j, pl.ds(row, g), :] for j in range(8)]
            ls = []
            for w in range(W):
                a = None
                for j in range(8):
                    term = q[j] * k_s[j, pl.ds(row + (PAD - DIL * w), g), :]
                    a = sp.link(ls[-1] if ls else None, term) if a is None else a + term
                ls.append(a)
            rs = [pltpu.roll(a, 64, 1) for a in ls]
            ls = [a + r for a, r in zip(ls, rs)]
            rs = [pltpu.roll(a, 32, 1) for a in ls]
            ls = [a + r for a, r in zip(ls, rs)]
            if masked:
                ri = row + lax.broadcasted_iota(i32, (g, 128), 0)
                ls = [ls[0]] + [jnp.where(ri >= DIL * w, ls[w], NEG) for w in range(1, W)]
            m = _tree(jnp.maximum, ls)
            ps = [jnp.exp2((l - m) * EXP2_SCALE) for l in ls]
            r = gs[pl.ds(row, g), :] / _tree(jnp.add, ps)
            outs = []
            for j in range(8):
                a = None
                for w in range(W):
                    term = ps[w] * v_s[j, pl.ds(row + (PAD - DIL * w), g), :]
                    a = sp.link(outs[-1] if outs else None, term) if a is None else a + term
                outs.append(a * r)
            for j in range(8):
                q_s[j, pl.ds(row, g), :] = outs[j]
            return sp.chain([outs[-1]], prev, 1)
        return run

    def attn_tasks(base, nrows, first=False):
        return [attn_group(base + (qq * Q + r), first and qq == 0 and r < PAD)
                for r in range(0, nrows, 8) for qq in range(4)]

    def pack_tasks(oa, base, hbase, nrows):
        def task(r, c):
            def run(prev):
                def blk(i1, i2, k1, k2):
                    return q_s[4 * k1 + 2 * k2 + c, pl.ds(base + (i1 * H + i2 * Q + r), 16), :]
                cs, tok = sp.two_level(_a_combos, blk, prev, DEPTH2)
                for t in range(49):
                    oa[t, pl.ds(hbase + r // 2, 8), c * 128:(c + 1) * 128] = cs[t]
                return tok
            return run
        return [task(r, c) for r in range(0, nrows, 16) for c in range(2)]

    GS = RB * (KH // 128) * (FC // 128) * 7 // (4 * SLOT)
    DS = 49
    PS = 2 * RB * (D // 128) * (D // 128) // (4 * SLOT)

    def glu(hs, ha):
        def finish(rb, m):
            glu_tasks(hs, rb, _c_combos(m), RB)[0](None)
            if rb >= 2:
                down_lhs(hs, rb - 2, ha)
        return finish

    def raw_first(rbs, n):
        lead = [(rb, t) for rb in rbs[:n] for t in ORDER[:2]]
        return lead + [(rb, t) for rb in rbs for t in ORDER if (rb, t) not in lead]

    def gu_src(j):
        return lambda r, c: wgu[j, r, c]

    def front(wqkv_vm, wp, wo_vm):
        in_q, in_k, in_v = [
            cp(wqkv_hbm.at[:, pl.ds(i * D, D)], wqkv_vm.at[:, pl.ds(i * D, D)], (6, 6, 5)[i])
            for i in range(3)]
        in_wo = cp(wo_hbm, wo_vm, 6)

        def plain(rb, hf, p):
            return sp.dot(x_vm[rows(rb, hf), :], wgu[0, :, p * CH:(p + 1) * CH])

        def plain_finish(rb, c):
            cs = [jnp.concatenate(c[2 * qd:2 * qd + 2], axis=1) for qd in range(4)]
            return glu_tasks(hs, rb, cs, 16)

        hs, bc, dc = {}, {}, {}
        wait(in0)
        start(in3)
        c0 = {(0, 0): plain(0, 0, 0)}
        wait(in1)
        c0[1, 0] = plain(0, 1, 0)
        wait(in2)
        start(in4)
        for hf in range(2):
            c0[hf, 1] = plain(0, hf, 1)
        wait(in3)
        start(in5)
        sp.block()
        bt = b_sum_tasks(gu_src(0), bc)
        sp.schedule(bt[:12], 3, 16)
        sp.schedule(prep_tasks(0, sums=False), 3, 16)
        for p in (2, 3):
            for hf in range(2):
                c0[hf, p] = plain(0, hf, p)
        c0 = [c0[hf, p] for hf in range(2) for p in range(4)]
        wait(in4)
        start([in_v])
        sp.block()
        sp.schedule(bt[12:], 3, 32)
        sp.schedule(prep_tasks(1, sums=False), 2, 10)
        sp.schedule(prep_tasks(2), 10, 32)
        c1 = [plain(1, hf, p) for hf in range(2) for p in range(4)]
        wait(in5 + [in_v])
        start([in_k, in_wo, in_q])
        sp.block()
        for j in range(8):
            k_s[j, 0:PAD, :] = jnp.zeros((PAD, 128), f32)
        ha = {}
        sp.schedule(prep_tasks(3), 2, GS)
        sp.schedule(plain_finish(0, c0), 2, GS)
        sp.schedule(plain_finish(1, c1), GS + 6, 2 * GS)
        sp.schedule(d_tasks(0, dc), GS - 2, 2 * GS)
        sp.schedule(perm_tasks(wqkv_vm, wp, 2, q_s), 2 * GS + 6, 2 * GS + DS - 8)
        strassen_x([(rb, t) for rb in (2, 3) for t in ORDER], b_rhs(gu_src(0), bc),
                   glu(hs, ha))
        ffn_down(ha, dc, True)

        wait([in_k, in_wo, in_q])
        start(in_ffn)
        sp.block()
        vb = {}
        v_src = lambda r, c: _unpack(wp[2, _half(r), c])
        wo_spread, wo_gather = wo_tasks(wo_vm)
        sp.schedule(b_sum_tasks(v_src, vb, VDEPTH), *VBC_SLOTS)
        sp.schedule(prep_tasks(0, gate=False) + prep_tasks(1, gate=False), *PREP01)
        sp.schedule(perm_tasks(wqkv_vm, wp, 1, k_s.at[:, PAD:, :]), *PERMK)
        sp.schedule(wo_spread, *WOS)
        strassen_x(raw_first((2, 3, 0, 1), 2), b_rhs(v_src, vb), v_finish)
        sp.schedule(perm_tasks(wqkv_vm, wp, 0, q_s), 4, 3 * PS)
        tok = None
        for t in wo_gather:
            tok = t(tok)
        for rb in range(NRB):
            proj(wp, 1, k_s, PAD, [(rb * Q, Q)])
        proj(wp, 0, q_s, 0, [(qq * Q, QA) for qq in range(4)])

        def q_rest(_, carry):
            sp.block()
            n = (Q - QA) // 2
            total = 4 * (Q - QA) * 64 // (4 * SLOT)
            sp.schedule(attn_tasks(0, A0, True), 4, total)
            for r0 in (QA, QA + n):
                proj(wp, 0, q_s, 0, [(qq * Q + r0, n) for qq in range(4)])
            return carry

        lax.fori_loop(0, zi[0], q_rest, 0)
        wait(in_ffn)

    def back(oa):
        def body(j, carry):
            sp.block()
            base = pl.multiple_of((j - 1) * AR, AR)
            hs, ha, bc, dc = {}, {}, {}, {}
            sp.schedule(b_sum_tasks(gu_src(j), bc), *BC_SLOTS)
            sp.schedule(attn_tasks(base + A0, AR), *ATTN_SLOTS)
            sp.schedule(pack_tasks(oa, base, pl.multiple_of((j - 1) * (AR // 2), AR // 2), AR),
                        *PACK_SLOTS)
            sp.schedule(d_tasks(j, dc), *DC_SLOTS)
            strassen_x(raw_first((0, 2, 1, 3), NRAW), b_rhs(gu_src(j), bc), glu(hs, ha))
            ffn_down(ha, dc, False)
            return carry

        lax.fori_loop(1, NC, body, 0)

        def out_copy(r0, i1, i2, cols):
            idx = (pl.ds(r0 + (i1 * H + i2 * Q), PB), cols)
            return cp(x_vm.at[idx], o2.at[idx], out_sem)

        def out_blocks(blocks):
            done_by = {ts[-1]: qd for ts, qd in _C_ORDER}
            todo = [(blk, t1, t2) for blk in range(len(blocks))
                    for ts1, _ in _C_ORDER for t1 in ts1 for ts2, _ in _C_ORDER for t2 in ts2]
            m, inner = {}, {}
            for i in range(0, len(todo), 2):
                pair = todo[i:i + 2]
                ps = sp.dots([(_unpack(oa[7 * t1 + t2, pl.ds(blocks[blk][1], PB // 2), :]),
                               _unpack(woc[7 * t1 + t2])) for blk, t1, t2 in pair])
                for (blk, t1, t2), p in zip(pair, ps):
                    r0, _, copies = blocks[blk]
                    m.setdefault((blk, t1), {})[t2] = acc[7 * t1 + t2, pl.ds(r0, PB), :] + p
                    if t2 not in done_by:
                        continue
                    q2 = done_by[t2]
                    inner.setdefault((blk, q2), {})[t1] = _c_quadrant(m[blk, t1], q2)
                    if t1 not in done_by:
                        continue
                    q1 = done_by[t1]
                    r = pl.ds(r0 + ((q1 // 2) * H + (q2 // 2) * Q), PB)
                    c = (q1 % 2) * KH + (q2 % 2) * KQ
                    x_vm[r, c:c + KQ] = _c_quadrant(inner[blk, q2], q1).astype(bf16)
                    start(copies.get((q1, q2), []))

        def whole(r0):
            return {(3, 3): [out_copy(r0, i1, i2, slice(None)) for i1 in range(2) for i2 in range(2)]}

        done = (NC - 1) * AR

        def out_body(i, carry):
            sp.block()
            half = pl.multiple_of(done // 2 + i * 24, 8)
            sp.schedule(pack_tasks(oa, 2 * half, half, 48), *PACK4)
            r0 = pl.multiple_of(i * PB, PB)
            out_blocks([(r0, pl.multiple_of(i * (PB // 2), PB // 2),
                         whole(r0))])
            return carry

        lax.fori_loop(0, 2, out_body, 0)
        sp.block()
        sp.schedule(pack_tasks(oa, done + 96, (done + 96) // 2, Q - done - 96), 4, 22)
        last = {(q1, 3): [out_copy(3 * PB, q1 // 2, i2, pl.ds((q1 % 2) * KH, KH))
                          for i2 in range(2)] for q1 in range(3)}
        for q2 in range(4):
            last[3, q2] = [out_copy(3 * PB, 1, q2 // 2, pl.ds(KH + (q2 % 2) * KQ, KQ))]
        copies = [whole(blk * PB) for blk in range(3)] + [last]
        out_blocks([(blk * PB, blk * PB // 2, copies[blk]) for blk in (2, 3)])
        for cs in copies:
            for key in cs:
                wait(cs[key])

    pl.run_scoped(front, pltpu.VMEM((D, 3 * D), bf16), pltpu.VMEM((3, D // 2, D), i32),
                  pltpu.VMEM((D, D), bf16))
    pl.run_scoped(back, pltpu.VMEM((49, Q // 2, KQ), i32))
    assert not sp.plan


_N_SEMS = 9


@jax.jit
def pallas_gated_mix__sliding_local_dilated__glu_gated_reglu__prompt_kernel(
    A_x: jax.Array,
    A_wqkv: jax.Array,
    A_wo: jax.Array,
    B_x: jax.Array,
    B_W_gate: jax.Array,
    B_W_up: jax.Array,
    B_W_down: jax.Array,
    gate_w: jax.Array,
):
    del B_x
    hbm = pl.BlockSpec(memory_space=pl.ANY)
    scratch = [
        pltpu.VMEM((S, D), bf16),
        pltpu.VMEM((S // 2, D), i32),
        pltpu.VMEM((5, H // 2, KH), i32),
        pltpu.VMEM((8, 128), bf16),
        pltpu.VMEM((NC, D, 2 * FC), bf16),
        pltpu.VMEM((NC, FC, D), bf16),
        pltpu.VMEM((49, Q, KQ), f32),
        pltpu.VMEM((8, S + QPAD, 128), f32),
        pltpu.VMEM((8, PAD + S, 128), f32),
        pltpu.VMEM((8, PAD + S, 128), f32),
        pltpu.VMEM((S, 128), f32),
        pltpu.VMEM((49, KQ // 2, KQ), i32),
        pltpu.VMEM((8, 128), i32),
        pltpu.SMEM((1,), i32),
        pltpu.SemaphoreType.DMA((_N_SEMS,)),
    ]
    return pl.pallas_call(
        _kernel,
        in_specs=[hbm] * 7,
        out_specs=hbm,
        out_shape=jax.ShapeDtypeStruct((1, S, D), bf16),
        scratch_shapes=scratch,
        compiler_params=pltpu.CompilerParams(vmem_limit_bytes=124 * 1024 * 1024),
    )(A_x, A_wqkv, A_wo, B_W_gate, B_W_up, B_W_down, gate_w.reshape(8, 128))
```

```python
import math

import jax
import jax.numpy as jnp
from jax import lax
import jax.experimental.pallas as pl
import jax.experimental.pallas.tpu as pltpu

f32 = jnp.float32
bf16 = jnp.bfloat16
i32 = jnp.int32

S = 2048
D = 1024
F = 3584
NH = 32
DH = D // NH
W = 8
DIL = 2
H = S // 2
Q = S // 4
KH = D // 2
KQ = D // 4
FC = 512
CH = FC // 2
CQ = FC // 4
NC = F // FC
RB = 256
NRB = H // RB
PB = 128
PAD = 16
TP = DH + 1
AR = 64
A0 = Q - 6 * AR
QA = 160
QPAD = 112

BC_SLOTS = (2, 24)
ATTN_SLOTS = (24, 106)
DC_SLOTS = (26, 98)
VDEPTH = 2
PDEPTH = 3
VBC_SLOTS = (2, 16)
PREP01 = (16, 56)
PERMK = (64, 106)
WOS = (70, 112)
PACK4 = (4, 24)
NRAW = 3
DEPTH = 3
DEPTH2 = 3
H_DEPTH = 3

SCALE = DH ** -0.5
EXP2_SCALE = SCALE * math.log2(math.e)
NEG = -1e9 / SCALE


def _a_combos(a11, a12, a21, a22):
    return [a11 + a22, a21 + a22, a11, a22, a11 + a12, a21 - a11, a12 - a22]


def _b_combos(b11, b12, b21, b22):
    return [b11 + b22, b11, b12 - b22, b21 - b11, b22, b11 + b12, b21 + b22]


_C_TERMS = (((1, 0), (1, 3), (-1, 4), (1, 6)), ((1, 2), (1, 4)), ((1, 1), (1, 3)),
            ((1, 0), (-1, 1), (1, 2), (1, 5)))
_C_ORDER = (((2, 4), 1), ((1, 3), 2), ((0, 6), 0), ((5,), 3))


def _c_quadrant(m, qd):
    out = m[_C_TERMS[qd][0][1]]
    for sign, t in _C_TERMS[qd][1:]:
        out = out + m[t] if sign > 0 else out - m[t]
    return out


def _c_combos(m):
    return [_c_quadrant(m, qd) for qd in range(4)]


_A_SLOT = {0: 0, 1: 1, 4: 2, 5: 3, 6: 4}
_B_SUMS = (2, 3, 0, 5, 6)
ORDER = (1, 4) + _B_SUMS


def _tree(op, xs):
    xs = list(xs)
    while len(xs) > 1:
        xs = [op(xs[i], xs[i + 1]) if i + 1 < len(xs) else xs[i] for i in range(0, len(xs), 2)]
    return xs[0]


def _pack(x):
    return pltpu.bitcast(x.astype(bf16), i32)


def _unpack(x):
    return pltpu.bitcast(x, bf16)


def _half(r):
    return slice(r.start // 2, r.stop // 2)


SLOT = 256


class _Spreader:
    def __init__(self, zero_ref):
        self.zero_ref = zero_ref
        self.plan = {}
        self.lists = 0
        self.now = 0

    def block(self):
        self.zero = self.zero_ref[...]
        self.never = self.zero != 0

    def link(self, after, x):
        if after is None:
            return x
        if after.dtype != x.dtype:
            after = pltpu.bitcast(after, x.dtype)
        return jnp.where(self.never, after, x)

    def chain(self, vals, prev, depth):
        for v in vals:
            v = pltpu.bitcast(v, i32) if v.dtype != i32 else v
            for r in range(0, v.shape[0], 8):
                for c in range(0, v.shape[1], 128):
                    tile = v[r:r + 8, c:c + 128]
                    if prev is None:
                        prev = tile
                        continue
                    prev = prev | tile
                    for i in range(depth - 1):
                        prev = (prev + self.zero) if i % 2 == 0 else (prev ^ self.zero)
        return prev

    def link_rows(self, after, x):
        return jnp.concatenate([self.link(after, x[r:r + 8, :]) for r in range(0, x.shape[0], 8)],
                               axis=0)

    def serial_combos(self, combos, x11, x12, x21, x22, after):
        return combos(self.link_rows(after, x11), x12, x21, self.link_rows(after, x22))

    def two_level(self, combos, blk, prev, depth, after=None):
        outer = [self.serial_combos(
            combos, *[blk(r1, r2, c1, c2) for r1 in range(2) for c1 in range(2)], after)
            for r2 in range(2) for c2 in range(2)]
        outs, tok = [], None
        for t in range(7):
            wide = _pack(jnp.concatenate(
                self.serial_combos(combos, *[o[t] for o in outer], tok), axis=1))
            outs += [wide[:, c:c + 128] for c in range(0, 7 * 128, 128)]
            tok = self.chain(outs[-7:], tok, depth)
        return outs, self.chain([tok], prev, 1)

    def schedule(self, tasks, first, last):
        self.lists += 1
        for i, t in enumerate(tasks):
            pos = self.now + first + ((i + 1) * (last - first) - 1) // len(tasks)
            self.plan.setdefault(pos, []).append((t, self.lists))

    def dots(self, pairs):
        m = pairs[0][0].shape[0]
        tiles = [(i, r, c) for i, (_, rhs) in enumerate(pairs)
                 for c in range(0, rhs.shape[1], 128) for r in range(0, rhs.shape[0], 128)]
        nslots = m * len(tiles) // (4 * SLOT)
        deps = {}
        for sl in range(nslots):
            ps = sl * SLOT // m
            toks = {}
            for t, lane in self.plan.pop(self.now + sl, []):
                tok = t(toks.get(lane))
                if tok is not None:
                    toks[lane] = tok
            for tok in toks.values():
                deps[ps] = tok | deps[ps] if ps in deps else tok
        self.now += nslots
        tied = {tile: d for ps, d in deps.items() for tile in tiles[4 * ps:4 * ps + 4]}
        outs = []
        for i, (lhs, rhs) in enumerate(pairs):
            if any(key[0] == i for key in tied):
                parts = []
                for r in range(0, rhs.shape[0], 128):
                    top = [rhs[r:r + 16, c:c + 128] for c in range(0, rhs.shape[1], 128)]
                    top = [_unpack(self.link(tied[i, r, c * 128], _pack(t0)))
                           if (i, r, c * 128) in tied else t0 for c, t0 in enumerate(top)]
                    parts += [jnp.concatenate(top, axis=1), rhs[r + 16:r + 128, :]]
                rhs = jnp.concatenate(parts, axis=0)
            outs.append(jnp.dot(lhs, rhs, preferred_element_type=f32))
        return outs

    def dot(self, lhs, rhs):
        return self.dots([(lhs, rhs)])[0]


def _kernel(x_hbm, wqkv_hbm, wo_hbm, wg_hbm, wu_hbm, wd_hbm, gw_hbm, out_hbm,
            x_vm, xn, xa, gw_vm, wgu, wd, acc, q_s, k_s, v_s, gs, woc, zs, zi, sems):
    def cp(src, dst, sem):
        return pltpu.make_async_copy(src, dst, sems.at[sem])

    def cp_gu(j, p, sem):
        return cp((wg_hbm, wu_hbm)[p % 2].at[:, pl.ds(j * FC + (p // 2) * CH, CH)],
                  wgu.at[j, :, pl.ds(p * CH, CH)], sem)

    def cp_d(j, sem):
        return cp(wd_hbm.at[pl.ds(j * FC, FC), :], wd.at[j], sem)

    def cp_x(rb, hf, sem):
        idx = (pl.ds(hf * H + rb * RB, RB), slice(None))
        return cp(x_hbm.at[0].at[idx], x_vm.at[idx], sem)

    o2 = out_hbm.at[0]
    in0 = [cp_x(0, 0, 0), cp_gu(0, 0, 0)]
    in1 = [cp_x(0, 1, 1)]
    in2 = [cp_gu(0, 1, 2)]
    in3 = [cp_gu(0, 2, 3), cp_gu(0, 3, 3), cp(gw_hbm, gw_vm, 3)]
    in4 = [cp_x(rb, hf, 4) for rb in (1, 2) for hf in range(2)]
    in5 = [cp_x(3, 0, 5), cp_x(3, 1, 5), cp_d(0, 5)]
    in_ffn = [c for j in range(1, NC) for c in [cp_gu(j, p, 7) for p in range(4)] + [cp_d(j, 7)]]
    out_sem = 8

    def start(cs):
        for c in cs:
            c.start()

    def wait(cs):
        for c in cs:
            c.wait()

    start(in0 + in1 + in2)

    zs[...] = jnp.zeros((8, 128), i32)
    zi[0] = 1
    sp = _Spreader(zs)

    def rows(rb, hf=0):
        return slice(hf * H + rb * RB, hf * H + (rb + 1) * RB)

    def x_lhs(t, rb):
        if t == 2:
            return _unpack(xn[_half(rows(rb, 0)), :KH])
        if t == 3:
            return _unpack(xn[_half(rows(rb, 1)), KH:])
        return _unpack(xa[_A_SLOT[t], _half(rows(rb)), :])

    def prep_tasks(rb, sums=True, gate=True):
        def task(s0):
            def run(first):
                prev = None
                gw = gw_vm[...].astype(f32)
                r = [slice(hf * H + rb * RB + s0, hf * H + rb * RB + s0 + 16) for hf in range(2)]
                z = [None, None]
                for c in range(4):
                    cols = [slice(kh * KH + c * 128, kh * KH + (c + 1) * 128) for kh in range(2)]
                    xs = [sp.link(prev, _pack(x_vm[r[qd // 2], cols[qd % 2]])) for qd in range(4)]
                    a = [_unpack(t).astype(f32) for t in xs]
                    outs = []
                    if sums:
                        for qd in range(4):
                            xn[_half(r[qd // 2]), cols[qd % 2]] = xs[qd]
                        cs = _a_combos(*a)
                        for t, slot in _A_SLOT.items():
                            outs.append(_pack(cs[t]))
                            xa[slot, _half(r[0]), cols[0]] = outs[-1]
                    if gate:
                        for qd in range(4):
                            g0 = (qd % 2) * 4 + c
                            term = a[qd] * gw[g0:g0 + 1, :]
                            z[qd // 2] = term if z[qd // 2] is None else z[qd // 2] + term
                        outs += z
                    prev = sp.chain(outs, prev, 1)
                if gate:
                    for hf in range(2):
                        g = jax.nn.sigmoid(jnp.sum(z[hf], axis=1, keepdims=True))
                        g = jnp.broadcast_to(g, (16, 128))
                        gs[r[hf], :] = g
                        prev = sp.chain([g], prev, 1)
                return sp.chain([prev], first, 1)
            return run
        return [task(s0) for s0 in range(0, RB, 16)]

    def b_sum_tasks(src, dst, depth=DEPTH):
        def task(r0):
            def run(prev):
                raw = [src(slice(a * KH + r0, a * KH + r0 + 16), slice(c * KH, (c + 1) * KH))
                       for a in range(2) for c in range(2)]
                cs = _b_combos(*[b.astype(f32) for b in raw])
                for t in _B_SUMS:
                    dst.setdefault(t, []).append(_pack(cs[t]))
                return sp.chain([dst[t][-1] for t in _B_SUMS], prev, depth)
            return run
        return [task(r0) for r0 in range(0, KH, 16)]

    def b_rhs(src, sums):
        def rhs(t):
            if t == 1:
                return src(slice(0, KH), slice(0, KH))
            if t == 4:
                return src(slice(KH, D), slice(KH, D))
            return _unpack(jnp.concatenate(sums[t], axis=0))
        return rhs

    def strassen_x(order, rhs, finish):
        m = {}
        for rb, t in order:
            m.setdefault(rb, {})[t] = sp.dot(x_lhs(t, rb), rhs(t))
            if len(m[rb]) == 7:
                finish(rb, m.pop(rb))

    def h_sums(rb, cs, r0, sub):
        h = []
        for qd, cc in enumerate(cs):
            g0 = (qd // 2) * H + rb * RB + r0
            omg = 1.0 - gs[g0:g0 + sub, :]
            omg = jnp.concatenate([omg] * (CH // 128), axis=1)
            h.append(jnp.maximum(cc[:, :CH], 0.0) * cc[:, CH:] * omg)
        return _a_combos(*h)

    def glu_tasks(hs, rb, cs, sub):
        hs[rb] = [[] for _ in range(7)]

        def task(r0):
            def run(prev):
                sums = h_sums(rb, [cc[r0:r0 + sub] for cc in cs], r0, sub)
                for t in range(7):
                    hs[rb][t].append(sums[t])
                if sub < RB:
                    return sp.chain([sums[t] for t in _A_SLOT], prev, DEPTH2)
            return run
        return [task(r0) for r0 in range(0, RB, sub)]

    def down_lhs(hs, b, ha):
        tok = None
        for t in range(7):
            s0, s1 = [jnp.concatenate(hs[rb][t], axis=0) for rb in (b, b + 2)]
            slabs = []
            for r in range(0, RB, 16):
                slabs.append(sp.serial_combos(
                    _a_combos, s0[r:r + 16, :CQ], s0[r:r + 16, CQ:],
                    s1[r:r + 16, :CQ], s1[r:r + 16, CQ:], tok))
                tok = sp.chain([slabs[-1][t2] for t2 in _A_SLOT], None, H_DEPTH)
            for t2 in range(7):
                ha[b, 7 * t + t2] = jnp.concatenate([sl[t2] for sl in slabs], axis=0).astype(bf16)
        ha['tok'] = tok

    def d_tasks(j, dst):
        def task(r0, c):
            def run(prev):
                def blk(k1, k2, n1, n2):
                    r, c0 = k1 * CH + k2 * CQ + r0, n1 * KH + n2 * KQ + c * 128
                    return wd[j, r:r + 16, c0:c0 + 128].astype(f32)
                cs, tok = sp.two_level(_b_combos, blk, prev, DEPTH2)
                for t in range(49):
                    dst.setdefault((t, c), []).append(cs[t])
                return tok
            return run
        return [task(r0, c) for r0 in range(0, CQ, 16) for c in range(2)]

    def ffn_down(ha, dc, first):
        rhs = [_unpack(jnp.concatenate([jnp.concatenate(dc[t, c], axis=0) for c in range(2)], axis=1))
               for t in range(49)]
        todo = [(b, t) for b in range(2) for t in range(49)]
        for i in range(0, len(todo), 2):
            pair = todo[i:i + 2]
            ps = sp.dots([(ha[b, t], rhs[t]) for b, t in pair])
            for (b, t), p in zip(pair, ps):
                if first:
                    acc[t, b * RB:(b + 1) * RB, :] = p
                else:
                    acc[t, b * RB:(b + 1) * RB, :] += p

    def perm_tasks(wqkv_vm, wp, i, tbuf):
        def fwd(rb, c):
            def run(prev):
                c0 = i * D + c * 128
                tt = pltpu.bitcast(wqkv_vm[rb * 256:(rb + 1) * 256, c0:c0 + 128], f32).T
                for hh in range(4):
                    tbuf[rb, pl.ds((4 * c + hh) * TP, DH), :] = tt[hh * DH:(hh + 1) * DH, :]
                return sp.chain([tt], prev, 1)
            return run

        def bwd(rb, j):
            def run(prev):
                g = jnp.concatenate(
                    [tbuf[rb, pl.ds(4 * j + dd, NH, stride=TP), :] for dd in range(4)], axis=0).T
                wp[i, rb * 128:(rb + 1) * 128, j * 128:(j + 1) * 128] = pltpu.bitcast(g, i32)
            return run
        tasks = []
        for rb in range(4):
            tasks += [fwd(rb, c) for c in range(8)] + [bwd(rb, j) for j in range(8)]
        return tasks

    def wo_tasks(wo_vm):
        def stage(c):
            return 4 + c % 4, (c // 4) * NH * TP

        def spread(h0):
            def run(prev):
                blk = wo_vm[h0 * DH:(h0 + 2) * DH, :].astype(f32)
                for h in range(2):
                    for c in range(8):
                        sl, r0 = stage(c)
                        q_s[sl, pl.ds(r0 + (h0 + h) * TP, DH), :] = (
                            blk[h * DH:(h + 1) * DH, c * 128:(c + 1) * 128])
                return sp.chain([blk], prev, 1)
            return run

        def gather(d, h0, c):
            def run(after):
                def blk(k1, k2, n1, n2):
                    sl, r0 = stage(4 * n1 + 2 * n2 + c)
                    r0 += h0 * TP + 16 * k1 + 8 * k2 + d
                    return q_s[sl, pl.ds(r0, 16, stride=TP), :]
                cs, tok = sp.two_level(_b_combos, blk, None, DEPTH2, after)
                r = (d * NH + h0) // 2
                for t in range(49):
                    woc[t, r:r + 8, c * 128:(c + 1) * 128] = cs[t]
                return tok
            return run
        return ([spread(h0) for h0 in range(0, NH, 2)],
                [gather(d, h0, c) for d in range(8) for h0 in (0, 16) for c in range(2)])

    def proj(wp, i, dst, pad, slabs):
        lhs = jnp.concatenate([xn[r0 // 2:(r0 + n) // 2, :] for r0, n in slabs], axis=0)
        p = sp.dot(_unpack(lhs), _unpack(wp[i]))
        at = 0
        for r0, n in slabs:
            for j in range(8):
                dst[j, pad + r0:pad + r0 + n, :] = p[at:at + n, j * 128:(j + 1) * 128]
            at += n

    def v_finish(rb, m):
        cs = _c_combos(m)
        for qd, cc in enumerate(cs):
            r0 = PAD + (qd // 2) * H + rb * RB
            for j in range(4):
                v_s[(qd % 2) * 4 + j, r0:r0 + RB, :] = cc[:, j * 128:(j + 1) * 128]
        if rb == 0:
            for j in range(8):
                src = cs[j // 4][0:1, (j % 4) * 128:(j % 4 + 1) * 128]
                v_s[j, 0:PAD, :] = jnp.broadcast_to(src, (PAD, 128))

    def attn_group(row, masked):
        def run(prev):
            g = 8
            q = [q_s[j, pl.ds(row, g), :] for j in range(8)]
            ls = []
            for w in range(W):
                a = None
                for j in range(8):
                    term = q[j] * k_s[j, pl.ds(row + (PAD - DIL * w), g), :]
                    a = sp.link(ls[-1] if ls else None, term) if a is None else a + term
                ls.append(a)
            rs = [pltpu.roll(a, 64, 1) for a in ls]
            ls = [a + r for a, r in zip(ls, rs)]
            rs = [pltpu.roll(a, 32, 1) for a in ls]
            ls = [a + r for a, r in zip(ls, rs)]
            if masked:
                ri = row + lax.broadcasted_iota(i32, (g, 128), 0)
                ls = [ls[0]] + [jnp.where(ri >= DIL * w, ls[w], NEG) for w in range(1, W)]
            m = _tree(jnp.maximum, ls)
            ps = [jnp.exp2((l - m) * EXP2_SCALE) for l in ls]
            r = gs[pl.ds(row, g), :] / _tree(jnp.add, ps)
            outs = []
            for j in range(8):
                a = None
                for w in range(W):
                    term = ps[w] * v_s[j, pl.ds(row + (PAD - DIL * w), g), :]
                    a = sp.link(outs[-1] if outs else None, term) if a is None else a + term
                outs.append(a * r)
            for j in range(8):
                q_s[j, pl.ds(row, g), :] = outs[j]
            return sp.chain([outs[-1]], prev, 1)
        return run

    def attn_tasks(base, nrows, first=False):
        return [attn_group(base + (qq * Q + r), first and qq == 0 and r < PAD)
                for r in range(0, nrows, 8) for qq in range(4)]

    def pack_tasks(oa, base, hbase, nrows):
        def task(r, c):
            def run(prev, after=None):
                def blk(i1, i2, k1, k2):
                    return q_s[4 * k1 + 2 * k2 + c, pl.ds(base + (i1 * H + i2 * Q + r), 16), :]
                cs, tok = sp.two_level(_a_combos, blk, prev, DEPTH2 if after is None else PDEPTH, after)
                for t in range(49):
                    oa[t, pl.ds(hbase + r // 2, 8), c * 128:(c + 1) * 128] = cs[t]
                return tok
            return run
        return [task(r, c) for r in range(0, nrows, 16) for c in range(2)]

    GS = RB * (KH // 128) * (FC // 128) * 7 // (4 * SLOT)
    DS = 49
    PS = 2 * RB * (D // 128) * (D // 128) // (4 * SLOT)

    def glu(hs, ha):
        def finish(rb, m):
            glu_tasks(hs, rb, _c_combos(m), RB)[0](None)
            if rb >= 2:
                down_lhs(hs, rb - 2, ha)
        return finish

    def raw_first(rbs, n):
        lead = [(rb, t) for rb in rbs[:n] for t in ORDER[:2]]
        return lead + [(rb, t) for rb in rbs for t in ORDER if (rb, t) not in lead]

    def gu_src(j):
        return lambda r, c: wgu[j, r, c]

    def front(wqkv_vm, wp, wo_vm):
        in_q, in_k, in_v = [
            cp(wqkv_hbm.at[:, pl.ds(i * D, D)], wqkv_vm.at[:, pl.ds(i * D, D)], (6, 6, 5)[i])
            for i in range(3)]
        in_wo = cp(wo_hbm, wo_vm, 6)

        def plain(rb, hf, p):
            return sp.dot(x_vm[rows(rb, hf), :], wgu[0, :, p * CH:(p + 1) * CH])

        def plain_finish(rb, c):
            cs = [jnp.concatenate(c[2 * qd:2 * qd + 2], axis=1) for qd in range(4)]
            return glu_tasks(hs, rb, cs, 16)

        hs, bc, dc = {}, {}, {}
        wait(in0)
        start(in3)
        c0 = {(0, 0): plain(0, 0, 0)}
        wait(in1)
        c0[1, 0] = plain(0, 1, 0)
        wait(in2)
        start(in4)
        for hf in range(2):
            c0[hf, 1] = plain(0, hf, 1)
        wait(in3)
        start(in5)
        sp.block()
        bt = b_sum_tasks(gu_src(0), bc)
        sp.schedule(bt[:12], 3, 16)
        sp.schedule(prep_tasks(0, sums=False), 3, 16)
        for p in (2, 3):
            for hf in range(2):
                c0[hf, p] = plain(0, hf, p)
        c0 = [c0[hf, p] for hf in range(2) for p in range(4)]
        wait(in4)
        start([in_v])
        sp.block()
        sp.schedule(bt[12:], 3, 32)
        sp.schedule(prep_tasks(1, sums=False), 2, 10)
        sp.schedule(prep_tasks(2), 10, 32)
        c1 = [plain(1, hf, p) for hf in range(2) for p in range(4)]
        wait(in5 + [in_v])
        start([in_k, in_wo, in_q])
        sp.block()
        for j in range(8):
            k_s[j, 0:PAD, :] = jnp.zeros((PAD, 128), f32)
        ha = {}
        sp.schedule(prep_tasks(3), 2, GS)
        sp.schedule(plain_finish(0, c0), 2, GS)
        sp.schedule(plain_finish(1, c1), GS + 6, 2 * GS)
        sp.schedule(d_tasks(0, dc), GS - 2, 2 * GS)
        sp.schedule(perm_tasks(wqkv_vm, wp, 2, q_s), 2 * GS + 6, 2 * GS + DS - 8)
        strassen_x([(rb, t) for rb in (2, 3) for t in ORDER], b_rhs(gu_src(0), bc),
                   glu(hs, ha))
        ffn_down(ha, dc, True)

        wait([in_k, in_wo, in_q])
        start(in_ffn)
        sp.block()
        vb = {}
        v_src = lambda r, c: _unpack(wp[2, _half(r), c])
        wo_spread, wo_gather = wo_tasks(wo_vm)
        sp.schedule(b_sum_tasks(v_src, vb, VDEPTH), *VBC_SLOTS)
        sp.schedule(prep_tasks(0, gate=False) + prep_tasks(1, gate=False), *PREP01)
        sp.schedule(perm_tasks(wqkv_vm, wp, 1, k_s.at[:, PAD:, :]), *PERMK)
        sp.schedule(wo_spread, *WOS)
        strassen_x(raw_first((2, 3, 0, 1), 2), b_rhs(v_src, vb), v_finish)
        sp.schedule(perm_tasks(wqkv_vm, wp, 0, q_s), 4, 3 * PS)
        tok = None
        for t in wo_gather:
            tok = t(tok)
        for rb in range(NRB):
            proj(wp, 1, k_s, PAD, [(rb * Q, Q)])
        proj(wp, 0, q_s, 0, [(qq * Q, QA) for qq in range(4)])

        def q_rest(_, carry):
            sp.block()
            n = (Q - QA) // 2
            total = 4 * (Q - QA) * 64 // (4 * SLOT)
            sp.schedule(attn_tasks(0, A0, True), 4, total)
            for r0 in (QA, QA + n):
                proj(wp, 0, q_s, 0, [(qq * Q + r0, n) for qq in range(4)])
            return carry

        lax.fori_loop(0, zi[0], q_rest, 0)
        wait(in_ffn)

    def back(oa):
        def body(j, carry):
            sp.block()
            base = pl.multiple_of((j - 1) * AR, AR)
            hs, ha, bc, dc = {}, {}, {}, {}
            sp.schedule(b_sum_tasks(gu_src(j), bc), *BC_SLOTS)
            sp.schedule(attn_tasks(base + A0, AR), *ATTN_SLOTS)
            packs = pack_tasks(oa, base, pl.multiple_of((j - 1) * (AR // 2), AR // 2), AR)
            sp.schedule(d_tasks(j, dc), *DC_SLOTS)
            strassen_x(raw_first((0, 2, 1, 3), NRAW), b_rhs(gu_src(j), bc), glu(hs, ha))
            tok = ha['tok']
            for t in packs:
                tok = t(None, tok)
            ffn_down(ha, dc, False)
            return carry

        lax.fori_loop(1, NC, body, 0)

        def out_copy(r0, i1, i2, cols):
            idx = (pl.ds(r0 + (i1 * H + i2 * Q), PB), cols)
            return cp(x_vm.at[idx], o2.at[idx], out_sem)

        def out_blocks(blocks):
            done_by = {ts[-1]: qd for ts, qd in _C_ORDER}
            todo = [(blk, t1, t2) for blk in range(len(blocks))
                    for ts1, _ in _C_ORDER for t1 in ts1 for ts2, _ in _C_ORDER for t2 in ts2]
            m, inner = {}, {}
            for i in range(0, len(todo), 2):
                pair = todo[i:i + 2]
                ps = sp.dots([(_unpack(oa[7 * t1 + t2, pl.ds(blocks[blk][1], PB // 2), :]),
                               _unpack(woc[7 * t1 + t2])) for blk, t1, t2 in pair])
                for (blk, t1, t2), p in zip(pair, ps):
                    r0, _, copies = blocks[blk]
                    m.setdefault((blk, t1), {})[t2] = acc[7 * t1 + t2, pl.ds(r0, PB), :] + p
                    if t2 not in done_by:
                        continue
                    q2 = done_by[t2]
                    inner.setdefault((blk, q2), {})[t1] = _c_quadrant(m[blk, t1], q2)
                    if t1 not in done_by:
                        continue
                    q1 = done_by[t1]
                    r = pl.ds(r0 + ((q1 // 2) * H + (q2 // 2) * Q), PB)
                    c = (q1 % 2) * KH + (q2 % 2) * KQ
                    x_vm[r, c:c + KQ] = _c_quadrant(inner[blk, q2], q1).astype(bf16)
                    start(copies.get((q1, q2), []))

        def whole(r0):
            return {(3, 3): [out_copy(r0, i1, i2, slice(None)) for i1 in range(2) for i2 in range(2)]}

        done = (NC - 1) * AR

        def out_body(i, carry):
            sp.block()
            half = pl.multiple_of(done // 2 + i * 24, 8)
            sp.schedule(pack_tasks(oa, 2 * half, half, 48), *PACK4)
            r0 = pl.multiple_of(i * PB, PB)
            out_blocks([(r0, pl.multiple_of(i * (PB // 2), PB // 2),
                         whole(r0))])
            return carry

        lax.fori_loop(0, 2, out_body, 0)
        sp.block()
        sp.schedule(pack_tasks(oa, done + 96, (done + 96) // 2, Q - done - 96), 4, 22)
        last = {(q1, 3): [out_copy(3 * PB, q1 // 2, i2, pl.ds((q1 % 2) * KH, KH))
                          for i2 in range(2)] for q1 in range(3)}
        for q2 in range(4):
            last[3, q2] = [out_copy(3 * PB, 1, q2 // 2, pl.ds(KH + (q2 % 2) * KQ, KQ))]
        copies = [whole(blk * PB) for blk in range(3)] + [last]
        out_blocks([(blk * PB, blk * PB // 2, copies[blk]) for blk in (2, 3)])
        for cs in copies:
            for key in cs:
                wait(cs[key])

    pl.run_scoped(front, pltpu.VMEM((D, 3 * D), bf16), pltpu.VMEM((3, D // 2, D), i32),
                  pltpu.VMEM((D, D), bf16))
    pl.run_scoped(back, pltpu.VMEM((49, Q // 2, KQ), i32))
    assert not sp.plan


_N_SEMS = 9


@jax.jit
def pallas_gated_mix__sliding_local_dilated__glu_gated_reglu__prompt_kernel(
    A_x: jax.Array,
    A_wqkv: jax.Array,
    A_wo: jax.Array,
    B_x: jax.Array,
    B_W_gate: jax.Array,
    B_W_up: jax.Array,
    B_W_down: jax.Array,
    gate_w: jax.Array,
):
    del B_x
    hbm = pl.BlockSpec(memory_space=pl.ANY)
    scratch = [
        pltpu.VMEM((S, D), bf16),
        pltpu.VMEM((S // 2, D), i32),
        pltpu.VMEM((5, H // 2, KH), i32),
        pltpu.VMEM((8, 128), bf16),
        pltpu.VMEM((NC, D, 2 * FC), bf16),
        pltpu.VMEM((NC, FC, D), bf16),
        pltpu.VMEM((49, Q, KQ), f32),
        pltpu.VMEM((8, S + QPAD, 128), f32),
        pltpu.VMEM((8, PAD + S, 128), f32),
        pltpu.VMEM((8, PAD + S, 128), f32),
        pltpu.VMEM((S, 128), f32),
        pltpu.VMEM((49, KQ // 2, KQ), i32),
        pltpu.VMEM((8, 128), i32),
        pltpu.SMEM((1,), i32),
        pltpu.SemaphoreType.DMA((_N_SEMS,)),
    ]
    return pl.pallas_call(
        _kernel,
        in_specs=[hbm] * 7,
        out_specs=hbm,
        out_shape=jax.ShapeDtypeStruct((1, S, D), bf16),
        scratch_shapes=scratch,
        compiler_params=pltpu.CompilerParams(vmem_limit_bytes=124 * 1024 * 1024),
    )(A_x, A_wqkv, A_wo, B_W_gate, B_W_up, B_W_down, gate_w.reshape(8, 128))
```

```python
import math

import jax
import jax.numpy as jnp
from jax import lax
import jax.experimental.pallas as pl
import jax.experimental.pallas.tpu as pltpu

f32 = jnp.float32
bf16 = jnp.bfloat16
i32 = jnp.int32

S = 2048
D = 1024
F = 3584
NH = 32
DH = D // NH
W = 8
DIL = 2
H = S // 2
Q = S // 4
KH = D // 2
KQ = D // 4
FC = 512
CH = FC // 2
CQ = FC // 4
NC = F // FC
RB = 256
NRB = H // RB
PB = 128
PAD = 16
TP = DH + 1
AR = 64
A0 = Q - 6 * AR
QA = 160
QPAD = 112

BC_SLOTS = (2, 24)
ATTN_SLOTS = (24, 106)
DC_SLOTS = (26, 98)
VDEPTH = 2
PDEPTH = 3
VBC_SLOTS = (2, 16)
PREP01 = (16, 56)
PERMK = (64, 106)
WOS = (70, 112)
PACK4 = (4, 24)
NRAW = 3
DEPTH = 3
DEPTH2 = 3
H_DEPTH = 3

SCALE = DH ** -0.5
EXP2_SCALE = SCALE * math.log2(math.e)
NEG = -1e9 / SCALE


def _a_combos(a11, a12, a21, a22):
    return [a11 + a22, a21 + a22, a11, a22, a11 + a12, a21 - a11, a12 - a22]


def _b_combos(b11, b12, b21, b22):
    return [b11 + b22, b11, b12 - b22, b21 - b11, b22, b11 + b12, b21 + b22]


_C_TERMS = (((1, 0), (1, 3), (-1, 4), (1, 6)), ((1, 2), (1, 4)), ((1, 1), (1, 3)),
            ((1, 0), (-1, 1), (1, 2), (1, 5)))
_C_ORDER = (((2, 4), 1), ((1, 3), 2), ((0, 6), 0), ((5,), 3))


def _c_quadrant(m, qd):
    out = m[_C_TERMS[qd][0][1]]
    for sign, t in _C_TERMS[qd][1:]:
        out = out + m[t] if sign > 0 else out - m[t]
    return out


def _c_combos(m):
    return [_c_quadrant(m, qd) for qd in range(4)]


_FLIP = (1, 4, 5, 6)
_A_SLOT = {0: 0, 1: 1, 4: 2, 5: 3, 6: 4}
_B_SUMS = (2, 3, 0, 5, 6)
ORDER = (1, 4) + _B_SUMS


def _tree(op, xs):
    xs = list(xs)
    while len(xs) > 1:
        xs = [op(xs[i], xs[i + 1]) if i + 1 < len(xs) else xs[i] for i in range(0, len(xs), 2)]
    return xs[0]


def _pack(x):
    return pltpu.bitcast(x.astype(bf16), i32)


def _unpack(x):
    return pltpu.bitcast(x, bf16)


def _half(r):
    return slice(r.start // 2, r.stop // 2)


SLOT = 256


class _Spreader:
    def __init__(self, zero_ref):
        self.zero_ref = zero_ref
        self.plan = {}
        self.lists = 0
        self.now = 0

    def block(self):
        self.zero = self.zero_ref[...]
        self.never = self.zero != 0

    def link(self, after, x):
        if after is None:
            return x
        if after.dtype != x.dtype:
            after = pltpu.bitcast(after, x.dtype)
        return jnp.where(self.never, after, x)

    def chain(self, vals, prev, depth):
        for v in vals:
            v = pltpu.bitcast(v, i32) if v.dtype != i32 else v
            for r in range(0, v.shape[0], 8):
                for c in range(0, v.shape[1], 128):
                    tile = v[r:r + 8, c:c + 128]
                    if prev is None:
                        prev = tile
                        continue
                    prev = prev | tile
                    for i in range(depth - 1):
                        prev = (prev + self.zero) if i % 2 == 0 else (prev ^ self.zero)
        return prev

    def link_rows(self, after, x):
        return jnp.concatenate([self.link(after, x[r:r + 8, :]) for r in range(0, x.shape[0], 8)],
                               axis=0)

    def serial_combos(self, combos, x11, x12, x21, x22, after):
        return combos(self.link_rows(after, x11), x12, x21, self.link_rows(after, x22))

    def two_level(self, combos, blk, prev, depth, after=None):
        outer = [self.serial_combos(
            combos, *[blk(r1, r2, c1, c2) for r1 in range(2) for c1 in range(2)], after)
            for r2 in range(2) for c2 in range(2)]
        outs, tok = [], None
        for t in range(7):
            flip = combos is _b_combos and t in _FLIP
            wide = _pack(jnp.concatenate(
                self.serial_combos(combos, *[outer[i ^ flip][t] for i in range(4)], tok), axis=1))
            outs += [wide[:, c:c + 128] for c in range(0, 7 * 128, 128)]
            tok = self.chain(outs[-7:], tok, depth)
        return outs, self.chain([tok], prev, 1)

    def schedule(self, tasks, first, last):
        self.lists += 1
        for i, t in enumerate(tasks):
            pos = self.now + first + ((i + 1) * (last - first) - 1) // len(tasks)
            self.plan.setdefault(pos, []).append((t, self.lists))

    def dots(self, pairs):
        m = pairs[0][0].shape[0]
        tiles = [(i, r, c) for i, (_, rhs) in enumerate(pairs)
                 for c in range(0, rhs.shape[1], 128) for r in range(0, rhs.shape[0], 128)]
        nslots = m * len(tiles) // (4 * SLOT)
        deps = {}
        for sl in range(nslots):
            ps = sl * SLOT // m
            toks = {}
            for t, lane in self.plan.pop(self.now + sl, []):
                tok = t(toks.get(lane))
                if tok is not None:
                    toks[lane] = tok
            for tok in toks.values():
                deps[ps] = tok | deps[ps] if ps in deps else tok
        self.now += nslots
        tied = {tile: d for ps, d in deps.items() for tile in tiles[4 * ps:4 * ps + 4]}
        outs = []
        for i, (lhs, rhs) in enumerate(pairs):
            if any(key[0] == i for key in tied):
                parts = []
                for r in range(0, rhs.shape[0], 128):
                    top = [rhs[r:r + 16, c:c + 128] for c in range(0, rhs.shape[1], 128)]
                    top = [_unpack(self.link(tied[i, r, c * 128], _pack(t0)))
                           if (i, r, c * 128) in tied else t0 for c, t0 in enumerate(top)]
                    parts += [jnp.concatenate(top, axis=1), rhs[r + 16:r + 128, :]]
                rhs = jnp.concatenate(parts, axis=0)
            outs.append(jnp.dot(lhs, rhs, preferred_element_type=f32))
        return outs

    def dot(self, lhs, rhs):
        return self.dots([(lhs, rhs)])[0]


def _kernel(x_hbm, wqkv_hbm, wo_hbm, wg_hbm, wu_hbm, wd_hbm, gw_hbm, out_hbm,
            x_vm, xn, xa, gw_vm, wgu, wd, acc, q_s, k_s, v_s, gs, woc, zs, zi, sems):
    def cp(src, dst, sem):
        return pltpu.make_async_copy(src, dst, sems.at[sem])

    def cp_gu(j, p, sem):
        return cp((wg_hbm, wu_hbm)[p % 2].at[:, pl.ds(j * FC + (p // 2) * CH, CH)],
                  wgu.at[j, :, pl.ds(p * CH, CH)], sem)

    def cp_d(j, sem):
        return cp(wd_hbm.at[pl.ds(j * FC, FC), :], wd.at[j], sem)

    def cp_x(rb, hf, sem):
        idx = (pl.ds(hf * H + rb * RB, RB), slice(None))
        return cp(x_hbm.at[0].at[idx], x_vm.at[idx], sem)

    o2 = out_hbm.at[0]
    in0 = [cp_x(0, 0, 0), cp_gu(0, 0, 0)]
    in1 = [cp_x(0, 1, 1)]
    in2 = [cp_gu(0, 1, 2)]
    in3 = [cp_gu(0, 2, 3), cp_gu(0, 3, 3), cp(gw_hbm, gw_vm, 3)]
    in4 = [cp_x(rb, hf, 4) for rb in (1, 2) for hf in range(2)]
    in5 = [cp_x(3, 0, 5), cp_x(3, 1, 5), cp_d(0, 5)]
    in_ffn = [c for j in range(1, NC) for c in [cp_gu(j, p, 7) for p in range(4)] + [cp_d(j, 7)]]
    out_sem = 8

    def start(cs):
        for c in cs:
            c.start()

    def wait(cs):
        for c in cs:
            c.wait()

    start(in0 + in1 + in2)

    zs[...] = jnp.zeros((8, 128), i32)
    zi[0] = 1
    sp = _Spreader(zs)

    def rows(rb, hf=0):
        return slice(hf * H + rb * RB, hf * H + (rb + 1) * RB)

    def x_lhs(t, rb):
        if t == 2:
            return _unpack(xn[_half(rows(rb, 0)), :KH])
        if t == 3:
            return _unpack(xn[_half(rows(rb, 1)), KH:])
        return _unpack(xa[_A_SLOT[t], _half(rows(rb)), :])

    def prep_tasks(rb, sums=True, gate=True):
        def task(s0):
            def run(first):
                prev = None
                gw = gw_vm[...].astype(f32)
                r = [slice(hf * H + rb * RB + s0, hf * H + rb * RB + s0 + 16) for hf in range(2)]
                z = [None, None]
                for c in range(4):
                    cols = [slice(kh * KH + c * 128, kh * KH + (c + 1) * 128) for kh in range(2)]
                    xs = [sp.link(prev, _pack(x_vm[r[qd // 2], cols[qd % 2]])) for qd in range(4)]
                    a = [_unpack(t).astype(f32) for t in xs]
                    outs = []
                    if sums:
                        for qd in range(4):
                            xn[_half(r[qd // 2]), cols[qd % 2]] = xs[qd]
                        cs = _a_combos(*a)
                        for t, slot in _A_SLOT.items():
                            outs.append(_pack(cs[t]))
                            xa[slot, _half(r[0]), cols[0]] = outs[-1]
                    if gate:
                        for qd in range(4):
                            g0 = (qd % 2) * 4 + c
                            term = a[qd] * gw[g0:g0 + 1, :]
                            z[qd // 2] = term if z[qd // 2] is None else z[qd // 2] + term
                        outs += z
                    prev = sp.chain(outs, prev, 1)
                if gate:
                    for hf in range(2):
                        g = jax.nn.sigmoid(jnp.sum(z[hf], axis=1, keepdims=True))
                        g = jnp.broadcast_to(g, (16, 128))
                        gs[r[hf], :] = g
                        prev = sp.chain([g], prev, 1)
                return sp.chain([prev], first, 1)
            return run
        return [task(s0) for s0 in range(0, RB, 16)]

    def b_sum_tasks(src, dst, depth=DEPTH):
        def task(r0):
            def run(prev):
                raw = [src(slice(a * KH + r0, a * KH + r0 + 16), slice(c * KH, (c + 1) * KH))
                       for a in range(2) for c in range(2)]
                cs = _b_combos(*[b.astype(f32) for b in raw])
                for t in _B_SUMS:
                    dst.setdefault(t, []).append(_pack(cs[t]))
                return sp.chain([dst[t][-1] for t in _B_SUMS], prev, depth)
            return run
        return [task(r0) for r0 in range(0, KH, 16)]

    def b_rhs(src, sums):
        def rhs(t):
            if t == 1:
                return src(slice(0, KH), slice(0, KH))
            if t == 4:
                return src(slice(KH, D), slice(KH, D))
            return _unpack(jnp.concatenate(sums[t], axis=0))
        return rhs

    def strassen_x(order, rhs, finish):
        m = {}
        for rb, t in order:
            m.setdefault(rb, {})[t] = sp.dot(x_lhs(t, rb), rhs(t))
            if len(m[rb]) == 7:
                finish(rb, m.pop(rb))

    def h_sums(rb, cs, r0, sub):
        h = []
        for qd, cc in enumerate(cs):
            g0 = (qd // 2) * H + rb * RB + r0
            omg = 1.0 - gs[g0:g0 + sub, :]
            omg = jnp.concatenate([omg] * (CH // 128), axis=1)
            h.append(jnp.maximum(cc[:, :CH], 0.0) * cc[:, CH:] * omg)
        return _a_combos(*h)

    def glu_tasks(hs, rb, cs, sub):
        hs[rb] = [[] for _ in range(7)]

        def task(r0):
            def run(prev):
                sums = h_sums(rb, [cc[r0:r0 + sub] for cc in cs], r0, sub)
                for t in range(7):
                    hs[rb][t].append(sums[t])
                if sub < RB:
                    return sp.chain([sums[t] for t in _A_SLOT], prev, DEPTH2)
            return run
        return [task(r0) for r0 in range(0, RB, sub)]

    def down_lhs(hs, b, ha):
        tok = None
        for t in range(7):
            s0, s1 = [jnp.concatenate(hs[rb][t], axis=0) for rb in (b, b + 2)]
            slabs = []
            for r in range(0, RB, 16):
                slabs.append(sp.serial_combos(
                    _a_combos, s0[r:r + 16, :CQ], s0[r:r + 16, CQ:],
                    s1[r:r + 16, :CQ], s1[r:r + 16, CQ:], tok))
                tok = sp.chain([slabs[-1][t2] for t2 in _A_SLOT], None, H_DEPTH)
            for t2 in range(7):
                ha[b, 7 * t + t2] = jnp.concatenate([sl[t2] for sl in slabs], axis=0).astype(bf16)
        ha['tok'] = tok

    def d_tasks(j, dst):
        def task(r0, c):
            def run(prev):
                def blk(k1, k2, n1, n2):
                    r, c0 = k1 * CH + k2 * CQ + r0, n1 * KH + n2 * KQ + c * 128
                    return wd[j, r:r + 16, c0:c0 + 128].astype(f32)
                cs, tok = sp.two_level(_b_combos, blk, prev, DEPTH2)
                for t in range(49):
                    dst.setdefault((t, c), []).append(cs[t])
                return tok
            return run
        return [task(r0, c) for r0 in range(0, CQ, 16) for c in range(2)]

    def ffn_down(ha, dc, first):
        rhs = [_unpack(jnp.concatenate([jnp.concatenate(dc[t, c], axis=0) for c in range(2)], axis=1))
               for t in range(49)]
        todo = [(b, t) for b in range(2) for t in range(49)]
        for i in range(0, len(todo), 2):
            pair = todo[i:i + 2]
            ps = sp.dots([(ha[b, t], rhs[t]) for b, t in pair])
            for (b, t), p in zip(pair, ps):
                if first:
                    acc[t, b * RB:(b + 1) * RB, :] = p
                else:
                    acc[t, b * RB:(b + 1) * RB, :] += p

    def perm_tasks(wqkv_vm, wp, i, tbuf):
        def fwd(rb, c):
            def run(prev):
                c0 = i * D + c * 128
                tt = pltpu.bitcast(wqkv_vm[rb * 256:(rb + 1) * 256, c0:c0 + 128], f32).T
                for hh in range(4):
                    tbuf[rb, pl.ds((4 * c + hh) * TP, DH), :] = tt[hh * DH:(hh + 1) * DH, :]
                return sp.chain([tt], prev, 1)
            return run

        def bwd(rb, j):
            def run(prev):
                g = jnp.concatenate(
                    [tbuf[rb, pl.ds(4 * j + dd, NH, stride=TP), :] for dd in range(4)], axis=0).T
                wp[i, rb * 128:(rb + 1) * 128, j * 128:(j + 1) * 128] = pltpu.bitcast(g, i32)
            return run
        tasks = []
        for rb in range(4):
            tasks += [fwd(rb, c) for c in range(8)] + [bwd(rb, j) for j in range(8)]
        return tasks

    def wo_tasks(wo_vm):
        def stage(c):
            return 4 + c % 4, (c // 4) * NH * TP

        def spread(h0):
            def run(prev):
                blk = wo_vm[h0 * DH:(h0 + 2) * DH, :].astype(f32)
                for h in range(2):
                    for c in range(8):
                        sl, r0 = stage(c)
                        q_s[sl, pl.ds(r0 + (h0 + h) * TP, DH), :] = (
                            blk[h * DH:(h + 1) * DH, c * 128:(c + 1) * 128])
                return sp.chain([blk], prev, 1)
            return run

        def gather(d, h0, c):
            def run(after):
                def blk(k1, k2, n1, n2):
                    sl, r0 = stage(4 * n1 + 2 * n2 + c)
                    r0 += h0 * TP + 16 * k1 + 8 * k2 + d
                    return q_s[sl, pl.ds(r0, 16, stride=TP), :]
                cs, tok = sp.two_level(_b_combos, blk, None, DEPTH2, after)
                r = (d * NH + h0) // 2
                for t in range(49):
                    woc[t, r:r + 8, c * 128:(c + 1) * 128] = cs[t]
                return tok
            return run
        return ([spread(h0) for h0 in range(0, NH, 2)],
                [gather(d, h0, c) for d in range(8) for h0 in (0, 16) for c in range(2)])

    def proj(wp, i, dst, pad, slabs):
        lhs = jnp.concatenate([xn[r0 // 2:(r0 + n) // 2, :] for r0, n in slabs], axis=0)
        p = sp.dot(_unpack(lhs), _unpack(wp[i]))
        at = 0
        for r0, n in slabs:
            for j in range(8):
                dst[j, pad + r0:pad + r0 + n, :] = p[at:at + n, j * 128:(j + 1) * 128]
            at += n

    def v_finish(rb, m):
        cs = _c_combos(m)
        for qd, cc in enumerate(cs):
            r0 = PAD + (qd // 2) * H + rb * RB
            for j in range(4):
                v_s[(qd % 2) * 4 + j, r0:r0 + RB, :] = cc[:, j * 128:(j + 1) * 128]
        if rb == 0:
            for j in range(8):
                src = cs[j // 4][0:1, (j % 4) * 128:(j % 4 + 1) * 128]
                v_s[j, 0:PAD, :] = jnp.broadcast_to(src, (PAD, 128))

    def attn_group(row, masked):
        def run(prev):
            g = 8
            q = [q_s[j, pl.ds(row, g), :] for j in range(8)]
            ls = []
            for w in range(W):
                a = None
                for j in range(8):
                    term = q[j] * k_s[j, pl.ds(row + (PAD - DIL * w), g), :]
                    a = sp.link(ls[-1] if ls else None, term) if a is None else a + term
                ls.append(a)
            rs = [pltpu.roll(a, 64, 1) for a in ls]
            ls = [a + r for a, r in zip(ls, rs)]
            rs = [pltpu.roll(a, 32, 1) for a in ls]
            ls = [a + r for a, r in zip(ls, rs)]
            if masked:
                ri = row + lax.broadcasted_iota(i32, (g, 128), 0)
                ls = [ls[0]] + [jnp.where(ri >= DIL * w, ls[w], NEG) for w in range(1, W)]
            m = _tree(jnp.maximum, ls)
            ps = [jnp.exp2((l - m) * EXP2_SCALE) for l in ls]
            r = gs[pl.ds(row, g), :] / _tree(jnp.add, ps)
            outs = []
            for j in range(8):
                a = None
                for w in range(W):
                    term = ps[w] * v_s[j, pl.ds(row + (PAD - DIL * w), g), :]
                    a = sp.link(outs[-1] if outs else None, term) if a is None else a + term
                outs.append(a * r)
            for j in range(8):
                q_s[j, pl.ds(row, g), :] = outs[j]
            return sp.chain([outs[-1]], prev, 1)
        return run

    def attn_tasks(base, nrows, first=False):
        return [attn_group(base + (qq * Q + r), first and qq == 0 and r < PAD)
                for r in range(0, nrows, 8) for qq in range(4)]

    def pack_tasks(oa, base, hbase, nrows):
        def task(r, c):
            def run(prev, after=None):
                def blk(i1, i2, k1, k2):
                    return q_s[4 * k1 + 2 * k2 + c, pl.ds(base + (i1 * H + i2 * Q + r), 16), :]
                cs, tok = sp.two_level(_a_combos, blk, prev, DEPTH2 if after is None else PDEPTH, after)
                for t in range(49):
                    oa[t, pl.ds(hbase + r // 2, 8), c * 128:(c + 1) * 128] = cs[t]
                return tok
            return run
        return [task(r, c) for r in range(0, nrows, 16) for c in range(2)]

    GS = RB * (KH // 128) * (FC // 128) * 7 // (4 * SLOT)
    DS = 49
    PS = 2 * RB * (D // 128) * (D // 128) // (4 * SLOT)

    def glu(hs, ha):
        def finish(rb, m):
            glu_tasks(hs, rb, _c_combos(m), RB)[0](None)
            if rb >= 2:
                down_lhs(hs, rb - 2, ha)
        return finish

    def raw_first(rbs, n):
        lead = [(rb, t) for rb in rbs[:n] for t in ORDER[:2]]
        return lead + [(rb, t) for rb in rbs for t in ORDER if (rb, t) not in lead]

    def gu_src(j):
        return lambda r, c: wgu[j, r, c]

    def front(wqkv_vm, wp, wo_vm):
        in_q, in_k, in_v = [
            cp(wqkv_hbm.at[:, pl.ds(i * D, D)], wqkv_vm.at[:, pl.ds(i * D, D)], (6, 6, 5)[i])
            for i in range(3)]
        in_wo = cp(wo_hbm, wo_vm, 6)

        def plain(rb, hf, p):
            return sp.dot(x_vm[rows(rb, hf), :], wgu[0, :, p * CH:(p + 1) * CH])

        def plain_finish(rb, c):
            cs = [jnp.concatenate(c[2 * qd:2 * qd + 2], axis=1) for qd in range(4)]
            return glu_tasks(hs, rb, cs, 16)

        hs, bc, dc = {}, {}, {}
        wait(in0)
        start(in3)
        c0 = {(0, 0): plain(0, 0, 0)}
        wait(in1)
        c0[1, 0] = plain(0, 1, 0)
        wait(in2)
        start(in4)
        for hf in range(2):
            c0[hf, 1] = plain(0, hf, 1)
        wait(in3)
        start(in5)
        sp.block()
        bt = b_sum_tasks(gu_src(0), bc)
        sp.schedule(bt[:12], 3, 16)
        sp.schedule(prep_tasks(0, sums=False), 3, 16)
        for p in (2, 3):
            for hf in range(2):
                c0[hf, p] = plain(0, hf, p)
        c0 = [c0[hf, p] for hf in range(2) for p in range(4)]
        wait(in4)
        start([in_v])
        sp.block()
        sp.schedule(bt[12:], 3, 32)
        sp.schedule(prep_tasks(1, sums=False), 2, 10)
        sp.schedule(prep_tasks(2), 10, 32)
        c1 = [plain(1, hf, p) for hf in range(2) for p in range(4)]
        wait(in5 + [in_v])
        start([in_k, in_wo, in_q])
        sp.block()
        for j in range(8):
            k_s[j, 0:PAD, :] = jnp.zeros((PAD, 128), f32)
        ha = {}
        sp.schedule(prep_tasks(3), 2, GS)
        sp.schedule(plain_finish(0, c0), 2, GS)
        sp.schedule(plain_finish(1, c1), GS + 6, 2 * GS)
        sp.schedule(d_tasks(0, dc), GS - 2, 2 * GS)
        sp.schedule(perm_tasks(wqkv_vm, wp, 2, q_s), 2 * GS + 6, 2 * GS + DS - 8)
        strassen_x([(rb, t) for rb in (2, 3) for t in ORDER], b_rhs(gu_src(0), bc),
                   glu(hs, ha))
        ffn_down(ha, dc, True)

        wait([in_k, in_wo, in_q])
        start(in_ffn)
        sp.block()
        vb = {}
        v_src = lambda r, c: _unpack(wp[2, _half(r), c])
        wo_spread, wo_gather = wo_tasks(wo_vm)
        sp.schedule(b_sum_tasks(v_src, vb, VDEPTH), *VBC_SLOTS)
        sp.schedule(prep_tasks(0, gate=False) + prep_tasks(1, gate=False), *PREP01)
        sp.schedule(perm_tasks(wqkv_vm, wp, 1, k_s.at[:, PAD:, :]), *PERMK)
        sp.schedule(wo_spread, *WOS)
        strassen_x(raw_first((2, 3, 0, 1), 2), b_rhs(v_src, vb), v_finish)
        sp.schedule(perm_tasks(wqkv_vm, wp, 0, q_s), 4, 3 * PS)
        tok = None
        for t in wo_gather:
            tok = t(tok)
        for rb in range(NRB):
            proj(wp, 1, k_s, PAD, [(rb * Q, Q)])
        proj(wp, 0, q_s, 0, [(qq * Q, QA) for qq in range(4)])

        def q_rest(_, carry):
            sp.block()
            n = (Q - QA) // 2
            total = 4 * (Q - QA) * 64 // (4 * SLOT)
            sp.schedule(attn_tasks(0, A0, True), 4, total)
            for r0 in (QA, QA + n):
                proj(wp, 0, q_s, 0, [(qq * Q + r0, n) for qq in range(4)])
            return carry

        lax.fori_loop(0, zi[0], q_rest, 0)
        wait(in_ffn)

    def back(oa):
        def body(j, carry):
            sp.block()
            base = pl.multiple_of((j - 1) * AR, AR)
            hs, ha, bc, dc = {}, {}, {}, {}
            sp.schedule(b_sum_tasks(gu_src(j), bc), *BC_SLOTS)
            sp.schedule(attn_tasks(base + A0, AR), *ATTN_SLOTS)
            packs = pack_tasks(oa, base, pl.multiple_of((j - 1) * (AR // 2), AR // 2), AR)
            sp.schedule(d_tasks(j, dc), *DC_SLOTS)
            strassen_x(raw_first((0, 2, 1, 3), NRAW), b_rhs(gu_src(j), bc), glu(hs, ha))
            tok = ha['tok']
            for t in packs:
                tok = t(None, tok)
            ffn_down(ha, dc, False)
            return carry

        lax.fori_loop(1, NC, body, 0)

        def out_copy(r0, i1, i2, cols):
            idx = (pl.ds(r0 + (i1 * H + i2 * Q), PB), cols)
            return cp(x_vm.at[idx], o2.at[idx], out_sem)

        def out_blocks(blocks):
            done_by = {ts[-1]: qd for ts, qd in _C_ORDER}
            todo = [(blk, t1, t2) for blk in range(len(blocks))
                    for ts1, _ in _C_ORDER for t1 in ts1 for ts2, _ in _C_ORDER for t2 in ts2]
            m, inner = {}, {}
            for i in range(0, len(todo), 2):
                pair = todo[i:i + 2]
                ps = sp.dots([(_unpack(oa[7 * t1 + t2, pl.ds(blocks[blk][1], PB // 2), :]),
                               _unpack(woc[7 * t1 + t2])) for blk, t1, t2 in pair])
                for (blk, t1, t2), p in zip(pair, ps):
                    r0, _, copies = blocks[blk]
                    m.setdefault((blk, t1), {})[t2] = acc[7 * t1 + t2, pl.ds(r0, PB), :] + p
                    if t2 not in done_by:
                        continue
                    q2 = done_by[t2] ^ (t1 in _FLIP)
                    inner.setdefault((blk, q2), {})[t1] = _c_quadrant(m[blk, t1], done_by[t2])
                    if t1 not in done_by:
                        continue
                    q1 = done_by[t1]
                    r = pl.ds(r0 + ((q1 // 2) * H + (q2 // 2) * Q), PB)
                    c = (q1 % 2) * KH + (q2 % 2) * KQ
                    x_vm[r, c:c + KQ] = _c_quadrant(inner[blk, q2], q1).astype(bf16)
                    start(copies.get((q1, q2), []))

        final = {q1: (q1, 3 ^ (ts[-1] in _FLIP)) for ts, q1 in _C_ORDER}

        def whole(r0):
            return {final[3]: [out_copy(r0, i1, i2, slice(None))
                               for i1 in range(2) for i2 in range(2)]}

        done = (NC - 1) * AR

        def out_body(i, carry):
            sp.block()
            half = pl.multiple_of(done // 2 + i * 24, 8)
            sp.schedule(pack_tasks(oa, 2 * half, half, 48), *PACK4)
            r0 = pl.multiple_of(i * PB, PB)
            out_blocks([(r0, pl.multiple_of(i * (PB // 2), PB // 2),
                         whole(r0))])
            return carry

        lax.fori_loop(0, 2, out_body, 0)
        sp.block()
        sp.schedule(pack_tasks(oa, done + 96, (done + 96) // 2, Q - done - 96), 4, 22)
        last = {final[q1]: [out_copy(3 * PB, q1 // 2, i2, pl.ds((q1 % 2) * KH, KH))
                            for i2 in range(2)] for q1 in range(3)}
        for q2 in range(4):
            last[3, q2] = [out_copy(3 * PB, 1, q2 // 2, pl.ds(KH + (q2 % 2) * KQ, KQ))]
        copies = [whole(blk * PB) for blk in range(3)] + [last]
        out_blocks([(blk * PB, blk * PB // 2, copies[blk]) for blk in (2, 3)])
        for cs in copies:
            for key in cs:
                wait(cs[key])

    pl.run_scoped(front, pltpu.VMEM((D, 3 * D), bf16), pltpu.VMEM((3, D // 2, D), i32),
                  pltpu.VMEM((D, D), bf16))
    pl.run_scoped(back, pltpu.VMEM((49, Q // 2, KQ), i32))
    assert not sp.plan


_N_SEMS = 9


@jax.jit
def pallas_gated_mix__sliding_local_dilated__glu_gated_reglu__prompt_kernel(
    A_x: jax.Array,
    A_wqkv: jax.Array,
    A_wo: jax.Array,
    B_x: jax.Array,
    B_W_gate: jax.Array,
    B_W_up: jax.Array,
    B_W_down: jax.Array,
    gate_w: jax.Array,
):
    del B_x
    hbm = pl.BlockSpec(memory_space=pl.ANY)
    scratch = [
        pltpu.VMEM((S, D), bf16),
        pltpu.VMEM((S // 2, D), i32),
        pltpu.VMEM((5, H // 2, KH), i32),
        pltpu.VMEM((8, 128), bf16),
        pltpu.VMEM((NC, D, 2 * FC), bf16),
        pltpu.VMEM((NC, FC, D), bf16),
        pltpu.VMEM((49, Q, KQ), f32),
        pltpu.VMEM((8, S + QPAD, 128), f32),
        pltpu.VMEM((8, PAD + S, 128), f32),
        pltpu.VMEM((8, PAD + S, 128), f32),
        pltpu.VMEM((S, 128), f32),
        pltpu.VMEM((49, KQ // 2, KQ), i32),
        pltpu.VMEM((8, 128), i32),
        pltpu.SMEM((1,), i32),
        pltpu.SemaphoreType.DMA((_N_SEMS,)),
    ]
    return pl.pallas_call(
        _kernel,
        in_specs=[hbm] * 7,
        out_specs=hbm,
        out_shape=jax.ShapeDtypeStruct((1, S, D), bf16),
        scratch_shapes=scratch,
        compiler_params=pltpu.CompilerParams(vmem_limit_bytes=124 * 1024 * 1024),
    )(A_x, A_wqkv, A_wo, B_W_gate, B_W_up, B_W_down, gate_w.reshape(8, 128))
```

```python
import math

import jax
import jax.numpy as jnp
from jax import lax
import jax.experimental.pallas as pl
import jax.experimental.pallas.tpu as pltpu

f32 = jnp.float32
bf16 = jnp.bfloat16
i32 = jnp.int32

S = 2048
D = 1024
F = 3584
NH = 32
DH = D // NH
W = 8
DIL = 2
H = S // 2
Q = S // 4
KH = D // 2
KQ = D // 4
FC = 512
CH = FC // 2
CQ = FC // 4
NC = F // FC
RB = 256
NRB = H // RB
PB = 128
PAD = 16
TP = DH + 1
AR = 64
A0 = Q - 6 * AR
QA = 160
QPAD = 112

BC_SLOTS = (2, 24)
ATTN_SLOTS = (24, 106)
DC_SLOTS = (26, 98)
VDEPTH = 2
PDEPTH = 3
VBC_SLOTS = (2, 16)
PREP01 = (16, 56)
PERMK = (64, 106)
WOS = (70, 112)
PACK4 = (4, 24)
NRAW = 3
DEPTH = 3
DEPTH2 = 3
H_DEPTH = 3

SCALE = DH ** -0.5
EXP2_SCALE = SCALE * math.log2(math.e)
NEG = -1e9 / SCALE


def _a_combos(a11, a12, a21, a22):
    return [a11 + a22, a21 + a22, a11, a22, a11 + a12, a21 - a11, a12 - a22]


def _b_combos(b11, b12, b21, b22):
    return [b11 + b22, b11, b12 - b22, b21 - b11, b22, b11 + b12, b21 + b22]


_C_TERMS = (((1, 0), (1, 3), (-1, 4), (1, 6)), ((1, 2), (1, 4)), ((1, 1), (1, 3)),
            ((1, 0), (-1, 1), (1, 2), (1, 5)))
_C_ORDER = (((2, 4), 1), ((1, 3), 2), ((0, 6), 0), ((5,), 3))


def _c_quadrant(m, qd):
    out = m[_C_TERMS[qd][0][1]]
    for sign, t in _C_TERMS[qd][1:]:
        out = out + m[t] if sign > 0 else out - m[t]
    return out


def _c_combos(m):
    return [_c_quadrant(m, qd) for qd in range(4)]


_FLIP = (1, 4, 5, 6)
_A_SLOT = {0: 0, 1: 1, 4: 2, 5: 3, 6: 4}
_B_SUMS = (2, 3, 0, 5, 6)
ORDER = (1, 4) + _B_SUMS


def _tree(op, xs):
    xs = list(xs)
    while len(xs) > 1:
        xs = [op(xs[i], xs[i + 1]) if i + 1 < len(xs) else xs[i] for i in range(0, len(xs), 2)]
    return xs[0]


def _pack(x):
    return pltpu.bitcast(x.astype(bf16), i32)


def _unpack(x):
    return pltpu.bitcast(x, bf16)


def _half(r):
    return slice(r.start // 2, r.stop // 2)


SLOT = 256


class _Spreader:
    def __init__(self, zero_ref):
        self.zero_ref = zero_ref
        self.plan = {}
        self.lists = 0
        self.now = 0

    def block(self):
        self.zero = self.zero_ref[...]
        self.never = self.zero != 0

    def link(self, after, x):
        if after is None:
            return x
        if after.dtype != x.dtype:
            after = pltpu.bitcast(after, x.dtype)
        return jnp.where(self.never, after, x)

    def chain(self, vals, prev, depth):
        for v in vals:
            v = pltpu.bitcast(v, i32) if v.dtype != i32 else v
            for r in range(0, v.shape[0], 8):
                for c in range(0, v.shape[1], 128):
                    tile = v[r:r + 8, c:c + 128]
                    if prev is None:
                        prev = tile
                        continue
                    prev = prev | tile
                    for i in range(depth - 1):
                        prev = (prev + self.zero) if i % 2 == 0 else (prev ^ self.zero)
        return prev

    def link_rows(self, after, x):
        return jnp.concatenate([self.link(after, x[r:r + 8, :]) for r in range(0, x.shape[0], 8)],
                               axis=0)

    def serial_combos(self, combos, x11, x12, x21, x22, after):
        return combos(self.link_rows(after, x11), x12, x21, self.link_rows(after, x22))

    def two_level(self, combos, blk, prev, depth, after=None):
        outer, outs, tok = [], [], after
        for r2 in range(2):
            for c2 in range(2):
                outer.append(self.serial_combos(
                    combos, *[blk(r1, r2, c1, c2) for r1 in range(2) for c1 in range(2)], tok))
                tok = self.chain([x[:8] for x in outer[-1]], None, 1)
        for t in range(7):
            flip = combos is _b_combos and t in _FLIP
            wide = _pack(jnp.concatenate(
                self.serial_combos(combos, *[outer[i ^ flip][t] for i in range(4)], tok), axis=1))
            outs += [wide[:, c:c + 128] for c in range(0, 7 * 128, 128)]
            tok = self.chain(outs[-7:], tok, depth)
        return outs, self.chain([tok], prev, 1)

    def schedule(self, tasks, first, last):
        self.lists += 1
        for i, t in enumerate(tasks):
            pos = self.now + first + ((i + 1) * (last - first) - 1) // len(tasks)
            self.plan.setdefault(pos, []).append((t, self.lists))

    def dots(self, pairs):
        m = pairs[0][0].shape[0]
        tiles = [(i, r, c) for i, (_, rhs) in enumerate(pairs)
                 for c in range(0, rhs.shape[1], 128) for r in range(0, rhs.shape[0], 128)]
        nslots = m * len(tiles) // (4 * SLOT)
        deps = {}
        for sl in range(nslots):
            ps = sl * SLOT // m
            toks = {}
            for t, lane in self.plan.pop(self.now + sl, []):
                tok = t(toks.get(lane))
                if tok is not None:
                    toks[lane] = tok
            for tok in toks.values():
                deps[ps] = tok | deps[ps] if ps in deps else tok
        self.now += nslots
        tied = {tile: d for ps, d in deps.items() for tile in tiles[4 * ps:4 * ps + 4]}
        outs = []
        for i, (lhs, rhs) in enumerate(pairs):
            if any(key[0] == i for key in tied):
                parts = []
                for r in range(0, rhs.shape[0], 128):
                    top = [rhs[r:r + 16, c:c + 128] for c in range(0, rhs.shape[1], 128)]
                    top = [_unpack(self.link(tied[i, r, c * 128], _pack(t0)))
                           if (i, r, c * 128) in tied else t0 for c, t0 in enumerate(top)]
                    parts += [jnp.concatenate(top, axis=1), rhs[r + 16:r + 128, :]]
                rhs = jnp.concatenate(parts, axis=0)
            outs.append(jnp.dot(lhs, rhs, preferred_element_type=f32))
        return outs

    def dot(self, lhs, rhs):
        return self.dots([(lhs, rhs)])[0]


def _kernel(x_hbm, wqkv_hbm, wo_hbm, wg_hbm, wu_hbm, wd_hbm, gw_hbm, out_hbm,
            x_vm, xn, xa, gw_vm, wgu, wd, acc, q_s, k_s, v_s, gs, woc, zs, zi, sems):
    def cp(src, dst, sem):
        return pltpu.make_async_copy(src, dst, sems.at[sem])

    def cp_gu(j, p, sem):
        return cp((wg_hbm, wu_hbm)[p % 2].at[:, pl.ds(j * FC + (p // 2) * CH, CH)],
                  wgu.at[j, :, pl.ds(p * CH, CH)], sem)

    def cp_d(j, sem):
        return cp(wd_hbm.at[pl.ds(j * FC, FC), :], wd.at[j], sem)

    def cp_x(rb, hf, sem):
        idx = (pl.ds(hf * H + rb * RB, RB), slice(None))
        return cp(x_hbm.at[0].at[idx], x_vm.at[idx], sem)

    o2 = out_hbm.at[0]
    in0 = [cp_x(0, 0, 0), cp_gu(0, 0, 0)]
    in1 = [cp_x(0, 1, 1)]
    in2 = [cp_gu(0, 1, 2)]
    in3 = [cp_gu(0, 2, 3), cp_gu(0, 3, 3), cp(gw_hbm, gw_vm, 3)]
    in4 = [cp_x(rb, hf, 4) for rb in (1, 2) for hf in range(2)]
    in5 = [cp_x(3, 0, 5), cp_x(3, 1, 5), cp_d(0, 5)]
    in_ffn = [c for j in range(1, NC) for c in [cp_gu(j, p, 7) for p in range(4)] + [cp_d(j, 7)]]
    out_sem = 8

    def start(cs):
        for c in cs:
            c.start()

    def wait(cs):
        for c in cs:
            c.wait()

    start(in0 + in1 + in2)

    zs[...] = jnp.zeros((8, 128), i32)
    zi[0] = 1
    sp = _Spreader(zs)

    def rows(rb, hf=0):
        return slice(hf * H + rb * RB, hf * H + (rb + 1) * RB)

    def x_lhs(t, rb):
        if t == 2:
            return _unpack(xn[_half(rows(rb, 0)), :KH])
        if t == 3:
            return _unpack(xn[_half(rows(rb, 1)), KH:])
        return _unpack(xa[_A_SLOT[t], _half(rows(rb)), :])

    def prep_tasks(rb, sums=True, gate=True):
        def task(s0):
            def run(first):
                prev = None
                gw = gw_vm[...].astype(f32)
                r = [slice(hf * H + rb * RB + s0, hf * H + rb * RB + s0 + 16) for hf in range(2)]
                z = [None, None]
                for c in range(4):
                    cols = [slice(kh * KH + c * 128, kh * KH + (c + 1) * 128) for kh in range(2)]
                    xs = [sp.link(prev, _pack(x_vm[r[qd // 2], cols[qd % 2]])) for qd in range(4)]
                    a = [_unpack(t).astype(f32) for t in xs]
                    outs = []
                    if sums:
                        for qd in range(4):
                            xn[_half(r[qd // 2]), cols[qd % 2]] = xs[qd]
                        cs = _a_combos(*a)
                        for t, slot in _A_SLOT.items():
                            outs.append(_pack(cs[t]))
                            xa[slot, _half(r[0]), cols[0]] = outs[-1]
                    if gate:
                        for qd in range(4):
                            g0 = (qd % 2) * 4 + c
                            term = a[qd] * gw[g0:g0 + 1, :]
                            z[qd // 2] = term if z[qd // 2] is None else z[qd // 2] + term
                        outs += z
                    prev = sp.chain(outs, prev, 1)
                if gate:
                    for hf in range(2):
                        g = jax.nn.sigmoid(jnp.sum(z[hf], axis=1, keepdims=True))
                        g = jnp.broadcast_to(g, (16, 128))
                        gs[r[hf], :] = g
                        prev = sp.chain([g], prev, 1)
                return sp.chain([prev], first, 1)
            return run
        return [task(s0) for s0 in range(0, RB, 16)]

    def b_sum_tasks(src, dst, depth=DEPTH):
        def task(r0):
            def run(prev):
                raw = [src(slice(a * KH + r0, a * KH + r0 + 16), slice(c * KH, (c + 1) * KH))
                       for a in range(2) for c in range(2)]
                cs = _b_combos(*[b.astype(f32) for b in raw])
                for t in _B_SUMS:
                    dst.setdefault(t, []).append(_pack(cs[t]))
                return sp.chain([dst[t][-1] for t in _B_SUMS], prev, depth)
            return run
        return [task(r0) for r0 in range(0, KH, 16)]

    def b_rhs(src, sums):
        def rhs(t):
            if t == 1:
                return src(slice(0, KH), slice(0, KH))
            if t == 4:
                return src(slice(KH, D), slice(KH, D))
            return _unpack(jnp.concatenate(sums[t], axis=0))
        return rhs

    def strassen_x(order, rhs, finish):
        m = {}
        for rb, t in order:
            m.setdefault(rb, {})[t] = sp.dot(x_lhs(t, rb), rhs(t))
            if len(m[rb]) == 7:
                finish(rb, m.pop(rb))

    def h_sums(rb, cs, r0, sub):
        h = []
        for qd, cc in enumerate(cs):
            g0 = (qd // 2) * H + rb * RB + r0
            omg = 1.0 - gs[g0:g0 + sub, :]
            omg = jnp.concatenate([omg] * (CH // 128), axis=1)
            h.append(jnp.maximum(cc[:, :CH], 0.0) * cc[:, CH:] * omg)
        return _a_combos(*h)

    def glu_tasks(hs, rb, cs, sub):
        hs[rb] = [[] for _ in range(7)]

        def task(r0):
            def run(prev):
                sums = h_sums(rb, [cc[r0:r0 + sub] for cc in cs], r0, sub)
                for t in range(7):
                    hs[rb][t].append(sums[t])
                if sub < RB:
                    return sp.chain([sums[t] for t in _A_SLOT], prev, DEPTH2)
            return run
        return [task(r0) for r0 in range(0, RB, sub)]

    def down_lhs(hs, b, ha):
        tok = None
        for t in range(7):
            s0, s1 = [jnp.concatenate(hs[rb][t], axis=0) for rb in (b, b + 2)]
            slabs = []
            for r in range(0, RB, 16):
                slabs.append(sp.serial_combos(
                    _a_combos, s0[r:r + 16, :CQ], s0[r:r + 16, CQ:],
                    s1[r:r + 16, :CQ], s1[r:r + 16, CQ:], tok))
                tok = sp.chain([slabs[-1][t2] for t2 in _A_SLOT], None, H_DEPTH)
            for t2 in range(7):
                ha[b, 7 * t + t2] = jnp.concatenate([sl[t2] for sl in slabs], axis=0).astype(bf16)
        ha['tok'] = tok

    def d_tasks(j, dst):
        def task(r0, c):
            def run(prev):
                def blk(k1, k2, n1, n2):
                    r, c0 = k1 * CH + k2 * CQ + r0, n1 * KH + n2 * KQ + c * 128
                    return wd[j, r:r + 16, c0:c0 + 128].astype(f32)
                cs, tok = sp.two_level(_b_combos, blk, prev, DEPTH2)
                for t in range(49):
                    dst.setdefault((t, c), []).append(cs[t])
                return tok
            return run
        return [task(r0, c) for r0 in range(0, CQ, 16) for c in range(2)]

    def ffn_down(ha, dc, first):
        rhs = [_unpack(jnp.concatenate([jnp.concatenate(dc[t, c], axis=0) for c in range(2)], axis=1))
               for t in range(49)]
        todo = [(b, t) for b in range(2) for t in range(49)]
        for i in range(0, len(todo), 2):
            pair = todo[i:i + 2]
            ps = sp.dots([(ha[b, t], rhs[t]) for b, t in pair])
            for (b, t), p in zip(pair, ps):
                if first:
                    acc[t, b * RB:(b + 1) * RB, :] = p
                else:
                    acc[t, b * RB:(b + 1) * RB, :] += p

    def perm_tasks(wqkv_vm, wp, i, tbuf):
        def fwd(rb, c):
            def run(prev):
                c0 = i * D + c * 128
                tt = pltpu.bitcast(wqkv_vm[rb * 256:(rb + 1) * 256, c0:c0 + 128], f32).T
                for hh in range(4):
                    tbuf[rb, pl.ds((4 * c + hh) * TP, DH), :] = tt[hh * DH:(hh + 1) * DH, :]
                return sp.chain([tt], prev, 1)
            return run

        def bwd(rb, j):
            def run(prev):
                g = jnp.concatenate(
                    [tbuf[rb, pl.ds(4 * j + dd, NH, stride=TP), :] for dd in range(4)], axis=0).T
                wp[i, rb * 128:(rb + 1) * 128, j * 128:(j + 1) * 128] = pltpu.bitcast(g, i32)
            return run
        tasks = []
        for rb in range(4):
            tasks += [fwd(rb, c) for c in range(8)] + [bwd(rb, j) for j in range(8)]
        return tasks

    def wo_tasks(wo_vm):
        def stage(c):
            return 4 + c % 4, (c // 4) * NH * TP

        def spread(h0):
            def run(prev):
                blk = wo_vm[h0 * DH:(h0 + 2) * DH, :].astype(f32)
                for h in range(2):
                    for c in range(8):
                        sl, r0 = stage(c)
                        q_s[sl, pl.ds(r0 + (h0 + h) * TP, DH), :] = (
                            blk[h * DH:(h + 1) * DH, c * 128:(c + 1) * 128])
                return sp.chain([blk], prev, 1)
            return run

        def gather(d, h0, c):
            def run(after):
                def blk(k1, k2, n1, n2):
                    sl, r0 = stage(4 * n1 + 2 * n2 + c)
                    r0 += h0 * TP + 16 * k1 + 8 * k2 + d
                    return q_s[sl, pl.ds(r0, 16, stride=TP), :]
                cs, tok = sp.two_level(_b_combos, blk, None, DEPTH2, after)
                r = (d * NH + h0) // 2
                for t in range(49):
                    woc[t, r:r + 8, c * 128:(c + 1) * 128] = cs[t]
                return tok
            return run
        return ([spread(h0) for h0 in range(0, NH, 2)],
                [gather(d, h0, c) for d in range(8) for h0 in (0, 16) for c in range(2)])

    def proj(wp, i, dst, pad, slabs):
        lhs = jnp.concatenate([xn[r0 // 2:(r0 + n) // 2, :] for r0, n in slabs], axis=0)
        p = sp.dot(_unpack(lhs), _unpack(wp[i]))
        at = 0
        for r0, n in slabs:
            for j in range(8):
                dst[j, pad + r0:pad + r0 + n, :] = p[at:at + n, j * 128:(j + 1) * 128]
            at += n

    def v_finish(rb, m):
        cs = _c_combos(m)
        for qd, cc in enumerate(cs):
            r0 = PAD + (qd // 2) * H + rb * RB
            for j in range(4):
                v_s[(qd % 2) * 4 + j, r0:r0 + RB, :] = cc[:, j * 128:(j + 1) * 128]
        if rb == 0:
            for j in range(8):
                src = cs[j // 4][0:1, (j % 4) * 128:(j % 4 + 1) * 128]
                v_s[j, 0:PAD, :] = jnp.broadcast_to(src, (PAD, 128))

    def attn_group(row, masked):
        def run(prev):
            g = 8
            q = [q_s[j, pl.ds(row, g), :] for j in range(8)]
            ls = []
            for w in range(W):
                a = None
                for j in range(8):
                    term = q[j] * k_s[j, pl.ds(row + (PAD - DIL * w), g), :]
                    a = sp.link(ls[-1] if ls else None, term) if a is None else a + term
                ls.append(a)
            rs = [pltpu.roll(a, 64, 1) for a in ls]
            ls = [a + r for a, r in zip(ls, rs)]
            rs = [pltpu.roll(a, 32, 1) for a in ls]
            ls = [a + r for a, r in zip(ls, rs)]
            if masked:
                ri = row + lax.broadcasted_iota(i32, (g, 128), 0)
                ls = [ls[0]] + [jnp.where(ri >= DIL * w, ls[w], NEG) for w in range(1, W)]
            m = _tree(jnp.maximum, ls)
            ps = [jnp.exp2((l - m) * EXP2_SCALE) for l in ls]
            r = gs[pl.ds(row, g), :] / _tree(jnp.add, ps)
            outs = []
            for j in range(8):
                a = None
                for w in range(W):
                    term = ps[w] * v_s[j, pl.ds(row + (PAD - DIL * w), g), :]
                    a = sp.link(outs[-1] if outs else None, term) if a is None else a + term
                outs.append(a * r)
            for j in range(8):
                q_s[j, pl.ds(row, g), :] = outs[j]
            return sp.chain([outs[-1]], prev, 1)
        return run

    def attn_tasks(base, nrows, first=False):
        return [attn_group(base + (qq * Q + r), first and qq == 0 and r < PAD)
                for r in range(0, nrows, 8) for qq in range(4)]

    def pack_tasks(oa, base, hbase, nrows):
        def task(r, c):
            def run(prev, after=None):
                def blk(i1, i2, k1, k2):
                    return q_s[4 * k1 + 2 * k2 + c, pl.ds(base + (i1 * H + i2 * Q + r), 16), :]
                cs, tok = sp.two_level(_a_combos, blk, prev, DEPTH2 if after is None else PDEPTH, after)
                for t in range(49):
                    oa[t, pl.ds(hbase + r // 2, 8), c * 128:(c + 1) * 128] = cs[t]
                return tok
            return run
        return [task(r, c) for r in range(0, nrows, 16) for c in range(2)]

    GS = RB * (KH // 128) * (FC // 128) * 7 // (4 * SLOT)
    DS = 49
    PS = 2 * RB * (D // 128) * (D // 128) // (4 * SLOT)

    def glu(hs, ha):
        def finish(rb, m):
            glu_tasks(hs, rb, _c_combos(m), RB)[0](None)
            if rb >= 2:
                down_lhs(hs, rb - 2, ha)
        return finish

    def raw_first(rbs, n):
        lead = [(rb, t) for rb in rbs[:n] for t in ORDER[:2]]
        return lead + [(rb, t) for rb in rbs for t in ORDER if (rb, t) not in lead]

    def gu_src(j):
        return lambda r, c: wgu[j, r, c]

    def front(wqkv_vm, wp, wo_vm):
        in_q, in_k, in_v = [
            cp(wqkv_hbm.at[:, pl.ds(i * D, D)], wqkv_vm.at[:, pl.ds(i * D, D)], (6, 6, 5)[i])
            for i in range(3)]
        in_wo = cp(wo_hbm, wo_vm, 6)

        def plain(rb, hf, p):
            return sp.dot(x_vm[rows(rb, hf), :], wgu[0, :, p * CH:(p + 1) * CH])

        def plain_finish(rb, c):
            cs = [jnp.concatenate(c[2 * qd:2 * qd + 2], axis=1) for qd in range(4)]
            return glu_tasks(hs, rb, cs, 16)

        hs, bc, dc = {}, {}, {}
        wait(in0)
        start(in3)
        c0 = {(0, 0): plain(0, 0, 0)}
        wait(in1)
        c0[1, 0] = plain(0, 1, 0)
        wait(in2)
        start(in4)
        for hf in range(2):
            c0[hf, 1] = plain(0, hf, 1)
        wait(in3)
        start(in5)
        sp.block()
        bt = b_sum_tasks(gu_src(0), bc)
        sp.schedule(bt[:12], 3, 16)
        sp.schedule(prep_tasks(0, sums=False), 3, 16)
        for p in (2, 3):
            for hf in range(2):
                c0[hf, p] = plain(0, hf, p)
        c0 = [c0[hf, p] for hf in range(2) for p in range(4)]
        wait(in4)
        start([in_v])
        sp.block()
        sp.schedule(bt[12:], 3, 32)
        sp.schedule(prep_tasks(1, sums=False), 2, 10)
        sp.schedule(prep_tasks(2), 10, 32)
        c1 = [plain(1, hf, p) for hf in range(2) for p in range(4)]
        wait(in5 + [in_v])
        start([in_k, in_wo, in_q])
        sp.block()
        for j in range(8):
            k_s[j, 0:PAD, :] = jnp.zeros((PAD, 128), f32)
        ha = {}
        sp.schedule(prep_tasks(3), 2, GS)
        sp.schedule(plain_finish(0, c0), 2, GS)
        sp.schedule(plain_finish(1, c1), GS + 6, 2 * GS)
        sp.schedule(d_tasks(0, dc), GS - 2, 2 * GS)
        sp.schedule(perm_tasks(wqkv_vm, wp, 2, q_s), 2 * GS + 6, 2 * GS + DS - 8)
        strassen_x([(rb, t) for rb in (2, 3) for t in ORDER], b_rhs(gu_src(0), bc),
                   glu(hs, ha))
        ffn_down(ha, dc, True)

        wait([in_k, in_wo, in_q])
        start(in_ffn)
        sp.block()
        vb = {}
        v_src = lambda r, c: _unpack(wp[2, _half(r), c])
        wo_spread, wo_gather = wo_tasks(wo_vm)
        sp.schedule(b_sum_tasks(v_src, vb, VDEPTH), *VBC_SLOTS)
        sp.schedule(prep_tasks(0, gate=False) + prep_tasks(1, gate=False), *PREP01)
        sp.schedule(perm_tasks(wqkv_vm, wp, 1, k_s.at[:, PAD:, :]), *PERMK)
        sp.schedule(wo_spread, *WOS)
        strassen_x(raw_first((2, 3, 0, 1), 2), b_rhs(v_src, vb), v_finish)
        sp.schedule(perm_tasks(wqkv_vm, wp, 0, q_s), 4, 3 * PS)
        tok = None
        for t in wo_gather:
            tok = t(tok)
        for rb in range(NRB):
            proj(wp, 1, k_s, PAD, [(rb * Q, Q)])
        proj(wp, 0, q_s, 0, [(qq * Q, QA) for qq in range(4)])

        def q_rest(_, carry):
            sp.block()
            n = (Q - QA) // 2
            total = 4 * (Q - QA) * 64 // (4 * SLOT)
            sp.schedule(attn_tasks(0, A0, True), 4, total)
            for r0 in (QA, QA + n):
                proj(wp, 0, q_s, 0, [(qq * Q + r0, n) for qq in range(4)])
            return carry

        lax.fori_loop(0, zi[0], q_rest, 0)
        wait(in_ffn)

    def back(oa):
        def body(j, carry):
            sp.block()
            base = pl.multiple_of((j - 1) * AR, AR)
            hs, ha, bc, dc = {}, {}, {}, {}
            sp.schedule(b_sum_tasks(gu_src(j), bc), *BC_SLOTS)
            sp.schedule(attn_tasks(base + A0, AR), *ATTN_SLOTS)
            packs = pack_tasks(oa, base, pl.multiple_of((j - 1) * (AR // 2), AR // 2), AR)
            sp.schedule(d_tasks(j, dc), *DC_SLOTS)
            strassen_x(raw_first((0, 2, 1, 3), NRAW), b_rhs(gu_src(j), bc), glu(hs, ha))
            tok = ha['tok']
            for t in packs:
                tok = t(None, tok)
            ffn_down(ha, dc, False)
            return carry

        lax.fori_loop(1, NC, body, 0)

        def out_copy(r0, i1, i2, cols):
            idx = (pl.ds(r0 + (i1 * H + i2 * Q), PB), cols)
            return cp(x_vm.at[idx], o2.at[idx], out_sem)

        def out_blocks(blocks):
            done_by = {ts[-1]: qd for ts, qd in _C_ORDER}
            todo = [(blk, t1, t2) for blk in range(len(blocks))
                    for ts1, _ in _C_ORDER for t1 in ts1 for ts2, _ in _C_ORDER for t2 in ts2]
            m, inner = {}, {}
            for i in range(0, len(todo), 2):
                pair = todo[i:i + 2]
                ps = sp.dots([(_unpack(oa[7 * t1 + t2, pl.ds(blocks[blk][1], PB // 2), :]),
                               _unpack(woc[7 * t1 + t2])) for blk, t1, t2 in pair])
                for (blk, t1, t2), p in zip(pair, ps):
                    r0, _, copies = blocks[blk]
                    m.setdefault((blk, t1), {})[t2] = acc[7 * t1 + t2, pl.ds(r0, PB), :] + p
                    if t2 not in done_by:
                        continue
                    q2 = done_by[t2] ^ (t1 in _FLIP)
                    inner.setdefault((blk, q2), {})[t1] = _c_quadrant(m[blk, t1], done_by[t2])
                    if t1 not in done_by:
                        continue
                    q1 = done_by[t1]
                    r = pl.ds(r0 + ((q1 // 2) * H + (q2 // 2) * Q), PB)
                    c = (q1 % 2) * KH + (q2 % 2) * KQ
                    x_vm[r, c:c + KQ] = _c_quadrant(inner[blk, q2], q1).astype(bf16)
                    start(copies.get((q1, q2), []))

        final = {q1: (q1, 3 ^ (ts[-1] in _FLIP)) for ts, q1 in _C_ORDER}

        def whole(r0):
            return {final[3]: [out_copy(r0, i1, i2, slice(None))
                               for i1 in range(2) for i2 in range(2)]}

        done = (NC - 1) * AR

        def out_body(i, carry):
            sp.block()
            half = pl.multiple_of(done // 2 + i * 24, 8)
            sp.schedule(pack_tasks(oa, 2 * half, half, 48), *PACK4)
            r0 = pl.multiple_of(i * PB, PB)
            out_blocks([(r0, pl.multiple_of(i * (PB // 2), PB // 2),
                         whole(r0))])
            return carry

        lax.fori_loop(0, 2, out_body, 0)
        sp.block()
        sp.schedule(pack_tasks(oa, done + 96, (done + 96) // 2, Q - done - 96), 4, 22)
        last = {final[q1]: [out_copy(3 * PB, q1 // 2, i2, pl.ds((q1 % 2) * KH, KH))
                            for i2 in range(2)] for q1 in range(3)}
        for q2 in range(4):
            last[3, q2] = [out_copy(3 * PB, 1, q2 // 2, pl.ds(KH + (q2 % 2) * KQ, KQ))]
        copies = [whole(blk * PB) for blk in range(3)] + [last]
        out_blocks([(blk * PB, blk * PB // 2, copies[blk]) for blk in (2, 3)])
        for cs in copies:
            for key in cs:
                wait(cs[key])

    pl.run_scoped(front, pltpu.VMEM((D, 3 * D), bf16), pltpu.VMEM((3, D // 2, D), i32),
                  pltpu.VMEM((D, D), bf16))
    pl.run_scoped(back, pltpu.VMEM((49, Q // 2, KQ), i32))
    assert not sp.plan


_N_SEMS = 9


@jax.jit
def pallas_gated_mix__sliding_local_dilated__glu_gated_reglu__prompt_kernel(
    A_x: jax.Array,
    A_wqkv: jax.Array,
    A_wo: jax.Array,
    B_x: jax.Array,
    B_W_gate: jax.Array,
    B_W_up: jax.Array,
    B_W_down: jax.Array,
    gate_w: jax.Array,
):
    del B_x
    hbm = pl.BlockSpec(memory_space=pl.ANY)
    scratch = [
        pltpu.VMEM((S, D), bf16),
        pltpu.VMEM((S // 2, D), i32),
        pltpu.VMEM((5, H // 2, KH), i32),
        pltpu.VMEM((8, 128), bf16),
        pltpu.VMEM((NC, D, 2 * FC), bf16),
        pltpu.VMEM((NC, FC, D), bf16),
        pltpu.VMEM((49, Q, KQ), f32),
        pltpu.VMEM((8, S + QPAD, 128), f32),
        pltpu.VMEM((8, PAD + S, 128), f32),
        pltpu.VMEM((8, PAD + S, 128), f32),
        pltpu.VMEM((S, 128), f32),
        pltpu.VMEM((49, KQ // 2, KQ), i32),
        pltpu.VMEM((8, 128), i32),
        pltpu.SMEM((1,), i32),
        pltpu.SemaphoreType.DMA((_N_SEMS,)),
    ]
    return pl.pallas_call(
        _kernel,
        in_specs=[hbm] * 7,
        out_specs=hbm,
        out_shape=jax.ShapeDtypeStruct((1, S, D), bf16),
        scratch_shapes=scratch,
        compiler_params=pltpu.CompilerParams(vmem_limit_bytes=124 * 1024 * 1024),
    )(A_x, A_wqkv, A_wo, B_W_gate, B_W_up, B_W_down, gate_w.reshape(8, 128))
```

```python
import math

import jax
import jax.numpy as jnp
from jax import lax
import jax.experimental.pallas as pl
import jax.experimental.pallas.tpu as pltpu

f32 = jnp.float32
bf16 = jnp.bfloat16
i32 = jnp.int32

S = 2048
D = 1024
F = 3584
NH = 32
DH = D // NH
W = 8
DIL = 2
H = S // 2
Q = S // 4
KH = D // 2
KQ = D // 4
FC = 512
CH = FC // 2
CQ = FC // 4
NC = F // FC
RB = 256
NRB = H // RB
PB = 128
PAD = 16
TP = DH + 1
AR = 64
A0 = Q - 6 * AR
QA = 160
QPAD = 112

BC_SLOTS = (2, 24)
ATTN_SLOTS = (24, 106)
DC_SLOTS = (26, 98)
VDEPTH = 2
PDEPTH = 3
VBC_SLOTS = (2, 16)
PREP01 = (16, 56)
PERMK = (64, 106)
WOS = (70, 112)
PACK4 = (4, 48)
NRAW = 3
DEPTH = 3
DEPTH2 = 3
H_DEPTH = 3

SCALE = DH ** -0.5
EXP2_SCALE = SCALE * math.log2(math.e)
NEG = -1e9 / SCALE


def _a_combos(a11, a12, a21, a22):
    return [a11 + a22, a21 + a22, a11, a22, a11 + a12, a21 - a11, a12 - a22]


def _b_combos(b11, b12, b21, b22):
    return [b11 + b22, b11, b12 - b22, b21 - b11, b22, b11 + b12, b21 + b22]


_C_TERMS = (((1, 0), (1, 3), (-1, 4), (1, 6)), ((1, 2), (1, 4)), ((1, 1), (1, 3)),
            ((1, 0), (-1, 1), (1, 2), (1, 5)))
_C_ORDER = (((2, 4), 1), ((1, 3), 2), ((0, 6), 0), ((5,), 3))


def _c_quadrant(m, qd):
    out = m[_C_TERMS[qd][0][1]]
    for sign, t in _C_TERMS[qd][1:]:
        out = out + m[t] if sign > 0 else out - m[t]
    return out


def _c_combos(m):
    return [_c_quadrant(m, qd) for qd in range(4)]


_FLIP = (1, 4, 5, 6)
_A_SLOT = {0: 0, 1: 1, 4: 2, 5: 3, 6: 4}
_B_SUMS = (2, 3, 0, 5, 6)
ORDER = (1, 4) + _B_SUMS


def _tree(op, xs):
    xs = list(xs)
    while len(xs) > 1:
        xs = [op(xs[i], xs[i + 1]) if i + 1 < len(xs) else xs[i] for i in range(0, len(xs), 2)]
    return xs[0]


def _pack(x):
    return pltpu.bitcast(x.astype(bf16), i32)


def _unpack(x):
    return pltpu.bitcast(x, bf16)


def _half(r):
    return slice(r.start // 2, r.stop // 2)


SLOT = 256


class _Spreader:
    def __init__(self, zero_ref):
        self.zero_ref = zero_ref
        self.plan = {}
        self.lists = 0
        self.now = 0

    def block(self):
        self.zero = self.zero_ref[...]
        self.never = self.zero != 0

    def link(self, after, x):
        if after is None:
            return x
        if after.dtype != x.dtype:
            after = pltpu.bitcast(after, x.dtype)
        return jnp.where(self.never, after, x)

    def chain(self, vals, prev, depth):
        for v in vals:
            v = pltpu.bitcast(v, i32) if v.dtype != i32 else v
            for r in range(0, v.shape[0], 8):
                for c in range(0, v.shape[1], 128):
                    tile = v[r:r + 8, c:c + 128]
                    if prev is None:
                        prev = tile
                        continue
                    prev = prev | tile
                    for i in range(depth - 1):
                        prev = (prev + self.zero) if i % 2 == 0 else (prev ^ self.zero)
        return prev

    def link_rows(self, after, x):
        return jnp.concatenate([self.link(after, x[r:r + 8, :]) for r in range(0, x.shape[0], 8)],
                               axis=0)

    def serial_combos(self, combos, x11, x12, x21, x22, after):
        return combos(self.link_rows(after, x11), x12, x21, self.link_rows(after, x22))

    def two_level(self, combos, blk, prev, depth, after=None):
        outer, outs, tok = [], [], after
        for r2 in range(2):
            for c2 in range(2):
                outer.append(self.serial_combos(
                    combos, *[blk(r1, r2, c1, c2) for r1 in range(2) for c1 in range(2)], tok))
                tok = self.chain([x[:8] for x in outer[-1]], None, 1)
        for t in range(7):
            flip = combos is _b_combos and t in _FLIP
            wide = _pack(jnp.concatenate(
                self.serial_combos(combos, *[outer[i ^ flip][t] for i in range(4)], tok), axis=1))
            outs += [wide[:, c:c + 128] for c in range(0, 7 * 128, 128)]
            tok = self.chain(outs[-7:], tok, depth)
        return outs, self.chain([tok], prev, 1)

    def schedule(self, tasks, first, last):
        self.lists += 1
        for i, t in enumerate(tasks):
            pos = self.now + first + ((i + 1) * (last - first) - 1) // len(tasks)
            self.plan.setdefault(pos, []).append((t, self.lists))

    def dots(self, pairs):
        m = pairs[0][0].shape[0]
        tiles = [(i, r, c) for i, (_, rhs) in enumerate(pairs)
                 for c in range(0, rhs.shape[1], 128) for r in range(0, rhs.shape[0], 128)]
        nslots = m * len(tiles) // (4 * SLOT)
        deps = {}
        for sl in range(nslots):
            ps = sl * SLOT // m
            toks = {}
            for t, lane in self.plan.pop(self.now + sl, []):
                tok = t(toks.get(lane))
                if tok is not None:
                    toks[lane] = tok
            for tok in toks.values():
                deps[ps] = tok | deps[ps] if ps in deps else tok
        self.now += nslots
        tied = {tile: d for ps, d in deps.items() for tile in tiles[4 * ps:4 * ps + 4]}
        outs = []
        for i, (lhs, rhs) in enumerate(pairs):
            if any(key[0] == i for key in tied):
                parts = []
                for r in range(0, rhs.shape[0], 128):
                    top = [rhs[r:r + 16, c:c + 128] for c in range(0, rhs.shape[1], 128)]
                    top = [_unpack(self.link(tied[i, r, c * 128], _pack(t0)))
                           if (i, r, c * 128) in tied else t0 for c, t0 in enumerate(top)]
                    parts += [jnp.concatenate(top, axis=1), rhs[r + 16:r + 128, :]]
                rhs = jnp.concatenate(parts, axis=0)
            outs.append(jnp.dot(lhs, rhs, preferred_element_type=f32))
        return outs

    def dot(self, lhs, rhs):
        return self.dots([(lhs, rhs)])[0]


def _kernel(x_hbm, wqkv_hbm, wo_hbm, wg_hbm, wu_hbm, wd_hbm, gw_hbm, out_hbm,
            x_vm, xn, xa, gw_vm, wgu, wd, acc, q_s, k_s, v_s, gs, woc, zs, zi, sems):
    def cp(src, dst, sem):
        return pltpu.make_async_copy(src, dst, sems.at[sem])

    def cp_gu(j, p, sem):
        return cp((wg_hbm, wu_hbm)[p % 2].at[:, pl.ds(j * FC + (p // 2) * CH, CH)],
                  wgu.at[j, :, pl.ds(p * CH, CH)], sem)

    def cp_d(j, sem):
        return cp(wd_hbm.at[pl.ds(j * FC, FC), :], wd.at[j], sem)

    def cp_x(rb, hf, sem):
        idx = (pl.ds(hf * H + rb * RB, RB), slice(None))
        return cp(x_hbm.at[0].at[idx], x_vm.at[idx], sem)

    o2 = out_hbm.at[0]
    in0 = [cp_x(0, 0, 0), cp_gu(0, 0, 0)]
    in1 = [cp_x(0, 1, 1)]
    in2 = [cp_gu(0, 1, 2)]
    in3 = [cp_gu(0, 2, 3), cp_gu(0, 3, 3), cp(gw_hbm, gw_vm, 3)]
    in4 = [cp_x(rb, hf, 4) for rb in (1, 2) for hf in range(2)]
    in5 = [cp_x(3, 0, 5), cp_x(3, 1, 5), cp_d(0, 5)]
    in_ffn = [c for j in range(1, NC) for c in [cp_gu(j, p, 7) for p in range(4)] + [cp_d(j, 7)]]
    out_sem = 8

    def start(cs):
        for c in cs:
            c.start()

    def wait(cs):
        for c in cs:
            c.wait()

    start(in0 + in1 + in2)

    zs[...] = jnp.zeros((8, 128), i32)
    zi[0] = 1
    sp = _Spreader(zs)

    def rows(rb, hf=0):
        return slice(hf * H + rb * RB, hf * H + (rb + 1) * RB)

    def x_lhs(t, rb):
        if t == 2:
            return _unpack(xn[_half(rows(rb, 0)), :KH])
        if t == 3:
            return _unpack(xn[_half(rows(rb, 1)), KH:])
        return _unpack(xa[_A_SLOT[t], _half(rows(rb)), :])

    def prep_tasks(rb, sums=True, gate=True):
        def task(s0):
            def run(first):
                prev = None
                gw = gw_vm[...].astype(f32)
                r = [slice(hf * H + rb * RB + s0, hf * H + rb * RB + s0 + 16) for hf in range(2)]
                z = [None, None]
                for c in range(4):
                    cols = [slice(kh * KH + c * 128, kh * KH + (c + 1) * 128) for kh in range(2)]
                    xs = [sp.link(prev, _pack(x_vm[r[qd // 2], cols[qd % 2]])) for qd in range(4)]
                    a = [_unpack(t).astype(f32) for t in xs]
                    outs = []
                    if sums:
                        for qd in range(4):
                            xn[_half(r[qd // 2]), cols[qd % 2]] = xs[qd]
                        cs = _a_combos(*a)
                        for t, slot in _A_SLOT.items():
                            outs.append(_pack(cs[t]))
                            xa[slot, _half(r[0]), cols[0]] = outs[-1]
                    if gate:
                        for qd in range(4):
                            g0 = (qd % 2) * 4 + c
                            term = a[qd] * gw[g0:g0 + 1, :]
                            z[qd // 2] = term if z[qd // 2] is None else z[qd // 2] + term
                        outs += z
                    prev = sp.chain(outs, prev, 1)
                if gate:
                    for hf in range(2):
                        g = jax.nn.sigmoid(jnp.sum(z[hf], axis=1, keepdims=True))
                        g = jnp.broadcast_to(g, (16, 128))
                        gs[r[hf], :] = g
                        prev = sp.chain([g], prev, 1)
                return sp.chain([prev], first, 1)
            return run
        return [task(s0) for s0 in range(0, RB, 16)]

    def b_sum_tasks(src, dst, depth=DEPTH):
        def task(r0):
            def run(prev):
                raw = [src(slice(a * KH + r0, a * KH + r0 + 16), slice(c * KH, (c + 1) * KH))
                       for a in range(2) for c in range(2)]
                cs = _b_combos(*[b.astype(f32) for b in raw])
                for t in _B_SUMS:
                    dst.setdefault(t, []).append(_pack(cs[t]))
                return sp.chain([dst[t][-1] for t in _B_SUMS], prev, depth)
            return run
        return [task(r0) for r0 in range(0, KH, 16)]

    def b_rhs(src, sums):
        def rhs(t):
            if t == 1:
                return src(slice(0, KH), slice(0, KH))
            if t == 4:
                return src(slice(KH, D), slice(KH, D))
            return _unpack(jnp.concatenate(sums[t], axis=0))
        return rhs

    def strassen_x(order, rhs, finish):
        m = {}
        for rb, t in order:
            m.setdefault(rb, {})[t] = sp.dot(x_lhs(t, rb), rhs(t))
            if len(m[rb]) == 7:
                finish(rb, m.pop(rb))

    def h_sums(rb, cs, r0, sub):
        h = []
        for qd, cc in enumerate(cs):
            g0 = (qd // 2) * H + rb * RB + r0
            omg = 1.0 - gs[g0:g0 + sub, :]
            omg = jnp.concatenate([omg] * (CH // 128), axis=1)
            h.append(jnp.maximum(cc[:, :CH], 0.0) * cc[:, CH:] * omg)
        return _a_combos(*h)

    def glu_tasks(hs, rb, cs, sub):
        hs[rb] = [[] for _ in range(7)]

        def task(r0):
            def run(prev):
                sums = h_sums(rb, [cc[r0:r0 + sub] for cc in cs], r0, sub)
                for t in range(7):
                    hs[rb][t].append(sums[t])
                if sub < RB:
                    return sp.chain([sums[t] for t in _A_SLOT], prev, DEPTH2)
            return run
        return [task(r0) for r0 in range(0, RB, sub)]

    def down_lhs(hs, b, ha):
        tok = None
        for t in range(7):
            s0, s1 = [jnp.concatenate(hs[rb][t], axis=0) for rb in (b, b + 2)]
            slabs = []
            for r in range(0, RB, 16):
                slabs.append(sp.serial_combos(
                    _a_combos, s0[r:r + 16, :CQ], s0[r:r + 16, CQ:],
                    s1[r:r + 16, :CQ], s1[r:r + 16, CQ:], tok))
                tok = sp.chain([slabs[-1][t2] for t2 in _A_SLOT], None, H_DEPTH)
            for t2 in range(7):
                ha[b, 7 * t + t2] = jnp.concatenate([sl[t2] for sl in slabs], axis=0).astype(bf16)
        ha['tok'] = tok

    def d_tasks(j, dst):
        def task(r0, c):
            def run(prev):
                def blk(k1, k2, n1, n2):
                    r, c0 = k1 * CH + k2 * CQ + r0, n1 * KH + n2 * KQ + c * 128
                    return wd[j, r:r + 16, c0:c0 + 128].astype(f32)
                cs, tok = sp.two_level(_b_combos, blk, prev, DEPTH2)
                for t in range(49):
                    dst.setdefault((t, c), []).append(cs[t])
                return tok
            return run
        return [task(r0, c) for r0 in range(0, CQ, 16) for c in range(2)]

    def ffn_down(ha, dc, first):
        rhs = [_unpack(jnp.concatenate([jnp.concatenate(dc[t, c], axis=0) for c in range(2)], axis=1))
               for t in range(49)]
        todo = [(b, t) for b in range(2) for t in range(49)]
        for i in range(0, len(todo), 2):
            pair = todo[i:i + 2]
            ps = sp.dots([(ha[b, t], rhs[t]) for b, t in pair])
            for (b, t), p in zip(pair, ps):
                if first:
                    acc[t, b * RB:(b + 1) * RB, :] = p
                else:
                    acc[t, b * RB:(b + 1) * RB, :] += p

    def perm_tasks(wqkv_vm, wp, i, tbuf):
        def fwd(rb, c):
            def run(prev):
                c0 = i * D + c * 128
                tt = pltpu.bitcast(wqkv_vm[rb * 256:(rb + 1) * 256, c0:c0 + 128], f32).T
                for hh in range(4):
                    tbuf[rb, pl.ds((4 * c + hh) * TP, DH), :] = tt[hh * DH:(hh + 1) * DH, :]
                return sp.chain([tt], prev, 1)
            return run

        def bwd(rb, j):
            def run(prev):
                g = jnp.concatenate(
                    [tbuf[rb, pl.ds(4 * j + dd, NH, stride=TP), :] for dd in range(4)], axis=0).T
                wp[i, rb * 128:(rb + 1) * 128, j * 128:(j + 1) * 128] = pltpu.bitcast(g, i32)
            return run
        tasks = []
        for rb in range(4):
            tasks += [fwd(rb, c) for c in range(8)] + [bwd(rb, j) for j in range(8)]
        return tasks

    def wo_tasks(wo_vm):
        def stage(c):
            return 4 + c % 4, (c // 4) * NH * TP

        def spread(h0):
            def run(prev):
                blk = wo_vm[h0 * DH:(h0 + 2) * DH, :].astype(f32)
                for h in range(2):
                    for c in range(8):
                        sl, r0 = stage(c)
                        q_s[sl, pl.ds(r0 + (h0 + h) * TP, DH), :] = (
                            blk[h * DH:(h + 1) * DH, c * 128:(c + 1) * 128])
                return sp.chain([blk], prev, 1)
            return run

        def gather(d, h0, c):
            def run(after):
                def blk(k1, k2, n1, n2):
                    sl, r0 = stage(4 * n1 + 2 * n2 + c)
                    r0 += h0 * TP + 16 * k1 + 8 * k2 + d
                    return q_s[sl, pl.ds(r0, 16, stride=TP), :]
                cs, tok = sp.two_level(_b_combos, blk, None, DEPTH2, after)
                r = (d * NH + h0) // 2
                for t in range(49):
                    woc[t, r:r + 8, c * 128:(c + 1) * 128] = cs[t]
                return tok
            return run
        return ([spread(h0) for h0 in range(0, NH, 2)],
                [gather(d, h0, c) for d in range(8) for h0 in (0, 16) for c in range(2)])

    def proj(wp, i, dst, pad, slabs):
        lhs = jnp.concatenate([xn[r0 // 2:(r0 + n) // 2, :] for r0, n in slabs], axis=0)
        p = sp.dot(_unpack(lhs), _unpack(wp[i]))
        at = 0
        for r0, n in slabs:
            for j in range(8):
                dst[j, pad + r0:pad + r0 + n, :] = p[at:at + n, j * 128:(j + 1) * 128]
            at += n

    def v_finish(rb, m):
        cs = _c_combos(m)
        for qd, cc in enumerate(cs):
            r0 = PAD + (qd // 2) * H + rb * RB
            for j in range(4):
                v_s[(qd % 2) * 4 + j, r0:r0 + RB, :] = cc[:, j * 128:(j + 1) * 128]
        if rb == 0:
            for j in range(8):
                src = cs[j // 4][0:1, (j % 4) * 128:(j % 4 + 1) * 128]
                v_s[j, 0:PAD, :] = jnp.broadcast_to(src, (PAD, 128))

    def attn_group(row, masked):
        def run(prev):
            g = 8
            q = [q_s[j, pl.ds(row, g), :] for j in range(8)]
            ls = []
            for w in range(W):
                a = None
                for j in range(8):
                    term = q[j] * k_s[j, pl.ds(row + (PAD - DIL * w), g), :]
                    a = sp.link(ls[-1] if ls else None, term) if a is None else a + term
                ls.append(a)
            rs = [pltpu.roll(a, 64, 1) for a in ls]
            ls = [a + r for a, r in zip(ls, rs)]
            rs = [pltpu.roll(a, 32, 1) for a in ls]
            ls = [a + r for a, r in zip(ls, rs)]
            if masked:
                ri = row + lax.broadcasted_iota(i32, (g, 128), 0)
                ls = [ls[0]] + [jnp.where(ri >= DIL * w, ls[w], NEG) for w in range(1, W)]
            m = _tree(jnp.maximum, ls)
            ps = [jnp.exp2((l - m) * EXP2_SCALE) for l in ls]
            r = gs[pl.ds(row, g), :] / _tree(jnp.add, ps)
            outs = []
            for j in range(8):
                a = None
                for w in range(W):
                    term = ps[w] * v_s[j, pl.ds(row + (PAD - DIL * w), g), :]
                    a = sp.link(outs[-1] if outs else None, term) if a is None else a + term
                outs.append(a * r)
            for j in range(8):
                q_s[j, pl.ds(row, g), :] = outs[j]
            return sp.chain([outs[-1]], prev, 1)
        return run

    def attn_tasks(base, nrows, first=False):
        return [attn_group(base + (qq * Q + r), first and qq == 0 and r < PAD)
                for r in range(0, nrows, 8) for qq in range(4)]

    def pack_tasks(oa, base, hbase, nrows):
        def task(r, c):
            def run(prev, after=None):
                def blk(i1, i2, k1, k2):
                    return q_s[4 * k1 + 2 * k2 + c, pl.ds(base + (i1 * H + i2 * Q + r), 16), :]
                cs, tok = sp.two_level(_a_combos, blk, prev, DEPTH2 if after is None else PDEPTH, after)
                for t in range(49):
                    oa[t, pl.ds(hbase + r // 2, 8), c * 128:(c + 1) * 128] = cs[t]
                return tok
            return run
        return [task(r, c) for r in range(0, nrows, 16) for c in range(2)]

    GS = RB * (KH // 128) * (FC // 128) * 7 // (4 * SLOT)
    DS = 49
    PS = 2 * RB * (D // 128) * (D // 128) // (4 * SLOT)

    def glu(hs, ha):
        def finish(rb, m):
            glu_tasks(hs, rb, _c_combos(m), RB)[0](None)
            if rb >= 2:
                down_lhs(hs, rb - 2, ha)
        return finish

    def raw_first(rbs, n):
        lead = [(rb, t) for rb in rbs[:n] for t in ORDER[:2]]
        return lead + [(rb, t) for rb in rbs for t in ORDER if (rb, t) not in lead]

    def gu_src(j):
        return lambda r, c: wgu[j, r, c]

    def front(wqkv_vm, wp, wo_vm):
        in_q, in_k, in_v = [
            cp(wqkv_hbm.at[:, pl.ds(i * D, D)], wqkv_vm.at[:, pl.ds(i * D, D)], (6, 6, 5)[i])
            for i in range(3)]
        in_wo = cp(wo_hbm, wo_vm, 6)

        def plain(rb, hf, p):
            return sp.dot(x_vm[rows(rb, hf), :], wgu[0, :, p * CH:(p + 1) * CH])

        def plain_finish(rb, c):
            cs = [jnp.concatenate(c[2 * qd:2 * qd + 2], axis=1) for qd in range(4)]
            return glu_tasks(hs, rb, cs, 16)

        hs, bc, dc = {}, {}, {}
        wait(in0)
        start(in3)
        c0 = {(0, 0): plain(0, 0, 0)}
        wait(in1)
        c0[1, 0] = plain(0, 1, 0)
        wait(in2)
        start(in4)
        for hf in range(2):
            c0[hf, 1] = plain(0, hf, 1)
        wait(in3)
        start(in5)
        sp.block()
        bt = b_sum_tasks(gu_src(0), bc)
        sp.schedule(bt[:12], 3, 16)
        sp.schedule(prep_tasks(0, sums=False), 3, 16)
        for p in (2, 3):
            for hf in range(2):
                c0[hf, p] = plain(0, hf, p)
        c0 = [c0[hf, p] for hf in range(2) for p in range(4)]
        wait(in4)
        start([in_v])
        sp.block()
        sp.schedule(bt[12:], 3, 32)
        sp.schedule(prep_tasks(1, sums=False), 2, 10)
        sp.schedule(prep_tasks(2), 10, 32)
        c1 = [plain(1, hf, p) for hf in range(2) for p in range(4)]
        wait(in5 + [in_v])
        start([in_k, in_wo, in_q])
        sp.block()
        for j in range(8):
            k_s[j, 0:PAD, :] = jnp.zeros((PAD, 128), f32)
        ha = {}
        sp.schedule(prep_tasks(3), 2, GS)
        sp.schedule(plain_finish(0, c0), 2, GS)
        sp.schedule(plain_finish(1, c1), GS + 6, 2 * GS)
        sp.schedule(d_tasks(0, dc), GS - 2, 2 * GS)
        sp.schedule(perm_tasks(wqkv_vm, wp, 2, q_s), 2 * GS + 6, 2 * GS + DS - 8)
        strassen_x([(rb, t) for rb in (2, 3) for t in ORDER], b_rhs(gu_src(0), bc),
                   glu(hs, ha))
        ffn_down(ha, dc, True)

        wait([in_k, in_wo, in_q])
        start(in_ffn)
        sp.block()
        vb = {}
        v_src = lambda r, c: _unpack(wp[2, _half(r), c])
        wo_spread, wo_gather = wo_tasks(wo_vm)
        sp.schedule(b_sum_tasks(v_src, vb, VDEPTH), *VBC_SLOTS)
        sp.schedule(prep_tasks(0, gate=False) + prep_tasks(1, gate=False), *PREP01)
        sp.schedule(perm_tasks(wqkv_vm, wp, 1, k_s.at[:, PAD:, :]), *PERMK)
        sp.schedule(wo_spread, *WOS)
        strassen_x(raw_first((2, 3, 0, 1), 2), b_rhs(v_src, vb), v_finish)
        sp.schedule(perm_tasks(wqkv_vm, wp, 0, q_s), 4, 3 * PS)
        tok = None
        for t in wo_gather:
            tok = t(tok)
        for rb in range(NRB):
            proj(wp, 1, k_s, PAD, [(rb * Q, Q)])
        proj(wp, 0, q_s, 0, [(qq * Q, QA) for qq in range(4)])

        def q_rest(_, carry):
            sp.block()
            n = (Q - QA) // 2
            total = 4 * (Q - QA) * 64 // (4 * SLOT)
            sp.schedule(attn_tasks(0, A0, True), 4, total)
            for r0 in (QA, QA + n):
                proj(wp, 0, q_s, 0, [(qq * Q + r0, n) for qq in range(4)])
            return carry

        lax.fori_loop(0, zi[0], q_rest, 0)
        wait(in_ffn)

    def back(oa):
        def body(j, carry):
            sp.block()
            base = pl.multiple_of((j - 1) * AR, AR)
            hs, ha, bc, dc = {}, {}, {}, {}
            sp.schedule(b_sum_tasks(gu_src(j), bc), *BC_SLOTS)
            sp.schedule(attn_tasks(base + A0, AR), *ATTN_SLOTS)
            packs = pack_tasks(oa, base, pl.multiple_of((j - 1) * (AR // 2), AR // 2), AR)
            sp.schedule(d_tasks(j, dc), *DC_SLOTS)
            strassen_x(raw_first((0, 2, 1, 3), NRAW), b_rhs(gu_src(j), bc), glu(hs, ha))
            tok = ha['tok']
            for t in packs:
                tok = t(None, tok)
            ffn_down(ha, dc, False)
            return carry

        lax.fori_loop(1, NC, body, 0)

        def out_copy(r0, n, i1, i2, cols):
            idx = (pl.ds(r0 + i1 * H + i2 * Q, n), cols)
            return cp(x_vm.at[idx], o2.at[idx], out_sem)

        def out_blocks(n, blocks):
            done_by = {ts[-1]: qd for ts, qd in _C_ORDER}
            todo = [(blk, t1, t2) for blk in range(len(blocks))
                    for ts1, _ in _C_ORDER for t1 in ts1 for ts2, _ in _C_ORDER for t2 in ts2]
            m, inner = {}, {}
            for i in range(0, len(todo), SLOT // n):
                group = todo[i:i + SLOT // n]
                ps = sp.dots([(_unpack(oa[7 * t1 + t2, pl.ds(blocks[blk][0] // 2, n // 2), :]),
                               _unpack(woc[7 * t1 + t2])) for blk, t1, t2 in group])
                for (blk, t1, t2), p in zip(group, ps):
                    r0, copies = blocks[blk]
                    m.setdefault((blk, t1), {})[t2] = acc[7 * t1 + t2, pl.ds(r0, n), :] + p
                    if t2 not in done_by:
                        continue
                    q2 = done_by[t2] ^ (t1 in _FLIP)
                    inner.setdefault((blk, q2), {})[t1] = _c_quadrant(m[blk, t1], done_by[t2])
                    if t1 not in done_by:
                        continue
                    q1 = done_by[t1]
                    r = pl.ds(r0 + (q1 // 2) * H + (q2 // 2) * Q, n)
                    c = (q1 % 2) * KH + (q2 % 2) * KQ
                    x_vm[r, c:c + KQ] = _c_quadrant(inner[blk, q2], q1).astype(bf16)
                    start(copies.get((q1, q2), []))

        final = {q1: (q1, 3 ^ (ts[-1] in _FLIP)) for ts, q1 in _C_ORDER}

        def whole(r0, n):
            return {final[3]: [out_copy(r0, n, i1, i2, slice(None))
                               for i1 in range(2) for i2 in range(2)]}

        done = (NC - 1) * AR
        sp.block()
        sp.schedule(pack_tasks(oa, done, done // 2, Q - done), *PACK4)
        last = {final[q1]: [out_copy(Q - PB, PB, q1 // 2, i2, pl.ds((q1 % 2) * KH, KH))
                            for i2 in range(2)] for q1 in range(3)}
        for q2 in range(4):
            last[3, q2] = [out_copy(Q - PB, PB, 1, q2 // 2, pl.ds(KH + (q2 % 2) * KQ, KQ))]
        copies = [whole(0, RB), whole(RB, PB), last]
        out_blocks(RB, [(0, copies[0])])
        out_blocks(PB, [(RB, copies[1]), (Q - PB, last)])
        for cs in copies:
            for key in cs:
                wait(cs[key])

    pl.run_scoped(front, pltpu.VMEM((D, 3 * D), bf16), pltpu.VMEM((3, D // 2, D), i32),
                  pltpu.VMEM((D, D), bf16))
    pl.run_scoped(back, pltpu.VMEM((49, Q // 2, KQ), i32))
    assert not sp.plan


_N_SEMS = 9


@jax.jit
def pallas_gated_mix__sliding_local_dilated__glu_gated_reglu__prompt_kernel(
    A_x: jax.Array,
    A_wqkv: jax.Array,
    A_wo: jax.Array,
    B_x: jax.Array,
    B_W_gate: jax.Array,
    B_W_up: jax.Array,
    B_W_down: jax.Array,
    gate_w: jax.Array,
):
    del B_x
    hbm = pl.BlockSpec(memory_space=pl.ANY)
    scratch = [
        pltpu.VMEM((S, D), bf16),
        pltpu.VMEM((S // 2, D), i32),
        pltpu.VMEM((5, H // 2, KH), i32),
        pltpu.VMEM((8, 128), bf16),
        pltpu.VMEM((NC, D, 2 * FC), bf16),
        pltpu.VMEM((NC, FC, D), bf16),
        pltpu.VMEM((49, Q, KQ), f32),
        pltpu.VMEM((8, S + QPAD, 128), f32),
        pltpu.VMEM((8, PAD + S, 128), f32),
        pltpu.VMEM((8, PAD + S, 128), f32),
        pltpu.VMEM((S, 128), f32),
        pltpu.VMEM((49, KQ // 2, KQ), i32),
        pltpu.VMEM((8, 128), i32),
        pltpu.SMEM((1,), i32),
        pltpu.SemaphoreType.DMA((_N_SEMS,)),
    ]
    return pl.pallas_call(
        _kernel,
        in_specs=[hbm] * 7,
        out_specs=hbm,
        out_shape=jax.ShapeDtypeStruct((1, S, D), bf16),
        scratch_shapes=scratch,
        compiler_params=pltpu.CompilerParams(vmem_limit_bytes=124 * 1024 * 1024),
    )(A_x, A_wqkv, A_wo, B_W_gate, B_W_up, B_W_down, gate_w.reshape(8, 128))
```

```python
import math

import jax
import jax.numpy as jnp
from jax import lax
import jax.experimental.pallas as pl
import jax.experimental.pallas.tpu as pltpu

f32 = jnp.float32
bf16 = jnp.bfloat16
i32 = jnp.int32

S = 2048
D = 1024
F = 3584
NH = 32
DH = D // NH
W = 8
DIL = 2
H = S // 2
Q = S // 4
KH = D // 2
KQ = D // 4
FC = 512
CH = FC // 2
CQ = FC // 4
NC = F // FC
RB = 256
NRB = H // RB
PB = 128
PAD = 16
TP = DH + 1
AR = 64
A0 = Q - 6 * AR
QA = 160
QPAD = 112

BC_SLOTS = (2, 24)
ATTN_SLOTS = (24, 106)
DC_SLOTS = (26, 98)
VDEPTH = 2
PDEPTH = 3
VBC_SLOTS = (2, 16)
PREP01 = (16, 56)
PERMK = (64, 106)
WOS = (70, 112)
PACK4 = (4, 48)
NRAW = 3
DEPTH = 3
DEPTH2 = 3
H_DEPTH = 3

SCALE = DH ** -0.5
EXP2_SCALE = SCALE * math.log2(math.e)
NEG = -1e9 / SCALE


def _a_combos(a11, a12, a21, a22):
    return [a11 + a22, a21 + a22, a11, a22, a11 + a12, a21 - a11, a12 - a22]


def _b_combos(b11, b12, b21, b22):
    return [b11 + b22, b11, b12 - b22, b21 - b11, b22, b11 + b12, b21 + b22]


_C_TERMS = (((1, 0), (1, 3), (-1, 4), (1, 6)), ((1, 2), (1, 4)), ((1, 1), (1, 3)),
            ((1, 0), (-1, 1), (1, 2), (1, 5)))
_C_ORDER = (((2, 4), 1), ((1, 3), 2), ((0, 6), 0), ((5,), 3))


def _c_quadrant(m, qd):
    out = m[_C_TERMS[qd][0][1]]
    for sign, t in _C_TERMS[qd][1:]:
        out = out + m[t] if sign > 0 else out - m[t]
    return out


def _c_combos(m):
    return [_c_quadrant(m, qd) for qd in range(4)]


_FLIP = (1, 4, 5, 6)
_A_SLOT = {0: 0, 1: 1, 4: 2, 5: 3, 6: 4}
_B_SUMS = (2, 3, 0, 5, 6)
ORDER = (1, 4) + _B_SUMS


def _tree(op, xs):
    xs = list(xs)
    while len(xs) > 1:
        xs = [op(xs[i], xs[i + 1]) if i + 1 < len(xs) else xs[i] for i in range(0, len(xs), 2)]
    return xs[0]


def _pack(x):
    return pltpu.bitcast(x.astype(bf16), i32)


def _unpack(x):
    return pltpu.bitcast(x, bf16)


def _half(r):
    return slice(r.start // 2, r.stop // 2)


SLOT = 256


class _Spreader:
    def __init__(self, zero_ref):
        self.zero_ref = zero_ref
        self.plan = {}
        self.lists = 0
        self.now = 0

    def block(self):
        self.zero = self.zero_ref[...]
        self.never = self.zero != 0

    def link(self, after, x):
        if after is None:
            return x
        if after.dtype != x.dtype:
            after = pltpu.bitcast(after, x.dtype)
        return jnp.where(self.never, after, x)

    def chain(self, vals, prev, depth):
        for v in vals:
            v = pltpu.bitcast(v, i32) if v.dtype != i32 else v
            for r in range(0, v.shape[0], 8):
                for c in range(0, v.shape[1], 128):
                    tile = v[r:r + 8, c:c + 128]
                    if prev is None:
                        prev = tile
                        continue
                    prev = prev | tile
                    for i in range(depth - 1):
                        prev = (prev + self.zero) if i % 2 == 0 else (prev ^ self.zero)
        return prev

    def link_rows(self, after, x):
        return jnp.concatenate([self.link(after, x[r:r + 8, :]) for r in range(0, x.shape[0], 8)],
                               axis=0)

    def serial_combos(self, combos, x11, x12, x21, x22, after):
        return combos(self.link_rows(after, x11), x12, x21, self.link_rows(after, x22))

    def two_level(self, combos, blk, prev, depth, after=None):
        outer, outs, tok = [], [], after
        for r2 in range(2):
            for c2 in range(2):
                outer.append(self.serial_combos(
                    combos, *[blk(r1, r2, c1, c2) for r1 in range(2) for c1 in range(2)], tok))
                tok = self.chain([x[:8] for x in outer[-1]], None, 1)
        for t in range(7):
            flip = combos is _b_combos and t in _FLIP
            wide = _pack(jnp.concatenate(
                self.serial_combos(combos, *[outer[i ^ flip][t] for i in range(4)], tok), axis=1))
            outs += [wide[:, c:c + 128] for c in range(0, 7 * 128, 128)]
            tok = self.chain(outs[-7:], tok, depth)
        return outs, self.chain([tok], prev, 1)

    def schedule(self, tasks, first, last):
        self.lists += 1
        for i, t in enumerate(tasks):
            pos = self.now + first + ((i + 1) * (last - first) - 1) // len(tasks)
            self.plan.setdefault(pos, []).append((t, self.lists))

    def dots(self, pairs):
        m = pairs[0][0].shape[0]
        tiles = [(i, r, c) for i, (_, rhs) in enumerate(pairs)
                 for c in range(0, rhs.shape[1], 128) for r in range(0, rhs.shape[0], 128)]
        nslots = m * len(tiles) // (4 * SLOT)
        deps = {}
        for sl in range(nslots):
            ps = sl * SLOT // m
            toks = {}
            for t, lane in self.plan.pop(self.now + sl, []):
                tok = t(toks.get(lane))
                if tok is not None:
                    toks[lane] = tok
            for tok in toks.values():
                deps[ps] = tok | deps[ps] if ps in deps else tok
        self.now += nslots
        tied = {tile: d for ps, d in deps.items() for tile in tiles[4 * ps:4 * ps + 4]}
        outs = []
        for i, (lhs, rhs) in enumerate(pairs):
            if any(key[0] == i for key in tied):
                parts = []
                for r in range(0, rhs.shape[0], 128):
                    top = [rhs[r:r + 16, c:c + 128] for c in range(0, rhs.shape[1], 128)]
                    top = [_unpack(self.link(tied[i, r, c * 128], _pack(t0)))
                           if (i, r, c * 128) in tied else t0 for c, t0 in enumerate(top)]
                    parts += [jnp.concatenate(top, axis=1), rhs[r + 16:r + 128, :]]
                rhs = jnp.concatenate(parts, axis=0)
            outs.append(jnp.dot(lhs, rhs, preferred_element_type=f32))
        return outs

    def dot(self, lhs, rhs):
        return self.dots([(lhs, rhs)])[0]


def _kernel(x_hbm, wqkv_hbm, wo_hbm, wg_hbm, wu_hbm, wd_hbm, gw_hbm, out_hbm,
            x_vm, xn, xa, gw_vm, wgu, wd, acc, q_s, k_s, v_s, gs, woc, zs, zi, sems):
    def cp(src, dst, sem):
        return pltpu.make_async_copy(src, dst, sems.at[sem])

    def cp_gu(j, p, sem):
        return cp((wg_hbm, wu_hbm)[p % 2].at[:, pl.ds(j * FC + (p // 2) * CH, CH)],
                  wgu.at[j, :, pl.ds(p * CH, CH)], sem)

    def cp_d(j, sem):
        return cp(wd_hbm.at[pl.ds(j * FC, FC), :], wd.at[j], sem)

    def cp_x(rb, hf, sem):
        idx = (pl.ds(hf * H + rb * RB, RB), slice(None))
        return cp(x_hbm.at[0].at[idx], x_vm.at[idx], sem)

    o2 = out_hbm.at[0]
    in0 = [cp_x(0, 0, 0), cp_gu(0, 0, 0)]
    in1 = [cp_x(0, 1, 1)]
    in2 = [cp_gu(0, 1, 2)]
    in3 = [cp_gu(0, 2, 3), cp_gu(0, 3, 3), cp(gw_hbm, gw_vm, 3)]
    in4 = [cp_x(rb, hf, 4) for rb in (1, 2) for hf in range(2)]
    in5 = [cp_x(3, 0, 5), cp_x(3, 1, 5), cp_d(0, 5)]
    in_ffn = [c for j in range(1, NC) for c in [cp_gu(j, p, 7) for p in range(4)] + [cp_d(j, 7)]]
    out_sem = 8

    def start(cs):
        for c in cs:
            c.start()

    def wait(cs):
        for c in cs:
            c.wait()

    start(in0 + in1 + in2)

    zs[...] = jnp.zeros((8, 128), i32)
    zi[0] = 1
    sp = _Spreader(zs)

    def rows(rb, hf=0):
        return slice(hf * H + rb * RB, hf * H + (rb + 1) * RB)

    def x_lhs(t, rb):
        if t == 2:
            return _unpack(xn[_half(rows(rb, 0)), :KH])
        if t == 3:
            return _unpack(xn[_half(rows(rb, 1)), KH:])
        return _unpack(xa[_A_SLOT[t], _half(rows(rb)), :])

    def prep_tasks(rb, sums=True, gate=True):
        def task(s0):
            def run(first):
                prev = None
                gw = gw_vm[...].astype(f32)
                r = [slice(hf * H + rb * RB + s0, hf * H + rb * RB + s0 + 16) for hf in range(2)]
                z = [None, None]
                for c in range(4):
                    cols = [slice(kh * KH + c * 128, kh * KH + (c + 1) * 128) for kh in range(2)]
                    xs = [sp.link(prev, _pack(x_vm[r[qd // 2], cols[qd % 2]])) for qd in range(4)]
                    a = [_unpack(t).astype(f32) for t in xs]
                    outs = []
                    if sums:
                        for qd in range(4):
                            xn[_half(r[qd // 2]), cols[qd % 2]] = xs[qd]
                        cs = _a_combos(*a)
                        for t, slot in _A_SLOT.items():
                            outs.append(_pack(cs[t]))
                            xa[slot, _half(r[0]), cols[0]] = outs[-1]
                    if gate:
                        for qd in range(4):
                            g0 = (qd % 2) * 4 + c
                            term = a[qd] * gw[g0:g0 + 1, :]
                            z[qd // 2] = term if z[qd // 2] is None else z[qd // 2] + term
                        outs += z
                    prev = sp.chain(outs, prev, 1)
                if gate:
                    for hf in range(2):
                        g = jax.nn.sigmoid(jnp.sum(z[hf], axis=1, keepdims=True))
                        g = jnp.broadcast_to(g, (16, 128))
                        gs[r[hf], :] = g
                        prev = sp.chain([g], prev, 1)
                return sp.chain([prev], first, 1)
            return run
        return [task(s0) for s0 in range(0, RB, 16)]

    def b_sum_tasks(src, dst, depth=DEPTH):
        def task(r0):
            def run(prev):
                raw = [src(slice(a * KH + r0, a * KH + r0 + 16), slice(c * KH, (c + 1) * KH))
                       for a in range(2) for c in range(2)]
                cs = _b_combos(*[b.astype(f32) for b in raw])
                for t in _B_SUMS:
                    dst.setdefault(t, []).append(_pack(cs[t]))
                return sp.chain([dst[t][-1] for t in _B_SUMS], prev, depth)
            return run
        return [task(r0) for r0 in range(0, KH, 16)]

    def b_rhs(src, sums):
        def rhs(t):
            if t == 1:
                return src(slice(0, KH), slice(0, KH))
            if t == 4:
                return src(slice(KH, D), slice(KH, D))
            return _unpack(jnp.concatenate(sums[t], axis=0))
        return rhs

    def strassen_x(order, rhs, finish):
        m = {}
        for rb, t in order:
            m.setdefault(rb, {})[t] = sp.dot(x_lhs(t, rb), rhs(t))
            if len(m[rb]) == 7:
                finish(rb, m.pop(rb))

    def h_sums(rb, cs, r0, sub):
        h = []
        for qd, cc in enumerate(cs):
            g0 = (qd // 2) * H + rb * RB + r0
            omg = 1.0 - gs[g0:g0 + sub, :]
            omg = jnp.concatenate([omg] * (CH // 128), axis=1)
            h.append(jnp.maximum(cc[:, :CH], 0.0) * cc[:, CH:] * omg)
        return _a_combos(*h)

    def glu_tasks(hs, rb, cs, sub):
        hs[rb] = [[] for _ in range(7)]

        def task(r0):
            def run(prev):
                sums = h_sums(rb, [cc[r0:r0 + sub] for cc in cs], r0, sub)
                for t in range(7):
                    hs[rb][t].append(sums[t])
                if sub < RB:
                    return sp.chain([sums[t] for t in _A_SLOT], prev, DEPTH2)
            return run
        return [task(r0) for r0 in range(0, RB, sub)]

    def down_lhs(hs, b, ha):
        tok = None
        for t in range(7):
            s0, s1 = [jnp.concatenate(hs[rb][t], axis=0) for rb in (b, b + 2)]
            slabs = []
            for r in range(0, RB, 16):
                slabs.append(sp.serial_combos(
                    _a_combos, s0[r:r + 16, :CQ], s0[r:r + 16, CQ:],
                    s1[r:r + 16, :CQ], s1[r:r + 16, CQ:], tok))
                tok = sp.chain([slabs[-1][t2] for t2 in _A_SLOT], None, H_DEPTH)
            for t2 in range(7):
                ha[b, 7 * t + t2] = jnp.concatenate([sl[t2] for sl in slabs], axis=0).astype(bf16)
        ha['tok'] = tok

    def d_tasks(j, dst):
        def task(r0, c):
            def run(prev):
                def blk(k1, k2, n1, n2):
                    r, c0 = k1 * CH + k2 * CQ + r0, n1 * KH + n2 * KQ + c * 128
                    return wd[j, r:r + 16, c0:c0 + 128].astype(f32)
                cs, tok = sp.two_level(_b_combos, blk, prev, DEPTH2)
                for t in range(49):
                    dst.setdefault((t, c), []).append(cs[t])
                return tok
            return run
        return [task(r0, c) for r0 in range(0, CQ, 16) for c in range(2)]

    def ffn_down(ha, dc, first):
        rhs = [_unpack(jnp.concatenate([jnp.concatenate(dc[t, c], axis=0) for c in range(2)], axis=1))
               for t in range(49)]
        todo = [(b, t) for b in range(2) for t in range(49)]
        for i in range(0, len(todo), 2):
            pair = todo[i:i + 2]
            ps = sp.dots([(ha[b, t], rhs[t]) for b, t in pair])
            for (b, t), p in zip(pair, ps):
                if first:
                    acc[t, b * RB:(b + 1) * RB, :] = p
                else:
                    acc[t, b * RB:(b + 1) * RB, :] += p

    def perm_tasks(wqkv_vm, wp, i, tbuf):
        def fwd(rb, c):
            def run(prev):
                c0 = i * D + c * 128
                tt = pltpu.bitcast(wqkv_vm[rb * 256:(rb + 1) * 256, c0:c0 + 128], f32).T
                for hh in range(4):
                    tbuf[rb, pl.ds((4 * c + hh) * TP, DH), :] = tt[hh * DH:(hh + 1) * DH, :]
                return sp.chain([tt], prev, 1)
            return run

        def bwd(rb, j):
            def run(prev):
                g = jnp.concatenate(
                    [tbuf[rb, pl.ds(4 * j + dd, NH, stride=TP), :] for dd in range(4)], axis=0).T
                wp[i, rb * 128:(rb + 1) * 128, j * 128:(j + 1) * 128] = pltpu.bitcast(g, i32)
            return run
        tasks = []
        for rb in range(4):
            tasks += [fwd(rb, c) for c in range(8)] + [bwd(rb, j) for j in range(8)]
        return tasks

    def wo_tasks(wo_vm):
        def stage(c):
            return 4 + c % 4, (c // 4) * NH * TP

        def spread(h0):
            def run(prev):
                blk = wo_vm[h0 * DH:(h0 + 2) * DH, :].astype(f32)
                for h in range(2):
                    for c in range(8):
                        sl, r0 = stage(c)
                        q_s[sl, pl.ds(r0 + (h0 + h) * TP, DH), :] = (
                            blk[h * DH:(h + 1) * DH, c * 128:(c + 1) * 128])
                return sp.chain([blk], prev, 1)
            return run

        def gather(d, h0, c):
            def run(after):
                def blk(k1, k2, n1, n2):
                    sl, r0 = stage(4 * n1 + 2 * n2 + c)
                    r0 += h0 * TP + 16 * k1 + 8 * k2 + d
                    return q_s[sl, pl.ds(r0, 16, stride=TP), :]
                cs, tok = sp.two_level(_b_combos, blk, None, DEPTH2, after)
                r = (d * NH + h0) // 2
                for t in range(49):
                    woc[t, r:r + 8, c * 128:(c + 1) * 128] = cs[t]
                return tok
            return run
        return ([spread(h0) for h0 in range(0, NH, 2)],
                [gather(d, h0, c) for d in range(8) for h0 in (0, 16) for c in range(2)])

    def proj(wp, i, dst, pad, slabs):
        lhs = jnp.concatenate([xn[r0 // 2:(r0 + n) // 2, :] for r0, n in slabs], axis=0)
        p = sp.dot(_unpack(lhs), _unpack(wp[i]))
        at = 0
        for r0, n in slabs:
            for j in range(8):
                dst[j, pad + r0:pad + r0 + n, :] = p[at:at + n, j * 128:(j + 1) * 128]
            at += n

    def v_finish(rb, m):
        cs = _c_combos(m)
        for qd, cc in enumerate(cs):
            r0 = PAD + (qd // 2) * H + rb * RB
            for j in range(4):
                v_s[(qd % 2) * 4 + j, r0:r0 + RB, :] = cc[:, j * 128:(j + 1) * 128]
        if rb == 0:
            for j in range(8):
                src = cs[j // 4][0:1, (j % 4) * 128:(j % 4 + 1) * 128]
                v_s[j, 0:PAD, :] = jnp.broadcast_to(src, (PAD, 128))

    def attn_group(row, masked):
        def run(prev):
            g = 8
            q = [q_s[j, pl.ds(row, g), :] for j in range(8)]
            ls = []
            for w in range(W):
                a = None
                for j in range(8):
                    term = q[j] * k_s[j, pl.ds(row + (PAD - DIL * w), g), :]
                    a = sp.link(ls[-1] if ls else None, term) if a is None else a + term
                ls.append(a)
            rs = [pltpu.roll(a, 64, 1) for a in ls]
            ls = [a + r for a, r in zip(ls, rs)]
            rs = [pltpu.roll(a, 32, 1) for a in ls]
            ls = [a + r for a, r in zip(ls, rs)]
            if masked:
                ri = row + lax.broadcasted_iota(i32, (g, 128), 0)
                ls = [ls[0]] + [jnp.where(ri >= DIL * w, ls[w], NEG) for w in range(1, W)]
            m = _tree(jnp.maximum, ls)
            ps = [jnp.exp2((l - m) * EXP2_SCALE) for l in ls]
            r = gs[pl.ds(row, g), :] / _tree(jnp.add, ps)
            outs = []
            for j in range(8):
                a = None
                for w in range(W):
                    term = ps[w] * v_s[j, pl.ds(row + (PAD - DIL * w), g), :]
                    a = sp.link(outs[-1] if outs else None, term) if a is None else a + term
                outs.append(a * r)
            for j in range(8):
                q_s[j, pl.ds(row, g), :] = outs[j]
            return sp.chain([outs[-1]], prev, 1)
        return run

    def attn_tasks(base, nrows, first=False):
        return [attn_group(base + (qq * Q + r), first and qq == 0 and r < PAD)
                for r in range(0, nrows, 8) for qq in range(4)]

    def pack_tasks(oa, base, hbase, nrows):
        def task(r, c):
            def run(prev, after=None):
                def blk(i1, i2, k1, k2):
                    return q_s[4 * k1 + 2 * k2 + c, pl.ds(base + (i1 * H + i2 * Q + r), 16), :]
                cs, tok = sp.two_level(_a_combos, blk, prev, DEPTH2 if after is None else PDEPTH, after)
                for t in range(49):
                    oa[t, pl.ds(hbase + r // 2, 8), c * 128:(c + 1) * 128] = cs[t]
                return tok
            return run
        return [task(r, c) for r in range(0, nrows, 16) for c in range(2)]

    GS = RB * (KH // 128) * (FC // 128) * 7 // (4 * SLOT)
    DS = 49
    PS = 2 * RB * (D // 128) * (D // 128) // (4 * SLOT)

    def glu(hs, ha):
        def finish(rb, m):
            glu_tasks(hs, rb, _c_combos(m), RB)[0](None)
            if rb >= 2:
                down_lhs(hs, rb - 2, ha)
        return finish

    def raw_first(rbs, n):
        lead = [(rb, t) for rb in rbs[:n] for t in ORDER[:2]]
        return lead + [(rb, t) for rb in rbs for t in ORDER if (rb, t) not in lead]

    def gu_src(j):
        return lambda r, c: wgu[j, r, c]

    def front(wqkv_vm, wp, wo_vm):
        in_q, in_k, in_v = [
            cp(wqkv_hbm.at[:, pl.ds(i * D, D)], wqkv_vm.at[:, pl.ds(i * D, D)], (6, 6, 5)[i])
            for i in range(3)]
        in_wo = cp(wo_hbm, wo_vm, 6)

        def plain(rb, hf, p):
            return sp.dot(x_vm[rows(rb, hf), :], wgu[0, :, p * CH:(p + 1) * CH])

        def plain_finish(hs, rb, c):
            cs = [jnp.concatenate(c[2 * qd:2 * qd + 2], axis=1) for qd in range(4)]
            return glu_tasks(hs, rb, cs, 16)

        def chunk0(_, carry):
            hs, bc, dc = {}, {}, {}
            wait(in0)
            start(in3)
            c0 = {(0, 0): plain(0, 0, 0)}
            wait(in1)
            c0[1, 0] = plain(0, 1, 0)
            wait(in2)
            start(in4)
            for hf in range(2):
                c0[hf, 1] = plain(0, hf, 1)
            wait(in3)
            start(in5)
            sp.block()
            bt = b_sum_tasks(gu_src(0), bc)
            sp.schedule(bt[:12], 3, 16)
            sp.schedule(prep_tasks(0, sums=False), 3, 16)
            for p in (2, 3):
                for hf in range(2):
                    c0[hf, p] = plain(0, hf, p)
            c0 = [c0[hf, p] for hf in range(2) for p in range(4)]
            wait(in4)
            start([in_v])
            sp.block()
            sp.schedule(bt[12:], 3, 32)
            sp.schedule(prep_tasks(1, sums=False), 2, 10)
            sp.schedule(prep_tasks(2), 10, 32)
            c1 = [plain(1, hf, p) for hf in range(2) for p in range(4)]
            wait(in5 + [in_v])
            start([in_k, in_wo, in_q])
            sp.block()
            for j in range(8):
                k_s[j, 0:PAD, :] = jnp.zeros((PAD, 128), f32)
            ha = {}
            sp.schedule(prep_tasks(3), 2, GS)
            sp.schedule(plain_finish(hs, 0, c0), 2, GS)
            sp.schedule(plain_finish(hs, 1, c1), GS + 6, 2 * GS)
            sp.schedule(d_tasks(0, dc), GS - 2, 2 * GS)
            sp.schedule(perm_tasks(wqkv_vm, wp, 2, q_s), 2 * GS + 6, 2 * GS + DS - 8)
            strassen_x([(rb, t) for rb in (2, 3) for t in ORDER], b_rhs(gu_src(0), bc),
                       glu(hs, ha))
            ffn_down(ha, dc, True)
            return carry

        lax.fori_loop(0, zi[0], chunk0, 0)

        wait([in_k, in_wo, in_q])
        start(in_ffn)
        sp.block()
        vb = {}
        v_src = lambda r, c: _unpack(wp[2, _half(r), c])
        wo_spread, wo_gather = wo_tasks(wo_vm)
        sp.schedule(b_sum_tasks(v_src, vb, VDEPTH), *VBC_SLOTS)
        sp.schedule(prep_tasks(0, gate=False) + prep_tasks(1, gate=False), *PREP01)
        sp.schedule(perm_tasks(wqkv_vm, wp, 1, k_s.at[:, PAD:, :]), *PERMK)
        sp.schedule(wo_spread, *WOS)
        strassen_x(raw_first((2, 3, 0, 1), 2), b_rhs(v_src, vb), v_finish)
        sp.schedule(perm_tasks(wqkv_vm, wp, 0, q_s), 4, 3 * PS)
        tok = None
        for t in wo_gather:
            tok = t(tok)
        for rb in range(NRB):
            proj(wp, 1, k_s, PAD, [(rb * Q, Q)])
        proj(wp, 0, q_s, 0, [(qq * Q, QA) for qq in range(4)])

        def q_rest(_, carry):
            sp.block()
            n = (Q - QA) // 2
            total = 4 * (Q - QA) * 64 // (4 * SLOT)
            sp.schedule(attn_tasks(0, A0, True), 4, total)
            for r0 in (QA, QA + n):
                proj(wp, 0, q_s, 0, [(qq * Q + r0, n) for qq in range(4)])
            return carry

        lax.fori_loop(0, zi[0], q_rest, 0)
        wait(in_ffn)

    def back(oa):
        def body(j, carry):
            sp.block()
            base = pl.multiple_of((j - 1) * AR, AR)
            hs, ha, bc, dc = {}, {}, {}, {}
            sp.schedule(b_sum_tasks(gu_src(j), bc), *BC_SLOTS)
            sp.schedule(attn_tasks(base + A0, AR), *ATTN_SLOTS)
            packs = pack_tasks(oa, base, pl.multiple_of((j - 1) * (AR // 2), AR // 2), AR)
            sp.schedule(d_tasks(j, dc), *DC_SLOTS)
            strassen_x(raw_first((0, 2, 1, 3), NRAW), b_rhs(gu_src(j), bc), glu(hs, ha))
            tok = ha['tok']
            for t in packs:
                tok = t(None, tok)
            ffn_down(ha, dc, False)
            return carry

        lax.fori_loop(1, NC, body, 0)

        def out_copy(r0, n, i1, i2, cols):
            idx = (pl.ds(r0 + i1 * H + i2 * Q, n), cols)
            return cp(x_vm.at[idx], o2.at[idx], out_sem)

        def out_blocks(n, blocks):
            done_by = {ts[-1]: qd for ts, qd in _C_ORDER}
            todo = [(blk, t1, t2) for blk in range(len(blocks))
                    for ts1, _ in _C_ORDER for t1 in ts1 for ts2, _ in _C_ORDER for t2 in ts2]
            m, inner = {}, {}
            for i in range(0, len(todo), SLOT // n):
                group = todo[i:i + SLOT // n]
                ps = sp.dots([(_unpack(oa[7 * t1 + t2, pl.ds(blocks[blk][0] // 2, n // 2), :]),
                               _unpack(woc[7 * t1 + t2])) for blk, t1, t2 in group])
                for (blk, t1, t2), p in zip(group, ps):
                    r0, copies = blocks[blk]
                    m.setdefault((blk, t1), {})[t2] = acc[7 * t1 + t2, pl.ds(r0, n), :] + p
                    if t2 not in done_by:
                        continue
                    q2 = done_by[t2] ^ (t1 in _FLIP)
                    inner.setdefault((blk, q2), {})[t1] = _c_quadrant(m[blk, t1], done_by[t2])
                    if t1 not in done_by:
                        continue
                    q1 = done_by[t1]
                    r = pl.ds(r0 + (q1 // 2) * H + (q2 // 2) * Q, n)
                    c = (q1 % 2) * KH + (q2 % 2) * KQ
                    x_vm[r, c:c + KQ] = _c_quadrant(inner[blk, q2], q1).astype(bf16)
                    start(copies.get((q1, q2), []))

        final = {q1: (q1, 3 ^ (ts[-1] in _FLIP)) for ts, q1 in _C_ORDER}

        def whole(r0, n):
            return {final[3]: [out_copy(r0, n, i1, i2, slice(None))
                               for i1 in range(2) for i2 in range(2)]}

        done = (NC - 1) * AR
        sp.block()
        sp.schedule(pack_tasks(oa, done, done // 2, Q - done), *PACK4)
        last = {final[q1]: [out_copy(Q - PB, PB, q1 // 2, i2, pl.ds((q1 % 2) * KH, KH))
                            for i2 in range(2)] for q1 in range(3)}
        for q2 in range(4):
            last[3, q2] = [out_copy(Q - PB, PB, 1, q2 // 2, pl.ds(KH + (q2 % 2) * KQ, KQ))]
        copies = [whole(0, RB), whole(RB, PB), last]
        out_blocks(RB, [(0, copies[0])])
        out_blocks(PB, [(RB, copies[1]), (Q - PB, last)])
        for cs in copies:
            for key in cs:
                wait(cs[key])

    pl.run_scoped(front, pltpu.VMEM((D, 3 * D), bf16), pltpu.VMEM((3, D // 2, D), i32),
                  pltpu.VMEM((D, D), bf16))
    pl.run_scoped(back, pltpu.VMEM((49, Q // 2, KQ), i32))
    assert not sp.plan


_N_SEMS = 9


@jax.jit
def pallas_gated_mix__sliding_local_dilated__glu_gated_reglu__prompt_kernel(
    A_x: jax.Array,
    A_wqkv: jax.Array,
    A_wo: jax.Array,
    B_x: jax.Array,
    B_W_gate: jax.Array,
    B_W_up: jax.Array,
    B_W_down: jax.Array,
    gate_w: jax.Array,
):
    del B_x
    hbm = pl.BlockSpec(memory_space=pl.ANY)
    scratch = [
        pltpu.VMEM((S, D), bf16),
        pltpu.VMEM((S // 2, D), i32),
        pltpu.VMEM((5, H // 2, KH), i32),
        pltpu.VMEM((8, 128), bf16),
        pltpu.VMEM((NC, D, 2 * FC), bf16),
        pltpu.VMEM((NC, FC, D), bf16),
        pltpu.VMEM((49, Q, KQ), f32),
        pltpu.VMEM((8, S + QPAD, 128), f32),
        pltpu.VMEM((8, PAD + S, 128), f32),
        pltpu.VMEM((8, PAD + S, 128), f32),
        pltpu.VMEM((S, 128), f32),
        pltpu.VMEM((49, KQ // 2, KQ), i32),
        pltpu.VMEM((8, 128), i32),
        pltpu.SMEM((1,), i32),
        pltpu.SemaphoreType.DMA((_N_SEMS,)),
    ]
    return pl.pallas_call(
        _kernel,
        in_specs=[hbm] * 7,
        out_specs=hbm,
        out_shape=jax.ShapeDtypeStruct((1, S, D), bf16),
        scratch_shapes=scratch,
        compiler_params=pltpu.CompilerParams(vmem_limit_bytes=124 * 1024 * 1024),
    )(A_x, A_wqkv, A_wo, B_W_gate, B_W_up, B_W_down, gate_w.reshape(8, 128))
```

```python
import math

import jax
import jax.numpy as jnp
from jax import lax
import jax.experimental.pallas as pl
import jax.experimental.pallas.tpu as pltpu

f32 = jnp.float32
bf16 = jnp.bfloat16
i32 = jnp.int32

S = 2048
D = 1024
F = 3584
NH = 32
DH = D // NH
W = 8
DIL = 2
H = S // 2
Q = S // 4
KH = D // 2
KQ = D // 4
FC = 512
CH = FC // 2
CQ = FC // 4
NC = F // FC
NW = NC - 1
RB = 256
NRB = H // RB
PB = 128
PAD = 16
TP = DH + 1
AR = 64
A0 = Q - 6 * AR
QA = 160
QPAD = 112

BC_SLOTS = (2, 24)
ATTN_SLOTS = (24, 106)
DC_SLOTS = (26, 98)
VDEPTH = 2
PDEPTH = 3
VBC_SLOTS = (2, 16)
PREP01 = (16, 56)
PERMK = (64, 106)
WOS = (70, 112)
PACK4 = (4, 48)
NRAW = 3
DEPTH = 3
DEPTH2 = 3
H_DEPTH = 3

SCALE = DH ** -0.5
EXP2_SCALE = SCALE * math.log2(math.e)
NEG = -1e9 / SCALE


def _a_combos(a11, a12, a21, a22):
    return [a11 + a22, a21 + a22, a11, a22, a11 + a12, a21 - a11, a12 - a22]


def _b_combos(b11, b12, b21, b22):
    return [b11 + b22, b11, b12 - b22, b21 - b11, b22, b11 + b12, b21 + b22]


_C_TERMS = (((1, 0), (1, 3), (-1, 4), (1, 6)), ((1, 2), (1, 4)), ((1, 1), (1, 3)),
            ((1, 0), (-1, 1), (1, 2), (1, 5)))
_C_ORDER = (((2, 4), 1), ((1, 3), 2), ((0, 6), 0), ((5,), 3))


def _c_quadrant(m, qd):
    out = m[_C_TERMS[qd][0][1]]
    for sign, t in _C_TERMS[qd][1:]:
        out = out + m[t] if sign > 0 else out - m[t]
    return out


def _c_combos(m):
    return [_c_quadrant(m, qd) for qd in range(4)]


_FLIP = (1, 4, 5, 6)
_A_SLOT = {0: 0, 1: 1, 4: 2, 5: 3, 6: 4}
_B_SUMS = (2, 3, 0, 5, 6)
ORDER = (1, 4) + _B_SUMS


def _tree(op, xs):
    xs = list(xs)
    while len(xs) > 1:
        xs = [op(xs[i], xs[i + 1]) if i + 1 < len(xs) else xs[i] for i in range(0, len(xs), 2)]
    return xs[0]


def _pack(x):
    return pltpu.bitcast(x.astype(bf16), i32)


def _unpack(x):
    return pltpu.bitcast(x, bf16)


def _half(r):
    return slice(r.start // 2, r.stop // 2)


SLOT = 256


class _Spreader:
    def __init__(self, zero_ref):
        self.zero_ref = zero_ref
        self.plan = {}
        self.lists = 0
        self.now = 0

    def block(self):
        self.zero = self.zero_ref[...]
        self.never = self.zero != 0

    def link(self, after, x):
        if after is None:
            return x
        if after.dtype != x.dtype:
            after = pltpu.bitcast(after, x.dtype)
        return jnp.where(self.never, after, x)

    def chain(self, vals, prev, depth):
        for v in vals:
            v = pltpu.bitcast(v, i32) if v.dtype != i32 else v
            for r in range(0, v.shape[0], 8):
                for c in range(0, v.shape[1], 128):
                    tile = v[r:r + 8, c:c + 128]
                    if prev is None:
                        prev = tile
                        continue
                    prev = prev | tile
                    for i in range(depth - 1):
                        prev = (prev + self.zero) if i % 2 == 0 else (prev ^ self.zero)
        return prev

    def link_rows(self, after, x):
        return jnp.concatenate([self.link(after, x[r:r + 8, :]) for r in range(0, x.shape[0], 8)],
                               axis=0)

    def serial_combos(self, combos, x11, x12, x21, x22, after):
        return combos(self.link_rows(after, x11), x12, x21, self.link_rows(after, x22))

    def two_level(self, combos, blk, prev, depth, after=None):
        outer, outs, tok = [], [], after
        for r2 in range(2):
            for c2 in range(2):
                outer.append(self.serial_combos(
                    combos, *[blk(r1, r2, c1, c2) for r1 in range(2) for c1 in range(2)], tok))
                tok = self.chain([x[:8] for x in outer[-1]], None, 1)
        for t in range(7):
            flip = combos is _b_combos and t in _FLIP
            wide = _pack(jnp.concatenate(
                self.serial_combos(combos, *[outer[i ^ flip][t] for i in range(4)], tok), axis=1))
            outs += [wide[:, c:c + 128] for c in range(0, 7 * 128, 128)]
            tok = self.chain(outs[-7:], tok, depth)
        return outs, self.chain([tok], prev, 1)

    def schedule(self, tasks, first, last):
        self.lists += 1
        for i, t in enumerate(tasks):
            pos = self.now + first + ((i + 1) * (last - first) - 1) // len(tasks)
            self.plan.setdefault(pos, []).append((t, self.lists))

    def dots(self, pairs):
        m = pairs[0][0].shape[0]
        tiles = [(i, r, c) for i, (_, rhs) in enumerate(pairs)
                 for c in range(0, rhs.shape[1], 128) for r in range(0, rhs.shape[0], 128)]
        nslots = m * len(tiles) // (4 * SLOT)
        deps = {}
        for sl in range(nslots):
            ps = sl * SLOT // m
            toks = {}
            for t, lane in self.plan.pop(self.now + sl, []):
                tok = t(toks.get(lane))
                if tok is not None:
                    toks[lane] = tok
            for tok in toks.values():
                deps[ps] = tok | deps[ps] if ps in deps else tok
        self.now += nslots
        tied = {tile: d for ps, d in deps.items() for tile in tiles[4 * ps:4 * ps + 4]}
        outs = []
        for i, (lhs, rhs) in enumerate(pairs):
            if any(key[0] == i for key in tied):
                parts = []
                for r in range(0, rhs.shape[0], 128):
                    top = [rhs[r:r + 16, c:c + 128] for c in range(0, rhs.shape[1], 128)]
                    top = [_unpack(self.link(tied[i, r, c * 128], _pack(t0)))
                           if (i, r, c * 128) in tied else t0 for c, t0 in enumerate(top)]
                    parts += [jnp.concatenate(top, axis=1), rhs[r + 16:r + 128, :]]
                rhs = jnp.concatenate(parts, axis=0)
            outs.append(jnp.dot(lhs, rhs, preferred_element_type=f32))
        return outs

    def dot(self, lhs, rhs):
        return self.dots([(lhs, rhs)])[0]


def _kernel(x_hbm, wqkv_hbm, wo_hbm, wg_hbm, wu_hbm, wd_hbm, gw_hbm, out_hbm,
            x_vm, xn, xa, gw_vm, wgu, wd, acc, q_s, k_s, v_s, gs, woc, zs, zi, sems):
    def cp(src, dst, sem):
        return pltpu.make_async_copy(src, dst, sems.at[sem])

    def cp_gu(j, p, sem):
        return cp((wg_hbm, wu_hbm)[p % 2].at[:, pl.ds(j * FC + (p // 2) * CH, CH)],
                  wgu.at[j % NW, :, pl.ds(p * CH, CH)], sem)

    def cp_d(j, sem):
        return cp(wd_hbm.at[pl.ds(j * FC, FC), :], wd.at[j % NW], sem)

    def cp_x(rb, hf, sem):
        idx = (pl.ds(hf * H + rb * RB, RB), slice(None))
        return cp(x_hbm.at[0].at[idx], x_vm.at[idx], sem)

    o2 = out_hbm.at[0]
    in0 = [cp_x(0, 0, 0), cp_gu(0, 0, 0)]
    in1 = [cp_x(0, 1, 1)]
    in2 = [cp_gu(0, 1, 2)]
    in3 = [cp_gu(0, 2, 3), cp_gu(0, 3, 3), cp(gw_hbm, gw_vm, 3)]
    in4 = [cp_x(rb, hf, 4) for rb in (1, 2) for hf in range(2)]
    in5 = [cp_x(3, 0, 5), cp_x(3, 1, 5), cp_d(0, 5)]
    in_ffn = [c for j in range(1, NC) for c in [cp_gu(j, p, 7) for p in range(4)] + [cp_d(j, 7)]]
    out_sem = 8

    def start(cs):
        for c in cs:
            c.start()

    def wait(cs):
        for c in cs:
            c.wait()

    start(in0 + in1 + in2)

    zs[...] = jnp.zeros((8, 128), i32)
    zi[0] = 1
    sp = _Spreader(zs)

    def rows(rb, hf=0):
        return slice(hf * H + rb * RB, hf * H + (rb + 1) * RB)

    def x_lhs(t, rb):
        if t == 2:
            return _unpack(xn[_half(rows(rb, 0)), :KH])
        if t == 3:
            return _unpack(xn[_half(rows(rb, 1)), KH:])
        return _unpack(xa[_A_SLOT[t], _half(rows(rb)), :])

    def prep_tasks(rb, sums=True, gate=True):
        def task(s0):
            def run(first):
                prev = None
                gw = gw_vm[...].astype(f32)
                r = [slice(hf * H + rb * RB + s0, hf * H + rb * RB + s0 + 16) for hf in range(2)]
                z = [None, None]
                for c in range(4):
                    cols = [slice(kh * KH + c * 128, kh * KH + (c + 1) * 128) for kh in range(2)]
                    xs = [sp.link(prev, _pack(x_vm[r[qd // 2], cols[qd % 2]])) for qd in range(4)]
                    a = [_unpack(t).astype(f32) for t in xs]
                    outs = []
                    if sums:
                        for qd in range(4):
                            xn[_half(r[qd // 2]), cols[qd % 2]] = xs[qd]
                        cs = _a_combos(*a)
                        for t, slot in _A_SLOT.items():
                            outs.append(_pack(cs[t]))
                            xa[slot, _half(r[0]), cols[0]] = outs[-1]
                    if gate:
                        for qd in range(4):
                            g0 = (qd % 2) * 4 + c
                            term = a[qd] * gw[g0:g0 + 1, :]
                            z[qd // 2] = term if z[qd // 2] is None else z[qd // 2] + term
                        outs += z
                    prev = sp.chain(outs, prev, 1)
                if gate:
                    for hf in range(2):
                        g = jax.nn.sigmoid(jnp.sum(z[hf], axis=1, keepdims=True))
                        g = jnp.broadcast_to(g, (16, 128))
                        gs[r[hf], :] = g
                        prev = sp.chain([g], prev, 1)
                return sp.chain([prev], first, 1)
            return run
        return [task(s0) for s0 in range(0, RB, 16)]

    def b_sum_tasks(src, dst, depth=DEPTH):
        def task(r0):
            def run(prev):
                raw = [src(slice(a * KH + r0, a * KH + r0 + 16), slice(c * KH, (c + 1) * KH))
                       for a in range(2) for c in range(2)]
                cs = _b_combos(*[b.astype(f32) for b in raw])
                for t in _B_SUMS:
                    dst.setdefault(t, []).append(_pack(cs[t]))
                return sp.chain([dst[t][-1] for t in _B_SUMS], prev, depth)
            return run
        return [task(r0) for r0 in range(0, KH, 16)]

    def b_rhs(src, sums):
        def rhs(t):
            if t == 1:
                return src(slice(0, KH), slice(0, KH))
            if t == 4:
                return src(slice(KH, D), slice(KH, D))
            return _unpack(jnp.concatenate(sums[t], axis=0))
        return rhs

    def strassen_x(order, rhs, finish):
        m = {}
        for rb, t in order:
            m.setdefault(rb, {})[t] = sp.dot(x_lhs(t, rb), rhs(t))
            if len(m[rb]) == 7:
                finish(rb, m.pop(rb))

    def h_sums(rb, cs, r0, sub):
        h = []
        for qd, cc in enumerate(cs):
            g0 = (qd // 2) * H + rb * RB + r0
            omg = 1.0 - gs[g0:g0 + sub, :]
            omg = jnp.concatenate([omg] * (CH // 128), axis=1)
            h.append(jnp.maximum(cc[:, :CH], 0.0) * cc[:, CH:] * omg)
        return _a_combos(*h)

    def glu_tasks(hs, rb, cs, sub):
        hs[rb] = [[] for _ in range(7)]

        def task(r0):
            def run(prev):
                sums = h_sums(rb, [cc[r0:r0 + sub] for cc in cs], r0, sub)
                for t in range(7):
                    hs[rb][t].append(sums[t])
                if sub < RB:
                    return sp.chain([sums[t] for t in _A_SLOT], prev, DEPTH2)
            return run
        return [task(r0) for r0 in range(0, RB, sub)]

    def down_lhs(hs, b, ha):
        tok = None
        for t in range(7):
            s0, s1 = [jnp.concatenate(hs[rb][t], axis=0) for rb in (b, b + 2)]
            slabs = []
            for r in range(0, RB, 16):
                slabs.append(sp.serial_combos(
                    _a_combos, s0[r:r + 16, :CQ], s0[r:r + 16, CQ:],
                    s1[r:r + 16, :CQ], s1[r:r + 16, CQ:], tok))
                tok = sp.chain([slabs[-1][t2] for t2 in _A_SLOT], None, H_DEPTH)
            for t2 in range(7):
                ha[b, 7 * t + t2] = jnp.concatenate([sl[t2] for sl in slabs], axis=0).astype(bf16)
        ha['tok'] = tok

    def d_tasks(j, dst):
        def task(r0, c):
            def run(prev):
                def blk(k1, k2, n1, n2):
                    r, c0 = k1 * CH + k2 * CQ + r0, n1 * KH + n2 * KQ + c * 128
                    return wd[j, r:r + 16, c0:c0 + 128].astype(f32)
                cs, tok = sp.two_level(_b_combos, blk, prev, DEPTH2)
                for t in range(49):
                    dst.setdefault((t, c), []).append(cs[t])
                return tok
            return run
        return [task(r0, c) for r0 in range(0, CQ, 16) for c in range(2)]

    def ffn_down(ha, dc, first):
        rhs = [_unpack(jnp.concatenate([jnp.concatenate(dc[t, c], axis=0) for c in range(2)], axis=1))
               for t in range(49)]
        todo = [(b, t) for b in range(2) for t in range(49)]
        for i in range(0, len(todo), 2):
            pair = todo[i:i + 2]
            ps = sp.dots([(ha[b, t], rhs[t]) for b, t in pair])
            for (b, t), p in zip(pair, ps):
                if first:
                    acc[t, b * RB:(b + 1) * RB, :] = p
                else:
                    acc[t, b * RB:(b + 1) * RB, :] += p

    def perm_tasks(wqkv_vm, wp, i, tbuf):
        def fwd(rb, c):
            def run(prev):
                c0 = i * D + c * 128
                tt = pltpu.bitcast(wqkv_vm[rb * 256:(rb + 1) * 256, c0:c0 + 128], f32).T
                for hh in range(4):
                    tbuf[rb, pl.ds((4 * c + hh) * TP, DH), :] = tt[hh * DH:(hh + 1) * DH, :]
                return sp.chain([tt], prev, 1)
            return run

        def bwd(rb, j):
            def run(prev):
                g = jnp.concatenate(
                    [tbuf[rb, pl.ds(4 * j + dd, NH, stride=TP), :] for dd in range(4)], axis=0).T
                wp[i, rb * 128:(rb + 1) * 128, j * 128:(j + 1) * 128] = pltpu.bitcast(g, i32)
            return run
        tasks = []
        for rb in range(4):
            tasks += [fwd(rb, c) for c in range(8)] + [bwd(rb, j) for j in range(8)]
        return tasks

    def wo_tasks(wo_vm):
        def stage(c):
            return 4 + c % 4, (c // 4) * NH * TP

        def spread(h0):
            def run(prev):
                blk = wo_vm[h0 * DH:(h0 + 2) * DH, :].astype(f32)
                for h in range(2):
                    for c in range(8):
                        sl, r0 = stage(c)
                        q_s[sl, pl.ds(r0 + (h0 + h) * TP, DH), :] = (
                            blk[h * DH:(h + 1) * DH, c * 128:(c + 1) * 128])
                return sp.chain([blk], prev, 1)
            return run

        def gather(d, h0, c):
            def run(after):
                def blk(k1, k2, n1, n2):
                    sl, r0 = stage(4 * n1 + 2 * n2 + c)
                    r0 += h0 * TP + 16 * k1 + 8 * k2 + d
                    return q_s[sl, pl.ds(r0, 16, stride=TP), :]
                cs, tok = sp.two_level(_b_combos, blk, None, DEPTH2, after)
                r = (d * NH + h0) // 2
                for t in range(49):
                    woc[t, r:r + 8, c * 128:(c + 1) * 128] = cs[t]
                return tok
            return run
        return ([spread(h0) for h0 in range(0, NH, 2)],
                [gather(d, h0, c) for d in range(8) for h0 in (0, 16) for c in range(2)])

    def proj(wp, i, dst, pad, slabs):
        lhs = jnp.concatenate([xn[r0 // 2:(r0 + n) // 2, :] for r0, n in slabs], axis=0)
        p = sp.dot(_unpack(lhs), _unpack(wp[i]))
        at = 0
        for r0, n in slabs:
            for j in range(8):
                dst[j, pad + r0:pad + r0 + n, :] = p[at:at + n, j * 128:(j + 1) * 128]
            at += n

    def v_finish(rb, m):
        cs = _c_combos(m)
        for qd, cc in enumerate(cs):
            r0 = PAD + (qd // 2) * H + rb * RB
            for j in range(4):
                v_s[(qd % 2) * 4 + j, r0:r0 + RB, :] = cc[:, j * 128:(j + 1) * 128]
        if rb == 0:
            for j in range(8):
                src = cs[j // 4][0:1, (j % 4) * 128:(j % 4 + 1) * 128]
                v_s[j, 0:PAD, :] = jnp.broadcast_to(src, (PAD, 128))

    def attn_group(row, masked):
        def run(prev):
            g = 8
            q = [q_s[j, pl.ds(row, g), :] for j in range(8)]
            ls = []
            for w in range(W):
                a = None
                for j in range(8):
                    term = q[j] * k_s[j, pl.ds(row + (PAD - DIL * w), g), :]
                    a = sp.link(ls[-1] if ls else None, term) if a is None else a + term
                ls.append(a)
            rs = [pltpu.roll(a, 64, 1) for a in ls]
            ls = [a + r for a, r in zip(ls, rs)]
            rs = [pltpu.roll(a, 32, 1) for a in ls]
            ls = [a + r for a, r in zip(ls, rs)]
            if masked:
                ri = row + lax.broadcasted_iota(i32, (g, 128), 0)
                ls = [ls[0]] + [jnp.where(ri >= DIL * w, ls[w], NEG) for w in range(1, W)]
            m = _tree(jnp.maximum, ls)
            ps = [jnp.exp2((l - m) * EXP2_SCALE) for l in ls]
            r = gs[pl.ds(row, g), :] / _tree(jnp.add, ps)
            outs = []
            for j in range(8):
                a = None
                for w in range(W):
                    term = ps[w] * v_s[j, pl.ds(row + (PAD - DIL * w), g), :]
                    a = sp.link(outs[-1] if outs else None, term) if a is None else a + term
                outs.append(a * r)
            for j in range(8):
                q_s[j, pl.ds(row, g), :] = outs[j]
            return sp.chain([outs[-1]], prev, 1)
        return run

    def attn_tasks(base, nrows, first=False):
        return [attn_group(base + (qq * Q + r), first and qq == 0 and r < PAD)
                for r in range(0, nrows, 8) for qq in range(4)]

    def pack_tasks(oa, base, hbase, nrows):
        def task(r, c):
            def run(prev, after=None):
                def blk(i1, i2, k1, k2):
                    return q_s[4 * k1 + 2 * k2 + c, pl.ds(base + (i1 * H + i2 * Q + r), 16), :]
                cs, tok = sp.two_level(_a_combos, blk, prev, DEPTH2 if after is None else PDEPTH, after)
                for t in range(49):
                    oa[t, pl.ds(hbase + r // 2, 8), c * 128:(c + 1) * 128] = cs[t]
                return tok
            return run
        return [task(r, c) for r in range(0, nrows, 16) for c in range(2)]

    GS = RB * (KH // 128) * (FC // 128) * 7 // (4 * SLOT)
    DS = 49
    PS = 2 * RB * (D // 128) * (D // 128) // (4 * SLOT)

    def glu(hs, ha):
        def finish(rb, m):
            glu_tasks(hs, rb, _c_combos(m), RB)[0](None)
            if rb >= 2:
                down_lhs(hs, rb - 2, ha)
        return finish

    def raw_first(rbs, n):
        lead = [(rb, t) for rb in rbs[:n] for t in ORDER[:2]]
        return lead + [(rb, t) for rb in rbs for t in ORDER if (rb, t) not in lead]

    def gu_src(j):
        return lambda r, c: wgu[j, r, c]

    def front(wqkv_vm, wp, wo_vm):
        in_q, in_k, in_v = [
            cp(wqkv_hbm.at[:, pl.ds(i * D, D)], wqkv_vm.at[:, pl.ds(i * D, D)], (6, 6, 5)[i])
            for i in range(3)]
        in_wo = cp(wo_hbm, wo_vm, 6)

        def plain(rb, hf, p):
            return sp.dot(x_vm[rows(rb, hf), :], wgu[0, :, p * CH:(p + 1) * CH])

        def plain_finish(hs, rb, c):
            cs = [jnp.concatenate(c[2 * qd:2 * qd + 2], axis=1) for qd in range(4)]
            return glu_tasks(hs, rb, cs, 16)

        def chunk0(_, carry):
            hs, bc, dc = {}, {}, {}
            wait(in0)
            start(in3)
            c0 = {(0, 0): plain(0, 0, 0)}
            wait(in1)
            c0[1, 0] = plain(0, 1, 0)
            wait(in2)
            start(in4)
            for hf in range(2):
                c0[hf, 1] = plain(0, hf, 1)
            wait(in3)
            start(in5)
            sp.block()
            bt = b_sum_tasks(gu_src(0), bc)
            sp.schedule(bt[:12], 3, 16)
            sp.schedule(prep_tasks(0, sums=False), 3, 16)
            for p in (2, 3):
                for hf in range(2):
                    c0[hf, p] = plain(0, hf, p)
            c0 = [c0[hf, p] for hf in range(2) for p in range(4)]
            wait(in4)
            start([in_v])
            sp.block()
            sp.schedule(bt[12:], 3, 32)
            sp.schedule(prep_tasks(1, sums=False), 2, 10)
            sp.schedule(prep_tasks(2), 10, 32)
            c1 = [plain(1, hf, p) for hf in range(2) for p in range(4)]
            wait(in5 + [in_v])
            start([in_k, in_wo, in_q])
            sp.block()
            for j in range(8):
                k_s[j, 0:PAD, :] = jnp.zeros((PAD, 128), f32)
            ha = {}
            sp.schedule(prep_tasks(3), 2, GS)
            sp.schedule(plain_finish(hs, 0, c0), 2, GS)
            sp.schedule(plain_finish(hs, 1, c1), GS + 6, 2 * GS)
            sp.schedule(d_tasks(0, dc), GS - 2, 2 * GS)
            sp.schedule(perm_tasks(wqkv_vm, wp, 2, q_s), 2 * GS + 6, 2 * GS + DS - 8)
            strassen_x([(rb, t) for rb in (2, 3) for t in ORDER], b_rhs(gu_src(0), bc),
                       glu(hs, ha))
            ffn_down(ha, dc, True)
            return carry

        lax.fori_loop(0, zi[0], chunk0, 0)

        wait([in_k, in_wo, in_q])
        start(in_ffn)
        sp.block()
        vb = {}
        v_src = lambda r, c: _unpack(wp[2, _half(r), c])
        wo_spread, wo_gather = wo_tasks(wo_vm)
        sp.schedule(b_sum_tasks(v_src, vb, VDEPTH), *VBC_SLOTS)
        sp.schedule(prep_tasks(0, gate=False) + prep_tasks(1, gate=False), *PREP01)
        sp.schedule(perm_tasks(wqkv_vm, wp, 1, k_s.at[:, PAD:, :]), *PERMK)
        sp.schedule(wo_spread, *WOS)
        strassen_x(raw_first((2, 3, 0, 1), 2), b_rhs(v_src, vb), v_finish)
        sp.schedule(perm_tasks(wqkv_vm, wp, 0, q_s), 4, 3 * PS)
        tok = None
        for t in wo_gather:
            tok = t(tok)
        for rb in range(NRB):
            proj(wp, 1, k_s, PAD, [(rb * Q, Q)])
        proj(wp, 0, q_s, 0, [(qq * Q, QA) for qq in range(4)])

        def q_rest(_, carry):
            sp.block()
            n = (Q - QA) // 2
            total = 4 * (Q - QA) * 64 // (4 * SLOT)
            sp.schedule(attn_tasks(0, A0, True), 4, total)
            for r0 in (QA, QA + n):
                proj(wp, 0, q_s, 0, [(qq * Q + r0, n) for qq in range(4)])
            return carry

        lax.fori_loop(0, zi[0], q_rest, 0)
        wait(in_ffn)

    def back(oa):
        def body(j, carry):
            sp.block()
            base = pl.multiple_of((j - 1) * AR, AR)
            hs, ha, bc, dc = {}, {}, {}, {}
            slot = jnp.where(j == NW, 0, j)
            sp.schedule(b_sum_tasks(gu_src(slot), bc), *BC_SLOTS)
            sp.schedule(attn_tasks(base + A0, AR), *ATTN_SLOTS)
            packs = pack_tasks(oa, base, pl.multiple_of((j - 1) * (AR // 2), AR // 2), AR)
            sp.schedule(d_tasks(slot, dc), *DC_SLOTS)
            strassen_x(raw_first((0, 2, 1, 3), NRAW), b_rhs(gu_src(slot), bc), glu(hs, ha))
            tok = ha['tok']
            for t in packs:
                tok = t(None, tok)
            ffn_down(ha, dc, False)
            return carry

        lax.fori_loop(1, NC, body, 0)

        def out_copy(r0, n, i1, i2, cols):
            idx = (pl.ds(r0 + i1 * H + i2 * Q, n), cols)
            return cp(x_vm.at[idx], o2.at[idx], out_sem)

        def out_blocks(n, blocks):
            done_by = {ts[-1]: qd for ts, qd in _C_ORDER}
            todo = [(blk, t1, t2) for blk in range(len(blocks))
                    for ts1, _ in _C_ORDER for t1 in ts1 for ts2, _ in _C_ORDER for t2 in ts2]
            m, inner = {}, {}
            for i in range(0, len(todo), SLOT // n):
                group = todo[i:i + SLOT // n]
                ps = sp.dots([(_unpack(oa[7 * t1 + t2, pl.ds(blocks[blk][0] // 2, n // 2), :]),
                               _unpack(woc[7 * t1 + t2])) for blk, t1, t2 in group])
                for (blk, t1, t2), p in zip(group, ps):
                    r0, copies = blocks[blk]
                    m.setdefault((blk, t1), {})[t2] = acc[7 * t1 + t2, pl.ds(r0, n), :] + p
                    if t2 not in done_by:
                        continue
                    q2 = done_by[t2] ^ (t1 in _FLIP)
                    inner.setdefault((blk, q2), {})[t1] = _c_quadrant(m[blk, t1], done_by[t2])
                    if t1 not in done_by:
                        continue
                    q1 = done_by[t1]
                    r = pl.ds(r0 + (q1 // 2) * H + (q2 // 2) * Q, n)
                    c = (q1 % 2) * KH + (q2 % 2) * KQ
                    x_vm[r, c:c + KQ] = _c_quadrant(inner[blk, q2], q1).astype(bf16)
                    start(copies.get((q1, q2), []))

        final = {q1: (q1, 3 ^ (ts[-1] in _FLIP)) for ts, q1 in _C_ORDER}

        def whole(r0, n):
            return {final[3]: [out_copy(r0, n, i1, i2, slice(None))
                               for i1 in range(2) for i2 in range(2)]}

        done = (NC - 1) * AR
        sp.block()
        sp.schedule(pack_tasks(oa, done, done // 2, Q - done), *PACK4)
        last = {final[q1]: [out_copy(Q - PB, PB, q1 // 2, i2, pl.ds((q1 % 2) * KH, KH))
                            for i2 in range(2)] for q1 in range(3)}
        for q2 in range(4):
            last[3, q2] = [out_copy(Q - PB, PB, 1, q2 // 2, pl.ds(KH + (q2 % 2) * KQ, KQ))]
        copies = [whole(0, RB), whole(RB, PB), last]
        out_blocks(RB, [(0, copies[0])])
        out_blocks(PB, [(RB, copies[1]), (Q - PB, last)])
        for cs in copies:
            for key in cs:
                wait(cs[key])

    pl.run_scoped(front, pltpu.VMEM((D, 3 * D), bf16), pltpu.VMEM((3, D // 2, D), i32),
                  pltpu.VMEM((D, D), bf16))
    pl.run_scoped(back, pltpu.VMEM((49, Q // 2, KQ), i32))
    assert not sp.plan


_N_SEMS = 9


@jax.jit
def pallas_gated_mix__sliding_local_dilated__glu_gated_reglu__prompt_kernel(
    A_x: jax.Array,
    A_wqkv: jax.Array,
    A_wo: jax.Array,
    B_x: jax.Array,
    B_W_gate: jax.Array,
    B_W_up: jax.Array,
    B_W_down: jax.Array,
    gate_w: jax.Array,
):
    del B_x
    hbm = pl.BlockSpec(memory_space=pl.ANY)
    scratch = [
        pltpu.VMEM((S, D), bf16),
        pltpu.VMEM((S // 2, D), i32),
        pltpu.VMEM((5, H // 2, KH), i32),
        pltpu.VMEM((8, 128), bf16),
        pltpu.VMEM((NW, D, 2 * FC), bf16),
        pltpu.VMEM((NW, FC, D), bf16),
        pltpu.VMEM((49, Q, KQ), f32),
        pltpu.VMEM((8, S + QPAD, 128), f32),
        pltpu.VMEM((8, PAD + S, 128), f32),
        pltpu.VMEM((8, PAD + S, 128), f32),
        pltpu.VMEM((S, 128), f32),
        pltpu.VMEM((49, KQ // 2, KQ), i32),
        pltpu.VMEM((8, 128), i32),
        pltpu.SMEM((1,), i32),
        pltpu.SemaphoreType.DMA((_N_SEMS,)),
    ]
    return pl.pallas_call(
        _kernel,
        in_specs=[hbm] * 7,
        out_specs=hbm,
        out_shape=jax.ShapeDtypeStruct((1, S, D), bf16),
        scratch_shapes=scratch,
        compiler_params=pltpu.CompilerParams(vmem_limit_bytes=127 * 1024 * 1024),
    )(A_x, A_wqkv, A_wo, B_W_gate, B_W_up, B_W_down, gate_w.reshape(8, 128))
```

```python
import math

import jax
import jax.numpy as jnp
from jax import lax
import jax.experimental.pallas as pl
import jax.experimental.pallas.tpu as pltpu

f32 = jnp.float32
bf16 = jnp.bfloat16
i32 = jnp.int32

S = 2048
D = 1024
F = 3584
NH = 32
DH = D // NH
W = 8
DIL = 2
H = S // 2
Q = S // 4
KH = D // 2
KQ = D // 4
FC = 512
CH = FC // 2
CQ = FC // 4
NC = F // FC
NW = NC - 1
RB = 256
NRB = H // RB
PB = 128
PAD = 16
TP = DH + 1
AR = 64
A0 = Q - 6 * AR
QA = 160
QPAD = 112

BC_SLOTS = (2, 24)
ATTN_SLOTS = (24, 106)
DC_SLOTS = (26, 98)
VBC_SLOTS = (2, 16)
PREP01 = (16, 56)
PERMK = (64, 106)
WOS = (70, 112)
PACK4 = (4, 48)
NRAW = 3
DEPTH = 3
VDEPTH = 2
DEPTH2 = 3
H_DEPTH = 3

SCALE = DH ** -0.5
EXP2_SCALE = SCALE * math.log2(math.e)
NEG = -1e9 / SCALE


def _a_combos(a11, a12, a21, a22):
    return [a11 + a22, a21 + a22, a11, a22, a11 + a12, a21 - a11, a12 - a22]


def _b_combos(b11, b12, b21, b22):
    return [b11 + b22, b11, b12 - b22, b21 - b11, b22, b11 + b12, b21 + b22]


_C_TERMS = (((1, 0), (1, 3), (-1, 4), (1, 6)), ((1, 2), (1, 4)), ((1, 1), (1, 3)),
            ((1, 0), (-1, 1), (1, 2), (1, 5)))
_C_ORDER = (((2, 4), 1), ((1, 3), 2), ((0, 6), 0), ((5,), 3))


def _c_quadrant(m, qd):
    out = m[_C_TERMS[qd][0][1]]
    for sign, t in _C_TERMS[qd][1:]:
        out = out + m[t] if sign > 0 else out - m[t]
    return out


def _c_combos(m):
    return [_c_quadrant(m, qd) for qd in range(4)]


_FLIP = (1, 4, 5, 6)
_A_SLOT = {0: 0, 1: 1, 4: 2, 5: 3, 6: 4}
_B_SUMS = (2, 3, 0, 5, 6)
ORDER = (1, 4) + _B_SUMS


def _tree(op, xs):
    xs = list(xs)
    while len(xs) > 1:
        xs = [op(xs[i], xs[i + 1]) if i + 1 < len(xs) else xs[i] for i in range(0, len(xs), 2)]
    return xs[0]


def _pack(x):
    return pltpu.bitcast(x.astype(bf16), i32)


def _unpack(x):
    return pltpu.bitcast(x, bf16)


def _half(r):
    return slice(r.start // 2, r.stop // 2)


SLOT = 256


class _Spreader:
    def __init__(self, zero_ref):
        self.zero_ref = zero_ref
        self.plan = {}
        self.lists = 0
        self.now = 0

    def block(self):
        self.zero = self.zero_ref[...]
        self.never = self.zero != 0

    def link(self, after, x):
        if after is None:
            return x
        if after.dtype != x.dtype:
            after = pltpu.bitcast(after, x.dtype)
        return jnp.where(self.never, after, x)

    def chain(self, vals, prev, depth):
        for v in vals:
            v = pltpu.bitcast(v, i32) if v.dtype != i32 else v
            for r in range(0, v.shape[0], 8):
                for c in range(0, v.shape[1], 128):
                    tile = v[r:r + 8, c:c + 128]
                    if prev is None:
                        prev = tile
                        continue
                    prev = prev | tile
                    for i in range(depth - 1):
                        prev = (prev + self.zero) if i % 2 == 0 else (prev ^ self.zero)
        return prev

    def link_rows(self, after, x):
        return jnp.concatenate([self.link(after, x[r:r + 8, :]) for r in range(0, x.shape[0], 8)],
                               axis=0)

    def serial_combos(self, combos, x11, x12, x21, x22, after):
        return combos(self.link_rows(after, x11), x12, x21, self.link_rows(after, x22))

    def two_level(self, combos, blk, prev, depth, after=None):
        outer, outs, tok = [], [], after
        for r2 in range(2):
            for c2 in range(2):
                outer.append(self.serial_combos(
                    combos, *[blk(r1, r2, c1, c2) for r1 in range(2) for c1 in range(2)], tok))
                tok = self.chain([x[:8] for x in outer[-1]], None, 1)
        for t in range(7):
            flip = combos is _b_combos and t in _FLIP
            wide = _pack(jnp.concatenate(
                self.serial_combos(combos, *[outer[i ^ flip][t] for i in range(4)], tok), axis=1))
            outs += [wide[:, c:c + 128] for c in range(0, 7 * 128, 128)]
            tok = self.chain(outs[-7:], tok, depth)
        return outs, self.chain([tok], prev, 1)

    def schedule(self, tasks, first, last):
        self.lists += 1
        for i, t in enumerate(tasks):
            pos = self.now + first + ((i + 1) * (last - first) - 1) // len(tasks)
            self.plan.setdefault(pos, []).append((t, self.lists))

    def dots(self, pairs):
        m = pairs[0][0].shape[0]
        tiles = [(i, r, c) for i, (_, rhs) in enumerate(pairs)
                 for c in range(0, rhs.shape[1], 128) for r in range(0, rhs.shape[0], 128)]
        nslots = m * len(tiles) // (4 * SLOT)
        deps = {}
        for sl in range(nslots):
            ps = sl * SLOT // m
            toks = {}
            for t, lane in self.plan.pop(self.now + sl, []):
                tok = t(toks.get(lane))
                if tok is not None:
                    toks[lane] = tok
            for tok in toks.values():
                deps[ps] = tok | deps[ps] if ps in deps else tok
        self.now += nslots
        tied = {tile: d for ps, d in deps.items() for tile in tiles[4 * ps:4 * ps + 4]}
        outs = []
        for i, (lhs, rhs) in enumerate(pairs):
            if any(key[0] == i for key in tied):
                parts = []
                for r in range(0, rhs.shape[0], 128):
                    top = [rhs[r:r + 16, c:c + 128] for c in range(0, rhs.shape[1], 128)]
                    top = [_unpack(self.link(tied[i, r, c * 128], _pack(t0)))
                           if (i, r, c * 128) in tied else t0 for c, t0 in enumerate(top)]
                    parts += [jnp.concatenate(top, axis=1), rhs[r + 16:r + 128, :]]
                rhs = jnp.concatenate(parts, axis=0)
            outs.append(jnp.dot(lhs, rhs, preferred_element_type=f32))
        return outs

    def dot(self, lhs, rhs):
        return self.dots([(lhs, rhs)])[0]


def _kernel(x_hbm, wqkv_hbm, wo_hbm, wg_hbm, wu_hbm, wd_hbm, gw_hbm, out_hbm,
            x_vm, xn, xa, gw_vm, wgu, wd, acc, q_s, k_s, v_s, gs, woc, zs, zi, sems):
    def cp(src, dst, sem):
        return pltpu.make_async_copy(src, dst, sems.at[sem])

    def cp_gu(j, p, sem):
        return cp((wg_hbm, wu_hbm)[p % 2].at[:, pl.ds(j * FC + (p // 2) * CH, CH)],
                  wgu.at[j % NW, :, pl.ds(p * CH, CH)], sem)

    def cp_d(j, sem):
        return cp(wd_hbm.at[pl.ds(j * FC, FC), :], wd.at[j % NW], sem)

    def cp_x(rb, hf, sem):
        idx = (pl.ds(hf * H + rb * RB, RB), slice(None))
        return cp(x_hbm.at[0].at[idx], x_vm.at[idx], sem)

    o2 = out_hbm.at[0]
    in0 = [cp_x(0, 0, 0), cp_gu(0, 0, 0)]
    in1 = [cp_x(0, 1, 1)]
    in2 = [cp_gu(0, 1, 2)]
    in3 = [cp_gu(0, 2, 3), cp_gu(0, 3, 3), cp(gw_hbm, gw_vm, 3)]
    in4 = [cp_x(rb, hf, 4) for rb in (1, 2) for hf in range(2)]
    in5 = [cp_x(3, 0, 5), cp_x(3, 1, 5), cp_d(0, 5)]
    in_ffn = [c for j in range(1, NC) for c in [cp_gu(j, p, 7) for p in range(4)] + [cp_d(j, 7)]]
    out_sem = 8

    def start(cs):
        for c in cs:
            c.start()

    def wait(cs):
        for c in cs:
            c.wait()

    start(in0 + in1 + in2)

    zs[...] = jnp.zeros((8, 128), i32)
    zi[0] = 1
    sp = _Spreader(zs)

    def rows(rb, hf=0):
        return slice(hf * H + rb * RB, hf * H + (rb + 1) * RB)

    def x_lhs(t, rb):
        if t == 2:
            return _unpack(xn[_half(rows(rb, 0)), :KH])
        if t == 3:
            return _unpack(xn[_half(rows(rb, 1)), KH:])
        return _unpack(xa[_A_SLOT[t], _half(rows(rb)), :])

    def prep_tasks(rb, sums=True, gate=True):
        def task(s0):
            def run(first):
                prev = None
                gw = gw_vm[...].astype(f32)
                r = [slice(hf * H + rb * RB + s0, hf * H + rb * RB + s0 + 16) for hf in range(2)]
                z = [None, None]
                for c in range(4):
                    cols = [slice(kh * KH + c * 128, kh * KH + (c + 1) * 128) for kh in range(2)]
                    xs = [sp.link(prev, _pack(x_vm[r[qd // 2], cols[qd % 2]])) for qd in range(4)]
                    a = [_unpack(t).astype(f32) for t in xs]
                    outs = []
                    if sums:
                        for qd in range(4):
                            xn[_half(r[qd // 2]), cols[qd % 2]] = xs[qd]
                        cs = _a_combos(*a)
                        for t, slot in _A_SLOT.items():
                            outs.append(_pack(cs[t]))
                            xa[slot, _half(r[0]), cols[0]] = outs[-1]
                    if gate:
                        for qd in range(4):
                            g0 = (qd % 2) * 4 + c
                            term = a[qd] * gw[g0:g0 + 1, :]
                            z[qd // 2] = term if z[qd // 2] is None else z[qd // 2] + term
                        outs += z
                    prev = sp.chain(outs, prev, 1)
                if gate:
                    for hf in range(2):
                        g = jax.nn.sigmoid(jnp.sum(z[hf], axis=1, keepdims=True))
                        g = jnp.broadcast_to(g, (16, 128))
                        gs[r[hf], :] = g
                        prev = sp.chain([g], prev, 1)
                return sp.chain([prev], first, 1)
            return run
        return [task(s0) for s0 in range(0, RB, 16)]

    def b_sum_tasks(src, dst, depth=DEPTH):
        def task(r0):
            def run(prev):
                raw = [src(slice(a * KH + r0, a * KH + r0 + 16), slice(c * KH, (c + 1) * KH))
                       for a in range(2) for c in range(2)]
                cs = _b_combos(*[b.astype(f32) for b in raw])
                for t in _B_SUMS:
                    dst.setdefault(t, []).append(_pack(cs[t]))
                return sp.chain([dst[t][-1] for t in _B_SUMS], prev, depth)
            return run
        return [task(r0) for r0 in range(0, KH, 16)]

    def b_rhs(src, sums):
        def rhs(t):
            if t == 1:
                return src(slice(0, KH), slice(0, KH))
            if t == 4:
                return src(slice(KH, D), slice(KH, D))
            return _unpack(jnp.concatenate(sums[t], axis=0))
        return rhs

    def strassen_x(order, rhs, finish):
        m = {}
        for rb, t in order:
            m.setdefault(rb, {})[t] = sp.dot(x_lhs(t, rb), rhs(t))
            if len(m[rb]) == 7:
                finish(rb, m.pop(rb))

    def h_sums(rb, cs, r0, sub):
        h = []
        for qd, cc in enumerate(cs):
            g0 = (qd // 2) * H + rb * RB + r0
            omg = 1.0 - gs[g0:g0 + sub, :]
            omg = jnp.concatenate([omg] * (CH // 128), axis=1)
            h.append(jnp.maximum(cc[:, :CH], 0.0) * cc[:, CH:] * omg)
        return _a_combos(*h)

    def glu_tasks(hs, rb, cs, sub):
        hs[rb] = [[] for _ in range(7)]

        def task(r0):
            def run(prev):
                sums = h_sums(rb, [cc[r0:r0 + sub] for cc in cs], r0, sub)
                for t in range(7):
                    hs[rb][t].append(sums[t])
                if sub < RB:
                    return sp.chain([sums[t] for t in _A_SLOT], prev, DEPTH2)
            return run
        return [task(r0) for r0 in range(0, RB, sub)]

    def down_lhs(hs, b, ha):
        tok = None
        for t in range(7):
            s0, s1 = [jnp.concatenate(hs[rb][t], axis=0) for rb in (b, b + 2)]
            slabs = []
            for r in range(0, RB, 16):
                slabs.append(sp.serial_combos(
                    _a_combos, s0[r:r + 16, :CQ], s0[r:r + 16, CQ:],
                    s1[r:r + 16, :CQ], s1[r:r + 16, CQ:], tok))
                tok = sp.chain([slabs[-1][t2] for t2 in _A_SLOT], None, H_DEPTH)
            for t2 in range(7):
                ha[b, 7 * t + t2] = jnp.concatenate([sl[t2] for sl in slabs], axis=0).astype(bf16)
        ha['tok'] = tok

    def d_tasks(j, dst):
        def task(r0, c):
            def run(prev):
                def blk(k1, k2, n1, n2):
                    r, c0 = k1 * CH + k2 * CQ + r0, n1 * KH + n2 * KQ + c * 128
                    return wd[j, r:r + 16, c0:c0 + 128].astype(f32)
                cs, tok = sp.two_level(_b_combos, blk, prev, DEPTH2)
                for t in range(49):
                    dst.setdefault((t, c), []).append(cs[t])
                return tok
            return run
        return [task(r0, c) for r0 in range(0, CQ, 16) for c in range(2)]

    def ffn_down(ha, dc, first):
        rhs = [_unpack(jnp.concatenate(
            [jnp.concatenate(dc[t, c], axis=0) for c in range(2)], axis=1)) for t in range(49)]
        todo = [(b, t) for b in range(2) for t in range(49)]
        for i in range(0, len(todo), 2):
            pair = todo[i:i + 2]
            ps = sp.dots([(ha[b, t], rhs[t]) for b, t in pair])
            for (b, t), p in zip(pair, ps):
                if first:
                    acc[t, b * RB:(b + 1) * RB, :] = p
                else:
                    acc[t, b * RB:(b + 1) * RB, :] += p

    def perm_tasks(wqkv_vm, wp, i, tbuf):
        def fwd(rb, c):
            def run(prev):
                c0 = i * D + c * 128
                tt = pltpu.bitcast(wqkv_vm[rb * 256:(rb + 1) * 256, c0:c0 + 128], f32).T
                for hh in range(4):
                    tbuf[rb, pl.ds((4 * c + hh) * TP, DH), :] = tt[hh * DH:(hh + 1) * DH, :]
                return sp.chain([tt], prev, 1)
            return run

        def bwd(rb, j):
            def run(prev):
                g = jnp.concatenate(
                    [tbuf[rb, pl.ds(4 * j + dd, NH, stride=TP), :] for dd in range(4)], axis=0).T
                wp[i, rb * 128:(rb + 1) * 128, j * 128:(j + 1) * 128] = pltpu.bitcast(g, i32)
            return run
        tasks = []
        for rb in range(4):
            tasks += [fwd(rb, c) for c in range(8)] + [bwd(rb, j) for j in range(8)]
        return tasks

    def wo_tasks(wo_vm):
        def stage(c):
            return 4 + c % 4, (c // 4) * NH * TP

        def spread(h0):
            def run(prev):
                blk = wo_vm[h0 * DH:(h0 + 2) * DH, :].astype(f32)
                for h in range(2):
                    for c in range(8):
                        sl, r0 = stage(c)
                        q_s[sl, pl.ds(r0 + (h0 + h) * TP, DH), :] = (
                            blk[h * DH:(h + 1) * DH, c * 128:(c + 1) * 128])
                return sp.chain([blk], prev, 1)
            return run

        def gather(d, h0, c):
            def run(after):
                def blk(k1, k2, n1, n2):
                    sl, r0 = stage(4 * n1 + 2 * n2 + c)
                    r0 += h0 * TP + 16 * k1 + 8 * k2 + d
                    return q_s[sl, pl.ds(r0, 16, stride=TP), :]
                cs, tok = sp.two_level(_b_combos, blk, None, DEPTH2, after)
                r = (d * NH + h0) // 2
                for t in range(49):
                    woc[t, r:r + 8, c * 128:(c + 1) * 128] = cs[t]
                return tok
            return run
        return ([spread(h0) for h0 in range(0, NH, 2)],
                [gather(d, h0, c) for d in range(8) for h0 in (0, 16) for c in range(2)])

    def proj(wp, i, dst, pad, slabs):
        lhs = jnp.concatenate([xn[r0 // 2:(r0 + n) // 2, :] for r0, n in slabs], axis=0)
        p = sp.dot(_unpack(lhs), _unpack(wp[i]))
        at = 0
        for r0, n in slabs:
            for j in range(8):
                dst[j, pad + r0:pad + r0 + n, :] = p[at:at + n, j * 128:(j + 1) * 128]
            at += n

    def v_finish(rb, m):
        cs = _c_combos(m)
        for qd, cc in enumerate(cs):
            r0 = PAD + (qd // 2) * H + rb * RB
            for j in range(4):
                v_s[(qd % 2) * 4 + j, r0:r0 + RB, :] = cc[:, j * 128:(j + 1) * 128]
        if rb == 0:
            for j in range(8):
                src = cs[j // 4][0:1, (j % 4) * 128:(j % 4 + 1) * 128]
                v_s[j, 0:PAD, :] = jnp.broadcast_to(src, (PAD, 128))

    def attn_group(row, masked):
        def run(prev):
            g = 8
            q = [q_s[j, pl.ds(row, g), :] for j in range(8)]
            ls = []
            for w in range(W):
                a = None
                for j in range(8):
                    term = q[j] * k_s[j, pl.ds(row + (PAD - DIL * w), g), :]
                    a = sp.link(ls[-1] if ls else None, term) if a is None else a + term
                ls.append(a)
            rs = [pltpu.roll(a, 64, 1) for a in ls]
            ls = [a + r for a, r in zip(ls, rs)]
            rs = [pltpu.roll(a, 32, 1) for a in ls]
            ls = [a + r for a, r in zip(ls, rs)]
            if masked:
                ri = row + lax.broadcasted_iota(i32, (g, 128), 0)
                ls = [ls[0]] + [jnp.where(ri >= DIL * w, ls[w], NEG) for w in range(1, W)]
            m = _tree(jnp.maximum, ls)
            ps = [jnp.exp2((l - m) * EXP2_SCALE) for l in ls]
            r = gs[pl.ds(row, g), :] / _tree(jnp.add, ps)
            outs = []
            for j in range(8):
                a = None
                for w in range(W):
                    term = ps[w] * v_s[j, pl.ds(row + (PAD - DIL * w), g), :]
                    a = sp.link(outs[-1] if outs else None, term) if a is None else a + term
                outs.append(a * r)
            for j in range(8):
                q_s[j, pl.ds(row, g), :] = outs[j]
            return sp.chain([outs[-1]], prev, 1)
        return run

    def attn_tasks(base, nrows, first=False):
        return [attn_group(base + (qq * Q + r), first and qq == 0 and r < PAD)
                for r in range(0, nrows, 8) for qq in range(4)]

    def pack_tasks(oa, base, hbase, nrows):
        def task(r, c):
            def run(prev, after=None):
                def blk(i1, i2, k1, k2):
                    return q_s[4 * k1 + 2 * k2 + c, pl.ds(base + (i1 * H + i2 * Q + r), 16), :]
                cs, tok = sp.two_level(_a_combos, blk, prev, DEPTH2, after)
                for t in range(49):
                    oa[t, pl.ds(hbase + r // 2, 8), c * 128:(c + 1) * 128] = cs[t]
                return tok
            return run
        return [task(r, c) for r in range(0, nrows, 16) for c in range(2)]

    GS = RB * (KH // 128) * (FC // 128) * 7 // (4 * SLOT)
    DS = 49
    PS = 2 * RB * (D // 128) * (D // 128) // (4 * SLOT)

    def glu(hs, ha):
        def finish(rb, m):
            glu_tasks(hs, rb, _c_combos(m), RB)[0](None)
            if rb >= 2:
                down_lhs(hs, rb - 2, ha)
        return finish

    def raw_first(rbs, n):
        lead = [(rb, t) for rb in rbs[:n] for t in ORDER[:2]]
        return lead + [(rb, t) for rb in rbs for t in ORDER if (rb, t) not in lead]

    def gu_src(j):
        return lambda r, c: wgu[j, r, c]

    def front(wqkv_vm, wp, wo_vm):
        in_q, in_k, in_v = [
            cp(wqkv_hbm.at[:, pl.ds(i * D, D)], wqkv_vm.at[:, pl.ds(i * D, D)], (6, 6, 5)[i])
            for i in range(3)]
        in_wo = cp(wo_hbm, wo_vm, 6)

        def plain(rb, hf, p):
            return sp.dot(x_vm[rows(rb, hf), :], wgu[0, :, p * CH:(p + 1) * CH])

        def plain_finish(hs, rb, c):
            cs = [jnp.concatenate(c[2 * qd:2 * qd + 2], axis=1) for qd in range(4)]
            return glu_tasks(hs, rb, cs, 16)

        def chunk0(_, carry):
            hs, bc, dc = {}, {}, {}
            wait(in0)
            start(in3)
            c0 = {(0, 0): plain(0, 0, 0)}
            wait(in1)
            c0[1, 0] = plain(0, 1, 0)
            wait(in2)
            start(in4)
            for hf in range(2):
                c0[hf, 1] = plain(0, hf, 1)
            wait(in3)
            start(in5)
            sp.block()
            bt = b_sum_tasks(gu_src(0), bc)
            sp.schedule(bt[:12], 3, 16)
            sp.schedule(prep_tasks(0, sums=False), 3, 16)
            for p in (2, 3):
                for hf in range(2):
                    c0[hf, p] = plain(0, hf, p)
            c0 = [c0[hf, p] for hf in range(2) for p in range(4)]
            wait(in4)
            start([in_v])
            sp.block()
            sp.schedule(bt[12:], 3, 32)
            sp.schedule(prep_tasks(1, sums=False), 2, 10)
            sp.schedule(prep_tasks(2), 10, 32)
            c1 = [plain(1, hf, p) for hf in range(2) for p in range(4)]
            wait(in5 + [in_v])
            start([in_k, in_wo, in_q])
            sp.block()
            for j in range(8):
                k_s[j, 0:PAD, :] = jnp.zeros((PAD, 128), f32)
            ha = {}
            sp.schedule(prep_tasks(3), 2, GS)
            sp.schedule(plain_finish(hs, 0, c0), 2, GS)
            sp.schedule(plain_finish(hs, 1, c1), GS + 6, 2 * GS)
            sp.schedule(d_tasks(0, dc), GS - 2, 2 * GS)
            sp.schedule(perm_tasks(wqkv_vm, wp, 2, q_s), 2 * GS + 6, 2 * GS + DS - 8)
            strassen_x([(rb, t) for rb in (2, 3) for t in ORDER], b_rhs(gu_src(0), bc),
                       glu(hs, ha))
            ffn_down(ha, dc, True)
            return carry

        lax.fori_loop(0, zi[0], chunk0, 0)

        wait([in_k, in_wo, in_q])
        start(in_ffn)
        sp.block()
        vb = {}
        v_src = lambda r, c: _unpack(wp[2, _half(r), c])
        wo_spread, wo_gather = wo_tasks(wo_vm)
        sp.schedule(b_sum_tasks(v_src, vb, VDEPTH), *VBC_SLOTS)
        sp.schedule(prep_tasks(0, gate=False) + prep_tasks(1, gate=False), *PREP01)
        sp.schedule(perm_tasks(wqkv_vm, wp, 1, k_s.at[:, PAD:, :]), *PERMK)
        sp.schedule(wo_spread, *WOS)
        strassen_x(raw_first((2, 3, 0, 1), 2), b_rhs(v_src, vb), v_finish)
        sp.schedule(perm_tasks(wqkv_vm, wp, 0, q_s), 4, 3 * PS)
        tok = None
        for t in wo_gather:
            tok = t(tok)
        for rb in range(NRB):
            proj(wp, 1, k_s, PAD, [(rb * Q, Q)])
        proj(wp, 0, q_s, 0, [(qq * Q, QA) for qq in range(4)])

        def q_rest(_, carry):
            sp.block()
            n = (Q - QA) // 2
            total = 4 * (Q - QA) * 64 // (4 * SLOT)
            sp.schedule(attn_tasks(0, A0, True), 4, total)
            for r0 in (QA, QA + n):
                proj(wp, 0, q_s, 0, [(qq * Q + r0, n) for qq in range(4)])
            return carry

        lax.fori_loop(0, zi[0], q_rest, 0)
        wait(in_ffn)

    def back(oa):
        def body(j, carry):
            sp.block()
            base = pl.multiple_of((j - 1) * AR, AR)
            hs, ha, bc, dc = {}, {}, {}, {}
            slot = jnp.where(j == NW, 0, j)
            sp.schedule(b_sum_tasks(gu_src(slot), bc), *BC_SLOTS)
            sp.schedule(attn_tasks(base + A0, AR), *ATTN_SLOTS)
            packs = pack_tasks(oa, base, pl.multiple_of((j - 1) * (AR // 2), AR // 2), AR)
            sp.schedule(d_tasks(slot, dc), *DC_SLOTS)
            strassen_x(raw_first((0, 2, 1, 3), NRAW), b_rhs(gu_src(slot), bc), glu(hs, ha))
            tok = ha['tok']
            for t in packs:
                tok = t(None, tok)
            ffn_down(ha, dc, False)
            return carry

        lax.fori_loop(1, NC, body, 0)

        def out_copy(r0, n, i1, i2, cols):
            idx = (pl.ds(r0 + i1 * H + i2 * Q, n), cols)
            return cp(x_vm.at[idx], o2.at[idx], out_sem)

        def out_blocks(n, blocks):
            done_by = {ts[-1]: qd for ts, qd in _C_ORDER}
            todo = [(blk, t1, t2) for blk in range(len(blocks))
                    for ts1, _ in _C_ORDER for t1 in ts1 for ts2, _ in _C_ORDER for t2 in ts2]
            m, inner = {}, {}
            for i in range(0, len(todo), SLOT // n):
                group = todo[i:i + SLOT // n]
                ps = sp.dots([(_unpack(oa[7 * t1 + t2, pl.ds(blocks[blk][0] // 2, n // 2), :]),
                               _unpack(woc[7 * t1 + t2])) for blk, t1, t2 in group])
                for (blk, t1, t2), p in zip(group, ps):
                    r0, copies = blocks[blk]
                    m.setdefault((blk, t1), {})[t2] = acc[7 * t1 + t2, pl.ds(r0, n), :] + p
                    if t2 not in done_by:
                        continue
                    q2 = done_by[t2] ^ (t1 in _FLIP)
                    inner.setdefault((blk, q2), {})[t1] = _c_quadrant(m[blk, t1], done_by[t2])
                    if t1 not in done_by:
                        continue
                    q1 = done_by[t1]
                    r = pl.ds(r0 + (q1 // 2) * H + (q2 // 2) * Q, n)
                    c = (q1 % 2) * KH + (q2 % 2) * KQ
                    x_vm[r, c:c + KQ] = _c_quadrant(inner[blk, q2], q1).astype(bf16)
                    start(copies.get((q1, q2), []))

        final = {q1: (q1, 3 ^ (ts[-1] in _FLIP)) for ts, q1 in _C_ORDER}

        def whole(r0, n):
            return {final[3]: [out_copy(r0, n, i1, i2, slice(None))
                               for i1 in range(2) for i2 in range(2)]}

        done = (NC - 1) * AR
        sp.block()
        sp.schedule(pack_tasks(oa, done, done // 2, Q - done), *PACK4)
        last = {final[q1]: [out_copy(Q - PB, PB, q1 // 2, i2, pl.ds((q1 % 2) * KH, KH))
                            for i2 in range(2)] for q1 in range(3)}
        for q2 in range(4):
            last[3, q2] = [out_copy(Q - PB, PB, 1, q2 // 2, pl.ds(KH + (q2 % 2) * KQ, KQ))]
        copies = [whole(0, RB), whole(RB, PB), last]
        out_blocks(RB, [(0, copies[0])])
        out_blocks(PB, [(RB, copies[1]), (Q - PB, last)])
        for cs in copies:
            for key in cs:
                wait(cs[key])

    pl.run_scoped(front, pltpu.VMEM((D, 3 * D), bf16), pltpu.VMEM((3, D // 2, D), i32),
                  pltpu.VMEM((D, D), bf16))
    pl.run_scoped(back, pltpu.VMEM((49, Q // 2, KQ), i32))
    assert not sp.plan


_N_SEMS = 9


@jax.jit
def pallas_gated_mix__sliding_local_dilated__glu_gated_reglu__prompt_kernel(
    A_x: jax.Array,
    A_wqkv: jax.Array,
    A_wo: jax.Array,
    B_x: jax.Array,
    B_W_gate: jax.Array,
    B_W_up: jax.Array,
    B_W_down: jax.Array,
    gate_w: jax.Array,
):
    del B_x
    hbm = pl.BlockSpec(memory_space=pl.ANY)
    scratch = [
        pltpu.VMEM((S, D), bf16),
        pltpu.VMEM((S // 2, D), i32),
        pltpu.VMEM((5, H // 2, KH), i32),
        pltpu.VMEM((8, 128), bf16),
        pltpu.VMEM((NW, D, 2 * FC), bf16),
        pltpu.VMEM((NW, FC, D), bf16),
        pltpu.VMEM((49, Q, KQ), f32),
        pltpu.VMEM((8, S + QPAD, 128), f32),
        pltpu.VMEM((8, PAD + S, 128), f32),
        pltpu.VMEM((8, PAD + S, 128), f32),
        pltpu.VMEM((S, 128), f32),
        pltpu.VMEM((49, KQ // 2, KQ), i32),
        pltpu.VMEM((8, 128), i32),
        pltpu.SMEM((1,), i32),
        pltpu.SemaphoreType.DMA((_N_SEMS,)),
    ]
    return pl.pallas_call(
        _kernel,
        in_specs=[hbm] * 7,
        out_specs=hbm,
        out_shape=jax.ShapeDtypeStruct((1, S, D), bf16),
        scratch_shapes=scratch,
        compiler_params=pltpu.CompilerParams(vmem_limit_bytes=127 * 1024 * 1024),
    )(A_x, A_wqkv, A_wo, B_W_gate, B_W_up, B_W_down, gate_w.reshape(8, 128))
```
